```python
import jax
import jax.numpy as jnp

def _softmax(x, axis=-1):
    return jax.nn.softmax(x, axis=axis)

def _gelu(x):
    return jax.nn.gelu(x, approximate=True)

def _silu(x):
    return jax.nn.silu(x)

def _sigmoid(x):
    return jax.nn.sigmoid(x)

def _layernorm(x, axis=-1, eps=1e-05):
    m = jnp.mean(x, axis=axis, keepdims=True)
    v = jnp.var(x, axis=axis, keepdims=True)
    return (x - m) / jnp.sqrt(v + eps)

def _scatter_add(tgt, idx, src, axis=0):
    return tgt.at[idx].add(src)

def _segment_sum(src, seg, n):
    return jax.ops.segment_sum(src, seg, n)

class _Rng:

    def __init__(self, key):
        self._k = key

    def _next(self):
        self._k, sub = jax.random.split(self._k)
        return sub

    def normal(self, shape):
        return jax.random.normal(self._next(), shape, dtype=jnp.bfloat16)

    def randint(self, lo, hi, shape):
        return jax.random.randint(self._next(), shape, lo, hi, dtype=jnp.int32)

    def uniform(self, shape, lo=0.0, hi=1.0):
        return jax.random.uniform(self._next(), shape, jnp.bfloat16, lo, hi)

    def permutation(self, n):
        return jax.random.permutation(self._next(), n)
kernel_name = 'adaLN_cond__memory_aug_recurrent_mem_tr__glu_gated_swiglu__prompt'

def setup_inputs():
    _rng = _Rng(jax.random.key(int.from_bytes(__import__("os").urandom(4), "little")))
    _w = lambda a: (lambda t: t.astype(jnp.bfloat16) if jnp.issubdtype(t.dtype, jnp.floating) else t)(jnp.asarray(a))

    def _A_setup():
        B, S, Dm = (1, 2048, 1024)
        H, Dh = (32, 128)
        M, seg = (8, 32)
        seg = min(seg, S)
        S = S // seg * seg
        return {'x': _w((lambda *s: _rng.normal(s) * 0.05)(B, S, Dm)), 'mem0': _w((lambda *s: _rng.normal(s) * 0.05)(B, M, Dm)), 'Wq': _w((lambda *s: _rng.normal(s) * 0.05)(Dm, H, Dh) * Dm ** (-0.5)), 'Wk': _w((lambda *s: _rng.normal(s) * 0.05)(Dm, H, Dh) * Dm ** (-0.5)), 'Wv': _w((lambda *s: _rng.normal(s) * 0.05)(Dm, H, Dh) * Dm ** (-0.5)), 'Wo': _w((lambda *s: _rng.normal(s) * 0.05)(H, Dh, Dm) * (H * Dh) ** (-0.5)), 'seg_len': seg}
    _A_in = _A_setup()

    def _B_setup():
        B, S, D, F = (1, 2048, 1024, 3584)
        return {'x': _w((lambda *s: _rng.normal(s) * 0.05)(B, S, D)), 'w1': _w((lambda *s: _rng.normal(s) * 0.05)(D, F) * (2.0 / D) ** 0.5), 'w3': _w((lambda *s: _rng.normal(s) * 0.05)(D, F) * (2.0 / D) ** 0.5), 'w2': _w((lambda *s: _rng.normal(s) * 0.05)(F, D) * (2.0 / F) ** 0.5)}
    _B_in = _B_setup()
    return {'A_x': _A_in['x'], 'A_mem0': _A_in['mem0'], 'A_Wq': _A_in['Wq'], 'A_Wk': _A_in['Wk'], 'A_Wv': _A_in['Wv'], 'A_Wo': _A_in['Wo'], 'A_seg_len': _A_in['seg_len'], 'B_x': _B_in['x'], 'B_w1': _B_in['w1'], 'B_w3': _B_in['w3'], 'B_w2': _B_in['w2'], 'c': _w((lambda *s: _rng.normal(s) * 0.05)(1, 1024)), 'w_mod': _w((lambda *s: _rng.normal(s) * 0.05)(1024, 6 * 1024) * 1024 ** (-0.5))}

def reference(A_x, A_mem0, A_Wq, A_Wk, A_Wv, A_Wo, A_seg_len, B_x, B_w1, B_w3, B_w2, c, w_mod):

    def _A_ref(x, mem0, Wq, Wk, Wv, Wo, seg_len):
        B, S, Dm = x.shape
        H, Dh = (Wq.shape[1], Wq.shape[2])
        M = mem0.shape[1]
        scale = Dh ** (-0.5)
        n_seg = S // seg_len
        L = M + seg_len
        idx = jnp.arange(L)
        mask = (idx[:, None] < M) | (idx[:, None] >= idx[None, :])
        mem = mem0
        outs = []
        for s in range(n_seg):
            xs = x[:, s * seg_len:(s + 1) * seg_len, :].copy()
            h = jnp.concatenate([mem, xs], axis=1)
            q = jnp.einsum('btd,dhe->bhte', h, Wq)
            k = jnp.einsum('btd,dhe->bhte', h, Wk)
            v = jnp.einsum('btd,dhe->bhte', h, Wv)
            scores = jnp.einsum('bhqe,bhke->bhqk', q, k) * scale
            scores = jnp.where(mask[None, None], scores, -1000000000.0)
            p = _softmax(scores, axis=-1)
            o = jnp.einsum('bhqk,bhke->bhqe', p, v)
            o = jnp.einsum('bhte,hed->btd', o, Wo)
            mem = o[:, :M, :].copy()
            outs.append(o[:, M:, :])
        return jnp.concatenate(outs, axis=1)

    def _B_ref(x, w1, w3, w2):
        gate = jnp.einsum('bsd,df->bsf', x, w1)
        up = jnp.einsum('bsd,df->bsf', x, w3)
        h = _silu(gate) * up
        out = jnp.einsum('bsf,fd->bsd', h, w2)
        return out
    x = A_x
    mod = (_silu(c) @ w_mod).reshape(c.shape[0], 6, 1, -1)
    sa, ca, ga, sb, cb, gb = (mod[:, 0].copy(), mod[:, 1].copy(), mod[:, 2].copy(), mod[:, 3].copy(), mod[:, 4].copy(), mod[:, 5].copy())
    h = _layernorm(x, axis=-1) * (1 + ca) + sa
    x = x + ga * _A_ref(h, A_mem0, A_Wq, A_Wk, A_Wv, A_Wo, A_seg_len)
    h = _layernorm(x, axis=-1) * (1 + cb) + sb
    x = x + gb * _B_ref(h, B_w1, B_w3, B_w2)
    return x
```

```python
import functools

import jax
import jax.numpy as jnp
from jax import lax
import jax.experimental.pallas as pl
import jax.experimental.pallas.tpu as pltpu

F32 = jnp.float32
BF16 = jnp.bfloat16
U32 = jnp.uint32

S = 2048
D = 1024
H = 32
DH = 128
HD = H * DH
MEM = 8
SEG = 32
FF = 3584
EPS = 1e-5

G = 8
HG = H // G
GW = HG * DH
PRO = 512
NPAIR = S // (2 * SEG)
PT = 2 * SEG
SLOT = 80
NSLOT = 9
LAG = 2
X0 = 768
FC = 256
NFC = FF // FC


def _w(ref, r0, r1, c0, c1):
    return pltpu.bitcast(ref[r0 // 2:r1 // 2, c0:c1], BF16)


def _dot(a, b):
    return jnp.dot(a, b, preferred_element_type=F32)


def _ln(x):
    m = jnp.mean(x, axis=-1, keepdims=True)
    xc = x - m
    v = jnp.mean(xc * xc, axis=-1, keepdims=True)
    return xc * lax.rsqrt(v + EPS)


def _masks():
    def pos(j):
        return jnp.where(j < 40, j, jnp.where(j < 48, j - 32, jnp.where(j < 56, j - 48, j - 40)))

    out = []
    for q0, nq, nk in ((0, 32, 48), (32, 48, 80)):
        qi = lax.broadcasted_iota(jnp.int32, (nq, nk), 0) + q0
        kj = lax.broadcasted_iota(jnp.int32, (nq, nk), 1)
        qp, kp = pos(qi), pos(kj)
        same = ((qi < 40) & (kj < 40)) | ((qi >= 40) & (kj >= 40))
        allowed = same & ((qp < MEM) | (qp >= kp))
        fill = jnp.where(same, jnp.float32(-1e9), jnp.float32(-jnp.inf))
        out.append((allowed, fill))
    return out


def _kernel(x_hbm, mem0_hbm, wq_hbm, wk_hbm, wv_hbm, wo_hbm, w1_hbm, w3_hbm, w2_hbm,
            c_hbm, wm_hbm, out_hbm,
            xv, outv, wo, w1, w3, w2, wm, cv, m0v, modv, h0,
            lhs_a, lhs_b, o32, abuf, yv, h2, hid, sem_in, sem_g, sem_out, *rest):
    ring = rest[:G]
    wg = rest[G:]
    scale = DH ** -0.5

    copies = {}

    def cp(name, src, dst):
        c = pltpu.make_async_copy(src, dst, sem_in.at[len(copies)])
        copies[name] = c
        c.start()

    def cols(hbm, ref, c0, c1):
        return hbm.bitcast(U32).at[:, c0:c1], ref.at[:, c0:c1]

    cp("c", c_hbm, cv)
    cp("mem0", mem0_hbm, m0v)
    cp("x0", x_hbm.at[0:X0], xv.at[0:X0])
    cp("wm0", *cols(wm_hbm, wm, 0, 2 * D))
    gcopies = []
    for g in range(G):
        lst = []
        for m, hbm in enumerate((wq_hbm, wk_hbm, wv_hbm)):
            for jj in range(HG // 2):
                for par in range(2):
                    c = pltpu.make_async_copy(
                        hbm.bitcast(U32).at[:, par, g * (HG // 2) + jj],
                        wg[g].at[m * HG + 2 * jj + par], sem_g.at[g])
                    c.start()
                    lst.append(c)
        gcopies.append(lst)
    cp("wo", wo_hbm.bitcast(U32), wo)
    cp("wm1", *cols(wm_hbm, wm, 2 * D, 6 * D))
    cp("w1", w1_hbm.bitcast(U32), w1)
    cp("w3", w3_hbm.bitcast(U32), w3)
    cp("w2", w2_hbm.bitcast(U32), w2)
    cp("x1", x_hbm.at[X0:S], xv.at[X0:S])

    def out_copy(r0, n):
        return pltpu.make_async_copy(outv.at[pl.ds(r0, n)], out_hbm.at[pl.ds(r0, n)], sem_out)

    def mod_part(c0, c1):
        cf = cv[...].astype(F32)
        sc = jnp.broadcast_to(cf * jax.nn.sigmoid(cf), (16, D)).astype(BF16)
        modv[:, c0:c1] = _dot(sc, _w(wm, 0, D, c0, c1))[0:8]

    def mvec(i):
        return modv[0:1, i * D:(i + 1) * D]

    def ln1(r0, n):
        xf = xv[pl.ds(r0, n), :].astype(F32)
        return _ln(xf) * (1.0 + mvec(1)) + mvec(0)

    def repack(g, r0, n):
        for t in range(0, 3 * HG, 2):
            a = wg[g][t, pl.ds(r0, n), :]
            b = wg[g][t + 1, pl.ds(r0, n), :]
            wg[g][t, pl.ds(r0, n), :] = (a & jnp.uint32(0xFFFF)) | (b << 16)
            wg[g][t + 1, pl.ds(r0, n), :] = (a >> 16) | (b & jnp.uint32(0xFFFF0000))

    def proj(lhs, g, rows):
        for t in range(3 * HG):
            r = _dot(lhs, pltpu.bitcast(wg[g][t], BF16))
            for i, row in enumerate(rows):
                ring[g][pl.ds(row, 8), t * DH:(t + 1) * DH] = r[8 * i:8 * i + 8].astype(BF16)

    def attn(g, base, q0, nq, nk, allowed, fill):
        qrow = pl.multiple_of(base + q0, 16)
        for hh in range(HG):
            c = hh * DH
            q = ring[g][pl.ds(qrow, nq), c:c + DH]
            k = ring[g][pl.ds(base, nk), GW + c:GW + c + DH]
            v = ring[g][pl.ds(base, nk), 2 * GW + c:2 * GW + c + DH]
            s = lax.dot_general(q, k, (((1,), (1,)), ((), ())), preferred_element_type=F32)
            s = jnp.where(allowed, s * scale, fill)
            m = jnp.max(s, axis=-1, keepdims=True)
            p = jnp.exp(s - m)
            l = jnp.sum(p, axis=-1, keepdims=True)
            o = _dot(p.astype(BF16), v) * (1.0 / l)
            col = (g * HG + hh) * DH
            o32[0:nq // 2, col:col + DH] = pltpu.bitcast(o.astype(BF16), U32)

    def wo_proj(nq, stores):
        o = _w(o32, 0, nq, 0, HD)
        cw = 256
        for cb in range(D // cw):
            r = _dot(o, _w(wo, 0, HD, cb * cw, (cb + 1) * cw))
            for r0, n, fn in stores:
                fn(slice(cb * cw, (cb + 1) * cw), r[r0:r0 + n])

    def post_attn(tok0, slot, n):
        x1 = xv[pl.ds(tok0, n), :].astype(F32) + mvec(2) * abuf[pl.ds(slot, n), :]
        yv[0:n, :] = x1
        hh = _ln(x1) * (1.0 + mvec(4)) + mvec(3)
        h2[0:n // 2, :] = pltpu.bitcast(hh.astype(BF16), U32)

    def ffn_up(c0, c1, n):
        a = _w(h2, 0, n, 0, D)
        for c in range(c0, c1):
            gt = _dot(a, _w(w1, 0, D, c * FC, (c + 1) * FC))
            up = _dot(a, _w(w3, 0, D, c * FC, (c + 1) * FC))
            hv = gt * jax.nn.sigmoid(gt) * up
            hid[0:n // 2, c * FC:(c + 1) * FC] = pltpu.bitcast(hv.astype(BF16), U32)

    def ffn_down(tok0, n, cb0, cb1):
        a = _w(hid, 0, n, 0, FF)
        cw = 256
        for cb in range(cb0, cb1):
            cs = slice(cb * cw, (cb + 1) * cw)
            r = _dot(a, _w(w2, 0, FF, cb * cw, (cb + 1) * cw))
            gb = modv[0:1, 5 * D + cb * cw:5 * D + (cb + 1) * cw]
            outv[pl.ds(tok0, n), cs] = (yv[0:n, cs] + gb * r).astype(BF16)

    def unit_row(u):
        r = u % 8
        return pl.multiple_of(((u // 8) % NSLOT) * SLOT + 8 + 8 * r + 8 * (r >= 5).astype(jnp.int32), 8)

    copies["c"].wait()
    copies["wm0"].wait()
    mod_part(0, 2 * D)
    copies["x0"].wait()
    copies["mem0"].wait()

    def ln_body(i, _):
        r0 = pl.multiple_of(i * 64, 64)
        h0[pl.ds(pl.multiple_of(i * 32, 32), 32), :] = pltpu.bitcast(ln1(r0, 64).astype(BF16), U32)
        return 0

    lax.fori_loop(0, PRO // 64, ln_body, 0)
    lhs_a[0:MEM, :] = m0v[...].astype(F32)
    lhs_a[MEM:32, :] = ln1(PRO, 24)

    RB = 128
    NRB = PRO // RB
    RP = D // 2 // NRB
    for c in gcopies[0]:
        c.wait()
    repack(0, 0, D // 2)
    for g in range(G):
        if g + 1 < G:
            for c in gcopies[g + 1]:
                c.wait()

        def pro_body(i, _, g=g):
            if g + 1 < G:
                repack(g + 1, pl.multiple_of(i * RP, RP), RP)
            a = pltpu.bitcast(h0[pl.ds(pl.multiple_of(i * (RB // 2), RB // 2), RB // 2), :], BF16)
            for t in range(3 * HG):
                r = _dot(a, pltpu.bitcast(wg[g][t], BF16))
                for pp in range(RB // PT):
                    base = (i * (RB // PT) + pp) * SLOT
                    ring[g][pl.ds(pl.multiple_of(base + 8, 8), 40), t * DH:(t + 1) * DH] = (
                        r[pp * PT:pp * PT + 40].astype(BF16))
                    ring[g][pl.ds(pl.multiple_of(base + 56, 8), 24), t * DH:(t + 1) * DH] = (
                        r[pp * PT + 40:pp * PT + 64].astype(BF16))
            return 0

        lax.fori_loop(0, NRB, pro_body, 0)

    def pair(p, with_ffn):
        (al_a, fi_a), (al_b, fi_b) = _masks()
        base = pl.multiple_of((p % NSLOT) * SLOT, 16)
        u0 = PRO // 8 + 6 * p
        tlead = PRO + 48 * p
        aslot = pl.multiple_of((p % LAG) * PT, PT)
        tok_f = pl.multiple_of((p - LAG) * PT, PT)

        if with_ffn:
            post_attn(tok_f, aslot, PT)

        lhs = lhs_a[...].astype(BF16)
        rows = [base, unit_row(u0), unit_row(u0 + 1), unit_row(u0 + 2)]
        lhs_b[MEM:32, :] = ln1(pl.multiple_of(tlead + 24, 8), 24)
        for g in range(G):
            proj(lhs, g, rows)
            if g > 0:
                attn(g - 1, base, 0, 32, 48, al_a, fi_a)
        if with_ffn:
            ffn_up(0, 2, PT)
        attn(G - 1, base, 0, 32, 48, al_a, fi_a)
        if with_ffn:
            ffn_up(2, 5, PT)

        def st_mem_b(cs, val):
            lhs_b[0:MEM, cs] = val.astype(BF16).astype(F32)

        def st_a(r0, n):
            def fn(cs, val):
                abuf[pl.ds(pl.multiple_of(aslot + r0, 8), n), cs] = val
            return fn

        wo_proj(32, [(0, 8, st_mem_b), (8, 24, st_a(0, 24))])
        if with_ffn:
            ffn_up(5, 9, PT)

        lhs = lhs_b[...].astype(BF16)
        rows = [pl.multiple_of(base + 48, 8), unit_row(u0 + 3), unit_row(u0 + 4), unit_row(u0 + 5)]
        nxt = pl.multiple_of(jnp.minimum(tlead + 48, S - 24), 8)
        lhs_a[MEM:32, :] = ln1(nxt, 24)
        for g in range(G):
            proj(lhs, g, rows)
            if g > 0:
                attn(g - 1, base, 32, 48, 80, al_b, fi_b)
        if with_ffn:
            ffn_up(9, 11, PT)
        attn(G - 1, base, 32, 48, 80, al_b, fi_b)
        if with_ffn:
            ffn_up(11, NFC, PT)

        def st_mem_a(cs, val):
            lhs_a[0:MEM, cs] = val.astype(BF16).astype(F32)

        wo_proj(48, [(16, 8, st_mem_a), (0, 16, st_a(24, 16)), (24, 24, st_a(40, 24))])
        if with_ffn:
            ffn_down(tok_f, PT, 0, 4)

    copies["wo"].wait()

    def pair_noffn(p, _):
        pair(p, False)
        return 0

    lax.fori_loop(0, LAG, pair_noffn, 0)

    copies["wm1"].wait()
    mod_part(2 * D, 6 * D)
    copies["w1"].wait()
    copies["w3"].wait()
    copies["w2"].wait()
    copies["x1"].wait()

    def pair_ffn(p, _):
        @pl.when(p > LAG)
        def _():
            out_copy(pl.multiple_of((p - LAG - 1) * PT, PT), PT).start()

        pair(p, True)
        return 0

    lax.fori_loop(LAG, NPAIR, pair_ffn, 0)

    out_copy((NPAIR - LAG - 1) * PT, PT).start()
    for p in range(NPAIR - LAG, NPAIR):
        post_attn(p * PT, (p % LAG) * PT, PT)
        ffn_up(0, NFC, PT)
        ffn_down(p * PT, PT, 0, 4)
        out_copy(p * PT, PT).start()
    out_copy(0, S).wait()


@functools.partial(jax.jit, static_argnames=("A_seg_len",))
def pallas_adaLN_cond__memory_aug_recurrent_mem_tr__glu_gated_swiglu__prompt_kernel(
    A_x, A_mem0, A_Wq, A_Wk, A_Wv, A_Wo, A_seg_len, B_x, B_w1, B_w3, B_w2, c, w_mod,
):
    assert A_seg_len == SEG
    assert A_x.shape == (1, S, D) and A_mem0.shape == (1, MEM, D)
    assert A_Wq.shape == (D, H, DH) and B_w1.shape == (D, FF)
    del B_x

    n_in_copies = 4 + 6
    scratch = [
        pltpu.VMEM((S, D), BF16),
        pltpu.VMEM((S, D), BF16),
        pltpu.VMEM((HD // 2, D), U32),
        pltpu.VMEM((D // 2, FF), U32),
        pltpu.VMEM((D // 2, FF), U32),
        pltpu.VMEM((FF // 2, D), U32),
        pltpu.VMEM((D // 2, 6 * D), U32),
        pltpu.VMEM((1, D), BF16),
        pltpu.VMEM((MEM, D), BF16),
        pltpu.VMEM((8, 6 * D), F32),
        pltpu.VMEM((PRO // 2, D), U32),
        pltpu.VMEM((32, D), F32),
        pltpu.VMEM((32, D), F32),
        pltpu.VMEM((24, HD), U32),
        pltpu.VMEM((LAG * PT, D), F32),
        pltpu.VMEM((PT, D), F32),
        pltpu.VMEM((PT // 2, D), U32),
        pltpu.VMEM((PT // 2, FF), U32),
        pltpu.SemaphoreType.DMA((n_in_copies,)),
        pltpu.SemaphoreType.DMA((G,)),
        pltpu.SemaphoreType.DMA,
    ] + [pltpu.VMEM((NSLOT * SLOT, 3 * GW), BF16) for _ in range(G)
    ] + [pltpu.VMEM((3 * HG, D // 2, DH), U32) for _ in range(G)]

    out = pl.pallas_call(
        _kernel,
        out_shape=jax.ShapeDtypeStruct((S, D), BF16),
        in_specs=[pl.BlockSpec(memory_space=pl.ANY)] * 11,
        out_specs=pl.BlockSpec(memory_space=pl.ANY),
        scratch_shapes=scratch,
        compiler_params=pltpu.CompilerParams(vmem_limit_bytes=120 * 1024 * 1024),
    )(
        A_x.reshape(S, D), A_mem0.reshape(MEM, D),
        A_Wq.reshape(D // 2, 2, H, DH), A_Wk.reshape(D // 2, 2, H, DH),
        A_Wv.reshape(D // 2, 2, H, DH), A_Wo.reshape(HD, D),
        B_w1, B_w3, B_w2, c, w_mod,
    )
    return out.reshape(1, S, D)
```

```python
import functools

import jax
import jax.numpy as jnp
from jax import lax
import jax.experimental.pallas as pl
import jax.experimental.pallas.tpu as pltpu

F32 = jnp.float32
BF16 = jnp.bfloat16
U32 = jnp.uint32

S = 2048
D = 1024
H = 32
DH = 128
HD = H * DH
MEM = 8
SEG = 32
FF = 3584
EPS = 1e-5

G = 8
HG = H // G
GW = HG * DH
PRO = 512
NPAIR = S // (2 * SEG)
PT = 2 * SEG
SLOT = 80
NSLOT = 9
LAG = 2
X0 = 768
FC = 256
NFC = FF // FC
MAIN_START = LAG
SCOPES = False
NO_LOOP_DMA = False
SKIP = ()


class _NoScope:
    def __enter__(self):
        return self

    def __exit__(self, *a):
        return False


def _scope(name):
    return jax.named_scope(name) if SCOPES else _NoScope()


def _w(ref, r0, r1, c0, c1):
    return pltpu.bitcast(ref[r0 // 2:r1 // 2, c0:c1], BF16)


def _dot(a, b):
    return jnp.dot(a, b, preferred_element_type=F32)


def _ln(x):
    m = jnp.mean(x, axis=-1, keepdims=True)
    xc = x - m
    v = jnp.mean(xc * xc, axis=-1, keepdims=True)
    return xc * lax.rsqrt(v + EPS)


def _masks():
    def pos(j):
        return jnp.where(j < 40, j, jnp.where(j < 48, j - 32, jnp.where(j < 56, j - 48, j - 40)))

    out = []
    for q0, nq, nk in ((0, 32, 48), (32, 48, 80)):
        qi = lax.broadcasted_iota(jnp.int32, (nq, nk), 0) + q0
        kj = lax.broadcasted_iota(jnp.int32, (nq, nk), 1)
        qp, kp = pos(qi), pos(kj)
        same = ((qi < 40) & (kj < 40)) | ((qi >= 40) & (kj >= 40))
        allowed = same & ((qp < MEM) | (qp >= kp))
        fill = jnp.where(same, jnp.float32(-1e9), jnp.float32(-jnp.inf))
        out.append((allowed, fill))
    return out


def _kernel(x_hbm, mem0_hbm, wq_hbm, wk_hbm, wv_hbm, wo_hbm, w1_hbm, w3_hbm, w2_hbm,
            c_hbm, wm_hbm, out_hbm,
            xv, outv, wo, w1, w3, w2, wm, cv, m0v, modv, h0,
            lhs_a, lhs_b, o32, abuf, yv, h2, hid, sem_in, sem_g, sem_out, *rest):
    rqk = rest[0:2]
    rv = rest[2:4]
    wg = rest[4:6]
    scale = DH ** -0.5

    copies = {}

    def mk(name, src, dst):
        copies[name] = pltpu.make_async_copy(src, dst, sem_in.at[len(copies)])

    def cols(hbm, ref, c0, c1):
        return hbm.bitcast(U32).at[:, c0:c1], ref.at[:, c0:c1]

    mk("c", c_hbm, cv)
    mk("mem0", mem0_hbm, m0v)
    mk("x0", x_hbm.at[0:X0], xv.at[0:X0])
    mk("wm0", *cols(wm_hbm, wm, 0, 2 * D))
    mk("wo", wo_hbm.bitcast(U32), wo)
    mk("wm1", *cols(wm_hbm, wm, 2 * D, 6 * D))
    mk("w1", w1_hbm.bitcast(U32), w1)
    mk("w3", w3_hbm.bitcast(U32), w3)
    mk("w2", w2_hbm.bitcast(U32), w2)
    mk("x1", x_hbm.at[X0:S], xv.at[X0:S])
    def gcopies(par_g, gi):
        lst = []
        for m, hbm in enumerate((wq_hbm, wk_hbm, wv_hbm)):
            for jj in range(HG // 2):
                for par in range(2):
                    lst.append(pltpu.make_async_copy(
                        hbm.bitcast(U32).at[:, par, (2 * gi + par_g) * (HG // 2) + jj],
                        wg[par_g].at[gi, m * HG + 2 * jj + par], sem_g.at[2 * gi + par_g]))
        return lst

    def start_group(par_g, gi):
        for c in gcopies(par_g, gi):
            c.start()

    def wait_group(par_g, gi):
        for c in gcopies(par_g, gi):
            c.wait()

    for n in ("c", "mem0", "x0", "wm0"):
        copies[n].start()
    start_group(0, 0)
    start_group(1, 0)

    def out_copy(r0, n):
        return pltpu.make_async_copy(outv.at[pl.ds(r0, n)], out_hbm.at[pl.ds(r0, n)], sem_out)

    def mod_part(c0, c1):
        cf = cv[...].astype(F32)
        sc = jnp.broadcast_to(cf * jax.nn.sigmoid(cf), (16, D)).astype(BF16)
        modv[:, c0:c1] = _dot(sc, _w(wm, 0, D, c0, c1))[0:8]

    def mvec(i):
        return modv[0:1, i * D:(i + 1) * D]

    def ln1(r0, n):
        xf = xv[pl.ds(r0, n), :].astype(F32)
        return _ln(xf) * (1.0 + mvec(1)) + mvec(0)

    def repack(par_g, gi, r0, n, enable=None):
        w = wg[par_g]
        for t in range(0, 3 * HG, 2):
            a = w[gi, t, pl.ds(r0, n), :]
            b = w[gi, t + 1, pl.ds(r0, n), :]
            e = (a & jnp.uint32(0xFFFF)) | (b << 16)
            o = (a >> 16) | (b & jnp.uint32(0xFFFF0000))
            if enable is not None:
                e = jnp.where(enable, e, a)
                o = jnp.where(enable, o, b)
            w[gi, t, pl.ds(r0, n), :] = e
            w[gi, t + 1, pl.ds(r0, n), :] = o

    def ring_store(par_g, gi, t, row, val):
        n = val.shape[0]
        if t < 2 * HG:
            rqk[par_g][gi, pl.ds(row, n), t * DH:(t + 1) * DH] = val.astype(BF16)
        else:
            t -= 2 * HG
            rv[par_g][gi, pl.ds(row, n), t * DH:(t + 1) * DH] = val.astype(BF16)

    def proj(lhs, par_g, gi, rows):
        for t in range(3 * HG):
            r = _dot(lhs, pltpu.bitcast(wg[par_g][gi, t], BF16))
            for i, row in enumerate(rows):
                ring_store(par_g, gi, t, row, r[8 * i:8 * i + 8])

    def attn_qk(par_g, gi, base, q0, nq, nk, allowed, fill):
        qrow = pl.multiple_of(base + q0, 16)
        ps = []
        for hh in range(HG):
            c = hh * DH
            q = rqk[par_g][gi, pl.ds(qrow, nq), c:c + DH]
            k = rqk[par_g][gi, pl.ds(base, nk), GW + c:GW + c + DH]
            s = lax.dot_general(q, k, (((1,), (1,)), ((), ())), preferred_element_type=F32)
            s = jnp.where(allowed, s * scale, fill)
            m = jnp.max(s, axis=-1, keepdims=True)
            p = jnp.exp(s - m)
            l = jnp.sum(p, axis=-1, keepdims=True)
            ps.append((p * (1.0 / l)).astype(BF16))
        return ps

    def attn_pv(g, base, nq, nk, ps):
        for hh in range(HG):
            v = rv[g % 2][g // 2, pl.ds(base, nk), hh * DH:(hh + 1) * DH]
            o = _dot(ps[hh], v)
            col = (g * HG + hh) * DH
            o32[0:nq // 2, col:col + DH] = pltpu.bitcast(o.astype(BF16), U32)

    def wo_proj(nq, stores):
        o = _w(o32, 0, nq, 0, HD)
        cw = 256
        for cb in range(D // cw):
            r = _dot(o, _w(wo, 0, HD, cb * cw, (cb + 1) * cw))
            for r0, n, fn in stores:
                fn(slice(cb * cw, (cb + 1) * cw), r[r0:r0 + n])

    def post_attn(tok0, slot, n):
        x1 = xv[pl.ds(tok0, n), :].astype(F32) + mvec(2) * abuf[pl.ds(slot, n), :]
        yv[0:n, :] = x1
        hh = _ln(x1) * (1.0 + mvec(4)) + mvec(3)
        h2[0:n // 2, :] = pltpu.bitcast(hh.astype(BF16), U32)

    def ffn_up(c0, c1, n):
        a = _w(h2, 0, n, 0, D)
        for c in range(c0, c1):
            gt = _dot(a, _w(w1, 0, D, c * FC, (c + 1) * FC))
            up = _dot(a, _w(w3, 0, D, c * FC, (c + 1) * FC))
            hv = gt * jax.nn.sigmoid(gt) * up
            hid[0:n // 2, c * FC:(c + 1) * FC] = pltpu.bitcast(hv.astype(BF16), U32)

    def ffn_down(tok0, n, cb0, cb1):
        a = _w(hid, 0, n, 0, FF)
        cw = 256
        for cb in range(cb0, cb1):
            cs = slice(cb * cw, (cb + 1) * cw)
            r = _dot(a, _w(w2, 0, FF, cb * cw, (cb + 1) * cw))
            gb = modv[0:1, 5 * D + cb * cw:5 * D + (cb + 1) * cw]
            outv[pl.ds(tok0, n), cs] = (yv[0:n, cs] + gb * r).astype(BF16)

    def unit_row(u):
        r = u % 8
        return pl.multiple_of(((u // 8) % NSLOT) * SLOT + 8 + 8 * r + 8 * (r >= 5).astype(jnp.int32), 8)

    with _scope("wait0"):
        copies["c"].wait()
        copies["wm0"].wait()
    mod_part(0, 2 * D)
    copies["x0"].wait()
    copies["mem0"].wait()

    def ln_body(i, _):
        r0 = pl.multiple_of(i * 64, 64)
        h0[pl.ds(pl.multiple_of(i * 32, 32), 32), :] = pltpu.bitcast(ln1(r0, 64).astype(BF16), U32)
        return 0

    lax.fori_loop(0, PRO // 64, ln_body, 0)
    lhs_a[0:MEM, :] = m0v[...].astype(F32)
    lhs_a[MEM:32, :] = ln1(PRO, 24)

    RB = 128
    NRB = PRO // RB
    RP = D // 2 // NRB
    with _scope("waitg0"):
        wait_group(0, 0)
    repack(0, 0, 0, D // 2)

    def pro_rows(par_g, gi, rp_par, rp_gi, enable=None):
        def body(i, _):
            repack(rp_par, rp_gi, pl.multiple_of(i * RP, RP), RP, enable)
            a = pltpu.bitcast(h0[pl.ds(pl.multiple_of(i * (RB // 2), RB // 2), RB // 2), :], BF16)
            for t in range(3 * HG):
                r = _dot(a, pltpu.bitcast(wg[par_g][gi, t], BF16))
                for pp in range(RB // PT):
                    base = (i * (RB // PT) + pp) * SLOT
                    ring_store(par_g, gi, t, pl.multiple_of(base + 8, 8), r[pp * PT:pp * PT + 40])
                    ring_store(par_g, gi, t, pl.multiple_of(base + 56, 8), r[pp * PT + 40:pp * PT + 64])
            return 0

        lax.fori_loop(0, NRB, body, 0)

    def pro_body(gi, _):
        last = G // 2 - 1

        @pl.when(gi < last)
        def _():
            start_group(0, gi + 1)
            start_group(1, gi + 1)

        @pl.when(gi == last)
        def _():
            copies["w3"].start()

        wait_group(1, gi)
        pro_rows(0, gi, 1, gi)

        for k, names in enumerate((("wo",), ("wm1",), ("w1",), ("w2", "x1"))):
            @pl.when(gi == k)
            def _(names=names):
                for n in names:
                    copies[n].start()

        @pl.when(gi < last)
        def _():
            wait_group(0, gi + 1)

        pro_rows(1, gi, 0, jnp.minimum(gi + 1, last), gi < last)
        return 0

    with _scope("pro"):
        lax.fori_loop(0, G // 2, pro_body, 0)

    def pair(p, with_ffn):
        (al_a, fi_a), (al_b, fi_b) = _masks()
        base = pl.multiple_of((p % NSLOT) * SLOT, 16)
        u0 = PRO // 8 + 6 * p
        tlead = PRO + 48 * p
        aslot = pl.multiple_of((p % LAG) * PT, PT)
        tok_f = pl.multiple_of((p - LAG) * PT, PT)

        if with_ffn:
            post_attn(tok_f, aslot, PT)

        def proj_attn(lhs, rows, q0, nq, nk, allowed, fill, f1, f2):
            ps = None
            for g in range(G):
                proj(lhs, g % 2, g // 2, rows)
                if g > 0:
                    attn_pv(g - 1, base, nq, nk, ps)
                ps = attn_qk(g % 2, g // 2, base, q0, nq, nk, allowed, fill)
            if with_ffn:
                ffn_up(*f1, PT)
            attn_pv(G - 1, base, nq, nk, ps)
            if with_ffn:
                ffn_up(*f2, PT)

        lhs = lhs_a[...].astype(BF16)
        rows = [base, unit_row(u0), unit_row(u0 + 1), unit_row(u0 + 2)]
        lhs_b[MEM:32, :] = ln1(pl.multiple_of(tlead + 24, 8), 24)
        proj_attn(lhs, rows, 0, 32, 48, al_a, fi_a, (0, 2), (2, 4))

        def st_mem_b(cs, val):
            lhs_b[0:MEM, cs] = val.astype(BF16).astype(F32)

        def st_a(r0, n):
            def fn(cs, val):
                abuf[pl.ds(pl.multiple_of(aslot + r0, 8), n), cs] = val
            return fn

        wo_proj(32, [(0, 8, st_mem_b), (8, 24, st_a(0, 24))])
        if with_ffn:
            ffn_up(4, 9, PT)

        lhs = lhs_b[...].astype(BF16)
        rows = [pl.multiple_of(base + 48, 8), unit_row(u0 + 3), unit_row(u0 + 4), unit_row(u0 + 5)]
        nxt = pl.multiple_of(jnp.minimum(tlead + 48, S - 24), 8)
        lhs_a[MEM:32, :] = ln1(nxt, 24)
        proj_attn(lhs, rows, 32, 48, 80, al_b, fi_b, (9, 11), (11, NFC))

        def st_mem_a(cs, val):
            lhs_a[0:MEM, cs] = val.astype(BF16).astype(F32)

        wo_proj(48, [(16, 8, st_mem_a), (0, 16, st_a(24, 16)), (24, 24, st_a(40, 24))])
        if with_ffn:
            ffn_down(tok_f, PT, 0, 4)

    with _scope("waitwo"):
        copies["wo"].wait()

    def pair_noffn(p, _):
        pair(p, False)
        return 0

    with _scope("noffn"):
        if "noffn" not in SKIP:
            lax.fori_loop(0, LAG, pair_noffn, 0)

    with _scope("mod2"):
        copies["wm1"].wait()
        mod_part(2 * D, 6 * D)
    with _scope("waitffn"):
        copies["w1"].wait()
        copies["w3"].wait()
        copies["w2"].wait()
        copies["x1"].wait()

    def pair_ffn(p, _):
        if not NO_LOOP_DMA:
            @pl.when(p > MAIN_START)
            def _():
                out_copy(pl.multiple_of((p - LAG - 1) * PT, PT), PT).start()

        pair(p, True)
        return 0

    with _scope("main"):
        lax.fori_loop(MAIN_START, NPAIR, pair_ffn, 0)

    if NO_LOOP_DMA:
        out_copy((MAIN_START - LAG) * PT, (NPAIR - MAIN_START) * PT).start()
    else:
        out_copy((NPAIR - LAG - 1) * PT, PT).start()
    with _scope("epi"):
        for p in range(NPAIR - LAG, NPAIR):
            if "epi" not in SKIP:
                post_attn(p * PT, (p % LAG) * PT, PT)
                ffn_up(0, NFC, PT)
                ffn_down(p * PT, PT, 0, 4)
            out_copy(p * PT, PT).start()
    with _scope("waitout"):
        out_copy(0, S - (MAIN_START - LAG) * PT).wait()


@functools.partial(jax.jit, static_argnames=("A_seg_len",))
def pallas_adaLN_cond__memory_aug_recurrent_mem_tr__glu_gated_swiglu__prompt_kernel(
    A_x, A_mem0, A_Wq, A_Wk, A_Wv, A_Wo, A_seg_len, B_x, B_w1, B_w3, B_w2, c, w_mod,
):
    assert A_seg_len == SEG
    assert A_x.shape == (1, S, D) and A_mem0.shape == (1, MEM, D)
    assert A_Wq.shape == (D, H, DH) and B_w1.shape == (D, FF)
    del B_x

    n_in_copies = 4 + 6
    scratch = [
        pltpu.VMEM((S, D), BF16),
        pltpu.VMEM((S, D), BF16),
        pltpu.VMEM((HD // 2, D), U32),
        pltpu.VMEM((D // 2, FF), U32),
        pltpu.VMEM((D // 2, FF), U32),
        pltpu.VMEM((FF // 2, D), U32),
        pltpu.VMEM((D // 2, 6 * D), U32),
        pltpu.VMEM((1, D), BF16),
        pltpu.VMEM((MEM, D), BF16),
        pltpu.VMEM((8, 6 * D), F32),
        pltpu.VMEM((PRO // 2, D), U32),
        pltpu.VMEM((32, D), F32),
        pltpu.VMEM((32, D), F32),
        pltpu.VMEM((24, HD), U32),
        pltpu.VMEM((LAG * PT, D), F32),
        pltpu.VMEM((PT, D), F32),
        pltpu.VMEM((PT // 2, D), U32),
        pltpu.VMEM((PT // 2, FF), U32),
        pltpu.SemaphoreType.DMA((n_in_copies,)),
        pltpu.SemaphoreType.DMA((G,)),
        pltpu.SemaphoreType.DMA,
    ] + [pltpu.VMEM((G // 2, NSLOT * SLOT, 2 * GW), BF16)] * 2 + [
        pltpu.VMEM((G // 2, NSLOT * SLOT, GW), BF16)] * 2 + [
        pltpu.VMEM((G // 2, 3 * HG, D // 2, DH), U32)] * 2

    out = pl.pallas_call(
        _kernel,
        out_shape=jax.ShapeDtypeStruct((S, D), BF16),
        in_specs=[pl.BlockSpec(memory_space=pl.ANY)] * 11,
        out_specs=pl.BlockSpec(memory_space=pl.ANY),
        scratch_shapes=scratch,
        compiler_params=pltpu.CompilerParams(vmem_limit_bytes=120 * 1024 * 1024),
    )(
        A_x.reshape(S, D), A_mem0.reshape(MEM, D),
        A_Wq.reshape(D // 2, 2, H, DH), A_Wk.reshape(D // 2, 2, H, DH),
        A_Wv.reshape(D // 2, 2, H, DH), A_Wo.reshape(HD, D),
        B_w1, B_w3, B_w2, c, w_mod,
    )
    return out.reshape(1, S, D)
```

```python
import functools

import jax
import jax.numpy as jnp
from jax import lax
import jax.experimental.pallas as pl
import jax.experimental.pallas.tpu as pltpu

F32 = jnp.float32
BF16 = jnp.bfloat16
U32 = jnp.uint32

S = 2048
D = 1024
H = 32
DH = 128
HD = H * DH
MEM = 8
SEG = 32
FF = 3584
EPS = 1e-5
LOG2E = 1.4426950408889634

G = 8
HG = H // G
GW = HG * DH
PRO = 512
NPAIR = S // (2 * SEG)
PT = 2 * SEG
SLOT = 80
NSLOT = 9
LAG = 2
X0 = 768
FC = 256
NFC = FF // FC
MAIN_START = LAG
SCOPES = False
NO_LOOP_DMA = False
SKIP = ()


class _NoScope:
    def __enter__(self):
        return self

    def __exit__(self, *a):
        return False


def _scope(name):
    return jax.named_scope(name) if SCOPES else _NoScope()


def _w(ref, r0, r1, c0, c1):
    return pltpu.bitcast(ref[r0 // 2:r1 // 2, c0:c1], BF16)


def _dot(a, b):
    return jnp.dot(a, b, preferred_element_type=F32)


def _ln(x):
    m = jnp.mean(x, axis=-1, keepdims=True)
    xc = x - m
    v = jnp.mean(xc * xc, axis=-1, keepdims=True)
    return xc * lax.rsqrt(v + EPS)


def _recip(x):
    r = pl.reciprocal(x, approx=True)
    return r * (2.0 - x * r)


def _silu(x):
    h = 0.5 * x
    return h + h * jnp.tanh(h)


def _masks():
    def pos(j):
        return jnp.where(j < 40, j, jnp.where(j < 48, j - 32, jnp.where(j < 56, j - 48, j - 40)))

    out = []
    for q0, nq, nk in ((0, 32, 48), (32, 48, 80)):
        qi = lax.broadcasted_iota(jnp.int32, (nq, nk), 0) + q0
        kj = lax.broadcasted_iota(jnp.int32, (nq, nk), 1)
        qp, kp = pos(qi), pos(kj)
        same = ((qi < 40) & (kj < 40)) | ((qi >= 40) & (kj >= 40))
        allowed = same & ((qp < MEM) | (qp >= kp))
        fill = jnp.where(same, jnp.float32(-1e9 * DH ** 0.5), jnp.float32(-jnp.inf))
        out.append((allowed, fill))
    return out


def _kernel(x_hbm, mem0_hbm, wq_hbm, wk_hbm, wv_hbm, wo_hbm, w1_hbm, w3_hbm, w2_hbm,
            c_hbm, wm_hbm, out_hbm,
            xv, outv, wo, w1, w3, w2, wm, cv, m0v, modv, h0,
            lhs_a, lhs_b, o32, abuf, yv, h2, hid, sem_in, sem_g, sem_out, *rest):
    rqk = rest[0:2]
    rv = rest[2:4]
    wg = rest[4:6]
    scale = DH ** -0.5

    copies = {}

    def mk(name, src, dst):
        copies[name] = pltpu.make_async_copy(src, dst, sem_in.at[len(copies)])

    def cols(hbm, ref, c0, c1):
        return hbm.bitcast(U32).at[:, c0:c1], ref.at[:, c0:c1]

    mk("c", c_hbm, cv)
    mk("mem0", mem0_hbm, m0v)
    mk("x0", x_hbm.at[0:X0], xv.at[0:X0])
    mk("wm0", *cols(wm_hbm, wm, 0, 2 * D))
    mk("wo", wo_hbm.bitcast(U32), wo)
    mk("wm1", *cols(wm_hbm, wm, 2 * D, 6 * D))
    mk("w1", w1_hbm.bitcast(U32), w1)
    mk("w3", w3_hbm.bitcast(U32), w3)
    mk("w2", w2_hbm.bitcast(U32), w2)
    mk("x1", x_hbm.at[X0:S], xv.at[X0:S])
    def gcopies(par_g, gi):
        lst = []
        for m, hbm in enumerate((wq_hbm, wk_hbm, wv_hbm)):
            for jj in range(HG // 2):
                for par in range(2):
                    lst.append(pltpu.make_async_copy(
                        hbm.bitcast(U32).at[:, par, (2 * gi + par_g) * (HG // 2) + jj],
                        wg[par_g].at[gi, m * HG + 2 * jj + par], sem_g.at[2 * gi + par_g]))
        return lst

    def start_group(par_g, gi):
        for c in gcopies(par_g, gi):
            c.start()

    def wait_group(par_g, gi):
        for c in gcopies(par_g, gi):
            c.wait()

    for n in ("c", "mem0", "x0", "wm0"):
        copies[n].start()
    start_group(0, 0)
    start_group(1, 0)

    def out_copy(r0, n):
        return pltpu.make_async_copy(outv.at[pl.ds(r0, n)], out_hbm.at[pl.ds(r0, n)], sem_out)

    def mod_part(c0, c1):
        cf = cv[...].astype(F32)
        sc = jnp.broadcast_to(_silu(cf), (16, D)).astype(BF16)
        modv[:, c0:c1] = _dot(sc, _w(wm, 0, D, c0, c1))[0:8]

    def mvec(i):
        return modv[0:1, i * D:(i + 1) * D]

    def ln1(r0, n):
        xf = xv[pl.ds(r0, n), :].astype(F32)
        return _ln(xf) * (1.0 + mvec(1)) + mvec(0)

    def repack(par_g, gi, r0, n, enable=None):
        w = wg[par_g]
        for t in range(0, 3 * HG, 2):
            a = w[gi, t, pl.ds(r0, n), :]
            b = w[gi, t + 1, pl.ds(r0, n), :]
            e = (a & jnp.uint32(0xFFFF)) | (b << 16)
            o = (a >> 16) | (b & jnp.uint32(0xFFFF0000))
            if enable is not None:
                e = jnp.where(enable, e, a)
                o = jnp.where(enable, o, b)
            w[gi, t, pl.ds(r0, n), :] = e
            w[gi, t + 1, pl.ds(r0, n), :] = o

    def ring_store(par_g, gi, t, row, val):
        n = val.shape[0]
        if t < 2 * HG:
            rqk[par_g][gi, pl.ds(row, n), t * DH:(t + 1) * DH] = val.astype(BF16)
        else:
            t -= 2 * HG
            rv[par_g][gi, pl.ds(row, n), t * DH:(t + 1) * DH] = val.astype(BF16)

    def proj(lhs, par_g, gi, rows):
        for t in range(3 * HG):
            r = _dot(lhs, pltpu.bitcast(wg[par_g][gi, t], BF16))
            for i, row in enumerate(rows):
                ring_store(par_g, gi, t, row, r[8 * i:8 * i + 8])

    def attn_qk(par_g, gi, base, q0, nq, nk, allowed, fill):
        qrow = pl.multiple_of(base + q0, 16)
        ps = []
        for hh in range(HG):
            c = hh * DH
            q = rqk[par_g][gi, pl.ds(qrow, nq), c:c + DH]
            k = rqk[par_g][gi, pl.ds(base, nk), GW + c:GW + c + DH]
            s = lax.dot_general(q, k, (((1,), (1,)), ((), ())), preferred_element_type=F32)
            s = jnp.where(allowed, s, fill)
            m = jnp.max(s, axis=-1, keepdims=True)
            p = jnp.exp2((s - m) * (scale * LOG2E))
            l = jnp.sum(p, axis=-1, keepdims=True)
            ps.append((p * _recip(l)).astype(BF16))
        return ps

    def attn_pv(g, base, nq, nk, ps):
        for hh in range(HG):
            v = rv[g % 2][g // 2, pl.ds(base, nk), hh * DH:(hh + 1) * DH]
            o = _dot(ps[hh], v)
            col = (g * HG + hh) * DH
            o32[0:nq // 2, col:col + DH] = pltpu.bitcast(o.astype(BF16), U32)

    def wo_proj(nq, stores):
        o = _w(o32, 0, nq, 0, HD)
        cw = 256
        for cb in range(D // cw):
            r = _dot(o, _w(wo, 0, HD, cb * cw, (cb + 1) * cw))
            for r0, n, fn in stores:
                fn(slice(cb * cw, (cb + 1) * cw), r[r0:r0 + n])

    def post_attn(tok0, slot, n):
        x1 = xv[pl.ds(tok0, n), :].astype(F32) + mvec(2) * abuf[pl.ds(slot, n), :]
        yv[0:n, :] = x1
        hh = _ln(x1) * (1.0 + mvec(4)) + mvec(3)
        h2[0:n // 2, :] = pltpu.bitcast(hh.astype(BF16), U32)

    def ffn_up(c0, c1, n):
        a = _w(h2, 0, n, 0, D)
        for c in range(c0, c1):
            gt = _dot(a, _w(w1, 0, D, c * FC, (c + 1) * FC))
            up = _dot(a, _w(w3, 0, D, c * FC, (c + 1) * FC))
            hv = _silu(gt) * up
            hid[0:n // 2, c * FC:(c + 1) * FC] = pltpu.bitcast(hv.astype(BF16), U32)

    def ffn_down(tok0, n, cb0, cb1):
        a = _w(hid, 0, n, 0, FF)
        cw = 256
        for cb in range(cb0, cb1):
            cs = slice(cb * cw, (cb + 1) * cw)
            r = _dot(a, _w(w2, 0, FF, cb * cw, (cb + 1) * cw))
            gb = modv[0:1, 5 * D + cb * cw:5 * D + (cb + 1) * cw]
            outv[pl.ds(tok0, n), cs] = (yv[0:n, cs] + gb * r).astype(BF16)

    def unit_row(u):
        r = u % 8
        return pl.multiple_of(((u // 8) % NSLOT) * SLOT + 8 + 8 * r + 8 * (r >= 5).astype(jnp.int32), 8)

    with _scope("wait0"):
        copies["c"].wait()
        copies["wm0"].wait()
    mod_part(0, 2 * D)
    copies["x0"].wait()
    copies["mem0"].wait()

    def ln_body(i, _):
        r0 = pl.multiple_of(i * 64, 64)
        h0[pl.ds(pl.multiple_of(i * 32, 32), 32), :] = pltpu.bitcast(ln1(r0, 64).astype(BF16), U32)
        return 0

    lax.fori_loop(0, PRO // 64, ln_body, 0)
    lhs_a[0:MEM, :] = m0v[...].astype(F32)
    lhs_a[MEM:32, :] = ln1(PRO, 24)

    RB = 128
    NRB = PRO // RB
    RP = D // 2 // NRB
    with _scope("waitg0"):
        wait_group(0, 0)
    repack(0, 0, 0, D // 2)

    def pro_rows(par_g, gi, rp_par, rp_gi, enable=None):
        def body(i, _):
            repack(rp_par, rp_gi, pl.multiple_of(i * RP, RP), RP, enable)
            a = pltpu.bitcast(h0[pl.ds(pl.multiple_of(i * (RB // 2), RB // 2), RB // 2), :], BF16)
            for t in range(3 * HG):
                r = _dot(a, pltpu.bitcast(wg[par_g][gi, t], BF16))
                for pp in range(RB // PT):
                    base = (i * (RB // PT) + pp) * SLOT
                    ring_store(par_g, gi, t, pl.multiple_of(base + 8, 8), r[pp * PT:pp * PT + 40])
                    ring_store(par_g, gi, t, pl.multiple_of(base + 56, 8), r[pp * PT + 40:pp * PT + 64])
            return 0

        lax.fori_loop(0, NRB, body, 0)

    def pro_body(gi, _):
        last = G // 2 - 1

        @pl.when(gi < last)
        def _():
            start_group(0, gi + 1)
            start_group(1, gi + 1)

        @pl.when(gi == last)
        def _():
            copies["w3"].start()

        wait_group(1, gi)
        pro_rows(0, gi, 1, gi)

        for k, names in enumerate((("wo",), ("wm1",), ("w1",), ("w2", "x1"))):
            @pl.when(gi == k)
            def _(names=names):
                for n in names:
                    copies[n].start()

        @pl.when(gi < last)
        def _():
            wait_group(0, gi + 1)

        pro_rows(1, gi, 0, jnp.minimum(gi + 1, last), gi < last)
        return 0

    with _scope("pro"):
        lax.fori_loop(0, G // 2, pro_body, 0)

    def pair(p, with_ffn):
        (al_a, fi_a), (al_b, fi_b) = _masks()
        base = pl.multiple_of((p % NSLOT) * SLOT, 16)
        u0 = PRO // 8 + 6 * p
        tlead = PRO + 48 * p
        aslot = pl.multiple_of((p % LAG) * PT, PT)
        tok_f = pl.multiple_of((p - LAG) * PT, PT)

        if with_ffn:
            post_attn(tok_f, aslot, PT)

        def proj_attn(lhs, rows, q0, nq, nk, allowed, fill, f1, f2):
            ps = None
            for g in range(G):
                proj(lhs, g % 2, g // 2, rows)
                if g > 0:
                    attn_pv(g - 1, base, nq, nk, ps)
                ps = attn_qk(g % 2, g // 2, base, q0, nq, nk, allowed, fill)
            if with_ffn:
                ffn_up(*f1, PT)
            attn_pv(G - 1, base, nq, nk, ps)
            if with_ffn:
                ffn_up(*f2, PT)

        lhs = lhs_a[...].astype(BF16)
        rows = [base, unit_row(u0), unit_row(u0 + 1), unit_row(u0 + 2)]
        lhs_b[MEM:32, :] = ln1(pl.multiple_of(tlead + 24, 8), 24)
        proj_attn(lhs, rows, 0, 32, 48, al_a, fi_a, (0, 2), (2, 4))

        def st_mem_b(cs, val):
            lhs_b[0:MEM, cs] = val.astype(BF16).astype(F32)

        def st_a(r0, n):
            def fn(cs, val):
                abuf[pl.ds(pl.multiple_of(aslot + r0, 8), n), cs] = val
            return fn

        wo_proj(32, [(0, 8, st_mem_b), (8, 24, st_a(0, 24))])
        if with_ffn:
            ffn_up(4, 9, PT)

        lhs = lhs_b[...].astype(BF16)
        rows = [pl.multiple_of(base + 48, 8), unit_row(u0 + 3), unit_row(u0 + 4), unit_row(u0 + 5)]
        nxt = pl.multiple_of(jnp.minimum(tlead + 48, S - 24), 8)
        lhs_a[MEM:32, :] = ln1(nxt, 24)
        proj_attn(lhs, rows, 32, 48, 80, al_b, fi_b, (9, 11), (11, NFC))

        def st_mem_a(cs, val):
            lhs_a[0:MEM, cs] = val.astype(BF16).astype(F32)

        wo_proj(48, [(16, 8, st_mem_a), (0, 16, st_a(24, 16)), (24, 24, st_a(40, 24))])
        if with_ffn:
            ffn_down(tok_f, PT, 0, 4)

    with _scope("waitwo"):
        copies["wo"].wait()

    def pair_noffn(p, _):
        pair(p, False)
        return 0

    with _scope("noffn"):
        if "noffn" not in SKIP:
            lax.fori_loop(0, LAG, pair_noffn, 0)

    with _scope("mod2"):
        copies["wm1"].wait()
        mod_part(2 * D, 6 * D)
    with _scope("waitffn"):
        copies["w1"].wait()
        copies["w3"].wait()
        copies["w2"].wait()
        copies["x1"].wait()

    def pair_ffn(p, _):
        if not NO_LOOP_DMA:
            @pl.when(p > MAIN_START)
            def _():
                out_copy(pl.multiple_of((p - LAG - 1) * PT, PT), PT).start()

        pair(p, True)
        return 0

    with _scope("main"):
        lax.fori_loop(MAIN_START, NPAIR, pair_ffn, 0)

    if NO_LOOP_DMA:
        out_copy((MAIN_START - LAG) * PT, (NPAIR - MAIN_START) * PT).start()
    else:
        out_copy((NPAIR - LAG - 1) * PT, PT).start()
    with _scope("epi"):
        for p in range(NPAIR - LAG, NPAIR):
            if "epi" not in SKIP:
                post_attn(p * PT, (p % LAG) * PT, PT)
                ffn_up(0, NFC, PT)
                ffn_down(p * PT, PT, 0, 4)
            out_copy(p * PT, PT).start()
    with _scope("waitout"):
        out_copy(0, S - (MAIN_START - LAG) * PT).wait()


@functools.partial(jax.jit, static_argnames=("A_seg_len",))
def pallas_adaLN_cond__memory_aug_recurrent_mem_tr__glu_gated_swiglu__prompt_kernel(
    A_x, A_mem0, A_Wq, A_Wk, A_Wv, A_Wo, A_seg_len, B_x, B_w1, B_w3, B_w2, c, w_mod,
):
    assert A_seg_len == SEG
    assert A_x.shape == (1, S, D) and A_mem0.shape == (1, MEM, D)
    assert A_Wq.shape == (D, H, DH) and B_w1.shape == (D, FF)
    del B_x

    n_in_copies = 4 + 6
    scratch = [
        pltpu.VMEM((S, D), BF16),
        pltpu.VMEM((S, D), BF16),
        pltpu.VMEM((HD // 2, D), U32),
        pltpu.VMEM((D // 2, FF), U32),
        pltpu.VMEM((D // 2, FF), U32),
        pltpu.VMEM((FF // 2, D), U32),
        pltpu.VMEM((D // 2, 6 * D), U32),
        pltpu.VMEM((1, D), BF16),
        pltpu.VMEM((MEM, D), BF16),
        pltpu.VMEM((8, 6 * D), F32),
        pltpu.VMEM((PRO // 2, D), U32),
        pltpu.VMEM((32, D), F32),
        pltpu.VMEM((32, D), F32),
        pltpu.VMEM((24, HD), U32),
        pltpu.VMEM((LAG * PT, D), F32),
        pltpu.VMEM((PT, D), F32),
        pltpu.VMEM((PT // 2, D), U32),
        pltpu.VMEM((PT // 2, FF), U32),
        pltpu.SemaphoreType.DMA((n_in_copies,)),
        pltpu.SemaphoreType.DMA((G,)),
        pltpu.SemaphoreType.DMA,
    ] + [pltpu.VMEM((G // 2, NSLOT * SLOT, 2 * GW), BF16)] * 2 + [
        pltpu.VMEM((G // 2, NSLOT * SLOT, GW), BF16)] * 2 + [
        pltpu.VMEM((G // 2, 3 * HG, D // 2, DH), U32)] * 2

    out = pl.pallas_call(
        _kernel,
        out_shape=jax.ShapeDtypeStruct((S, D), BF16),
        in_specs=[pl.BlockSpec(memory_space=pl.ANY)] * 11,
        out_specs=pl.BlockSpec(memory_space=pl.ANY),
        scratch_shapes=scratch,
        compiler_params=pltpu.CompilerParams(vmem_limit_bytes=120 * 1024 * 1024),
    )(
        A_x.reshape(S, D), A_mem0.reshape(MEM, D),
        A_Wq.reshape(D // 2, 2, H, DH), A_Wk.reshape(D // 2, 2, H, DH),
        A_Wv.reshape(D // 2, 2, H, DH), A_Wo.reshape(HD, D),
        B_w1, B_w3, B_w2, c, w_mod,
    )
    return out.reshape(1, S, D)
```

```python
import functools

import jax
import jax.numpy as jnp
from jax import lax
import jax.experimental.pallas as pl
import jax.experimental.pallas.tpu as pltpu

F32 = jnp.float32
BF16 = jnp.bfloat16
U32 = jnp.uint32

S = 2048
D = 1024
H = 32
DH = 128
HD = H * DH
MEM = 8
SEG = 32
FF = 3584
EPS = 1e-5
LOG2E = 1.4426950408889634

G = 8
HG = H // G
GW = HG * DH
PRO = 512
NPAIR = S // (2 * SEG)
PT = 2 * SEG
SLOT = 80
NSLOT = 9
LAG = 1
X0 = 544
X1 = 800
NM0 = 4
M0W = 2 * D // NM0
FILL = (0, 2, 4, 9, 11, 14)
EPI_UP = 7
EPI_DOWN = 2
J0 = 7
FC = 256
NFC = FF // FC
MAIN_START = LAG
SCOPES = False
NO_LOOP_DMA = False
SKIP = ()


class _NoScope:
    def __enter__(self):
        return self

    def __exit__(self, *a):
        return False


def _scope(name):
    return jax.named_scope(name) if SCOPES else _NoScope()


def _w(ref, r0, r1, c0, c1):
    return pltpu.bitcast(ref[r0 // 2:r1 // 2, c0:c1], BF16)


def _dot(a, b):
    return jnp.dot(a, b, preferred_element_type=F32)


def _ln(x):
    m = jnp.mean(x, axis=-1, keepdims=True)
    xc = x - m
    v = jnp.mean(xc * xc, axis=-1, keepdims=True)
    return xc * lax.rsqrt(v + EPS)


def _recip(x):
    r = pl.reciprocal(x, approx=True)
    return r * (2.0 - x * r)


def _silu(x):
    h = 0.5 * x
    return h + h * jnp.tanh(h)


def _masks():
    def pos(j):
        return jnp.where(j < 40, j, jnp.where(j < 48, j - 32, jnp.where(j < 56, j - 48, j - 40)))

    out = []
    for q0, nq, nk in ((0, 32, 48), (32, 48, 80)):
        qi = lax.broadcasted_iota(jnp.int32, (nq, nk), 0) + q0
        kj = lax.broadcasted_iota(jnp.int32, (nq, nk), 1)
        qp, kp = pos(qi), pos(kj)
        same = ((qi < 40) & (kj < 40)) | ((qi >= 40) & (kj >= 40))
        allowed = same & ((qp < MEM) | (qp >= kp))
        fill = jnp.where(same, jnp.float32(-1e9 * DH ** 0.5), jnp.float32(-jnp.inf))
        out.append((allowed, fill))
    return out


def _kernel(x_hbm, mem0_hbm, wq_hbm, wk_hbm, wv_hbm, wo_hbm, w1_hbm, w3_hbm, w2_hbm,
            c_hbm, wm_hbm, out_hbm,
            xv, outv, wo, w1, w3, w2, wm, cv, m0v, modv, xh, h0,
            lhs_a, lhs_b, o32, abuf, yv, h2, hid, sem_in, sem_k, sem_out, *rest):
    rqk = rest[0:2]
    rv = rest[2:4]
    wg = rest[4:6]
    scale = DH ** -0.5

    copies = {}

    def mk(name, src, dst):
        copies[name] = pltpu.make_async_copy(src, dst, sem_in.at[len(copies)])

    def cols(hbm, ref, c0, c1):
        return hbm.bitcast(U32).at[:, c0:c1], ref.at[:, c0:c1]

    mk("c", c_hbm, cv)
    mk("mem0", mem0_hbm, m0v)
    mk("x0", x_hbm.at[0:X0], xv.at[0:X0])
    for i in range(NM0):
        mk(f"wm0{i}", *cols(wm_hbm, wm, i * M0W, (i + 1) * M0W))
    mk("x1", x_hbm.at[X0:X1], xv.at[X0:X1])
    mk("wo", wo_hbm.bitcast(U32), wo)
    mk("wm1", *cols(wm_hbm, wm, 2 * D, 6 * D))
    mk("w1", w1_hbm.bitcast(U32), w1)
    mk("w3", w3_hbm.bitcast(U32), w3)
    mk("w2", w2_hbm.bitcast(U32), w2)
    mk("x2", x_hbm.at[X1:S], xv.at[X1:S])

    w_hbm = (wq_hbm, wk_hbm, wv_hbm)

    def chunk_copies(k, gi, m, t0, jj):
        return [
            pltpu.make_async_copy(
                w_hbm[m].bitcast(U32).at[:, par, (2 * gi + pg) * (HG // 2) + jj],
                wg[pg].at[gi, t0 + par], sem_k.at[k])
            for pg in range(2) for par in range(2)]

    def start_chunks(j, m):
        gi = j >> 1 if m < 2 else j - G
        for jj in range(HG // 2):
            for c in chunk_copies(2 * j + jj, gi, m, m * HG + 2 * jj, jj):
                c.start()

    def chunk_pos(k):
        is_v = k >= 2 * G
        gi = jnp.where(is_v, (k >> 1) - G, k >> 2)
        t0 = jnp.where(is_v, 2 * HG + 2 * (k & 1), 2 * (k & 3))
        return gi, t0

    def wait_chunk(k, gi, t0):
        for c in chunk_copies(k, gi, 0, t0, 0):
            c.wait()

    for n in ["c", "mem0", "x0"] + [f"wm0{i}" for i in range(NM0)]:
        copies[n].start()
    for j in range(J0):
        start_chunks(j, j % 2)

    def out_copy(r0, n):
        return pltpu.make_async_copy(outv.at[pl.ds(r0, n)], out_hbm.at[pl.ds(r0, n)], sem_out)

    def mod_part(c0, c1):
        cf = cv[...].astype(F32)
        sc = jnp.broadcast_to(_silu(cf), (16, D)).astype(BF16)
        modv[:, c0:c1] = _dot(sc, _w(wm, 0, D, c0, c1))[0:8]

    def mvec(i):
        return modv[0:1, i * D:(i + 1) * D]

    def ln1(r0, n):
        xf = xv[pl.ds(r0, n), :].astype(F32)
        return _ln(xf) * (1.0 + mvec(1)) + mvec(0)

    def repack(gi, t0, enable=None):
        for w in wg:
            for r0 in range(0, D // 2, 32):
                a = w[gi, t0, r0:r0 + 32, :]
                b = w[gi, t0 + 1, r0:r0 + 32, :]
                e = (a & jnp.uint32(0xFFFF)) | (b << 16)
                o = (a >> 16) | (b & jnp.uint32(0xFFFF0000))
                if enable is not None:
                    e = jnp.where(enable, e, a)
                    o = jnp.where(enable, o, b)
                w[gi, t0, r0:r0 + 32, :] = e
                w[gi, t0 + 1, r0:r0 + 32, :] = o

    def proj(lhs, pg, gi, rows):
        for t in range(3 * HG):
            r = _dot(lhs, pltpu.bitcast(wg[pg][gi, t], BF16))
            dst, td = (rqk[pg], t) if t < 2 * HG else (rv[pg], t - 2 * HG)
            for i, row in enumerate(rows):
                dst[gi, td, pl.ds(row, 8), :] = r[8 * i:8 * i + 8].astype(BF16)

    def attn_qk(par_g, gi, base, q0, nq, nk, allowed, fill):
        qrow = pl.multiple_of(base + q0, 16)
        ps = []
        for hh in range(HG):
            q = rqk[par_g][gi, hh, pl.ds(qrow, nq), :]
            k = rqk[par_g][gi, HG + hh, pl.ds(base, nk), :]
            s = lax.dot_general(q, k, (((1,), (1,)), ((), ())), preferred_element_type=F32)
            s = jnp.where(allowed, s, fill)
            m = jnp.max(s, axis=-1, keepdims=True)
            p = jnp.exp2((s - m) * (scale * LOG2E))
            l = jnp.sum(p, axis=-1, keepdims=True)
            ps.append((p * _recip(l)).astype(BF16))
        return ps

    def attn_pv(g, base, nq, nk, ps):
        for hh in range(HG):
            v = rv[g % 2][g // 2, hh, pl.ds(base, nk), :]
            o = _dot(ps[hh], v)
            col = (g * HG + hh) * DH
            o32[0:nq // 2, col:col + DH] = pltpu.bitcast(o.astype(BF16), U32)

    def wo_proj(nq, stores):
        o = _w(o32, 0, nq, 0, HD)
        cw = 256
        for cb in range(D // cw):
            r = _dot(o, _w(wo, 0, HD, cb * cw, (cb + 1) * cw))
            for r0, n, fn in stores:
                fn(slice(cb * cw, (cb + 1) * cw), r[r0:r0 + n])

    def post_attn(tok0, slot, n):
        x1 = xv[pl.ds(tok0, n), :].astype(F32) + mvec(2) * abuf[pl.ds(slot, n), :]
        yv[0:n, :] = x1
        hh = _ln(x1) * (1.0 + mvec(4)) + mvec(3)
        h2[0:n // 2, :] = pltpu.bitcast(hh.astype(BF16), U32)

    def cslice(off, c, w):
        if isinstance(off, int):
            return slice(off + c * w, off + (c + 1) * w)
        return pl.ds(pl.multiple_of(off + c * w, w), w)

    def ffn_up(c0, c1, n, off=0):
        a = _w(h2, 0, n, 0, D)
        for c in range(c0, c1):
            cs = cslice(off, c, FC)
            gt = _dot(a, pltpu.bitcast(w1[:, cs], BF16))
            up = _dot(a, pltpu.bitcast(w3[:, cs], BF16))
            hv = _silu(gt) * up
            hid[0:n // 2, cs] = pltpu.bitcast(hv.astype(BF16), U32)

    def ffn_down(tok0, n, cb0, cb1, off=0):
        a = _w(hid, 0, n, 0, FF)
        cw = 256
        for cb in range(cb0, cb1):
            cs = cslice(off, cb, cw)
            r = _dot(a, pltpu.bitcast(w2[:, cs], BF16))
            gb = modv[0:1, cslice(off + 5 * D, cb, cw)]
            outv[pl.ds(tok0, n), cs] = (yv[0:n, cs] + gb * r).astype(BF16)

    def unit_row(u):
        r = u & 7
        slot = lax.rem(u >> 3, NSLOT)
        return pl.multiple_of(slot * SLOT + 8 + 8 * r + 8 * (r >= 5).astype(jnp.int32), 8)

    with _scope("waitx0"):
        copies["x0"].wait()
    with _scope("ln0"):

        def ln_body(i, _):
            r0 = pl.multiple_of(i * 32, 32)
            xh[pl.ds(r0, 32), :] = _ln(xv[pl.ds(r0, 32), :].astype(F32))
            return 0

        lax.fori_loop(0, X0 // 32, ln_body, 0)
        copies["c"].wait()
        copies["mem0"].wait()
        lhs_a[0:MEM, :] = m0v[...].astype(F32)

    with _scope("mod0"):
        for i in range(NM0):
            with _scope(f"waitwm{i}"):
                copies[f"wm0{i}"].wait()
            mod_part(i * M0W, (i + 1) * M0W)

    with _scope("modulate"):
        def mod_body(i, _):
            hh = xh[pl.ds(pl.multiple_of(i * 128, 128), 128), :] * (1.0 + mvec(1)) + mvec(0)
            h0[pl.ds(pl.multiple_of(i * 64, 64), 64), :] = pltpu.bitcast(hh.astype(BF16), U32)
            return 0

        lax.fori_loop(0, PRO // 128, mod_body, 0)
        lhs_a[MEM:32, :] = xh[PRO:PRO + 24, :] * (1.0 + mvec(1)) + mvec(0)

    with _scope("first"):
        wait_chunk(0, 0, 0)
        repack(0, 0)

    def pro_body(k, is_v):
        last = 3 * G - 1
        kn = jnp.minimum(k + 1, last)
        gn, tn = chunk_pos(kn)
        if is_v:
            prefetch = k < last
        else:
            prefetch = k > 0

            @pl.when(k == 1)
            def _():
                wait_chunk(1, 0, 2)
                repack(0, 2)

        @pl.when(prefetch)
        def _():
            wait_chunk(kn, gn, tn)

        gi, t0 = chunk_pos(k)
        a = pltpu.bitcast(h0[...], BF16)
        for pg in range(2):
            dst, td = (rv[pg], t0 - 2 * HG) if is_v else (rqk[pg], t0)
            for d in range(2):
                r = _dot(a, pltpu.bitcast(wg[pg][gi, t0 + d], BF16))
                for pp in range(PRO // PT):
                    dst[gi, td + d, pp * SLOT + 8:pp * SLOT + 48, :] = (
                        r[pp * PT:pp * PT + 40].astype(BF16))
                    dst[gi, td + d, pp * SLOT + 56:pp * SLOT + 80, :] = (
                        r[pp * PT + 40:pp * PT + 64].astype(BF16))
        repack(jnp.where(prefetch, gn, gi), jnp.where(prefetch, tn, t0), prefetch)
        return 0

    def pro_outer(o, _):
        @pl.when(o == 1)
        def _():
            for j in range(J0, G + G // 2):
                start_chunks(j, j % 2 if j < G else 2)

        @pl.when(o == 2)
        def _():
            for n in ("x1", "wo", "wm1", "w1", "w3", "w2", "x2"):
                copies[n].start()

        lax.fori_loop(4 * o, 4 * o + 4, lambda k, _: pro_body(k, False), 0)
        return 0

    with _scope("pro"):
        lax.fori_loop(0, G // 2, pro_outer, 0)
        lax.fori_loop(2 * G, 3 * G, lambda k, _: pro_body(k, True), 0)

    def pair(p, with_ffn, with_mod=False):
        (al_a, fi_a), (al_b, fi_b) = _masks()
        base = pl.multiple_of(lax.rem(p, NSLOT) * SLOT, 16)
        u0 = PRO // 8 + 6 * p
        tlead = PRO + 48 * p
        aslot = pl.multiple_of(lax.rem(p, LAG) * PT, PT)
        tok_f = pl.multiple_of((p - LAG) * PT, PT)

        if with_ffn:
            post_attn(tok_f, aslot, PT)

        def filler(i):
            if with_ffn:
                if i < 5:
                    ffn_up(FILL[i], FILL[i + 1], PT)
                else:
                    ffn_down(tok_f, PT, 0, 4)
            elif with_mod and i in (0, 2, 3, 4):
                c0 = (2 + (0, 0, 1, 2, 3)[i]) * D
                mod_part(c0, c0 + D)

        def proj_attn(lhs, rows, q0, nq, nk, allowed, fill, f):
            ps = None
            for g in range(G):
                proj(lhs, g % 2, g // 2, rows)
                if g > 0:
                    attn_pv(g - 1, base, nq, nk, ps)
                ps = attn_qk(g % 2, g // 2, base, q0, nq, nk, allowed, fill)
            filler(f)
            attn_pv(G - 1, base, nq, nk, ps)
            filler(f + 1)

        lhs = lhs_a[...].astype(BF16)
        rows = [base, unit_row(u0), unit_row(u0 + 1), unit_row(u0 + 2)]
        lhs_b[MEM:32, :] = ln1(pl.multiple_of(tlead + 24, 8), 24)
        proj_attn(lhs, rows, 0, 32, 48, al_a, fi_a, 0)

        def st_mem_b(cs, val):
            lhs_b[0:MEM, cs] = val.astype(BF16).astype(F32)

        def st_a(r0, n):
            def fn(cs, val):
                abuf[pl.ds(pl.multiple_of(aslot + r0, 8), n), cs] = val
            return fn

        wo_proj(32, [(0, 8, st_mem_b), (8, 24, st_a(0, 24))])
        filler(2)

        lhs = lhs_b[...].astype(BF16)
        rows = [pl.multiple_of(base + 48, 8), unit_row(u0 + 3), unit_row(u0 + 4), unit_row(u0 + 5)]
        nxt = pl.multiple_of(jnp.minimum(tlead + 48, S - 24), 8)
        lhs_a[MEM:32, :] = ln1(nxt, 24)
        proj_attn(lhs, rows, 32, 48, 80, al_b, fi_b, 3)

        def st_mem_a(cs, val):
            lhs_a[0:MEM, cs] = val.astype(BF16).astype(F32)

        wo_proj(48, [(16, 8, st_mem_a), (0, 16, st_a(24, 16)), (24, 24, st_a(40, 24))])
        filler(5)

    with _scope("waitwo"):
        copies["x1"].wait()
        copies["wo"].wait()
        copies["wm1"].wait()

    with _scope("noffn"):
        if LAG == 1:
            pair(jnp.int32(0), False, True)
        else:
            def pair_noffn(p, _):
                pair(p, False, True)
                return 0

            lax.fori_loop(0, LAG, pair_noffn, 0)

    with _scope("waitffn"):
        copies["w1"].wait()
        copies["w3"].wait()
        copies["w2"].wait()

    def pair_ffn(p, _):
        @pl.when(p == MAIN_START + 2)
        def _():
            copies["x2"].wait()

        if not NO_LOOP_DMA:
            @pl.when(p > MAIN_START)
            def _():
                out_copy(pl.multiple_of((p - LAG - 1) * PT, PT), PT).start()

        pair(p, True)
        return 0

    with _scope("main"):
        lax.fori_loop(MAIN_START, NPAIR, pair_ffn, 0)

    if NO_LOOP_DMA:
        out_copy((MAIN_START - LAG) * PT, (NPAIR - MAIN_START) * PT).start()
    else:
        out_copy((NPAIR - LAG - 1) * PT, PT).start()
    with _scope("epi"):
        n = LAG * PT
        tok0 = S - n
        assert (NPAIR - LAG) % LAG == 0
        post_attn(tok0, 0, n)

        def up_body(i, _):
            ffn_up(0, EPI_UP, n, i * (EPI_UP * FC))
            return 0

        def down_body(i, _):
            ffn_down(tok0, n, 0, EPI_DOWN, i * (EPI_DOWN * 256))
            return 0

        lax.fori_loop(0, NFC // EPI_UP, up_body, 0)
        lax.fori_loop(0, 4 // EPI_DOWN, down_body, 0)
        out_copy(tok0, n).start()
    with _scope("waitout"):
        out_copy(0, S - (MAIN_START - LAG) * PT).wait()


@functools.partial(jax.jit, static_argnames=("A_seg_len",))
def pallas_adaLN_cond__memory_aug_recurrent_mem_tr__glu_gated_swiglu__prompt_kernel(
    A_x, A_mem0, A_Wq, A_Wk, A_Wv, A_Wo, A_seg_len, B_x, B_w1, B_w3, B_w2, c, w_mod,
):
    assert A_seg_len == SEG
    assert A_x.shape == (1, S, D) and A_mem0.shape == (1, MEM, D)
    assert A_Wq.shape == (D, H, DH) and B_w1.shape == (D, FF)
    del B_x

    n_in_copies = 3 + NM0 + 7
    scratch = [
        pltpu.VMEM((S, D), BF16),
        pltpu.VMEM((S, D), BF16),
        pltpu.VMEM((HD // 2, D), U32),
        pltpu.VMEM((D // 2, FF), U32),
        pltpu.VMEM((D // 2, FF), U32),
        pltpu.VMEM((FF // 2, D), U32),
        pltpu.VMEM((D // 2, 6 * D), U32),
        pltpu.VMEM((1, D), BF16),
        pltpu.VMEM((MEM, D), BF16),
        pltpu.VMEM((8, 6 * D), F32),
        pltpu.VMEM((X0, D), F32),
        pltpu.VMEM((PRO // 2, D), U32),
        pltpu.VMEM((32, D), F32),
        pltpu.VMEM((32, D), F32),
        pltpu.VMEM((24, HD), U32),
        pltpu.VMEM((LAG * PT, D), F32),
        pltpu.VMEM((LAG * PT, D), F32),
        pltpu.VMEM((LAG * PT // 2, D), U32),
        pltpu.VMEM((LAG * PT // 2, FF), U32),
        pltpu.SemaphoreType.DMA((n_in_copies,)),
        pltpu.SemaphoreType.DMA((3 * G,)),
        pltpu.SemaphoreType.DMA,
    ] + [pltpu.VMEM((G // 2, 2 * HG, NSLOT * SLOT, DH), BF16)] * 2 + [
        pltpu.VMEM((G // 2, HG, NSLOT * SLOT, DH), BF16)] * 2 + [
        pltpu.VMEM((G // 2, 3 * HG, D // 2, DH), U32)] * 2

    out = pl.pallas_call(
        _kernel,
        out_shape=jax.ShapeDtypeStruct((S, D), BF16),
        in_specs=[pl.BlockSpec(memory_space=pl.ANY)] * 11,
        out_specs=pl.BlockSpec(memory_space=pl.ANY),
        scratch_shapes=scratch,
        compiler_params=pltpu.CompilerParams(
            vmem_limit_bytes=120 * 1024 * 1024, disable_bounds_checks=True),
    )(
        A_x.reshape(S, D), A_mem0.reshape(MEM, D),
        A_Wq.reshape(D // 2, 2, H, DH), A_Wk.reshape(D // 2, 2, H, DH),
        A_Wv.reshape(D // 2, 2, H, DH), A_Wo.reshape(HD, D),
        B_w1, B_w3, B_w2, c, w_mod,
    )
    return out.reshape(1, S, D)
```

```python
import functools

import jax
import jax.numpy as jnp
from jax import lax
import jax.experimental.pallas as pl
import jax.experimental.pallas.tpu as pltpu

F32 = jnp.float32
BF16 = jnp.bfloat16
U32 = jnp.uint32

S = 2048
D = 1024
H = 32
DH = 128
HD = H * DH
MEM = 8
SEG = 32
FF = 3584
EPS = 1e-5
LOG2E = 1.4426950408889634

G = 8
HG = H // G
GW = HG * DH
PRO = 512
NPAIR = S // (2 * SEG)
PT = 2 * SEG
SLOT = 80
NSLOT = 9
LAG = 1
X0 = 544
X1 = 800
NM0 = 4
M0W = 2 * D // NM0
FILL = (0, 2, 4, 9, 11, 14)
EPI_UP = 7
EPI_DOWN = 2
J0 = 7
FC = 256
NFC = FF // FC
MAIN_START = LAG
SCOPES = False
NO_LOOP_DMA = False
SKIP = ()
DBG_STATIC = False


class _NoScope:
    def __enter__(self):
        return self

    def __exit__(self, *a):
        return False


def _scope(name):
    return jax.named_scope(name) if SCOPES else _NoScope()


def _w(ref, r0, r1, c0, c1):
    return pltpu.bitcast(ref[r0 // 2:r1 // 2, c0:c1], BF16)


def _pack(x):
    return pltpu.bitcast(x.astype(BF16), U32)


def _dot(a, b):
    return jnp.dot(a, b, preferred_element_type=F32)


def _ln(x):
    m = jnp.mean(x, axis=-1, keepdims=True)
    xc = x - m
    v = jnp.mean(xc * xc, axis=-1, keepdims=True)
    return xc * lax.rsqrt(v + EPS)


def _recip(x):
    r = pl.reciprocal(x, approx=True)
    return r * (2.0 - x * r)


def _silu(x):
    h = 0.5 * x
    return h + h * jnp.tanh(h)


def _masks():
    def pos(j):
        return jnp.where(j < 40, j, jnp.where(j < 48, j - 32, jnp.where(j < 56, j - 48, j - 40)))

    out = []
    for q0, nq, nk in ((0, 32, 48), (32, 48, 80)):
        qi = lax.broadcasted_iota(jnp.int32, (nq, nk), 0) + q0
        kj = lax.broadcasted_iota(jnp.int32, (nq, nk), 1)
        qp, kp = pos(qi), pos(kj)
        same = ((qi < 40) & (kj < 40)) | ((qi >= 40) & (kj >= 40))
        allowed = same & ((qp < MEM) | (qp >= kp))
        fill = jnp.where(same, jnp.float32(-1e9 * DH ** 0.5), jnp.float32(-jnp.inf))
        out.append((allowed, fill))
    return out


def _kernel(x_hbm, mem0_hbm, wq_hbm, wk_hbm, wv_hbm, wo_hbm, w1_hbm, w3_hbm, w2_hbm,
            c_hbm, wm_hbm, out_hbm,
            xv, outv, wo, w1, w3, w2, wm, cv, m0v, modv, xh, h0,
            lhs_a, lhs_b, o32, abuf, yv, h2, hid, sem_in, sem_k, sem_out, *rest):
    rqk = rest[0:2]
    rv = rest[2:4]
    wg = rest[4:6]
    scale = DH ** -0.5

    copies = {}

    def mk(name, src, dst):
        copies[name] = pltpu.make_async_copy(src, dst, sem_in.at[len(copies)])

    def cols(hbm, ref, c0, c1):
        return hbm.bitcast(U32).at[:, c0:c1], ref.at[:, c0:c1]

    mk("c", c_hbm, cv)
    mk("mem0", mem0_hbm, m0v)
    mk("x0", x_hbm.at[0:X0], xv.at[0:X0])
    for i in range(NM0):
        mk(f"wm0{i}", *cols(wm_hbm, wm, i * M0W, (i + 1) * M0W))
    mk("x1", x_hbm.at[X0:X1], xv.at[X0:X1])
    mk("wo", wo_hbm.bitcast(U32), wo)
    mk("wm1", *cols(wm_hbm, wm, 2 * D, 6 * D))
    mk("w1", w1_hbm.bitcast(U32), w1)
    mk("w3", w3_hbm.bitcast(U32), w3)
    mk("w2", w2_hbm.bitcast(U32), w2)
    mk("x2", x_hbm.at[X1:S], xv.at[X1:S])

    w_hbm = (wq_hbm, wk_hbm, wv_hbm)

    def chunk_copies(k, gi, m, t0, jj):
        return [
            pltpu.make_async_copy(
                w_hbm[m].bitcast(U32).at[:, par, (2 * gi + pg) * (HG // 2) + jj],
                wg[pg].at[gi, t0 + par], sem_k.at[k])
            for pg in range(2) for par in range(2)]

    def start_chunks(j, m):
        gi = j >> 1 if m < 2 else j - G
        for jj in range(HG // 2):
            for c in chunk_copies(2 * j + jj, gi, m, m * HG + 2 * jj, jj):
                c.start()

    def chunk_pos(k):
        is_v = k >= 2 * G
        gi = jnp.where(is_v, (k >> 1) - G, k >> 2)
        t0 = jnp.where(is_v, 2 * HG + 2 * (k & 1), 2 * (k & 3))
        return gi, t0

    def wait_chunk(k, gi, t0):
        for c in chunk_copies(k, gi, 0, t0, 0):
            c.wait()

    for n in ["c", "mem0", "x0"] + [f"wm0{i}" for i in range(NM0)]:
        copies[n].start()
    for j in range(J0):
        start_chunks(j, j % 2)

    def out_copy(r0, n):
        return pltpu.make_async_copy(outv.at[pl.ds(r0, n)], out_hbm.at[pl.ds(r0, n)], sem_out)

    def mod_part(c0, c1):
        cf = cv[...].astype(F32)
        sc = jnp.broadcast_to(_silu(cf), (16, D)).astype(BF16)
        modv[:, c0:c1] = _dot(sc, _w(wm, 0, D, c0, c1))[0:8]

    def mvec(i):
        return modv[0:1, i * D:(i + 1) * D]

    def ln1(r0, n):
        xf = xv[pl.ds(r0, n), :].astype(F32)
        return _ln(xf) * (1.0 + mvec(1)) + mvec(0)

    def repack(gi, t0, enable=None):
        for w in wg:
            for r0 in range(0, D // 2, 32):
                a = w[gi, t0, r0:r0 + 32, :]
                b = w[gi, t0 + 1, r0:r0 + 32, :]
                e = (a & jnp.uint32(0xFFFF)) | (b << 16)
                o = (a >> 16) | (b & jnp.uint32(0xFFFF0000))
                if enable is not None:
                    e = jnp.where(enable, e, a)
                    o = jnp.where(enable, o, b)
                w[gi, t0, r0:r0 + 32, :] = e
                w[gi, t0 + 1, r0:r0 + 32, :] = o

    def proj(lhs, pg, gi, rows):
        for t in range(3 * HG):
            r = _dot(lhs, pltpu.bitcast(wg[pg][gi, t], BF16))
            dst, td = (rqk[pg], t) if t < 2 * HG else (rv[pg], t - 2 * HG)
            for i, row in enumerate(rows):
                dst[gi, td, pl.ds(row, 4), :] = _pack(r[8 * i:8 * i + 8])

    def attn_qk(par_g, gi, base, q0, nq, nk, allowed, fill):
        qrow = base + q0 // 2 if isinstance(base, int) else pl.multiple_of(base + q0 // 2, 8)
        ps = []
        for hh in range(HG):
            q = pltpu.bitcast(rqk[par_g][gi, hh, pl.ds(qrow, nq // 2), :], BF16)
            k = pltpu.bitcast(rqk[par_g][gi, HG + hh, pl.ds(base, nk // 2), :], BF16)
            s = lax.dot_general(q, k, (((1,), (1,)), ((), ())), preferred_element_type=F32)
            s = jnp.where(allowed, s, fill)
            m = jnp.max(s, axis=-1, keepdims=True)
            p = jnp.exp2((s - m) * (scale * LOG2E))
            l = jnp.sum(p, axis=-1, keepdims=True)
            ps.append((p * _recip(l)).astype(BF16))
        return ps

    def attn_pv(g, base, nq, nk, ps):
        for hh in range(HG):
            v = pltpu.bitcast(rv[g % 2][g // 2, hh, pl.ds(base, nk // 2), :], BF16)
            o = _dot(ps[hh], v)
            col = (g * HG + hh) * DH
            o32[0:nq // 2, col:col + DH] = pltpu.bitcast(o.astype(BF16), U32)

    def wo_proj(nq, stores):
        o = _w(o32, 0, nq, 0, HD)
        cw = 256
        for cb in range(D // cw):
            r = _dot(o, _w(wo, 0, HD, cb * cw, (cb + 1) * cw))
            for r0, n, fn in stores:
                fn(slice(cb * cw, (cb + 1) * cw), r[r0:r0 + n])

    def post_attn(tok0, slot, n):
        x1 = xv[pl.ds(tok0, n), :].astype(F32) + mvec(2) * abuf[pl.ds(slot, n), :]
        yv[0:n, :] = x1
        hh = _ln(x1) * (1.0 + mvec(4)) + mvec(3)
        h2[0:n // 2, :] = pltpu.bitcast(hh.astype(BF16), U32)

    def cslice(off, c, w):
        if isinstance(off, int):
            return slice(off + c * w, off + (c + 1) * w)
        return pl.ds(pl.multiple_of(off + c * w, w), w)

    def ffn_up(c0, c1, n, off=0):
        a = _w(h2, 0, n, 0, D)
        for c in range(c0, c1):
            cs = cslice(off, c, FC)
            gt = _dot(a, pltpu.bitcast(w1[:, cs], BF16))
            up = _dot(a, pltpu.bitcast(w3[:, cs], BF16))
            hv = _silu(gt) * up
            hid[0:n // 2, cs] = pltpu.bitcast(hv.astype(BF16), U32)

    def ffn_down(tok0, n, cb0, cb1, off=0):
        a = _w(hid, 0, n, 0, FF)
        cw = 256
        for cb in range(cb0, cb1):
            cs = cslice(off, cb, cw)
            r = _dot(a, pltpu.bitcast(w2[:, cs], BF16))
            gb = modv[0:1, cslice(off + 5 * D, cb, cw)]
            outv[pl.ds(tok0, n), cs] = (yv[0:n, cs] + gb * r).astype(BF16)

    def unit_row(u):
        if DBG_STATIC:
            return u
        r = u & 7
        slot = lax.rem(u >> 3, NSLOT)
        return pl.multiple_of(slot * (SLOT // 2) + 4 + 4 * r + 4 * (r >= 5).astype(jnp.int32), 4)

    with _scope("waitx0"):
        copies["x0"].wait()
    with _scope("ln0"):

        def ln_body(i, _):
            r0 = pl.multiple_of(i * 32, 32)
            xh[pl.ds(r0, 32), :] = _ln(xv[pl.ds(r0, 32), :].astype(F32))
            return 0

        lax.fori_loop(0, X0 // 32, ln_body, 0)
        copies["c"].wait()
        copies["mem0"].wait()
        lhs_a[0:MEM, :] = m0v[...].astype(F32)

    with _scope("mod0"):
        for i in range(NM0):
            with _scope(f"waitwm{i}"):
                copies[f"wm0{i}"].wait()
            mod_part(i * M0W, (i + 1) * M0W)

    with _scope("modulate"):
        def mod_body(i, _):
            hh = xh[pl.ds(pl.multiple_of(i * 128, 128), 128), :] * (1.0 + mvec(1)) + mvec(0)
            h0[pl.ds(pl.multiple_of(i * 64, 64), 64), :] = pltpu.bitcast(hh.astype(BF16), U32)
            return 0

        lax.fori_loop(0, PRO // 128, mod_body, 0)
        lhs_a[MEM:32, :] = xh[PRO:PRO + 24, :] * (1.0 + mvec(1)) + mvec(0)

    with _scope("first"):
        wait_chunk(0, 0, 0)
        repack(0, 0)

    def pro_body(k, is_v):
        last = 3 * G - 1
        kn = jnp.minimum(k + 1, last)
        gn, tn = chunk_pos(kn)
        if is_v:
            prefetch = k < last
        else:
            prefetch = k > 0

            @pl.when(k == 1)
            def _():
                wait_chunk(1, 0, 2)
                repack(0, 2)

        @pl.when(prefetch)
        def _():
            wait_chunk(kn, gn, tn)

        gi, t0 = chunk_pos(k)
        a = pltpu.bitcast(h0[...], BF16)
        for pg in range(2):
            dst, td = (rv[pg], t0 - 2 * HG) if is_v else (rqk[pg], t0)
            for d in range(2):
                r = _dot(a, pltpu.bitcast(wg[pg][gi, t0 + d], BF16))
                for pp in range(PRO // PT):
                    b0, r0 = pp * (SLOT // 2), pp * PT
                    dst[gi, td + d, b0 + 4:b0 + 8, :] = _pack(r[r0:r0 + 8])
                    dst[gi, td + d, b0 + 8:b0 + 24, :] = _pack(r[r0 + 8:r0 + 40])
                    dst[gi, td + d, b0 + 28:b0 + 32, :] = _pack(r[r0 + 40:r0 + 48])
                    dst[gi, td + d, b0 + 32:b0 + 40, :] = _pack(r[r0 + 48:r0 + 64])
        repack(jnp.where(prefetch, gn, gi), jnp.where(prefetch, tn, t0), prefetch)
        return 0

    def pro_outer(o, _):
        @pl.when(o == 1)
        def _():
            for j in range(J0, G + G // 2):
                start_chunks(j, j % 2 if j < G else 2)

        @pl.when(o == 2)
        def _():
            for n in ("x1", "wo", "wm1", "w1", "w3", "w2", "x2"):
                copies[n].start()

        lax.fori_loop(4 * o, 4 * o + 4, lambda k, _: pro_body(k, False), 0)
        return 0

    with _scope("pro"):
        lax.fori_loop(0, G // 2, pro_outer, 0)
        lax.fori_loop(2 * G, 3 * G, lambda k, _: pro_body(k, True), 0)

    def pair(p, with_ffn, with_mod=False):
        (al_a, fi_a), (al_b, fi_b) = _masks()
        base = pl.multiple_of(lax.rem(p, NSLOT) * (SLOT // 2), 8)
        u0 = PRO // 8 + 6 * p
        if DBG_STATIC:
            base = 0
            class _U:
                def __add__(self, i):
                    return 44 + 4 * i
            u0 = _U()
        tlead = PRO + 48 * p
        aslot = pl.multiple_of(lax.rem(p, LAG) * PT, PT)
        tok_f = pl.multiple_of((p - LAG) * PT, PT)

        if with_ffn:
            post_attn(tok_f, aslot, PT)

        def filler(i):
            if with_ffn:
                if i < 5:
                    ffn_up(FILL[i], FILL[i + 1], PT)
                else:
                    ffn_down(tok_f, PT, 0, 4)
            elif with_mod and i in (0, 2, 3, 4):
                c0 = (2 + (0, 0, 1, 2, 3)[i]) * D
                mod_part(c0, c0 + D)

        def proj_attn(lhs, rows, q0, nq, nk, allowed, fill, f):
            ps = None
            for g in range(G):
                proj(lhs, g % 2, g // 2, rows)
                if g > 0:
                    attn_pv(g - 1, base, nq, nk, ps)
                ps = attn_qk(g % 2, g // 2, base, q0, nq, nk, allowed, fill)
            filler(f)
            attn_pv(G - 1, base, nq, nk, ps)
            filler(f + 1)

        lhs = lhs_a[...].astype(BF16)
        rows = [base, unit_row(u0 + 0), unit_row(u0 + 1), unit_row(u0 + 2)]
        lhs_b[MEM:32, :] = ln1(pl.multiple_of(tlead + 24, 8), 24)
        proj_attn(lhs, rows, 0, 32, 48, al_a, fi_a, 0)

        def st_mem_b(cs, val):
            lhs_b[0:MEM, cs] = val.astype(BF16).astype(F32)

        def st_a(r0, n):
            def fn(cs, val):
                abuf[pl.ds(pl.multiple_of(aslot + r0, 8), n), cs] = val
            return fn

        wo_proj(32, [(0, 8, st_mem_b), (8, 24, st_a(0, 24))])
        filler(2)

        lhs = lhs_b[...].astype(BF16)
        rows = [base + 24 if DBG_STATIC else pl.multiple_of(base + 24, 8), unit_row(u0 + 3), unit_row(u0 + 4), unit_row(u0 + 5)]
        nxt = pl.multiple_of(jnp.minimum(tlead + 48, S - 24), 8)
        lhs_a[MEM:32, :] = ln1(nxt, 24)
        proj_attn(lhs, rows, 32, 48, 80, al_b, fi_b, 3)

        def st_mem_a(cs, val):
            lhs_a[0:MEM, cs] = val.astype(BF16).astype(F32)

        wo_proj(48, [(16, 8, st_mem_a), (0, 16, st_a(24, 16)), (24, 24, st_a(40, 24))])
        filler(5)

    with _scope("waitwo"):
        copies["x1"].wait()
        copies["wo"].wait()
        copies["wm1"].wait()

    with _scope("noffn"):
        if LAG == 1:
            pair(jnp.int32(0), False, True)
        else:
            def pair_noffn(p, _):
                pair(p, False, True)
                return 0

            lax.fori_loop(0, LAG, pair_noffn, 0)

    with _scope("waitffn"):
        copies["w1"].wait()
        copies["w3"].wait()
        copies["w2"].wait()

    def pair_ffn(p, _):
        @pl.when(p == MAIN_START + 2)
        def _():
            copies["x2"].wait()

        if not NO_LOOP_DMA:
            @pl.when(p > MAIN_START)
            def _():
                out_copy(pl.multiple_of((p - LAG - 1) * PT, PT), PT).start()

        pair(p, True)
        return 0

    with _scope("main"):
        lax.fori_loop(MAIN_START, NPAIR, pair_ffn, 0)

    if NO_LOOP_DMA:
        out_copy((MAIN_START - LAG) * PT, (NPAIR - MAIN_START) * PT).start()
    else:
        out_copy((NPAIR - LAG - 1) * PT, PT).start()
    with _scope("epi"):
        n = LAG * PT
        tok0 = S - n
        assert (NPAIR - LAG) % LAG == 0
        post_attn(tok0, 0, n)

        def up_body(i, _):
            ffn_up(0, EPI_UP, n, i * (EPI_UP * FC))
            return 0

        def down_body(i, _):
            ffn_down(tok0, n, 0, EPI_DOWN, i * (EPI_DOWN * 256))
            return 0

        lax.fori_loop(0, NFC // EPI_UP, up_body, 0)
        lax.fori_loop(0, 4 // EPI_DOWN, down_body, 0)
        out_copy(tok0, n).start()
    with _scope("waitout"):
        out_copy(0, S - (MAIN_START - LAG) * PT).wait()


@functools.partial(jax.jit, static_argnames=("A_seg_len",))
def pallas_adaLN_cond__memory_aug_recurrent_mem_tr__glu_gated_swiglu__prompt_kernel(
    A_x, A_mem0, A_Wq, A_Wk, A_Wv, A_Wo, A_seg_len, B_x, B_w1, B_w3, B_w2, c, w_mod,
):
    assert A_seg_len == SEG
    assert A_x.shape == (1, S, D) and A_mem0.shape == (1, MEM, D)
    assert A_Wq.shape == (D, H, DH) and B_w1.shape == (D, FF)
    del B_x

    n_in_copies = 3 + NM0 + 7
    scratch = [
        pltpu.VMEM((S, D), BF16),
        pltpu.VMEM((S, D), BF16),
        pltpu.VMEM((HD // 2, D), U32),
        pltpu.VMEM((D // 2, FF), U32),
        pltpu.VMEM((D // 2, FF), U32),
        pltpu.VMEM((FF // 2, D), U32),
        pltpu.VMEM((D // 2, 6 * D), U32),
        pltpu.VMEM((1, D), BF16),
        pltpu.VMEM((MEM, D), BF16),
        pltpu.VMEM((8, 6 * D), F32),
        pltpu.VMEM((X0, D), F32),
        pltpu.VMEM((PRO // 2, D), U32),
        pltpu.VMEM((32, D), F32),
        pltpu.VMEM((32, D), F32),
        pltpu.VMEM((24, HD), U32),
        pltpu.VMEM((LAG * PT, D), F32),
        pltpu.VMEM((LAG * PT, D), F32),
        pltpu.VMEM((LAG * PT // 2, D), U32),
        pltpu.VMEM((LAG * PT // 2, FF), U32),
        pltpu.SemaphoreType.DMA((n_in_copies,)),
        pltpu.SemaphoreType.DMA((3 * G,)),
        pltpu.SemaphoreType.DMA,
    ] + [pltpu.VMEM((G // 2, 2 * HG, NSLOT * SLOT // 2, DH), U32)] * 2 + [
        pltpu.VMEM((G // 2, HG, NSLOT * SLOT // 2, DH), U32)] * 2 + [
        pltpu.VMEM((G // 2, 3 * HG, D // 2, DH), U32)] * 2

    out = pl.pallas_call(
        _kernel,
        out_shape=jax.ShapeDtypeStruct((S, D), BF16),
        in_specs=[pl.BlockSpec(memory_space=pl.ANY)] * 11,
        out_specs=pl.BlockSpec(memory_space=pl.ANY),
        scratch_shapes=scratch,
        compiler_params=pltpu.CompilerParams(
            vmem_limit_bytes=120 * 1024 * 1024, disable_bounds_checks=True),
    )(
        A_x.reshape(S, D), A_mem0.reshape(MEM, D),
        A_Wq.reshape(D // 2, 2, H, DH), A_Wk.reshape(D // 2, 2, H, DH),
        A_Wv.reshape(D // 2, 2, H, DH), A_Wo.reshape(HD, D),
        B_w1, B_w3, B_w2, c, w_mod,
    )
    return out.reshape(1, S, D)
```

```python
import functools

import jax
import jax.numpy as jnp
from jax import lax
import jax.experimental.pallas as pl
import jax.experimental.pallas.tpu as pltpu

F32 = jnp.float32
BF16 = jnp.bfloat16
U32 = jnp.uint32

S = 2048
D = 1024
H = 32
DH = 128
HD = H * DH
MEM = 8
SEG = 32
FF = 3584
EPS = 1e-5
LOG2E = 1.4426950408889634

G = 8
HG = H // G
PRO = 512
NPAIR = S // (2 * SEG)
PT = 2 * SEG
SLOT = 40
NSLOT = 9
LAG = 2
X0 = 544
FC = 256
NFC = FF // FC
KT = D // DH
NJ = 3 * G // 2
FILL = (0, 2, 4, 9, 11, 14)
QKPOS = 3
EPI_UP = 2
EPI_DOWN = 1
MAIN_START = LAG
SCOPES = False


class _NoScope:
    def __enter__(self):
        return self

    def __exit__(self, *a):
        return False


def _scope(name):
    return jax.named_scope(name) if SCOPES else _NoScope()


def _unpack(x):
    return pltpu.bitcast(x, BF16)


def _pack(x):
    return pltpu.bitcast(x.astype(BF16), U32)


def _dot(a, b):
    return jnp.dot(a, b, preferred_element_type=F32)


def _ln(x):
    m = jnp.mean(x, axis=-1, keepdims=True)
    xc = x - m
    v = jnp.mean(xc * xc, axis=-1, keepdims=True)
    return xc * lax.rsqrt(v + EPS)


def _recip(x):
    r = pl.reciprocal(x, approx=True)
    return r * (2.0 - x * r)


def _silu(x):
    h = 0.5 * x
    return h + h * jnp.tanh(h)


def _cols(off, w):
    if isinstance(off, int):
        return slice(off, off + w)
    return pl.ds(pl.multiple_of(off, w), w)


def _rarely(cond, fn):
    def body(_, c):
        fn()
        return c

    lax.fori_loop(0, cond.astype(jnp.int32), body, 0)


def _masks():
    def pos(j):
        return jnp.where(j < 40, j, jnp.where(j < 48, j - 32, jnp.where(j < 56, j - 48, j - 40)))

    out = []
    for q0, nq, nk in ((0, 32, 48), (32, 48, 80)):
        qi = lax.broadcasted_iota(jnp.int32, (nq, nk), 0) + q0
        kj = lax.broadcasted_iota(jnp.int32, (nq, nk), 1)
        qp, kp = pos(qi), pos(kj)
        same = ((qi < 40) & (kj < 40)) | ((qi >= 40) & (kj >= 40))
        allowed = same & ((qp < MEM) | (qp >= kp))
        fill = jnp.where(same, jnp.float32(-1e9 * DH ** 0.5), jnp.float32(-jnp.inf))
        out.append((allowed, fill))
    return out


def _kernel(x_hbm, mem0_hbm, wq_hbm, wk_hbm, wv_hbm, wo_hbm, w1_hbm, w3_hbm, w2_hbm,
            c_hbm, wm_hbm, out_hbm,
            xv, outv, wo, w1, w3, w2, wm, cv, m0v, modv, xh, h0, acc,
            lhs_a, lhs_b, o32, abuf, yv, h2, hid, sem_in, sem_m, sem_w, sem_out, *rest):
    ring = rest[0:2]
    wg = rest[2:4]
    scale = DH ** -0.5

    copies = {}

    def mk(name, src, dst):
        copies[name] = pltpu.make_async_copy(src, dst, sem_in.at[len(copies)])

    wm_u = wm_hbm.bitcast(U32)
    mk("c", c_hbm, cv)
    mk("mem0", mem0_hbm, m0v)
    mk("x0", x_hbm.at[0:X0], xv.at[0:X0])
    mk("x1", x_hbm.at[X0:S], xv.at[X0:S])
    mk("wo", wo_hbm.bitcast(U32), wo)
    mk("wm1", wm_u.at[:, 2 * D:6 * D], wm.at[:, 2 * D:6 * D])
    mk("w1", w1_hbm.bitcast(U32), w1)
    mk("w3", w3_hbm.bitcast(U32), w3)
    mk("w2", w2_hbm.bitcast(U32), w2)

    def mod_copies(kt):
        return [pltpu.make_async_copy(wm_u.at[:, _cols(i * D + kt * DH, DH)],
                                      wm.at[:, _cols(i * D + kt * DH, DH)], sem_m.at[kt])
                for i in range(2)]

    w_hbm = (wq_hbm, wk_hbm, wv_hbm)

    def block_copies(j, m, gi, t0):
        return [
            pltpu.make_async_copy(
                w_hbm[m].bitcast(U32).at[:, par, (2 * gi + pg) * (HG // 2) + jj],
                wg[pg].at[gi, t0 + 2 * jj + par], sem_w.at[j])
            for pg in range(2) for jj in range(HG // 2) for par in range(2)]

    def start_block(j):
        for c in block_copies(j, j // 4, j % 4, (j // 4) * HG):
            c.start()

    def wait_block(j, gi, t0):
        for c in block_copies(j, 0, gi, t0):
            c.wait()

    for n in ("c", "mem0", "x0"):
        copies[n].start()
    start_block(0)
    for kt in range(KT):
        for c in mod_copies(kt):
            c.start()
    for j in range(1, 4):
        start_block(j)

    def out_copy(r0, n):
        return pltpu.make_async_copy(outv.at[pl.ds(r0, n)], out_hbm.at[pl.ds(r0, n)], sem_out)

    def silu_c():
        return jnp.broadcast_to(_silu(cv[...].astype(F32)), (16, D)).astype(BF16)

    def mod_part(off, w):
        r = _dot(silu_c(), _unpack(wm[:, _cols(off, w)]))[0:8]
        modv[:, _cols(off, w)] = r
        return r[0:1]

    def mvec(i):
        return modv[0:1, i * D:(i + 1) * D]

    def ln1(r0, n):
        xf = xv[pl.ds(r0, n), :].astype(F32)
        return _ln(xf) * (1.0 + mvec(1)) + mvec(0)

    def repack_slot(w, gi, t, enable=None):
        for r0 in range(0, D // 2, 32):
            a = w[gi, t, r0:r0 + 32, :]
            b = w[gi, t + 1, r0:r0 + 32, :]
            e = (a & jnp.uint32(0xFFFF)) | (b << 16)
            o = (a >> 16) | (b & jnp.uint32(0xFFFF0000))
            if enable is not None:
                e = jnp.where(enable, e, a)
                o = jnp.where(enable, o, b)
            w[gi, t, r0:r0 + 32, :] = e
            w[gi, t + 1, r0:r0 + 32, :] = o

    def repack_now(gi, t0):
        def body(i, c):
            for w in wg:
                repack_slot(w, gi, t0 + 2 * i)
            return c

        lax.fori_loop(0, HG // 2, body, 0)

    def store_tokens(dst, gi, t, r):
        for pp in range(PRO // PT):
            b0, r0 = pp * SLOT, pp * PT
            dst[gi, t, b0 + 4:b0 + 8, :] = _pack(r[r0:r0 + 8])
            dst[gi, t, b0 + 8:b0 + 24, :] = _pack(r[r0 + 8:r0 + 40])
            dst[gi, t, b0 + 28:b0 + 32, :] = _pack(r[r0 + 40:r0 + 48])
            dst[gi, t, b0 + 32:b0 + 40, :] = _pack(r[r0 + 48:r0 + 64])

    def proj(lhs, g, rows, ts):
        for t in ts:
            r = _dot(lhs, _unpack(wg[g % 2][g // 2, t]))
            for i, row in enumerate(rows):
                ring[g % 2][g // 2, t, pl.ds(row, 4), :] = _pack(r[8 * i:8 * i + 8])

    def attn_qk(g, base, q0, nq, nk, allowed, fill):
        qrow = pl.multiple_of(base + q0 // 2, 8)
        ps = []
        for hh in range(HG):
            q = _unpack(ring[g % 2][g // 2, hh, pl.ds(qrow, nq // 2), :])
            k = _unpack(ring[g % 2][g // 2, HG + hh, pl.ds(base, nk // 2), :])
            s = lax.dot_general(q, k, (((1,), (1,)), ((), ())), preferred_element_type=F32)
            s = jnp.where(allowed, s, fill)
            m = jnp.max(s, axis=-1, keepdims=True)
            p = jnp.exp2((s - m) * (scale * LOG2E))
            l = jnp.sum(p, axis=-1, keepdims=True)
            ps.append((p * _recip(l)).astype(BF16))
        return ps

    def attn_pv(g, base, nq, nk, ps):
        for hh in range(HG):
            v = _unpack(ring[g % 2][g // 2, 2 * HG + hh, pl.ds(base, nk // 2), :])
            col = (g * HG + hh) * DH
            o32[0:nq // 2, col:col + DH] = _pack(_dot(ps[hh], v))

    def wo_proj(nq, stores):
        o = _unpack(o32[0:nq // 2, :])
        cw = 256
        for cb in range(D // cw):
            cs = slice(cb * cw, (cb + 1) * cw)
            r = _dot(o, _unpack(wo[:, cs]))
            for r0, n, fn in stores:
                fn(cs, r[r0:r0 + n])

    def post_attn(tok0, slot, n):
        x1 = xv[pl.ds(tok0, n), :].astype(F32) + mvec(2) * abuf[pl.ds(slot, n), :]
        yv[0:n, :] = x1
        h2[0:n // 2, :] = _pack(_ln(x1) * (1.0 + mvec(4)) + mvec(3))

    def ffn_up(c0, c1, n, off=0):
        a = _unpack(h2[0:n // 2, :])
        for c in range(c0, c1):
            cs = _cols(off + c * FC, FC)
            gt = _dot(a, _unpack(w1[:, cs]))
            up = _dot(a, _unpack(w3[:, cs]))
            hid[0:n // 2, cs] = _pack(_silu(gt) * up)

    def ffn_down(tok0, n, cb0, cb1, off=0):
        a = _unpack(hid[0:n // 2, :])
        cw = 256
        for cb in range(cb0, cb1):
            cs = _cols(off + cb * cw, cw)
            r = _dot(a, _unpack(w2[:, cs]))
            gb = modv[0:1, _cols(off + 5 * D + cb * cw, cw)]
            outv[pl.ds(tok0, n), cs] = (yv[0:n, cs] + gb * r).astype(BF16)

    def unit_row(u):
        r = u & 7
        slot = lax.rem(u >> 3, NSLOT)
        return pl.multiple_of(slot * SLOT + 4 + 4 * r + 4 * (r >= 5).astype(jnp.int32), 4)

    with _scope("ln0"):
        acc[...] = jnp.zeros(acc.shape, F32)
        copies["x0"].wait()

        def ln_body(i, c):
            r0 = pl.multiple_of(i * 136, 8)
            xh[pl.ds(r0, 136), :] = _ln(xv[pl.ds(r0, 136), :].astype(F32))
            return c

        lax.fori_loop(0, X0 // 136, ln_body, 0)
        copies["c"].wait()
        copies["mem0"].wait()
        lhs_a[0:MEM, :] = m0v[...].astype(F32)

    def modulate(kt):
        sa = mod_part(kt * DH, DH)
        ca = mod_part(D + kt * DH, DH)
        a = _pack(xh[0:PRO, _cols(kt * DH, DH)] * (1.0 + ca) + sa)
        h0[:, _cols(kt * DH, DH)] = a
        return a

    with _scope("first"):
        wait_block(0, 0, 0)
        repack_now(0, 0)
        for c in mod_copies(0):
            c.wait()
        a0 = modulate(0)

    def kmajor(kt, a):
        kn = jnp.minimum(kt + 1, KT - 1)

        @pl.when(kt < KT - 1)
        def _():
            for c in mod_copies(kn):
                c.wait()

        rows = pl.ds(pl.multiple_of(kt * (DH // 2), DH // 2), DH // 2)
        a_next = None
        for pg in range(2):
            for t in range(HG):
                acc[pg * HG + t] += _dot(_unpack(a), _unpack(wg[pg][0, t, rows, :]))
            if pg == 0:
                a_next = modulate(kn)
        return a_next

    with _scope("kmajor"):
        lax.fori_loop(0, KT, kmajor, a0)
        lhs_a[MEM:32, :] = xh[PRO:PRO + 24, :] * (1.0 + mvec(1)) + mvec(0)

        def flush(t, c):
            for pg in range(2):
                store_tokens(ring[pg], 0, t, acc[pg * HG + t])
            return c

        lax.fori_loop(0, HG, flush, 0)

    def pro_body(j, c):
        gi, t0 = j & 3, (j >> 2) * HG
        jn = jnp.minimum(j + 1, NJ - 1)
        gn, tn = jn & 3, (jn >> 2) * HG
        prefetch = (j > 1) & (j < NJ - 1)

        def batch(js, names):
            def fn():
                for jj in js:
                    start_block(jj)
                for n in names:
                    copies[n].start()
            return fn

        def late():
            wait_block(j, gi, t0)
            repack_now(gi, t0)

        _rarely(j == 1, batch(range(4, 9), ()))
        _rarely(j == 3, batch(range(9, NJ), ("x1", "wo", "wm1", "w1", "w3", "w2")))
        _rarely(j <= 2, late)

        @pl.when(prefetch)
        def _():
            wait_block(jn, gn, tn)

        a = _unpack(h0[...])
        for pg in range(2):
            for t in range(HG):
                store_tokens(ring[pg], gi, t0 + t, _dot(a, _unpack(wg[pg][gi, t0 + t])))
        gr, tr = jnp.where(prefetch, gn, gi), jnp.where(prefetch, tn, t0)
        for w in wg:
            for t in range(0, HG, 2):
                repack_slot(w, gr, tr + t, prefetch)
        return c

    with _scope("pro"):
        lax.fori_loop(1, NJ, pro_body, 0)

    def pair(p, with_ffn):
        (al_a, fi_a), (al_b, fi_b) = _masks()
        base = pl.multiple_of(lax.rem(p, NSLOT) * SLOT, 8)
        u0 = PRO // 8 + 6 * p
        tlead = PRO + 48 * p
        aslot = pl.multiple_of((p & (LAG - 1)) * PT, PT)
        tok_f = pl.multiple_of((p - LAG) * PT, PT)

        if with_ffn:
            post_attn(tok_f, aslot, PT)

        def filler(i, c0=None, c1=None):
            if not with_ffn:
                if i is not None:
                    w = 4 * D // LAG // 4
                    mod_part(2 * D + (p * 4 + i) * w, w)
            elif c0 is None:
                ffn_down(tok_f, PT, 0, 4)
            else:
                ffn_up(c0, c1, PT)

        def proj_attn(lhs, rows, q0, nq, nk, allowed, fill, f, m0, m1):
            order = list(range(2 * HG, 3 * HG)) + list(range(2 * HG))
            ps = None
            for g in range(G):
                proj(lhs, g, rows, order[:QKPOS])
                if g > 0:
                    ps = attn_qk(g - 1, base, q0, nq, nk, allowed, fill)
                proj(lhs, g, rows, order[QKPOS:])
                if g > 0:
                    attn_pv(g - 1, base, nq, nk, ps)
            filler(None, FILL[f], FILL[f] + 1)
            ps = attn_qk(G - 1, base, q0, nq, nk, allowed, fill)
            filler(m0, FILL[f] + 1, FILL[f + 1])
            attn_pv(G - 1, base, nq, nk, ps)
            filler(m1, FILL[f + 1], FILL[f + 2])

        def st_lhs(ref):
            def fn(cs, val):
                ref[0:MEM, cs] = val.astype(BF16).astype(F32)
            return fn

        def st_a(r0, n):
            def fn(cs, val):
                abuf[pl.ds(pl.multiple_of(aslot + r0, 8), n), cs] = val
            return fn

        lhs = lhs_a[...].astype(BF16)
        rows = [base, unit_row(u0), unit_row(u0 + 1), unit_row(u0 + 2)]
        lhs_b[MEM:32, :] = ln1(pl.multiple_of(tlead + 24, 8), 24)
        proj_attn(lhs, rows, 0, 32, 48, al_a, fi_a, 0, 0, None)
        wo_proj(32, [(0, 8, st_lhs(lhs_b)), (8, 24, st_a(0, 24))])
        filler(1, FILL[2], FILL[3])

        lhs = lhs_b[...].astype(BF16)
        rows = [pl.multiple_of(base + 24, 8), unit_row(u0 + 3), unit_row(u0 + 4), unit_row(u0 + 5)]
        nxt = pl.multiple_of(jnp.minimum(tlead + 48, S - 24), 8)
        lhs_a[MEM:32, :] = ln1(nxt, 24)
        proj_attn(lhs, rows, 32, 48, 80, al_b, fi_b, 3, 2, 3)
        wo_proj(48, [(16, 8, st_lhs(lhs_a)), (0, 16, st_a(24, 16)), (24, 24, st_a(40, 24))])
        filler(None)

    with _scope("waitwo"):
        copies["x1"].wait()
        copies["wo"].wait()
        copies["wm1"].wait()

    def pair_noffn(p, c):
        pair(p, False)
        return c

    with _scope("noffn"):
        lax.fori_loop(0, LAG, pair_noffn, 0)

    with _scope("waitffn"):
        copies["w1"].wait()
        copies["w3"].wait()
        copies["w2"].wait()

    def pair_ffn(p, c):
        @pl.when(p > MAIN_START)
        def _():
            out_copy(pl.multiple_of((p - LAG - 1) * PT, PT), PT).start()

        pair(p, True)
        return c

    with _scope("main"):
        lax.fori_loop(MAIN_START, NPAIR, pair_ffn, 0)

    out_copy((NPAIR - LAG - 1) * PT, PT).start()
    with _scope("epi"):
        n = LAG * PT
        tok0 = S - n
        post_attn(tok0, 0, n)

        def up_body(i, c):
            ffn_up(0, EPI_UP, n, i * (EPI_UP * FC))
            return c

        def down_body(i, c):
            ffn_down(tok0, n, 0, EPI_DOWN, i * (EPI_DOWN * 256))
            return c

        lax.fori_loop(0, NFC // EPI_UP, up_body, 0)
        lax.fori_loop(0, 4 // EPI_DOWN, down_body, 0)
        out_copy(tok0, n).start()
    with _scope("waitout"):
        out_copy(0, S - (MAIN_START - LAG) * PT).wait()


@functools.partial(jax.jit, static_argnames=("A_seg_len",))
def pallas_adaLN_cond__memory_aug_recurrent_mem_tr__glu_gated_swiglu__prompt_kernel(
    A_x, A_mem0, A_Wq, A_Wk, A_Wv, A_Wo, A_seg_len, B_x, B_w1, B_w3, B_w2, c, w_mod,
):
    assert A_seg_len == SEG
    assert A_x.shape == (1, S, D) and A_mem0.shape == (1, MEM, D)
    assert A_Wq.shape == (D, H, DH) and B_w1.shape == (D, FF)
    del B_x

    scratch = [
        pltpu.VMEM((S, D), BF16),
        pltpu.VMEM((S, D), BF16),
        pltpu.VMEM((HD // 2, D), U32),
        pltpu.VMEM((D // 2, FF), U32),
        pltpu.VMEM((D // 2, FF), U32),
        pltpu.VMEM((FF // 2, D), U32),
        pltpu.VMEM((D // 2, 6 * D), U32),
        pltpu.VMEM((1, D), BF16),
        pltpu.VMEM((MEM, D), BF16),
        pltpu.VMEM((8, 6 * D), F32),
        pltpu.VMEM((X0, D), F32),
        pltpu.VMEM((PRO // 2, D), U32),
        pltpu.VMEM((2 * HG, PRO, DH), F32),
        pltpu.VMEM((32, D), F32),
        pltpu.VMEM((32, D), F32),
        pltpu.VMEM((24, HD), U32),
        pltpu.VMEM((LAG * PT, D), F32),
        pltpu.VMEM((LAG * PT, D), F32),
        pltpu.VMEM((LAG * PT // 2, D), U32),
        pltpu.VMEM((LAG * PT // 2, FF), U32),
        pltpu.SemaphoreType.DMA((9,)),
        pltpu.SemaphoreType.DMA((KT,)),
        pltpu.SemaphoreType.DMA((NJ,)),
        pltpu.SemaphoreType.DMA,
    ] + [pltpu.VMEM((G // 2, 3 * HG, NSLOT * SLOT, DH), U32)] * 2 + [
        pltpu.VMEM((G // 2, 3 * HG, D // 2, DH), U32)] * 2

    out = pl.pallas_call(
        _kernel,
        out_shape=jax.ShapeDtypeStruct((S, D), BF16),
        in_specs=[pl.BlockSpec(memory_space=pl.ANY)] * 11,
        out_specs=pl.BlockSpec(memory_space=pl.ANY),
        scratch_shapes=scratch,
        compiler_params=pltpu.CompilerParams(
            vmem_limit_bytes=120 * 1024 * 1024, disable_bounds_checks=True),
    )(
        A_x.reshape(S, D), A_mem0.reshape(MEM, D),
        A_Wq.reshape(D // 2, 2, H, DH), A_Wk.reshape(D // 2, 2, H, DH),
        A_Wv.reshape(D // 2, 2, H, DH), A_Wo.reshape(HD, D),
        B_w1, B_w3, B_w2, c, w_mod,
    )
    return out.reshape(1, S, D)
```

```python
import functools

import jax
import jax.numpy as jnp
from jax import lax
import jax.experimental.pallas as pl
import jax.experimental.pallas.tpu as pltpu

F32 = jnp.float32
BF16 = jnp.bfloat16
U32 = jnp.uint32

S = 2048
D = 1024
H = 32
DH = 128
HD = H * DH
MEM = 8
SEG = 32
FF = 3584
EPS = 1e-5
LOG2E = 1.4426950408889634

G = 8
HG = H // G
PRO = 512
NPAIR = S // (2 * SEG)
PT = 2 * SEG
SLOT = 40
NSLOT = 9
X0 = 544
X1 = 640
FC = 256
NFC = FF // FC
KT = D // DH
NJ = 3 * G // 2
FILL = (0, 2, 4, 9, 11, 14)
QKPOS = 3
MODF = (0, 1, 4, 5, 7, 8, 11, 12)
EPI_UP = 7
EPI_DOWN = 2
MAIN_START = 1
SCOPES = False


class _NoScope:
    def __enter__(self):
        return self

    def __exit__(self, *a):
        return False


def _scope(name):
    return jax.named_scope(name) if SCOPES else _NoScope()


def _unpack(x):
    return pltpu.bitcast(x, BF16)


def _pack(x):
    return pltpu.bitcast(x.astype(BF16), U32)


def _dot(a, b):
    return jnp.dot(a, b, preferred_element_type=F32)


def _ln(x):
    m = jnp.mean(x, axis=-1, keepdims=True)
    xc = x - m
    v = jnp.mean(xc * xc, axis=-1, keepdims=True)
    return xc * lax.rsqrt(v + EPS)


def _recip(x):
    r = pl.reciprocal(x, approx=True)
    return r * (2.0 - x * r)


def _silu(x):
    h = 0.5 * x
    return h + h * jnp.tanh(h)


def _cols(off, w):
    if isinstance(off, int):
        return slice(off, off + w)
    return pl.ds(pl.multiple_of(off, w), w)


def _rarely(cond, fn):
    def body(_, c):
        fn()
        return c

    lax.fori_loop(0, cond.astype(jnp.int32), body, 0)


def _masks():
    def pos(j):
        return jnp.where(j < 40, j, jnp.where(j < 48, j - 32, jnp.where(j < 56, j - 48, j - 40)))

    out = []
    for q0, nq, nk in ((0, 32, 48), (32, 48, 80)):
        qi = lax.broadcasted_iota(jnp.int32, (nq, nk), 0) + q0
        kj = lax.broadcasted_iota(jnp.int32, (nq, nk), 1)
        qp, kp = pos(qi), pos(kj)
        same = ((qi < 40) & (kj < 40)) | ((qi >= 40) & (kj >= 40))
        allowed = same & ((qp < MEM) | (qp >= kp))
        fill = jnp.where(same, jnp.float32(-1e9 * DH ** 0.5), jnp.float32(-jnp.inf))
        out.append((allowed, fill))
    return out


def _kernel(x_hbm, mem0_hbm, wq_hbm, wk_hbm, wv_hbm, wo_hbm, w1_hbm, w3_hbm, w2_hbm,
            c_hbm, wm_hbm, out_hbm,
            xv, outv, wo, w1, w3, w2, wm, cv, m0v, modv, xh, h0, acc,
            lhs_a, lhs_b, o32, abuf, yv, fv, h2, hid, sem_in, sem_m, sem_w, sem_out, *rest):
    ring = rest[0:2]
    wg = rest[2:4]
    scale = DH ** -0.5

    copies = {}

    def mk(name, src, dst):
        copies[name] = pltpu.make_async_copy(src, dst, sem_in.at[len(copies)])

    wm_u = wm_hbm.bitcast(U32)
    mk("c", c_hbm, cv)
    mk("mem0", mem0_hbm, m0v)
    mk("x0", x_hbm.at[0:X0], xv.at[0:X0])
    mk("x1", x_hbm.at[X0:X1], xv.at[X0:X1])
    mk("wo", wo_hbm.bitcast(U32), wo)
    mk("wm1", wm_u.at[:, 2 * D:5 * D], wm.at[:, 2 * D:5 * D])
    mk("w1", w1_hbm.bitcast(U32), w1)
    mk("w3", w3_hbm.bitcast(U32), w3)
    mk("w2", w2_hbm.bitcast(U32), w2)
    mk("wm2", wm_u.at[:, 5 * D:6 * D], wm.at[:, 5 * D:6 * D])
    mk("x2", x_hbm.at[X1:S], xv.at[X1:S])

    def mod_copies(kt):
        return [pltpu.make_async_copy(wm_u.at[:, _cols(i * D + kt * DH, DH)],
                                      wm.at[:, _cols(i * D + kt * DH, DH)], sem_m.at[kt])
                for i in range(2)]

    w_hbm = (wq_hbm, wk_hbm, wv_hbm)

    def block_copies(j, m, gi, t0):
        return [
            pltpu.make_async_copy(
                w_hbm[m].bitcast(U32).at[:, par, (2 * gi + pg) * (HG // 2) + jj],
                wg[pg].at[gi, t0 + 2 * jj + par], sem_w.at[j])
            for pg in range(2) for jj in range(HG // 2) for par in range(2)]

    def start_block(j):
        for c in block_copies(j, j // 4, j % 4, (j // 4) * HG):
            c.start()

    def wait_block(j, gi, t0):
        for c in block_copies(j, 0, gi, t0):
            c.wait()

    for n in ("c", "mem0", "x0"):
        copies[n].start()
    start_block(0)
    for kt in range(KT):
        for c in mod_copies(kt):
            c.start()
    for j in range(1, 4):
        start_block(j)

    def out_copy(r0, n):
        return pltpu.make_async_copy(outv.at[pl.ds(r0, n)], out_hbm.at[pl.ds(r0, n)], sem_out)

    def silu_c():
        return jnp.broadcast_to(_silu(cv[...].astype(F32)), (16, D)).astype(BF16)

    def mod_part(off, w):
        r = _dot(silu_c(), _unpack(wm[:, _cols(off, w)]))[0:8]
        modv[:, _cols(off, w)] = r
        return r[0:1]

    def mvec(i):
        return modv[0:1, i * D:(i + 1) * D]

    def ln1(r0, n):
        xf = xv[pl.ds(r0, n), :].astype(F32)
        return _ln(xf) * (1.0 + mvec(1)) + mvec(0)

    def repack_slot(w, gi, t, enable=None):
        for r0 in range(0, D // 2, 32):
            a = w[gi, t, r0:r0 + 32, :]
            b = w[gi, t + 1, r0:r0 + 32, :]
            e = (a & jnp.uint32(0xFFFF)) | (b << 16)
            o = (a >> 16) | (b & jnp.uint32(0xFFFF0000))
            if enable is not None:
                e = jnp.where(enable, e, a)
                o = jnp.where(enable, o, b)
            w[gi, t, r0:r0 + 32, :] = e
            w[gi, t + 1, r0:r0 + 32, :] = o

    def repack_now(gi, t0):
        def body(i, c):
            for w in wg:
                repack_slot(w, gi, t0 + 2 * i)
            return c

        lax.fori_loop(0, HG // 2, body, 0)

    def store_tokens(dst, gi, t, r):
        for pp in range(PRO // PT):
            b0, r0 = pp * SLOT, pp * PT
            dst[gi, t, b0 + 4:b0 + 8, :] = _pack(r[r0:r0 + 8])
            dst[gi, t, b0 + 8:b0 + 24, :] = _pack(r[r0 + 8:r0 + 40])
            dst[gi, t, b0 + 28:b0 + 32, :] = _pack(r[r0 + 40:r0 + 48])
            dst[gi, t, b0 + 32:b0 + 40, :] = _pack(r[r0 + 48:r0 + 64])

    def proj(lhs, g, rows, ts):
        for t in ts:
            r = _dot(lhs, _unpack(wg[g % 2][g // 2, t]))
            for i, row in enumerate(rows):
                ring[g % 2][g // 2, t, pl.ds(row, 4), :] = _pack(r[8 * i:8 * i + 8])

    def attn_qk(g, base, q0, nq, nk, allowed, fill):
        qrow = pl.multiple_of(base + q0 // 2, 8)
        ps = []
        for hh in range(HG):
            q = _unpack(ring[g % 2][g // 2, hh, pl.ds(qrow, nq // 2), :])
            k = _unpack(ring[g % 2][g // 2, HG + hh, pl.ds(base, nk // 2), :])
            s = lax.dot_general(q, k, (((1,), (1,)), ((), ())), preferred_element_type=F32)
            s = jnp.where(allowed, s, fill)
            m = jnp.max(s, axis=-1, keepdims=True)
            p = jnp.exp2((s - m) * (scale * LOG2E))
            l = jnp.sum(p, axis=-1, keepdims=True)
            ps.append((p * _recip(l)).astype(BF16))
        return ps

    def attn_pv(g, base, nq, nk, ps):
        for hh in range(HG):
            v = _unpack(ring[g % 2][g // 2, 2 * HG + hh, pl.ds(base, nk // 2), :])
            col = (g * HG + hh) * DH
            o32[0:nq // 2, col:col + DH] = _pack(_dot(ps[hh], v))

    def wo_proj(nq, stores):
        o = _unpack(o32[0:nq // 2, :])
        cw = 256
        for cb in range(D // cw):
            cs = slice(cb * cw, (cb + 1) * cw)
            r = _dot(o, _unpack(wo[:, cs]))
            for r0, n, fn in stores:
                fn(cs, r[r0:r0 + n])

    def post_attn(tok0):
        x1 = xv[pl.ds(tok0, PT), :].astype(F32) + mvec(2) * abuf[...]
        yv[...] = x1
        h2[...] = _pack(_ln(x1) * (1.0 + mvec(4)) + mvec(3))

    def ffn_up(c0, c1, off=0):
        a = _unpack(h2[...])
        for c in range(c0, c1):
            cs = _cols(off + c * FC, FC)
            gt = _dot(a, _unpack(w1[:, cs]))
            up = _dot(a, _unpack(w3[:, cs]))
            hid[:, cs] = _pack(_silu(gt) * up)

    def ffn_down(cb0, cb1, off=0, tok0=None):
        a = _unpack(hid[...])
        cw = 256
        for cb in range(cb0, cb1):
            cs = _cols(off + cb * cw, cw)
            r = _dot(a, _unpack(w2[:, cs]))
            if tok0 is None:
                fv[:, cs] = r
            else:
                gb = modv[0:1, _cols(off + 5 * D + cb * cw, cw)]
                outv[pl.ds(tok0, PT), cs] = (yv[:, cs] + gb * r).astype(BF16)

    def finish(tok0):
        outv[pl.ds(tok0, PT), :] = (yv[...] + mvec(5) * fv[...]).astype(BF16)

    def unit_row(u):
        r = u & 7
        slot = lax.rem(u >> 3, NSLOT)
        return pl.multiple_of(slot * SLOT + 4 + 4 * r + 4 * (r >= 5).astype(jnp.int32), 4)

    with _scope("ln0"):
        acc[...] = jnp.zeros(acc.shape, F32)
        copies["x0"].wait()

        def ln_body(i, c):
            r0 = pl.multiple_of(i * 136, 8)
            xh[pl.ds(r0, 136), :] = _ln(xv[pl.ds(r0, 136), :].astype(F32))
            return c

        lax.fori_loop(0, X0 // 136, ln_body, 0)
        copies["c"].wait()
        copies["mem0"].wait()
        lhs_a[0:MEM, :] = m0v[...].astype(F32)

    def modulate(kt):
        sa = mod_part(kt * DH, DH)
        ca = mod_part(D + kt * DH, DH)
        a = _pack(xh[0:PRO, _cols(kt * DH, DH)] * (1.0 + ca) + sa)
        h0[:, _cols(kt * DH, DH)] = a
        return a

    with _scope("first"):
        wait_block(0, 0, 0)
        repack_now(0, 0)
        for c in mod_copies(0):
            c.wait()
        a0 = modulate(0)

    def kmajor(kt, a):
        kn = jnp.minimum(kt + 1, KT - 1)

        @pl.when(kt < KT - 1)
        def _():
            for c in mod_copies(kn):
                c.wait()

        rows = pl.ds(pl.multiple_of(kt * (DH // 2), DH // 2), DH // 2)
        a_next = None
        for pg in range(2):
            for t in range(HG):
                acc[pg * HG + t] += _dot(_unpack(a), _unpack(wg[pg][0, t, rows, :]))
            if pg == 0:
                a_next = modulate(kn)
        return a_next

    with _scope("kmajor"):
        lax.fori_loop(0, KT, kmajor, a0)
        lhs_a[MEM:32, :] = xh[PRO:PRO + 24, :] * (1.0 + mvec(1)) + mvec(0)

        def flush(t, c):
            for pg in range(2):
                store_tokens(ring[pg], 0, t, acc[pg * HG + t])
            return c

        lax.fori_loop(0, HG, flush, 0)

    def pro_body(j, c):
        gi, t0 = j & 3, (j >> 2) * HG
        jn = jnp.minimum(j + 1, NJ - 1)
        gn, tn = jn & 3, (jn >> 2) * HG
        prefetch = (j > 1) & (j < NJ - 1)

        def batch(js, names):
            def fn():
                for jj in js:
                    start_block(jj)
                for n in names:
                    copies[n].start()
            return fn

        def late():
            wait_block(j, gi, t0)
            repack_now(gi, t0)

        _rarely(j == 1, batch(range(4, 9), ()))
        _rarely(j == 3, batch(range(9, NJ), ("x1", "wo", "wm1", "w1", "w3", "w2", "wm2", "x2")))
        _rarely(j <= 2, late)

        @pl.when(prefetch)
        def _():
            wait_block(jn, gn, tn)

        a = _unpack(h0[...])
        for pg in range(2):
            for t in range(HG):
                store_tokens(ring[pg], gi, t0 + t, _dot(a, _unpack(wg[pg][gi, t0 + t])))
        gr, tr = jnp.where(prefetch, gn, gi), jnp.where(prefetch, tn, t0)
        for w in wg:
            for t in range(0, HG, 2):
                repack_slot(w, gr, tr + t, prefetch)
        return c

    with _scope("pro"):
        lax.fori_loop(1, NJ, pro_body, 0)

    def pair(p, with_ffn):
        (al_a, fi_a), (al_b, fi_b) = _masks()
        base = pl.multiple_of(lax.rem(p, NSLOT) * SLOT, 8)
        u0 = PRO // 8 + 6 * p
        tlead = PRO + 48 * p

        if with_ffn:
            finish(pl.multiple_of(jnp.maximum(p - 2, 0) * PT, PT))
            post_attn(pl.multiple_of((p - 1) * PT, PT))

        def filler(i, c0=None, c1=None):
            if not with_ffn:
                if i is not None:
                    mod_part(2 * D + MODF[i] * 256, (MODF[i + 1] - MODF[i]) * 256)
            elif c0 is None:
                ffn_down(0, 4)
            else:
                ffn_up(c0, c1)

        def proj_attn(lhs, rows, q0, nq, nk, allowed, fill, f, m0):
            order = list(range(2 * HG, 3 * HG)) + list(range(2 * HG))
            ps = None
            for g in range(G):
                proj(lhs, g, rows, order[:QKPOS])
                if g > 0:
                    ps = attn_qk(g - 1, base, q0, nq, nk, allowed, fill)
                proj(lhs, g, rows, order[QKPOS:])
                if g > 0:
                    attn_pv(g - 1, base, nq, nk, ps)
            filler(m0, FILL[f], FILL[f] + 1)
            ps = attn_qk(G - 1, base, q0, nq, nk, allowed, fill)
            filler(m0 + 1, FILL[f] + 1, FILL[f + 1])
            attn_pv(G - 1, base, nq, nk, ps)
            filler(m0 + 2, FILL[f + 1], FILL[f + 2])

        def st_lhs(ref):
            def fn(cs, val):
                ref[0:MEM, cs] = val.astype(BF16).astype(F32)
            return fn

        def st_a(r0, n):
            def fn(cs, val):
                abuf[r0:r0 + n, cs] = val
            return fn

        lhs = lhs_a[...].astype(BF16)
        rows = [base, unit_row(u0), unit_row(u0 + 1), unit_row(u0 + 2)]
        lhs_b[MEM:32, :] = ln1(pl.multiple_of(tlead + 24, 8), 24)
        proj_attn(lhs, rows, 0, 32, 48, al_a, fi_a, 0, 0)
        wo_proj(32, [(0, 8, st_lhs(lhs_b)), (8, 24, st_a(0, 24))])
        filler(3, FILL[2], FILL[3])

        lhs = lhs_b[...].astype(BF16)
        rows = [pl.multiple_of(base + 24, 8), unit_row(u0 + 3), unit_row(u0 + 4), unit_row(u0 + 5)]
        nxt = pl.multiple_of(jnp.minimum(tlead + 48, S - 24), 8)
        lhs_a[MEM:32, :] = ln1(nxt, 24)
        proj_attn(lhs, rows, 32, 48, 80, al_b, fi_b, 3, 4)
        wo_proj(48, [(16, 8, st_lhs(lhs_a)), (0, 16, st_a(24, 16)), (24, 24, st_a(40, 24))])
        filler(None)

    with _scope("waitwo"):
        copies["x1"].wait()
        copies["wo"].wait()
        copies["wm1"].wait()

    with _scope("noffn"):
        yv[...] = jnp.zeros(yv.shape, F32)
        fv[...] = jnp.zeros(fv.shape, F32)
        modv[:, 5 * D:6 * D] = jnp.zeros((8, D), F32)
        pair(jnp.int32(0), False)

    with _scope("waitffn"):
        copies["w1"].wait()
        copies["w3"].wait()
        copies["w2"].wait()

    def late_inputs():
        copies["wm2"].wait()
        copies["x2"].wait()
        mod_part(5 * D, D)

    def pair_ffn(p, c):
        _rarely(p == MAIN_START + 1, late_inputs)

        @pl.when(p > MAIN_START + 1)
        def _():
            out_copy(pl.multiple_of((p - 3) * PT, PT), PT).start()

        pair(p, True)
        return c

    with _scope("main"):
        lax.fori_loop(MAIN_START, NPAIR, pair_ffn, 0)

    with _scope("epi"):
        out_copy((NPAIR - 3) * PT, PT).start()
        finish((NPAIR - 2) * PT)
        post_attn((NPAIR - 1) * PT)
        out_copy((NPAIR - 2) * PT, PT).start()

        def up_body(i, c):
            ffn_up(0, EPI_UP, i * (EPI_UP * FC))
            return c

        def down_body(i, c):
            ffn_down(0, EPI_DOWN, i * (EPI_DOWN * 256), (NPAIR - 1) * PT)
            return c

        lax.fori_loop(0, NFC // EPI_UP, up_body, 0)
        lax.fori_loop(0, 4 // EPI_DOWN, down_body, 0)
        out_copy((NPAIR - 1) * PT, PT).start()
    with _scope("waitout"):
        out_copy(0, S - (MAIN_START - 1) * PT).wait()


@functools.partial(jax.jit, static_argnames=("A_seg_len",))
def pallas_adaLN_cond__memory_aug_recurrent_mem_tr__glu_gated_swiglu__prompt_kernel(
    A_x, A_mem0, A_Wq, A_Wk, A_Wv, A_Wo, A_seg_len, B_x, B_w1, B_w3, B_w2, c, w_mod,
):
    assert A_seg_len == SEG
    assert A_x.shape == (1, S, D) and A_mem0.shape == (1, MEM, D)
    assert A_Wq.shape == (D, H, DH) and B_w1.shape == (D, FF)
    del B_x

    scratch = [
        pltpu.VMEM((S, D), BF16),
        pltpu.VMEM((S, D), BF16),
        pltpu.VMEM((HD // 2, D), U32),
        pltpu.VMEM((D // 2, FF), U32),
        pltpu.VMEM((D // 2, FF), U32),
        pltpu.VMEM((FF // 2, D), U32),
        pltpu.VMEM((D // 2, 6 * D), U32),
        pltpu.VMEM((1, D), BF16),
        pltpu.VMEM((MEM, D), BF16),
        pltpu.VMEM((8, 6 * D), F32),
        pltpu.VMEM((X0, D), F32),
        pltpu.VMEM((PRO // 2, D), U32),
        pltpu.VMEM((2 * HG, PRO, DH), F32),
        pltpu.VMEM((32, D), F32),
        pltpu.VMEM((32, D), F32),
        pltpu.VMEM((24, HD), U32),
        pltpu.VMEM((PT, D), F32),
        pltpu.VMEM((PT, D), F32),
        pltpu.VMEM((PT, D), F32),
        pltpu.VMEM((PT // 2, D), U32),
        pltpu.VMEM((PT // 2, FF), U32),
        pltpu.SemaphoreType.DMA((11,)),
        pltpu.SemaphoreType.DMA((KT,)),
        pltpu.SemaphoreType.DMA((NJ,)),
        pltpu.SemaphoreType.DMA,
    ] + [pltpu.VMEM((G // 2, 3 * HG, NSLOT * SLOT, DH), U32)] * 2 + [
        pltpu.VMEM((G // 2, 3 * HG, D // 2, DH), U32)] * 2

    out = pl.pallas_call(
        _kernel,
        out_shape=jax.ShapeDtypeStruct((S, D), BF16),
        in_specs=[pl.BlockSpec(memory_space=pl.ANY)] * 11,
        out_specs=pl.BlockSpec(memory_space=pl.ANY),
        scratch_shapes=scratch,
        compiler_params=pltpu.CompilerParams(
            vmem_limit_bytes=120 * 1024 * 1024, disable_bounds_checks=True),
    )(
        A_x.reshape(S, D), A_mem0.reshape(MEM, D),
        A_Wq.reshape(D // 2, 2, H, DH), A_Wk.reshape(D // 2, 2, H, DH),
        A_Wv.reshape(D // 2, 2, H, DH), A_Wo.reshape(HD, D),
        B_w1, B_w3, B_w2, c, w_mod,
    )
    return out.reshape(1, S, D)
```

```python
import functools

import jax
import jax.numpy as jnp
from jax import lax
import jax.experimental.pallas as pl
import jax.experimental.pallas.tpu as pltpu

F32 = jnp.float32
BF16 = jnp.bfloat16
U32 = jnp.uint32

S = 2048
D = 1024
H = 32
DH = 128
HD = H * DH
MEM = 8
SEG = 32
FF = 3584
EPS = 1e-5
LOG2E = 1.4426950408889634

G = 8
HG = H // G
PRO = 512
NPAIR = S // (2 * SEG)
PT = 2 * SEG
SLOT = 40
NSLOT = 9
X0 = 544
X1 = 640
FC = 256
NFC = FF // FC
KW = 128
KT = D // KW
MW = 128
KPM = MW // KW
NJ = 3 * G // 2
FILL = (0, 2, 4, 9, 11, 14)
QKPOS = 3
MODF = (0, 1, 4, 5, 7, 8, 11, 12)
EPI_UP = 7
EPI_DOWN = 2
MAIN_START = 1
SCOPES = False
KSTART = 4


class _NoScope:
    def __enter__(self):
        return self

    def __exit__(self, *a):
        return False


def _scope(name):
    return jax.named_scope(name) if SCOPES else _NoScope()


def _unpack(x):
    return pltpu.bitcast(x, BF16)


def _pack(x):
    return pltpu.bitcast(x.astype(BF16), U32)


def _dot(a, b):
    return jnp.dot(a, b, preferred_element_type=F32)


def _ln(x):
    m = jnp.mean(x, axis=-1, keepdims=True)
    xc = x - m
    v = jnp.mean(xc * xc, axis=-1, keepdims=True)
    return xc * lax.rsqrt(v + EPS)


def _recip(x):
    r = pl.reciprocal(x, approx=True)
    return r * (2.0 - x * r)


def _silu(x):
    h = 0.5 * x
    return h + h * jnp.tanh(h)


def _cols(off, w):
    if isinstance(off, int):
        return slice(off, off + w)
    return pl.ds(pl.multiple_of(off, w), w)


def _rarely(cond, fn):
    def body(_, c):
        fn()
        return c

    lax.fori_loop(0, cond.astype(jnp.int32), body, 0)


def _masks():
    def pos(j):
        return jnp.where(j < 40, j, jnp.where(j < 48, j - 32, jnp.where(j < 56, j - 48, j - 40)))

    out = []
    for q0, nq, nk in ((0, 32, 48), (32, 48, 80)):
        qi = lax.broadcasted_iota(jnp.int32, (nq, nk), 0) + q0
        kj = lax.broadcasted_iota(jnp.int32, (nq, nk), 1)
        qp, kp = pos(qi), pos(kj)
        same = ((qi < 40) & (kj < 40)) | ((qi >= 40) & (kj >= 40))
        allowed = same & ((qp < MEM) | (qp >= kp))
        fill = jnp.where(same, jnp.float32(-1e9 * DH ** 0.5), jnp.float32(-jnp.inf))
        out.append((allowed, fill))
    return out


def _kernel(x_hbm, mem0_hbm, wq_hbm, wk_hbm, wv_hbm, wo_hbm, w1_hbm, w3_hbm, w2_hbm,
            c_hbm, wm_hbm, out_hbm,
            xv, outv, wo, w1, w3, w2, wm, cv, m0v, modv, xh, h0, acc,
            lhs_a, lhs_b, o32, abuf, yv, fv, h2, hid, sem_in, sem_m, sem_w, sem_out, *rest):
    ring = rest[0:2]
    wg = rest[2:4]
    scale = DH ** -0.5

    copies = {}

    def mk(name, src, dst):
        copies[name] = pltpu.make_async_copy(src, dst, sem_in.at[len(copies)])

    wm_u = wm_hbm.bitcast(U32)
    mk("c", c_hbm, cv)
    mk("mem0", mem0_hbm, m0v)
    mk("x0", x_hbm.at[0:X0], xv.at[0:X0])
    mk("x1", x_hbm.at[X0:X1], xv.at[X0:X1])
    mk("wo", wo_hbm.bitcast(U32), wo)
    mk("wm1", wm_u.at[:, 2 * D:5 * D], wm.at[:, 2 * D:5 * D])
    mk("w1", w1_hbm.bitcast(U32), w1)
    mk("w3", w3_hbm.bitcast(U32), w3)
    mk("w2", w2_hbm.bitcast(U32), w2)
    mk("wm2", wm_u.at[:, 5 * D:6 * D], wm.at[:, 5 * D:6 * D])
    mk("x2", x_hbm.at[X1:S], xv.at[X1:S])

    def mod_copies(kt):
        return [pltpu.make_async_copy(wm_u.at[:, _cols(i * D + kt * MW, MW)],
                                      wm.at[:, _cols(i * D + kt * MW, MW)], sem_m.at[kt])
                for i in range(2)]

    w_hbm = (wq_hbm, wk_hbm, wv_hbm)

    def block_copies(j, m, gi, t0):
        return [
            pltpu.make_async_copy(
                w_hbm[m].bitcast(U32).at[:, par, (2 * gi + pg) * (HG // 2) + jj],
                wg[pg].at[gi, t0 + 2 * jj + par], sem_w.at[j])
            for pg in range(2) for jj in range(HG // 2) for par in range(2)]

    def start_block(j):
        for c in block_copies(j, j // 4, j % 4, (j // 4) * HG):
            c.start()

    def wait_block(j, gi, t0):
        for c in block_copies(j, 0, gi, t0):
            c.wait()

    for n in ("x0", "c", "mem0"):
        copies[n].start()

    def zero(i, c):
        acc[i] = jnp.zeros(acc.shape[1:], F32)
        return c

    lax.fori_loop(0, 2 * HG, zero, 0)
    start_block(0)
    for kt in range(D // MW):
        for c in mod_copies(kt):
            c.start()

    def out_copy(r0, n):
        return pltpu.make_async_copy(outv.at[pl.ds(r0, n)], out_hbm.at[pl.ds(r0, n)], sem_out)

    def silu_c():
        return jnp.broadcast_to(_silu(cv[...].astype(F32)), (16, D)).astype(BF16)

    def mod_part(off, w):
        r = _dot(silu_c(), _unpack(wm[:, _cols(off, w)]))[0:8]
        modv[:, _cols(off, w)] = r
        return r[0:1]

    def mvec(i):
        return modv[0:1, i * D:(i + 1) * D]

    def ln1(r0, n):
        xf = xv[pl.ds(r0, n), :].astype(F32)
        return _ln(xf) * (1.0 + mvec(1)) + mvec(0)

    def repack_slot(w, gi, t, enable=None):
        for r0 in range(0, D // 2, 32):
            a = w[gi, t, r0:r0 + 32, :]
            b = w[gi, t + 1, r0:r0 + 32, :]
            e = (a & jnp.uint32(0xFFFF)) | (b << 16)
            o = (a >> 16) | (b & jnp.uint32(0xFFFF0000))
            if enable is not None:
                e = jnp.where(enable, e, a)
                o = jnp.where(enable, o, b)
            w[gi, t, r0:r0 + 32, :] = e
            w[gi, t + 1, r0:r0 + 32, :] = o

    def repack_now(gi, t0):
        def body(i, c):
            for w in wg:
                repack_slot(w, gi, t0 + 2 * i)
            return c

        lax.fori_loop(0, HG // 2, body, 0)

    def store_tokens(dst, gi, t, r):
        for pp in range(PRO // PT):
            b0, r0 = pp * SLOT, pp * PT
            dst[gi, t, b0 + 4:b0 + 8, :] = _pack(r[r0:r0 + 8])
            dst[gi, t, b0 + 8:b0 + 24, :] = _pack(r[r0 + 8:r0 + 40])
            dst[gi, t, b0 + 28:b0 + 32, :] = _pack(r[r0 + 40:r0 + 48])
            dst[gi, t, b0 + 32:b0 + 40, :] = _pack(r[r0 + 48:r0 + 64])

    def proj(lhs, g, rows, ts):
        for t in ts:
            r = _dot(lhs, _unpack(wg[g % 2][g // 2, t]))
            for i, row in enumerate(rows):
                ring[g % 2][g // 2, t, pl.ds(row, 4), :] = _pack(r[8 * i:8 * i + 8])

    def attn_qk(g, base, q0, nq, nk, allowed, fill):
        qrow = pl.multiple_of(base + q0 // 2, 8)
        ps = []
        for hh in range(HG):
            q = _unpack(ring[g % 2][g // 2, hh, pl.ds(qrow, nq // 2), :])
            k = _unpack(ring[g % 2][g // 2, HG + hh, pl.ds(base, nk // 2), :])
            s = lax.dot_general(q, k, (((1,), (1,)), ((), ())), preferred_element_type=F32)
            s = jnp.where(allowed, s, fill)
            m = jnp.max(s, axis=-1, keepdims=True)
            p = jnp.exp2((s - m) * (scale * LOG2E))
            l = jnp.sum(p, axis=-1, keepdims=True)
            ps.append((p * _recip(l)).astype(BF16))
        return ps

    def attn_pv(g, base, nq, nk, ps):
        for hh in range(HG):
            v = _unpack(ring[g % 2][g // 2, 2 * HG + hh, pl.ds(base, nk // 2), :])
            col = (g * HG + hh) * DH
            o32[0:nq // 2, col:col + DH] = _pack(_dot(ps[hh], v))

    def wo_proj(nq, stores):
        o = _unpack(o32[0:nq // 2, :])
        cw = 256
        for cb in range(D // cw):
            cs = slice(cb * cw, (cb + 1) * cw)
            r = _dot(o, _unpack(wo[:, cs]))
            for r0, n, fn in stores:
                fn(cs, r[r0:r0 + n])

    def post_attn(tok0):
        x1 = xv[pl.ds(tok0, PT), :].astype(F32) + mvec(2) * abuf[...]
        yv[...] = x1
        h2[...] = _pack(_ln(x1) * (1.0 + mvec(4)) + mvec(3))

    def ffn_up(c0, c1, off=0):
        a = _unpack(h2[...])
        for c in range(c0, c1):
            cs = _cols(off + c * FC, FC)
            gt = _dot(a, _unpack(w1[:, cs]))
            up = _dot(a, _unpack(w3[:, cs]))
            hid[:, cs] = _pack(_silu(gt) * up)

    def ffn_down(cb0, cb1, off=0, tok0=None):
        a = _unpack(hid[...])
        cw = 256
        for cb in range(cb0, cb1):
            cs = _cols(off + cb * cw, cw)
            r = _dot(a, _unpack(w2[:, cs]))
            if tok0 is None:
                fv[:, cs] = r
            else:
                gb = modv[0:1, _cols(off + 5 * D + cb * cw, cw)]
                outv[pl.ds(tok0, PT), cs] = (yv[:, cs] + gb * r).astype(BF16)

    def finish(tok0):
        outv[pl.ds(tok0, PT), :] = (yv[...] + mvec(5) * fv[...]).astype(BF16)

    def unit_row(u):
        r = u & 7
        slot = lax.rem(u >> 3, NSLOT)
        return pl.multiple_of(slot * SLOT + 4 + 4 * r + 4 * (r >= 5).astype(jnp.int32), 4)

    with _scope("waitx0"):
        copies["x0"].wait()
    with _scope("ln0"):

        def ln_body(i, c):
            r0 = pl.multiple_of(i * 136, 8)
            xh[pl.ds(r0, 136), :] = _ln(xv[pl.ds(r0, 136), :].astype(F32))
            return c

        lax.fori_loop(0, X0 // 136, ln_body, 0)
    with _scope("waitc"):
        copies["c"].wait()
        copies["mem0"].wait()
        lhs_a[0:MEM, :] = m0v[...].astype(F32)

    def modulate(kt):
        sa = mod_part(kt * KW, KW)
        ca = mod_part(D + kt * KW, KW)
        a = _pack(xh[0:PRO, _cols(kt * KW, KW)] * (1.0 + ca) + sa)
        h0[:, _cols(kt * KW, KW)] = a
        return a

    with _scope("waitw0"):
        wait_block(0, 0, 0)
    with _scope("first"):
        repack_now(0, 0)
        with _scope("waitm0"):
            for c in mod_copies(0):
                c.wait()
        a0 = modulate(0)

    def kmajor(kt, a):
        kn = jnp.minimum(kt + 1, KT - 1)

        def more():
            for j in range(1, 4):
                start_block(j)

        _rarely(kt == KSTART, more)

        @pl.when((kt < KT - 1) & (lax.rem(kn, KPM) == 0))
        def _():
            for c in mod_copies(lax.div(kn, KPM)):
                c.wait()

        rows = pl.ds(pl.multiple_of(kt * (KW // 2), KW // 2), KW // 2)
        a_next = None
        for pg in range(2):
            for t in range(HG):
                acc[pg * HG + t] += _dot(_unpack(a), _unpack(wg[pg][0, t, rows, :]))
            if pg == 0:
                a_next = modulate(kn)
        return a_next

    with _scope("kmajor"):
        lax.fori_loop(0, KT, kmajor, a0)
        lhs_a[MEM:32, :] = xh[PRO:PRO + 24, :] * (1.0 + mvec(1)) + mvec(0)

        def flush(t, c):
            for pg in range(2):
                store_tokens(ring[pg], 0, t, acc[pg * HG + t])
            return c

        lax.fori_loop(0, HG, flush, 0)

    def pro_body(j, c):
        gi, t0 = j & 3, (j >> 2) * HG
        jn = jnp.minimum(j + 1, NJ - 1)
        gn, tn = jn & 3, (jn >> 2) * HG
        prefetch = (j > 1) & (j < NJ - 1)

        def batch(js, names):
            def fn():
                for jj in js:
                    start_block(jj)
                for n in names:
                    copies[n].start()
            return fn

        def late():
            with _scope("waitlate"):
                wait_block(j, gi, t0)
            repack_now(gi, t0)

        _rarely(j == 1, batch(range(4, 9), ()))
        _rarely(j == 3, batch(range(9, NJ), ("x1", "wo", "wm1", "w1", "w3", "w2", "wm2", "x2")))
        _rarely(j <= 2, late)

        @pl.when(prefetch)
        def _():
            wait_block(jn, gn, tn)

        a = _unpack(h0[...])
        for pg in range(2):
            for t in range(HG):
                store_tokens(ring[pg], gi, t0 + t, _dot(a, _unpack(wg[pg][gi, t0 + t])))
        gr, tr = jnp.where(prefetch, gn, gi), jnp.where(prefetch, tn, t0)
        for w in wg:
            for t in range(0, HG, 2):
                repack_slot(w, gr, tr + t, prefetch)
        return c

    with _scope("pro"):
        lax.fori_loop(1, NJ, pro_body, 0)

    def pair(p, with_ffn):
        (al_a, fi_a), (al_b, fi_b) = _masks()
        base = pl.multiple_of(lax.rem(p, NSLOT) * SLOT, 8)
        u0 = PRO // 8 + 6 * p
        tlead = PRO + 48 * p

        if with_ffn:
            finish(pl.multiple_of(jnp.maximum(p - 2, 0) * PT, PT))
            post_attn(pl.multiple_of((p - 1) * PT, PT))

        def filler(i, c0=None, c1=None):
            if not with_ffn:
                if i is not None:
                    mod_part(2 * D + MODF[i] * 256, (MODF[i + 1] - MODF[i]) * 256)
            elif c0 is None:
                ffn_down(0, 4)
            else:
                ffn_up(c0, c1)

        def proj_attn(lhs, rows, q0, nq, nk, allowed, fill, f, m0):
            order = list(range(2 * HG, 3 * HG)) + list(range(2 * HG))
            ps = None
            for g in range(G):
                proj(lhs, g, rows, order[:QKPOS])
                if g > 0:
                    ps = attn_qk(g - 1, base, q0, nq, nk, allowed, fill)
                proj(lhs, g, rows, order[QKPOS:])
                if g > 0:
                    attn_pv(g - 1, base, nq, nk, ps)
            filler(m0, FILL[f], FILL[f] + 1)
            ps = attn_qk(G - 1, base, q0, nq, nk, allowed, fill)
            filler(m0 + 1, FILL[f] + 1, FILL[f + 1])
            attn_pv(G - 1, base, nq, nk, ps)
            filler(m0 + 2, FILL[f + 1], FILL[f + 2])

        def st_lhs(ref):
            def fn(cs, val):
                ref[0:MEM, cs] = val.astype(BF16).astype(F32)
            return fn

        def st_a(r0, n):
            def fn(cs, val):
                abuf[r0:r0 + n, cs] = val
            return fn

        lhs = lhs_a[...].astype(BF16)
        rows = [base, unit_row(u0), unit_row(u0 + 1), unit_row(u0 + 2)]
        lhs_b[MEM:32, :] = ln1(pl.multiple_of(tlead + 24, 8), 24)
        proj_attn(lhs, rows, 0, 32, 48, al_a, fi_a, 0, 0)
        wo_proj(32, [(0, 8, st_lhs(lhs_b)), (8, 24, st_a(0, 24))])
        filler(3, FILL[2], FILL[3])

        lhs = lhs_b[...].astype(BF16)
        rows = [pl.multiple_of(base + 24, 8), unit_row(u0 + 3), unit_row(u0 + 4), unit_row(u0 + 5)]
        nxt = pl.multiple_of(jnp.minimum(tlead + 48, S - 24), 8)
        lhs_a[MEM:32, :] = ln1(nxt, 24)
        proj_attn(lhs, rows, 32, 48, 80, al_b, fi_b, 3, 4)
        wo_proj(48, [(16, 8, st_lhs(lhs_a)), (0, 16, st_a(24, 16)), (24, 24, st_a(40, 24))])
        filler(None)

    with _scope("waitwo"):
        copies["x1"].wait()
        copies["wo"].wait()
        copies["wm1"].wait()

    with _scope("noffn"):
        yv[...] = jnp.zeros(yv.shape, F32)
        fv[...] = jnp.zeros(fv.shape, F32)
        modv[:, 5 * D:6 * D] = jnp.zeros((8, D), F32)
        pair(jnp.int32(0), False)

    with _scope("waitffn"):
        copies["w1"].wait()
        copies["w3"].wait()
        copies["w2"].wait()

    def late_inputs():
        copies["wm2"].wait()
        copies["x2"].wait()
        mod_part(5 * D, D)

    def pair_ffn(p, c):
        _rarely(p == MAIN_START + 1, late_inputs)

        @pl.when(p > MAIN_START + 1)
        def _():
            out_copy(pl.multiple_of((p - 3) * PT, PT), PT).start()

        pair(p, True)
        return c

    with _scope("main"):
        lax.fori_loop(MAIN_START, NPAIR, pair_ffn, 0)

    with _scope("epi"):
        out_copy((NPAIR - 3) * PT, PT).start()
        finish((NPAIR - 2) * PT)
        post_attn((NPAIR - 1) * PT)
        out_copy((NPAIR - 2) * PT, PT).start()

        def up_body(i, c):
            ffn_up(0, EPI_UP, i * (EPI_UP * FC))
            return c

        def down_body(i, c):
            ffn_down(0, EPI_DOWN, i * (EPI_DOWN * 256), (NPAIR - 1) * PT)
            return c

        lax.fori_loop(0, NFC // EPI_UP, up_body, 0)
        lax.fori_loop(0, 4 // EPI_DOWN, down_body, 0)
        out_copy((NPAIR - 1) * PT, PT).start()
    with _scope("waitout"):
        out_copy(0, S - (MAIN_START - 1) * PT).wait()


@functools.partial(jax.jit, static_argnames=("A_seg_len",))
def pallas_adaLN_cond__memory_aug_recurrent_mem_tr__glu_gated_swiglu__prompt_kernel(
    A_x, A_mem0, A_Wq, A_Wk, A_Wv, A_Wo, A_seg_len, B_x, B_w1, B_w3, B_w2, c, w_mod,
):
    assert A_seg_len == SEG
    assert A_x.shape == (1, S, D) and A_mem0.shape == (1, MEM, D)
    assert A_Wq.shape == (D, H, DH) and B_w1.shape == (D, FF)
    del B_x

    scratch = [
        pltpu.VMEM((S, D), BF16),
        pltpu.VMEM((S, D), BF16),
        pltpu.VMEM((HD // 2, D), U32),
        pltpu.VMEM((D // 2, FF), U32),
        pltpu.VMEM((D // 2, FF), U32),
        pltpu.VMEM((FF // 2, D), U32),
        pltpu.VMEM((D // 2, 6 * D), U32),
        pltpu.VMEM((1, D), BF16),
        pltpu.VMEM((MEM, D), BF16),
        pltpu.VMEM((8, 6 * D), F32),
        pltpu.VMEM((X0, D), F32),
        pltpu.VMEM((PRO // 2, D), U32),
        pltpu.VMEM((2 * HG, PRO, DH), F32),
        pltpu.VMEM((32, D), F32),
        pltpu.VMEM((32, D), F32),
        pltpu.VMEM((24, HD), U32),
        pltpu.VMEM((PT, D), F32),
        pltpu.VMEM((PT, D), F32),
        pltpu.VMEM((PT, D), F32),
        pltpu.VMEM((PT // 2, D), U32),
        pltpu.VMEM((PT // 2, FF), U32),
        pltpu.SemaphoreType.DMA((11,)),
        pltpu.SemaphoreType.DMA((KT,)),
        pltpu.SemaphoreType.DMA((NJ,)),
        pltpu.SemaphoreType.DMA,
    ] + [pltpu.VMEM((G // 2, 3 * HG, NSLOT * SLOT, DH), U32)] * 2 + [
        pltpu.VMEM((G // 2, 3 * HG, D // 2, DH), U32)] * 2

    out = pl.pallas_call(
        _kernel,
        out_shape=jax.ShapeDtypeStruct((S, D), BF16),
        in_specs=[pl.BlockSpec(memory_space=pl.ANY)] * 11,
        out_specs=pl.BlockSpec(memory_space=pl.ANY),
        scratch_shapes=scratch,
        compiler_params=pltpu.CompilerParams(
            vmem_limit_bytes=120 * 1024 * 1024, disable_bounds_checks=True),
    )(
        A_x.reshape(S, D), A_mem0.reshape(MEM, D),
        A_Wq.reshape(D // 2, 2, H, DH), A_Wk.reshape(D // 2, 2, H, DH),
        A_Wv.reshape(D // 2, 2, H, DH), A_Wo.reshape(HD, D),
        B_w1, B_w3, B_w2, c, w_mod,
    )
    return out.reshape(1, S, D)
```

```python
import functools

import jax
import jax.numpy as jnp
from jax import lax
import jax.experimental.pallas as pl
import jax.experimental.pallas.tpu as pltpu

F32 = jnp.float32
BF16 = jnp.bfloat16
U32 = jnp.uint32

S = 2048
D = 1024
H = 32
DH = 128
HD = H * DH
MEM = 8
SEG = 32
FF = 3584
EPS = 1e-5
LOG2E = 1.4426950408889634

G = 8
HG = H // G
PRO = 512
NPAIR = S // (2 * SEG)
PT = 2 * SEG
SLOT = 40
NSLOT = 9
X0 = 544
X1 = 640
FC = 256
NFC = FF // FC
KW = 128
KT = D // KW
MW = 128
KPM = MW // KW
NJ = 3 * G // 2
FILL = (0, 2, 4, 9, 11, 14)
MODF = (0, 4, 5, 7, 11, 12)
EPI_UP = 7
EPI_DOWN = 2
MAIN_START = 1
SCOPES = False
KSTART = 4


class _NoScope:
    def __enter__(self):
        return self

    def __exit__(self, *a):
        return False


def _scope(name):
    return jax.named_scope(name) if SCOPES else _NoScope()


def _unpack(x):
    return pltpu.bitcast(x, BF16)


def _pack(x):
    return pltpu.bitcast(x.astype(BF16), U32)


def _dot(a, b):
    return jnp.dot(a, b, preferred_element_type=F32)


def _ln(x):
    m = jnp.mean(x, axis=-1, keepdims=True)
    xc = x - m
    v = jnp.mean(xc * xc, axis=-1, keepdims=True)
    return xc * lax.rsqrt(v + EPS)


def _recip(x):
    r = pl.reciprocal(x, approx=True)
    return r * (2.0 - x * r)


def _silu(x):
    h = 0.5 * x
    return h + h * jnp.tanh(h)


def _cols(off, w):
    if isinstance(off, int):
        return slice(off, off + w)
    return pl.ds(pl.multiple_of(off, w), w)


def _rarely(cond, fn):
    def body(_, c):
        fn()
        return c

    lax.fori_loop(0, cond.astype(jnp.int32), body, 0)


def _masks():
    def pos(j):
        return jnp.where(j < 40, j, jnp.where(j < 48, j - 32, jnp.where(j < 56, j - 48, j - 40)))

    out = []
    for q0, nq, nk in ((0, 32, 48), (32, 48, 80)):
        qi = lax.broadcasted_iota(jnp.int32, (nq, nk), 0) + q0
        kj = lax.broadcasted_iota(jnp.int32, (nq, nk), 1)
        qp, kp = pos(qi), pos(kj)
        same = ((qi < 40) & (kj < 40)) | ((qi >= 40) & (kj >= 40))
        allowed = same & ((qp < MEM) | (qp >= kp))
        fill = jnp.where(same, jnp.float32(-1e9 * DH ** 0.5), jnp.float32(-jnp.inf))
        out.append((allowed, fill))
    return out


def _kernel(x_hbm, mem0_hbm, wq_hbm, wk_hbm, wv_hbm, wo_hbm, w1_hbm, w3_hbm, w2_hbm,
            c_hbm, wm_hbm, out_hbm,
            xv, outv, wo, w1, w3, w2, wm, cv, m0v, modv, xh, h0, acc,
            lhs_a, lhs_b, o32, abuf, yv, fv, h2, hid, sem_in, sem_m, sem_w, sem_out, *rest):
    ring = rest[0:2]
    wg = rest[2:4]

    def side(g, t):
        return (g % 2) ^ int(t >= 2 * HG)

    scale = DH ** -0.5

    copies = {}

    def mk(name, src, dst):
        copies[name] = pltpu.make_async_copy(src, dst, sem_in.at[len(copies)])

    wm_u = wm_hbm.bitcast(U32)
    mk("c", c_hbm, cv)
    mk("mem0", mem0_hbm, m0v)
    mk("x0", x_hbm.at[0:X0], xv.at[0:X0])
    mk("x1", x_hbm.at[X0:X1], xv.at[X0:X1])
    mk("wo", wo_hbm.bitcast(U32), wo)
    mk("wm1", wm_u.at[:, 2 * D:5 * D], wm.at[:, 2 * D:5 * D])
    mk("w1", w1_hbm.bitcast(U32), w1)
    mk("w3", w3_hbm.bitcast(U32), w3)
    mk("w2", w2_hbm.bitcast(U32), w2)
    mk("wm2", wm_u.at[:, 5 * D:6 * D], wm.at[:, 5 * D:6 * D])
    mk("x2", x_hbm.at[X1:S], xv.at[X1:S])

    def mod_copies(kt):
        return [pltpu.make_async_copy(wm_u.at[:, _cols(i * D + kt * MW, MW)],
                                      wm.at[:, _cols(i * D + kt * MW, MW)], sem_m.at[kt])
                for i in range(2)]

    w_hbm = (wq_hbm, wk_hbm, wv_hbm)

    def block_copies(j, m, gi, t0):
        return [
            pltpu.make_async_copy(
                w_hbm[m].bitcast(U32).at[:, par, (2 * gi + pg) * (HG // 2) + jj],
                wg[side(pg, m * HG)].at[gi, t0 + 2 * jj + par], sem_w.at[j])
            for pg in range(2) for jj in range(HG // 2) for par in range(2)]

    def start_block(j):
        for c in block_copies(j, j // 4, j % 4, (j // 4) * HG):
            c.start()

    def wait_block(j, gi, t0):
        for c in block_copies(j, 0, gi, t0):
            c.wait()

    for n in ("x0", "c", "mem0"):
        copies[n].start()

    def zero(i, c):
        acc[i] = jnp.zeros(acc.shape[1:], F32)
        return c

    lax.fori_loop(0, 2 * HG, zero, 0)
    start_block(0)
    for kt in range(D // MW):
        for c in mod_copies(kt):
            c.start()

    def out_copy(r0, n):
        return pltpu.make_async_copy(outv.at[pl.ds(r0, n)], out_hbm.at[pl.ds(r0, n)], sem_out)

    def silu_c():
        return jnp.broadcast_to(_silu(cv[...].astype(F32)), (16, D)).astype(BF16)

    def mod_part(off, w):
        r = _dot(silu_c(), _unpack(wm[:, _cols(off, w)]))[0:8]
        modv[:, _cols(off, w)] = r
        return r[0:1]

    def mvec(i):
        return modv[0:1, i * D:(i + 1) * D]

    def ln1(r0, n):
        xf = xv[pl.ds(r0, n), :].astype(F32)
        return _ln(xf) * (1.0 + mvec(1)) + mvec(0)

    def repack_slot(w, gi, t, enable=None):
        for r0 in range(0, D // 2, 32):
            a = w[gi, t, r0:r0 + 32, :]
            b = w[gi, t + 1, r0:r0 + 32, :]
            e = (a & jnp.uint32(0xFFFF)) | (b << 16)
            o = (a >> 16) | (b & jnp.uint32(0xFFFF0000))
            if enable is not None:
                e = jnp.where(enable, e, a)
                o = jnp.where(enable, o, b)
            w[gi, t, r0:r0 + 32, :] = e
            w[gi, t + 1, r0:r0 + 32, :] = o

    def repack_now(gi, t0):
        def body(i, c):
            for w in wg:
                repack_slot(w, gi, t0 + 2 * i)
            return c

        lax.fori_loop(0, HG // 2, body, 0)

    def store_tokens(dst, gi, t, r):
        for pp in range(PRO // PT):
            b0, r0 = pp * SLOT, pp * PT
            dst[gi, t, b0 + 4:b0 + 8, :] = _pack(r[r0:r0 + 8])
            dst[gi, t, b0 + 8:b0 + 24, :] = _pack(r[r0 + 8:r0 + 40])
            dst[gi, t, b0 + 28:b0 + 32, :] = _pack(r[r0 + 40:r0 + 48])
            dst[gi, t, b0 + 32:b0 + 40, :] = _pack(r[r0 + 48:r0 + 64])

    def proj(lhs, g, rows):
        for t in range(3 * HG):
            r = _dot(lhs, _unpack(wg[side(g, t)][g // 2, t]))
            for i, row in enumerate(rows):
                ring[side(g, t)][g // 2, t, pl.ds(row, 4), :] = _pack(r[8 * i:8 * i + 8])

    def attn_qk(g, base, q0, nq, nk, allowed, fill):
        qrow = pl.multiple_of(base + q0 // 2, 8)
        ps = []
        for hh in range(HG):
            q = _unpack(ring[g % 2][g // 2, hh, pl.ds(qrow, nq // 2), :])
            k = _unpack(ring[g % 2][g // 2, HG + hh, pl.ds(base, nk // 2), :])
            s = lax.dot_general(q, k, (((1,), (1,)), ((), ())), preferred_element_type=F32)
            s = jnp.where(allowed, s, fill)
            m = jnp.max(s, axis=-1, keepdims=True)
            p = jnp.exp2((s - m) * (scale * LOG2E))
            l = jnp.sum(p, axis=-1, keepdims=True)
            ps.append((p * _recip(l)).astype(BF16))
        return ps

    def attn_pv(g, base, nq, nk, ps):
        for hh in range(HG):
            v = _unpack(ring[1 - g % 2][g // 2, 2 * HG + hh, pl.ds(base, nk // 2), :])
            col = (g * HG + hh) * DH
            o32[0:nq // 2, col:col + DH] = _pack(_dot(ps[hh], v))

    def wo_proj(nq, stores):
        o = _unpack(o32[0:nq // 2, :])
        cw = 256
        for cb in range(D // cw):
            cs = slice(cb * cw, (cb + 1) * cw)
            r = _dot(o, _unpack(wo[:, cs]))
            for r0, n, fn in stores:
                fn(cs, r[r0:r0 + n])

    def post_attn(tok0):
        x1 = xv[pl.ds(tok0, PT), :].astype(F32) + mvec(2) * abuf[...]
        yv[...] = x1
        h2[...] = _pack(_ln(x1) * (1.0 + mvec(4)) + mvec(3))

    def ffn_up(c0, c1, off=0):
        a = _unpack(h2[...])
        for c in range(c0, c1):
            cs = _cols(off + c * FC, FC)
            gt = _dot(a, _unpack(w1[:, cs]))
            up = _dot(a, _unpack(w3[:, cs]))
            hid[:, cs] = _pack(_silu(gt) * up)

    def ffn_down(cb0, cb1, off=0, tok0=None):
        a = _unpack(hid[...])
        cw = 256
        for cb in range(cb0, cb1):
            cs = _cols(off + cb * cw, cw)
            r = _dot(a, _unpack(w2[:, cs]))
            if tok0 is None:
                fv[:, cs] = r
            else:
                gb = modv[0:1, _cols(off + 5 * D + cb * cw, cw)]
                outv[pl.ds(tok0, PT), cs] = (yv[:, cs] + gb * r).astype(BF16)

    def finish(tok0):
        outv[pl.ds(tok0, PT), :] = (yv[...] + mvec(5) * fv[...]).astype(BF16)

    def unit_row(u):
        r = u & 7
        slot = lax.rem(u >> 3, NSLOT)
        return pl.multiple_of(slot * SLOT + 4 + 4 * r + 4 * (r >= 5).astype(jnp.int32), 4)

    with _scope("waitx0"):
        copies["x0"].wait()
    with _scope("ln0"):

        def ln_body(i, c):
            r0 = pl.multiple_of(i * 136, 8)
            xh[pl.ds(r0, 136), :] = _ln(xv[pl.ds(r0, 136), :].astype(F32))
            return c

        lax.fori_loop(0, X0 // 136, ln_body, 0)
    with _scope("waitc"):
        copies["c"].wait()
        copies["mem0"].wait()
        lhs_a[0:MEM, :] = m0v[...].astype(F32)

    def modulate(kt):
        sa = mod_part(kt * KW, KW)
        ca = mod_part(D + kt * KW, KW)
        a = _pack(xh[0:PRO, _cols(kt * KW, KW)] * (1.0 + ca) + sa)
        h0[:, _cols(kt * KW, KW)] = a
        return a

    with _scope("waitw0"):
        wait_block(0, 0, 0)
    with _scope("first"):
        repack_now(0, 0)
        with _scope("waitm0"):
            for c in mod_copies(0):
                c.wait()
        a0 = modulate(0)

    def kmajor(kt, a):
        kn = jnp.minimum(kt + 1, KT - 1)

        def more():
            for j in range(1, 4):
                start_block(j)

        _rarely(kt == KSTART, more)

        @pl.when((kt < KT - 1) & (lax.rem(kn, KPM) == 0))
        def _():
            for c in mod_copies(lax.div(kn, KPM)):
                c.wait()

        rows = pl.ds(pl.multiple_of(kt * (KW // 2), KW // 2), KW // 2)
        a_next = None
        for pg in range(2):
            for t in range(HG):
                acc[pg * HG + t] += _dot(_unpack(a), _unpack(wg[pg][0, t, rows, :]))
            if pg == 0:
                a_next = modulate(kn)
        return a_next

    with _scope("kmajor"):
        lax.fori_loop(0, KT, kmajor, a0)
        lhs_a[MEM:32, :] = xh[PRO:PRO + 24, :] * (1.0 + mvec(1)) + mvec(0)

        def flush(t, c):
            for pg in range(2):
                store_tokens(ring[pg], 0, t, acc[pg * HG + t])
            return c

        lax.fori_loop(0, HG, flush, 0)

    def pro_body(j, c):
        gi, t0 = j & 3, (j >> 2) * HG
        jn = jnp.minimum(j + 1, NJ - 1)
        gn, tn = jn & 3, (jn >> 2) * HG
        prefetch = (j > 1) & (j < NJ - 1)

        def batch(js, names):
            def fn():
                for jj in js:
                    start_block(jj)
                for n in names:
                    copies[n].start()
            return fn

        def late():
            with _scope("waitlate"):
                wait_block(j, gi, t0)
            repack_now(gi, t0)

        _rarely(j == 1, batch(range(4, 9), ()))
        _rarely(j == 3, batch(range(9, NJ), ("x1", "wo", "wm1", "w1", "w3", "w2", "wm2", "x2")))
        _rarely(j <= 2, late)

        @pl.when(prefetch)
        def _():
            wait_block(jn, gn, tn)

        a = _unpack(h0[...])
        for pg in range(2):
            for t in range(HG):
                store_tokens(ring[pg], gi, t0 + t, _dot(a, _unpack(wg[pg][gi, t0 + t])))
        gr, tr = jnp.where(prefetch, gn, gi), jnp.where(prefetch, tn, t0)
        for w in wg:
            for t in range(0, HG, 2):
                repack_slot(w, gr, tr + t, prefetch)
        return c

    with _scope("pro"):
        lax.fori_loop(1, NJ, pro_body, 0)

    def pair(p, with_ffn):
        (al_a, fi_a), (al_b, fi_b) = _masks()
        base = pl.multiple_of(lax.rem(p, NSLOT) * SLOT, 8)
        u0 = PRO // 8 + 6 * p
        tlead = PRO + 48 * p

        if with_ffn:
            finish(pl.multiple_of(jnp.maximum(p - 2, 0) * PT, PT))
            post_attn(pl.multiple_of((p - 1) * PT, PT))

        def filler(i, c0=None, c1=None):
            if not with_ffn:
                if i is not None:
                    mod_part(2 * D + MODF[i] * 256, (MODF[i + 1] - MODF[i]) * 256)
            elif c0 is None:
                ffn_down(0, 4)
            else:
                ffn_up(c0, c1)

        def proj_attn(lhs, rows, q0, nq, nk, allowed, fill, f):
            ps = None
            for g in range(G):
                proj(lhs, g, rows)
                if g > 0:
                    attn_pv(g - 1, base, nq, nk, ps)
                ps = attn_qk(g, base, q0, nq, nk, allowed, fill)
            filler(f, FILL[f], FILL[f + 1])
            attn_pv(G - 1, base, nq, nk, ps)
            filler(f + 1, FILL[f + 1], FILL[f + 2])

        def st_lhs(ref):
            def fn(cs, val):
                ref[0:MEM, cs] = val.astype(BF16).astype(F32)
            return fn

        def st_a(r0, n):
            def fn(cs, val):
                abuf[r0:r0 + n, cs] = val
            return fn

        lhs = lhs_a[...].astype(BF16)
        rows = [base, unit_row(u0), unit_row(u0 + 1), unit_row(u0 + 2)]
        lhs_b[MEM:32, :] = ln1(pl.multiple_of(tlead + 24, 8), 24)
        proj_attn(lhs, rows, 0, 32, 48, al_a, fi_a, 0)
        wo_proj(32, [(0, 8, st_lhs(lhs_b)), (8, 24, st_a(0, 24))])
        filler(2, FILL[2], FILL[3])

        lhs = lhs_b[...].astype(BF16)
        rows = [pl.multiple_of(base + 24, 8), unit_row(u0 + 3), unit_row(u0 + 4), unit_row(u0 + 5)]
        nxt = pl.multiple_of(jnp.minimum(tlead + 48, S - 24), 8)
        lhs_a[MEM:32, :] = ln1(nxt, 24)
        proj_attn(lhs, rows, 32, 48, 80, al_b, fi_b, 3)
        wo_proj(48, [(16, 8, st_lhs(lhs_a)), (0, 16, st_a(24, 16)), (24, 24, st_a(40, 24))])
        filler(None)

    with _scope("waitwo"):
        copies["x1"].wait()
        copies["wo"].wait()
        copies["wm1"].wait()

    with _scope("noffn"):
        yv[...] = jnp.zeros(yv.shape, F32)
        fv[...] = jnp.zeros(fv.shape, F32)
        modv[:, 5 * D:6 * D] = jnp.zeros((8, D), F32)
        pair(jnp.int32(0), False)

    with _scope("waitffn"):
        copies["w1"].wait()
        copies["w3"].wait()
        copies["w2"].wait()

    def late_inputs():
        copies["wm2"].wait()
        copies["x2"].wait()
        mod_part(5 * D, D)

    def pair_ffn(p, c):
        _rarely(p == MAIN_START + 1, late_inputs)

        @pl.when(p > MAIN_START + 1)
        def _():
            out_copy(pl.multiple_of((p - 3) * PT, PT), PT).start()

        pair(p, True)
        return c

    with _scope("main"):
        lax.fori_loop(MAIN_START, NPAIR, pair_ffn, 0)

    with _scope("epi"):
        out_copy((NPAIR - 3) * PT, PT).start()
        finish((NPAIR - 2) * PT)
        post_attn((NPAIR - 1) * PT)
        out_copy((NPAIR - 2) * PT, PT).start()

        def up_body(i, c):
            ffn_up(0, EPI_UP, i * (EPI_UP * FC))
            return c

        def down_body(i, c):
            ffn_down(0, EPI_DOWN, i * (EPI_DOWN * 256), (NPAIR - 1) * PT)
            return c

        lax.fori_loop(0, NFC // EPI_UP, up_body, 0)
        lax.fori_loop(0, 4 // EPI_DOWN, down_body, 0)
        out_copy((NPAIR - 1) * PT, PT).start()
    with _scope("waitout"):
        out_copy(0, S - (MAIN_START - 1) * PT).wait()


@functools.partial(jax.jit, static_argnames=("A_seg_len",))
def pallas_adaLN_cond__memory_aug_recurrent_mem_tr__glu_gated_swiglu__prompt_kernel(
    A_x, A_mem0, A_Wq, A_Wk, A_Wv, A_Wo, A_seg_len, B_x, B_w1, B_w3, B_w2, c, w_mod,
):
    assert A_seg_len == SEG
    assert A_x.shape == (1, S, D) and A_mem0.shape == (1, MEM, D)
    assert A_Wq.shape == (D, H, DH) and B_w1.shape == (D, FF)
    del B_x

    scratch = [
        pltpu.VMEM((S, D), BF16),
        pltpu.VMEM((S, D), BF16),
        pltpu.VMEM((HD // 2, D), U32),
        pltpu.VMEM((D // 2, FF), U32),
        pltpu.VMEM((D // 2, FF), U32),
        pltpu.VMEM((FF // 2, D), U32),
        pltpu.VMEM((D // 2, 6 * D), U32),
        pltpu.VMEM((1, D), BF16),
        pltpu.VMEM((MEM, D), BF16),
        pltpu.VMEM((8, 6 * D), F32),
        pltpu.VMEM((X0, D), F32),
        pltpu.VMEM((PRO // 2, D), U32),
        pltpu.VMEM((2 * HG, PRO, DH), F32),
        pltpu.VMEM((32, D), F32),
        pltpu.VMEM((32, D), F32),
        pltpu.VMEM((24, HD), U32),
        pltpu.VMEM((PT, D), F32),
        pltpu.VMEM((PT, D), F32),
        pltpu.VMEM((PT, D), F32),
        pltpu.VMEM((PT // 2, D), U32),
        pltpu.VMEM((PT // 2, FF), U32),
        pltpu.SemaphoreType.DMA((11,)),
        pltpu.SemaphoreType.DMA((KT,)),
        pltpu.SemaphoreType.DMA((NJ,)),
        pltpu.SemaphoreType.DMA,
    ] + [pltpu.VMEM((G // 2, 3 * HG, NSLOT * SLOT, DH), U32)] * 2 + [
        pltpu.VMEM((G // 2, 3 * HG, D // 2, DH), U32)] * 2

    out = pl.pallas_call(
        _kernel,
        out_shape=jax.ShapeDtypeStruct((S, D), BF16),
        in_specs=[pl.BlockSpec(memory_space=pl.ANY)] * 11,
        out_specs=pl.BlockSpec(memory_space=pl.ANY),
        scratch_shapes=scratch,
        compiler_params=pltpu.CompilerParams(
            vmem_limit_bytes=120 * 1024 * 1024, disable_bounds_checks=True),
    )(
        A_x.reshape(S, D), A_mem0.reshape(MEM, D),
        A_Wq.reshape(D // 2, 2, H, DH), A_Wk.reshape(D // 2, 2, H, DH),
        A_Wv.reshape(D // 2, 2, H, DH), A_Wo.reshape(HD, D),
        B_w1, B_w3, B_w2, c, w_mod,
    )
    return out.reshape(1, S, D)
```

```python
import functools

import jax
import jax.numpy as jnp
from jax import lax
import jax.experimental.pallas as pl
import jax.experimental.pallas.tpu as pltpu

F32 = jnp.float32
BF16 = jnp.bfloat16
U32 = jnp.uint32

S = 2048
D = 1024
H = 32
DH = 128
HD = H * DH
MEM = 8
SEG = 32
FF = 3584
EPS = 1e-5
LOG2E = 1.4426950408889634

G = 8
HG = H // G
PRO = 512
NPAIR = S // (2 * SEG)
PT = 2 * SEG
SLOT = 40
NSLOT = 9
X0 = 544
X1 = 640
FC = 256
NFC = FF // FC
KW = 128
KT = D // KW
MW = 128
KPM = MW // KW
NJ = 3 * G // 2
FILL = (0, 2, 4, 9, 11, 14)
QKPOS = 1
PVPOS = 11
MODF = (0, 5, 6, 8, 11, 12)
PROM = PRO + 32
EPI_UP = 7
EPI_DOWN = 2
MAIN_START = 1
SCOPES = False
KSTART = 4


class _NoScope:
    def __enter__(self):
        return self

    def __exit__(self, *a):
        return False


def _scope(name):
    return jax.named_scope(name) if SCOPES else _NoScope()


def _unpack(x):
    return pltpu.bitcast(x, BF16)


def _pack(x):
    return pltpu.bitcast(x.astype(BF16), U32)


def _dot(a, b):
    return jnp.dot(a, b, preferred_element_type=F32)


def _ln(x):
    m = jnp.mean(x, axis=-1, keepdims=True)
    xc = x - m
    v = jnp.mean(xc * xc, axis=-1, keepdims=True)
    return xc * lax.rsqrt(v + EPS)


def _recip(x):
    r = pl.reciprocal(x, approx=True)
    return r * (2.0 - x * r)


def _silu(x):
    h = 0.5 * x
    return h + h * jnp.tanh(h)


def _cols(off, w):
    if isinstance(off, int):
        return slice(off, off + w)
    return pl.ds(pl.multiple_of(off, w), w)


def _rarely(cond, fn):
    def body(_, c):
        fn()
        return c

    lax.fori_loop(0, cond.astype(jnp.int32), body, 0)


def _masks():
    def pos(j):
        return jnp.where(j < 40, j, jnp.where(j < 48, j - 32, jnp.where(j < 56, j - 48, j - 40)))

    out = []
    for q0, nq, nk in ((0, 32, 48), (32, 48, 80)):
        qi = lax.broadcasted_iota(jnp.int32, (nq, nk), 0) + q0
        kj = lax.broadcasted_iota(jnp.int32, (nq, nk), 1)
        qp, kp = pos(qi), pos(kj)
        same = ((qi < 40) & (kj < 40)) | ((qi >= 40) & (kj >= 40))
        allowed = same & ((qp < MEM) | (qp >= kp))
        fill = jnp.where(same, jnp.float32(-1e9 * DH ** 0.5), jnp.float32(-jnp.inf))
        out.append((allowed, fill))
    return out


def _kernel(x_hbm, mem0_hbm, wq_hbm, wk_hbm, wv_hbm, wo_hbm, w1_hbm, w3_hbm, w2_hbm,
            c_hbm, wm_hbm, out_hbm,
            xv, outv, wo, w1, w3, w2, wm, cv, m0v, modv, xh, h0, acc,
            lhs_a, lhs_b, o32, abuf, yv, fv, h2, hid, sem_in, sem_m, sem_w, sem_out, *rest):
    ring = rest[0:2]
    wg = rest[2:4]

    def side(g, t):
        return (g % 2) ^ int(t >= 2 * HG)

    scale = DH ** -0.5

    copies = {}

    def mk(name, src, dst):
        copies[name] = pltpu.make_async_copy(src, dst, sem_in.at[len(copies)])

    wm_u = wm_hbm.bitcast(U32)
    mk("c", c_hbm, cv)
    mk("mem0", mem0_hbm, m0v)
    mk("x0", x_hbm.at[0:X0], xv.at[0:X0])
    mk("x1", x_hbm.at[X0:X1], xv.at[X0:X1])
    mk("wo", wo_hbm.bitcast(U32), wo)
    mk("wm1", wm_u.at[:, 2 * D:5 * D], wm.at[:, 2 * D:5 * D])
    mk("w1", w1_hbm.bitcast(U32), w1)
    mk("w3", w3_hbm.bitcast(U32), w3)
    mk("w2", w2_hbm.bitcast(U32), w2)
    mk("wm2", wm_u.at[:, 5 * D:6 * D], wm.at[:, 5 * D:6 * D])
    mk("x2", x_hbm.at[X1:S], xv.at[X1:S])

    def mod_copies(kt):
        return [pltpu.make_async_copy(wm_u.at[:, _cols(i * D + kt * MW, MW)],
                                      wm.at[:, _cols(i * D + kt * MW, MW)], sem_m.at[kt])
                for i in range(2)]

    w_hbm = (wq_hbm, wk_hbm, wv_hbm)

    def block_copies(j, m, gi, t0):
        return [
            pltpu.make_async_copy(
                w_hbm[m].bitcast(U32).at[:, par, (2 * gi + pg) * (HG // 2) + jj],
                wg[side(pg, m * HG)].at[gi, t0 + 2 * jj + par], sem_w.at[j])
            for pg in range(2) for jj in range(HG // 2) for par in range(2)]

    def start_block(j):
        for c in block_copies(j, j // 4, j % 4, (j // 4) * HG):
            c.start()

    def wait_block(j, gi, t0):
        for w in wg:
            buf = w.at[gi, pl.ds(t0, HG)]
            pltpu.make_async_copy(buf, buf, sem_w.at[j]).wait()

    for n in ("x0", "c", "mem0"):
        copies[n].start()

    def zero(i, c):
        acc[i] = jnp.zeros(acc.shape[1:], F32)
        return c

    lax.fori_loop(0, 2 * HG, zero, 0)
    start_block(0)
    for kt in range(D // MW):
        for c in mod_copies(kt):
            c.start()

    def out_copy(r0, n):
        return pltpu.make_async_copy(outv.at[pl.ds(r0, n)], out_hbm.at[pl.ds(r0, n)], sem_out)

    def silu_c():
        return jnp.broadcast_to(_silu(cv[...].astype(F32)), (16, D)).astype(BF16)

    def mod_part(off, w):
        r = _dot(silu_c(), _unpack(wm[:, _cols(off, w)]))[0:8]
        modv[:, _cols(off, w)] = r
        return r[0:1]

    def mvec(i):
        return modv[0:1, i * D:(i + 1) * D]

    def ln1(r0, n):
        xf = xv[pl.ds(r0, n), :].astype(F32)
        return _ln(xf) * (1.0 + mvec(1)) + mvec(0)

    def repack_slot(w, gi, t, enable=None):
        for r0 in range(0, D // 2, 32):
            a = w[gi, t, r0:r0 + 32, :]
            b = w[gi, t + 1, r0:r0 + 32, :]
            e = (a & jnp.uint32(0xFFFF)) | (b << 16)
            o = (a >> 16) | (b & jnp.uint32(0xFFFF0000))
            if enable is not None:
                e = jnp.where(enable, e, a)
                o = jnp.where(enable, o, b)
            w[gi, t, r0:r0 + 32, :] = e
            w[gi, t + 1, r0:r0 + 32, :] = o

    def repack_now(gi, t0):
        def body(i, c):
            for w in wg:
                repack_slot(w, gi, t0 + 2 * i)
            return c

        lax.fori_loop(0, HG // 2, body, 0)

    def store_tokens(dst, gi, t, r):
        for pp in range(PRO // PT):
            b0, r0 = pp * SLOT, pp * PT
            dst[gi, t, b0 + 4:b0 + 8, :] = _pack(r[r0:r0 + 8])
            dst[gi, t, b0 + 8:b0 + 24, :] = _pack(r[r0 + 8:r0 + 40])
            dst[gi, t, b0 + 28:b0 + 32, :] = _pack(r[r0 + 40:r0 + 48])
            dst[gi, t, b0 + 32:b0 + 40, :] = _pack(r[r0 + 48:r0 + 64])
        b0 = (PRO // PT) * SLOT
        dst[gi, t, 0:4, :] = _pack(r[PRO:PRO + 8])
        dst[gi, t, b0 + 4:b0 + 8, :] = _pack(r[PRO + 8:PRO + 16])
        dst[gi, t, b0 + 8:b0 + 16, :] = _pack(r[PRO + 16:PRO + 32])

    def proj(lhs, g, rows, t0, t1):
        for t in range(t0, t1):
            r = _dot(lhs, _unpack(wg[side(g, t)][g // 2, t]))
            for i, row in enumerate(rows):
                ring[side(g, t)][g // 2, t, pl.ds(row, 4), :] = _pack(r[8 * i:8 * i + 8])

    def attn_qk(g, base, q0, nq, nk, allowed, fill):
        qrow = pl.multiple_of(base + q0 // 2, 8)
        ps = []
        for hh in range(HG):
            q = _unpack(ring[g % 2][g // 2, hh, pl.ds(qrow, nq // 2), :])
            k = _unpack(ring[g % 2][g // 2, HG + hh, pl.ds(base, nk // 2), :])
            s = lax.dot_general(q, k, (((1,), (1,)), ((), ())), preferred_element_type=F32)
            s = jnp.where(allowed, s, fill)
            m = jnp.max(s, axis=-1, keepdims=True)
            p = jnp.exp2((s - m) * (scale * LOG2E))
            l = jnp.sum(p, axis=-1, keepdims=True)
            ps.append((p * _recip(l)).astype(BF16))
        return ps

    def attn_pv(g, base, nq, nk, ps):
        for hh in range(HG):
            v = _unpack(ring[1 - g % 2][g // 2, 2 * HG + hh, pl.ds(base, nk // 2), :])
            col = (g * HG + hh) * DH
            o32[0:nq // 2, col:col + DH] = _pack(_dot(ps[hh], v))

    def wo_proj(nq, stores):
        o = _unpack(o32[0:nq // 2, :])
        cw = 256
        for cb in range(D // cw):
            cs = slice(cb * cw, (cb + 1) * cw)
            r = _dot(o, _unpack(wo[:, cs]))
            for r0, n, fn in stores:
                fn(cs, r[r0:r0 + n])

    def post_attn(tok0):
        x1 = xv[pl.ds(tok0, PT), :].astype(F32) + mvec(2) * abuf[...]
        yv[...] = x1
        h2[...] = _pack(_ln(x1) * (1.0 + mvec(4)) + mvec(3))

    def ffn_up(c0, c1, off=0):
        a = _unpack(h2[...])
        for c in range(c0, c1):
            cs = _cols(off + c * FC, FC)
            gt = _dot(a, _unpack(w1[:, cs]))
            up = _dot(a, _unpack(w3[:, cs]))
            hid[:, cs] = _pack(_silu(gt) * up)

    def ffn_down(cb0, cb1, off=0, tok0=None):
        a = _unpack(hid[...])
        cw = 256
        for cb in range(cb0, cb1):
            cs = _cols(off + cb * cw, cw)
            r = _dot(a, _unpack(w2[:, cs]))
            if tok0 is None:
                fv[:, cs] = r
            else:
                gb = modv[0:1, _cols(off + 5 * D + cb * cw, cw)]
                outv[pl.ds(tok0, PT), cs] = (yv[:, cs] + gb * r).astype(BF16)

    def finish(tok0):
        outv[pl.ds(tok0, PT), :] = (yv[...] + mvec(5) * fv[...]).astype(BF16)

    def unit_row(u):
        r = u & 7
        slot = lax.rem(u >> 3, NSLOT)
        return pl.multiple_of(slot * SLOT + 4 + 4 * r + 4 * (r >= 5).astype(jnp.int32), 4)

    with _scope("waitx0"):
        copies["x0"].wait()
    with _scope("ln0"):

        def ln_body(i, c):
            r0 = pl.multiple_of(i * 136, 8)
            xh[pl.ds(r0, 136), :] = _ln(xv[pl.ds(r0, 136), :].astype(F32))
            return c

        lax.fori_loop(0, X0 // 136, ln_body, 0)
    with _scope("waitc"):
        copies["c"].wait()
        copies["mem0"].wait()

    def modulate(kt):
        sa = mod_part(kt * KW, KW)
        ca = mod_part(D + kt * KW, KW)
        cs = _cols(kt * KW, KW)
        hh = xh[0:PRO + 24, cs] * (1.0 + ca) + sa
        a = _pack(jnp.concatenate([hh[0:PRO], m0v[:, cs].astype(F32), hh[PRO:]], axis=0))
        h0[:, _cols(kt * KW, KW)] = a
        return a

    with _scope("waitw0"):
        wait_block(0, 0, 0)
    with _scope("first"):
        repack_now(0, 0)
        with _scope("waitm0"):
            for c in mod_copies(0):
                c.wait()
        a0 = modulate(0)

    def kmajor(kt, a):
        kn = jnp.minimum(kt + 1, KT - 1)

        def more():
            for j in range(1, 4):
                start_block(j)

        _rarely(kt == KSTART, more)

        @pl.when((kt < KT - 1) & (lax.rem(kn, KPM) == 0))
        def _():
            for c in mod_copies(lax.div(kn, KPM)):
                c.wait()

        rows = pl.ds(pl.multiple_of(kt * (KW // 2), KW // 2), KW // 2)
        a_next = None
        for pg in range(2):
            for t in range(HG):
                acc[pg * HG + t] += _dot(_unpack(a), _unpack(wg[pg][0, t, rows, :]))
            if pg == 0:
                a_next = modulate(kn)
        return a_next

    with _scope("kmajor"):
        lax.fori_loop(0, KT, kmajor, a0)

        def flush(t, c):
            for pg in range(2):
                store_tokens(ring[pg], 0, t, acc[pg * HG + t])
            return c

        lax.fori_loop(0, HG, flush, 0)

    def pro_body(j, c):
        gi, t0 = j & 3, (j >> 2) * HG
        jn = jnp.minimum(j + 1, NJ - 1)
        gn, tn = jn & 3, (jn >> 2) * HG
        prefetch = (j > 1) & (j < NJ - 1)

        def batch(js, names):
            def fn():
                for jj in js:
                    start_block(jj)
                for n in names:
                    copies[n].start()
            return fn

        def late():
            with _scope("waitlate"):
                wait_block(j, gi, t0)
            repack_now(gi, t0)

        _rarely(j == 1, batch(range(4, 9), ()))
        _rarely(j == 3, batch(range(9, NJ), ("x1", "wo", "wm1", "w1", "w3", "w2", "wm2", "x2")))
        _rarely(j <= 2, late)

        @pl.when(prefetch)
        def _():
            wait_block(jn, gn, tn)

        a = _unpack(h0[...])
        for pg in range(2):
            for t in range(HG):
                store_tokens(ring[pg], gi, t0 + t, _dot(a, _unpack(wg[pg][gi, t0 + t])))
        gr, tr = jnp.where(prefetch, gn, gi), jnp.where(prefetch, tn, t0)
        for w in wg:
            for t in range(0, HG, 2):
                repack_slot(w, gr, tr + t, prefetch)
        return c

    with _scope("pro"):
        lax.fori_loop(1, NJ, pro_body, 0)

    def pair(p, with_ffn):
        (al_a, fi_a), (al_b, fi_b) = _masks()
        base = pl.multiple_of(lax.rem(p, NSLOT) * SLOT, 8)
        u0 = PRO // 8 + 6 * p
        tlead = PRO + 48 * p

        if with_ffn:
            finish(pl.multiple_of(jnp.maximum(p - 2, 0) * PT, PT))
            post_attn(pl.multiple_of((p - 1) * PT, PT))

        def filler(i, c0=None, c1=None):
            if not with_ffn:
                if i is not None:
                    mod_part(2 * D + MODF[i] * 256, (MODF[i + 1] - MODF[i]) * 256)
            elif c0 is None:
                ffn_down(0, 4)
            else:
                ffn_up(c0, c1)

        def proj_attn(lhs, rows, q0, nq, nk, allowed, fill, f):
            ps = None
            for g in range(G):
                proj(lhs, g, rows, 0, QKPOS)
                if g > 0 and QKPOS > 0:
                    ps = attn_qk(g - 1, base, q0, nq, nk, allowed, fill)
                proj(lhs, g, rows, QKPOS, PVPOS)
                if g > 0:
                    attn_pv(g - 1, base, nq, nk, ps)
                proj(lhs, g, rows, PVPOS, 3 * HG)
                if QKPOS == 0 or g == G - 1:
                    ps = attn_qk(g, base, q0, nq, nk, allowed, fill)
            filler(f, FILL[f], FILL[f + 1])
            attn_pv(G - 1, base, nq, nk, ps)
            filler(f + 1, FILL[f + 1], FILL[f + 2])

        def st_lhs(ref):
            def fn(cs, val):
                ref[0:MEM, cs] = val.astype(BF16).astype(F32)
            return fn

        def st_a(r0, n):
            def fn(cs, val):
                abuf[r0:r0 + n, cs] = val
            return fn

        lhs_b[MEM:32, :] = ln1(pl.multiple_of(tlead + 24, 8), 24)
        if with_ffn:
            lhs = lhs_a[...].astype(BF16)
            rows = [base, unit_row(u0), unit_row(u0 + 1), unit_row(u0 + 2)]
            proj_attn(lhs, rows, 0, 32, 48, al_a, fi_a, 0)
        else:
            ps = [attn_qk(g, base, 0, 32, 48, al_a, fi_a) for g in range(G)]
            filler(0)
            for g in range(G):
                attn_pv(g, base, 32, 48, ps[g])
            filler(1)
        wo_proj(32, [(0, 8, st_lhs(lhs_b)), (8, 24, st_a(0, 24))])
        filler(2, FILL[2], FILL[3])

        lhs = lhs_b[...].astype(BF16)
        rows = [pl.multiple_of(base + 24, 8), unit_row(u0 + 3), unit_row(u0 + 4), unit_row(u0 + 5)]
        nxt = pl.multiple_of(jnp.minimum(tlead + 48, S - 24), 8)
        lhs_a[MEM:32, :] = ln1(nxt, 24)
        proj_attn(lhs, rows, 32, 48, 80, al_b, fi_b, 3)
        wo_proj(48, [(16, 8, st_lhs(lhs_a)), (0, 16, st_a(24, 16)), (24, 24, st_a(40, 24))])
        filler(None)

    with _scope("waitwo"):
        copies["x1"].wait()
        copies["wo"].wait()
        copies["wm1"].wait()

    with _scope("noffn"):
        yv[...] = jnp.zeros(yv.shape, F32)
        fv[...] = jnp.zeros(fv.shape, F32)
        modv[:, 5 * D:6 * D] = jnp.zeros((8, D), F32)
        pair(jnp.int32(0), False)

    with _scope("waitffn"):
        copies["w1"].wait()
        copies["w3"].wait()
        copies["w2"].wait()

    def late_inputs():
        copies["wm2"].wait()
        copies["x2"].wait()
        mod_part(5 * D, D)

    def pair_ffn(p, c):
        _rarely(p == MAIN_START + 1, late_inputs)

        @pl.when(p > MAIN_START + 1)
        def _():
            out_copy(pl.multiple_of((p - 3) * PT, PT), PT).start()

        pair(p, True)
        return c

    with _scope("main"):
        lax.fori_loop(MAIN_START, NPAIR, pair_ffn, 0)

    with _scope("epi"):
        out_copy((NPAIR - 3) * PT, PT).start()
        finish((NPAIR - 2) * PT)
        post_attn((NPAIR - 1) * PT)
        out_copy((NPAIR - 2) * PT, PT).start()

        def up_body(i, c):
            ffn_up(0, EPI_UP, i * (EPI_UP * FC))
            return c

        def down_body(i, c):
            ffn_down(0, EPI_DOWN, i * (EPI_DOWN * 256), (NPAIR - 1) * PT)
            return c

        lax.fori_loop(0, NFC // EPI_UP, up_body, 0)
        lax.fori_loop(0, 4 // EPI_DOWN, down_body, 0)
        out_copy((NPAIR - 1) * PT, PT).start()
    with _scope("waitout"):
        out_copy(0, S - (MAIN_START - 1) * PT).wait()


@functools.partial(jax.jit, static_argnames=("A_seg_len",))
def pallas_adaLN_cond__memory_aug_recurrent_mem_tr__glu_gated_swiglu__prompt_kernel(
    A_x, A_mem0, A_Wq, A_Wk, A_Wv, A_Wo, A_seg_len, B_x, B_w1, B_w3, B_w2, c, w_mod,
):
    assert A_seg_len == SEG
    assert A_x.shape == (1, S, D) and A_mem0.shape == (1, MEM, D)
    assert A_Wq.shape == (D, H, DH) and B_w1.shape == (D, FF)
    del B_x

    scratch = [
        pltpu.VMEM((S, D), BF16),
        pltpu.VMEM((S, D), BF16),
        pltpu.VMEM((HD // 2, D), U32),
        pltpu.VMEM((D // 2, FF), U32),
        pltpu.VMEM((D // 2, FF), U32),
        pltpu.VMEM((FF // 2, D), U32),
        pltpu.VMEM((D // 2, 6 * D), U32),
        pltpu.VMEM((1, D), BF16),
        pltpu.VMEM((MEM, D), BF16),
        pltpu.VMEM((8, 6 * D), F32),
        pltpu.VMEM((X0, D), F32),
        pltpu.VMEM((PROM // 2, D), U32),
        pltpu.VMEM((2 * HG, PROM, DH), F32),
        pltpu.VMEM((32, D), F32),
        pltpu.VMEM((32, D), F32),
        pltpu.VMEM((24, HD), U32),
        pltpu.VMEM((PT, D), F32),
        pltpu.VMEM((PT, D), F32),
        pltpu.VMEM((PT, D), F32),
        pltpu.VMEM((PT // 2, D), U32),
        pltpu.VMEM((PT // 2, FF), U32),
        pltpu.SemaphoreType.DMA((11,)),
        pltpu.SemaphoreType.DMA((KT,)),
        pltpu.SemaphoreType.DMA((NJ,)),
        pltpu.SemaphoreType.DMA,
    ] + [pltpu.VMEM((G // 2, 3 * HG, NSLOT * SLOT, DH), U32)] * 2 + [
        pltpu.VMEM((G // 2, 3 * HG, D // 2, DH), U32)] * 2

    out = pl.pallas_call(
        _kernel,
        out_shape=jax.ShapeDtypeStruct((S, D), BF16),
        in_specs=[pl.BlockSpec(memory_space=pl.ANY)] * 11,
        out_specs=pl.BlockSpec(memory_space=pl.ANY),
        scratch_shapes=scratch,
        compiler_params=pltpu.CompilerParams(
            vmem_limit_bytes=120 * 1024 * 1024, disable_bounds_checks=True),
    )(
        A_x.reshape(S, D), A_mem0.reshape(MEM, D),
        A_Wq.reshape(D // 2, 2, H, DH), A_Wk.reshape(D // 2, 2, H, DH),
        A_Wv.reshape(D // 2, 2, H, DH), A_Wo.reshape(HD, D),
        B_w1, B_w3, B_w2, c, w_mod,
    )
    return out.reshape(1, S, D)
```

```python
import functools

import jax
import jax.numpy as jnp
from jax import lax
import jax.experimental.pallas as pl
import jax.experimental.pallas.tpu as pltpu

F32 = jnp.float32
BF16 = jnp.bfloat16
U32 = jnp.uint32

S = 2048
D = 1024
H = 32
DH = 128
HD = H * DH
MEM = 8
SEG = 32
FF = 3584
EPS = 1e-5
LOG2E = 1.4426950408889634

G = 8
HG = H // G
PRO = 512
NPAIR = S // (2 * SEG)
PT = 2 * SEG
SLOT = 40
NSLOT = 9
X0 = 544
X1 = 640
FC = 256
NFC = FF // FC
KW = 128
KT = D // KW
MW = 128
KPM = MW // KW
NJ = 3 * G // 2
FILL = (0, 2, 4, 9, 11, 14)
QKPOS = 1
PVPOS = 11
MODF = (0, 5, 6, 8, 11, 12)
PROM = PRO + 32
MAIN_START = 1
SCOPES = False
KSTART = 4


class _NoScope:
    def __enter__(self):
        return self

    def __exit__(self, *a):
        return False


def _scope(name):
    return jax.named_scope(name) if SCOPES else _NoScope()


def _unpack(x):
    return pltpu.bitcast(x, BF16)


def _pack(x):
    return pltpu.bitcast(x.astype(BF16), U32)


def _dot(a, b):
    return jnp.dot(a, b, preferred_element_type=F32)


def _ln(x):
    m = jnp.mean(x, axis=-1, keepdims=True)
    xc = x - m
    v = jnp.mean(xc * xc, axis=-1, keepdims=True)
    return xc * lax.rsqrt(v + EPS)


def _recip(x):
    r = pl.reciprocal(x, approx=True)
    return r * (2.0 - x * r)


def _silu(x):
    h = 0.5 * x
    return h + h * jnp.tanh(h)


def _cols(off, w):
    if isinstance(off, int):
        return slice(off, off + w)
    return pl.ds(pl.multiple_of(off, w), w)


def _rarely(cond, fn):
    def body(_, c):
        fn()
        return c

    lax.fori_loop(0, cond.astype(jnp.int32), body, 0)


def _masks():
    def pos(j):
        return jnp.where(j < 40, j, jnp.where(j < 48, j - 32, jnp.where(j < 56, j - 48, j - 40)))

    out = []
    for q0, nq, nk in ((0, 32, 48), (32, 48, 80)):
        qi = lax.broadcasted_iota(jnp.int32, (nq, nk), 0) + q0
        kj = lax.broadcasted_iota(jnp.int32, (nq, nk), 1)
        qp, kp = pos(qi), pos(kj)
        same = ((qi < 40) & (kj < 40)) | ((qi >= 40) & (kj >= 40))
        allowed = same & ((qp < MEM) | (qp >= kp))
        fill = jnp.where(same, jnp.float32(-1e9 * DH ** 0.5), jnp.float32(-jnp.inf))
        out.append((allowed, fill))
    return out


def _kernel(x_hbm, mem0_hbm, wq_hbm, wk_hbm, wv_hbm, wo_hbm, w1_hbm, w3_hbm, w2_hbm,
            c_hbm, wm_hbm, out_hbm,
            xv, outv, wo, w1, w3, w2, wm, cv, m0v, modv, xh, h0, acc,
            lhs_a, lhs_b, o32, abuf, yv, fv, h2, hid, sem_in, sem_m, sem_w, sem_out, *rest):
    ring = rest[0:2]
    wg = rest[2:4]

    def side(g, t):
        return (g % 2) ^ int(t >= 2 * HG)

    scale = DH ** -0.5

    copies = {}

    def mk(name, src, dst):
        copies[name] = pltpu.make_async_copy(src, dst, sem_in.at[len(copies)])

    wm_u = wm_hbm.bitcast(U32)
    mk("c", c_hbm, cv)
    mk("mem0", mem0_hbm, m0v)
    mk("x0", x_hbm.at[0:X0], xv.at[0:X0])
    mk("x1", x_hbm.at[X0:X1], xv.at[X0:X1])
    mk("wo", wo_hbm.bitcast(U32), wo)
    mk("wm1", wm_u.at[:, 2 * D:5 * D], wm.at[:, 2 * D:5 * D])
    mk("w1", w1_hbm.bitcast(U32), w1)
    mk("w3", w3_hbm.bitcast(U32), w3)
    mk("w2", w2_hbm.bitcast(U32), w2)
    mk("wm2", wm_u.at[:, 5 * D:6 * D], wm.at[:, 5 * D:6 * D])
    mk("x2", x_hbm.at[X1:S], xv.at[X1:S])

    def mod_copies(kt):
        return [pltpu.make_async_copy(wm_u.at[:, _cols(i * D + kt * MW, MW)],
                                      wm.at[:, _cols(i * D + kt * MW, MW)], sem_m.at[kt])
                for i in range(2)]

    w_hbm = (wq_hbm, wk_hbm, wv_hbm)

    def block_copies(j, m, gi, t0):
        return [
            pltpu.make_async_copy(
                w_hbm[m].bitcast(U32).at[:, par, (2 * gi + pg) * (HG // 2) + jj],
                wg[side(pg, m * HG)].at[gi, t0 + 2 * jj + par], sem_w.at[j])
            for pg in range(2) for jj in range(HG // 2) for par in range(2)]

    def start_block(j):
        for c in block_copies(j, j // 4, j % 4, (j // 4) * HG):
            c.start()

    def wait_block(j, gi, t0):
        for w in wg:
            buf = w.at[gi, pl.ds(t0, HG)]
            pltpu.make_async_copy(buf, buf, sem_w.at[j]).wait()

    for n in ("x0", "c", "mem0"):
        copies[n].start()

    def zero(i, c):
        acc[i] = jnp.zeros(acc.shape[1:], F32)
        return c

    lax.fori_loop(0, 2 * HG, zero, 0)
    start_block(0)
    for kt in range(D // MW):
        for c in mod_copies(kt):
            c.start()

    def out_copy(r0, n):
        return pltpu.make_async_copy(outv.at[pl.ds(r0, n)], out_hbm.at[pl.ds(r0, n)], sem_out)

    def silu_c():
        return jnp.broadcast_to(_silu(cv[...].astype(F32)), (16, D)).astype(BF16)

    def mod_part(off, w):
        r = _dot(silu_c(), _unpack(wm[:, _cols(off, w)]))[0:8]
        modv[:, _cols(off, w)] = r
        return r[0:1]

    def mvec(i):
        return modv[0:1, i * D:(i + 1) * D]

    def ln1(r0, n):
        xf = xv[pl.ds(r0, n), :].astype(F32)
        return _ln(xf) * (1.0 + mvec(1)) + mvec(0)

    def repack_slot(w, gi, t, enable=None):
        for r0 in range(0, D // 2, 32):
            a = w[gi, t, r0:r0 + 32, :]
            b = w[gi, t + 1, r0:r0 + 32, :]
            e = (a & jnp.uint32(0xFFFF)) | (b << 16)
            o = (a >> 16) | (b & jnp.uint32(0xFFFF0000))
            if enable is not None:
                e = jnp.where(enable, e, a)
                o = jnp.where(enable, o, b)
            w[gi, t, r0:r0 + 32, :] = e
            w[gi, t + 1, r0:r0 + 32, :] = o

    def repack_now(gi, t0):
        def body(i, c):
            for w in wg:
                repack_slot(w, gi, t0 + 2 * i)
            return c

        lax.fori_loop(0, HG // 2, body, 0)

    def store_tokens(dst, gi, t, r):
        for pp in range(PRO // PT):
            b0, r0 = pp * SLOT, pp * PT
            dst[gi, t, b0 + 4:b0 + 8, :] = _pack(r[r0:r0 + 8])
            dst[gi, t, b0 + 8:b0 + 24, :] = _pack(r[r0 + 8:r0 + 40])
            dst[gi, t, b0 + 28:b0 + 32, :] = _pack(r[r0 + 40:r0 + 48])
            dst[gi, t, b0 + 32:b0 + 40, :] = _pack(r[r0 + 48:r0 + 64])
        b0 = (PRO // PT) * SLOT
        dst[gi, t, 0:4, :] = _pack(r[PRO:PRO + 8])
        dst[gi, t, b0 + 4:b0 + 8, :] = _pack(r[PRO + 8:PRO + 16])
        dst[gi, t, b0 + 8:b0 + 16, :] = _pack(r[PRO + 16:PRO + 32])

    def proj(lhs, g, rows, t0, t1):
        for t in range(t0, t1):
            r = _dot(lhs, _unpack(wg[side(g, t)][g // 2, t]))
            for i, row in enumerate(rows):
                ring[side(g, t)][g // 2, t, pl.ds(row, 4), :] = _pack(r[8 * i:8 * i + 8])

    def attn_qk(g, base, q0, nq, nk, allowed, fill):
        qrow = pl.multiple_of(base + q0 // 2, 8)
        ps = []
        for hh in range(HG):
            q = _unpack(ring[g % 2][g // 2, hh, pl.ds(qrow, nq // 2), :])
            k = _unpack(ring[g % 2][g // 2, HG + hh, pl.ds(base, nk // 2), :])
            s = lax.dot_general(q, k, (((1,), (1,)), ((), ())), preferred_element_type=F32)
            s = jnp.where(allowed, s, fill)
            m = jnp.max(s, axis=-1, keepdims=True)
            p = jnp.exp2((s - m) * (scale * LOG2E))
            l = jnp.sum(p, axis=-1, keepdims=True)
            ps.append((p * _recip(l)).astype(BF16))
        return ps

    def attn_pv(g, base, nq, nk, ps):
        for hh in range(HG):
            v = _unpack(ring[1 - g % 2][g // 2, 2 * HG + hh, pl.ds(base, nk // 2), :])
            col = (g * HG + hh) * DH
            o32[0:nq // 2, col:col + DH] = _pack(_dot(ps[hh], v))

    def wo_proj(nq, stores):
        o = _unpack(o32[0:nq // 2, :])
        cw = 256
        for cb in range(D // cw):
            cs = slice(cb * cw, (cb + 1) * cw)
            r = _dot(o, _unpack(wo[:, cs]))
            for r0, n, fn in stores:
                fn(cs, r[r0:r0 + n])

    def post_attn(tok0):
        x1 = xv[pl.ds(tok0, PT), :].astype(F32) + mvec(2) * abuf[...]
        yv[...] = x1
        h2[...] = _pack(_ln(x1) * (1.0 + mvec(4)) + mvec(3))

    def ffn_up(c0, c1):
        a = _unpack(h2[...])
        for c in range(c0, c1):
            cs = slice(c * FC, (c + 1) * FC)
            gt = _dot(a, _unpack(w1[:, cs]))
            up = _dot(a, _unpack(w3[:, cs]))
            hid[:, cs] = _pack(_silu(gt) * up)

    def ffn_down(cb0, cb1, tok0=None):
        a = _unpack(hid[...])
        cw = 256
        for cb in range(cb0, cb1):
            cs = slice(cb * cw, (cb + 1) * cw)
            r = _dot(a, _unpack(w2[:, cs]))
            if tok0 is None:
                fv[:, cs] = r
            else:
                gb = modv[0:1, 5 * D + cb * cw:5 * D + (cb + 1) * cw]
                outv[pl.ds(tok0, PT), cs] = (yv[:, cs] + gb * r).astype(BF16)

    def finish(tok0):
        outv[pl.ds(tok0, PT), :] = (yv[...] + mvec(5) * fv[...]).astype(BF16)

    def unit_row(u):
        r = u & 7
        slot = lax.rem(u >> 3, NSLOT)
        return pl.multiple_of(slot * SLOT + 4 + 4 * r + 4 * (r >= 5).astype(jnp.int32), 4)

    with _scope("waitx0"):
        copies["x0"].wait()
    with _scope("ln0"):

        def ln_body(i, c):
            r0 = pl.multiple_of(i * 136, 8)
            xh[pl.ds(r0, 136), :] = _ln(xv[pl.ds(r0, 136), :].astype(F32))
            return c

        lax.fori_loop(0, X0 // 136, ln_body, 0)
    with _scope("waitc"):
        copies["c"].wait()
        copies["mem0"].wait()

    def modulate(kt):
        sa = mod_part(kt * KW, KW)
        ca = mod_part(D + kt * KW, KW)
        cs = _cols(kt * KW, KW)
        hh = xh[0:PRO + 24, cs] * (1.0 + ca) + sa
        a = _pack(jnp.concatenate([hh[0:PRO], m0v[:, cs].astype(F32), hh[PRO:]], axis=0))
        h0[:, _cols(kt * KW, KW)] = a
        return a

    with _scope("waitw0"):
        wait_block(0, 0, 0)
    with _scope("first"):
        repack_now(0, 0)
        with _scope("waitm0"):
            for c in mod_copies(0):
                c.wait()
        a0 = modulate(0)

    def kmajor(kt, a):
        kn = jnp.minimum(kt + 1, KT - 1)

        def more():
            for j in range(1, 4):
                start_block(j)

        _rarely(kt == KSTART, more)

        @pl.when((kt < KT - 1) & (lax.rem(kn, KPM) == 0))
        def _():
            for c in mod_copies(lax.div(kn, KPM)):
                c.wait()

        rows = pl.ds(pl.multiple_of(kt * (KW // 2), KW // 2), KW // 2)
        a_next = None
        for pg in range(2):
            for t in range(HG):
                r = acc[pg * HG + t] + _dot(_unpack(a), _unpack(wg[pg][0, t, rows, :]))
                acc[pg * HG + t] = r
                store_tokens(ring[pg], 0, t, r)
            if pg == 0:
                a_next = modulate(kn)
        return a_next

    with _scope("kmajor"):
        lax.fori_loop(0, KT, kmajor, a0)

    def pro_body(j, c):
        gi, t0 = j & 3, (j >> 2) * HG
        jn = jnp.minimum(j + 1, NJ - 1)
        gn, tn = jn & 3, (jn >> 2) * HG
        prefetch = (j > 1) & (j < NJ - 1)

        def batch(js, names):
            def fn():
                for jj in js:
                    start_block(jj)
                for n in names:
                    copies[n].start()
            return fn

        def late():
            with _scope("waitlate"):
                wait_block(j, gi, t0)
            repack_now(gi, t0)

        _rarely(j == 1, batch(range(4, 9), ()))
        _rarely(j == 3, batch(range(9, NJ), ("x1", "wo", "wm1", "w1", "w3", "w2", "wm2", "x2")))
        _rarely(j <= 2, late)

        @pl.when(prefetch)
        def _():
            wait_block(jn, gn, tn)

        a = _unpack(h0[...])
        for pg in range(2):
            for t in range(HG):
                store_tokens(ring[pg], gi, t0 + t, _dot(a, _unpack(wg[pg][gi, t0 + t])))
        gr, tr = jnp.where(prefetch, gn, gi), jnp.where(prefetch, tn, t0)
        for w in wg:
            for t in range(0, HG, 2):
                repack_slot(w, gr, tr + t, prefetch)
        return c

    with _scope("pro"):
        lax.fori_loop(1, NJ, pro_body, 0)

    def pair(p, with_ffn):
        (al_a, fi_a), (al_b, fi_b) = _masks()
        base = pl.multiple_of(lax.rem(p, NSLOT) * SLOT, 8)
        u0 = PRO // 8 + 6 * p
        tlead = PRO + 48 * p

        if with_ffn:
            finish(pl.multiple_of(jnp.maximum(p - 2, 0) * PT, PT))
            post_attn(pl.multiple_of((p - 1) * PT, PT))

        def filler(i, c0=None, c1=None):
            if not with_ffn:
                if i is not None:
                    mod_part(2 * D + MODF[i] * 256, (MODF[i + 1] - MODF[i]) * 256)
            elif c0 is None:
                ffn_down(0, 4)
            else:
                ffn_up(c0, c1)

        def proj_attn(lhs, rows, q0, nq, nk, allowed, fill, f):
            ps = None
            for g in range(G):
                proj(lhs, g, rows, 0, QKPOS)
                if g > 0 and QKPOS > 0:
                    ps = attn_qk(g - 1, base, q0, nq, nk, allowed, fill)
                proj(lhs, g, rows, QKPOS, PVPOS)
                if g > 0:
                    attn_pv(g - 1, base, nq, nk, ps)
                proj(lhs, g, rows, PVPOS, 3 * HG)
                if QKPOS == 0 or g == G - 1:
                    ps = attn_qk(g, base, q0, nq, nk, allowed, fill)
            filler(f, FILL[f], FILL[f + 1])
            attn_pv(G - 1, base, nq, nk, ps)
            filler(f + 1, FILL[f + 1], FILL[f + 2])

        def st_lhs(ref):
            def fn(cs, val):
                ref[0:MEM, cs] = val.astype(BF16).astype(F32)
            return fn

        def st_a(r0, n):
            def fn(cs, val):
                abuf[r0:r0 + n, cs] = val
            return fn

        lhs_b[MEM:32, :] = ln1(pl.multiple_of(tlead + 24, 8), 24)
        if with_ffn:
            lhs = lhs_a[...].astype(BF16)
            rows = [base, unit_row(u0), unit_row(u0 + 1), unit_row(u0 + 2)]
            proj_attn(lhs, rows, 0, 32, 48, al_a, fi_a, 0)
        else:
            ps = [attn_qk(g, base, 0, 32, 48, al_a, fi_a) for g in range(G)]
            filler(0)
            for g in range(G):
                attn_pv(g, base, 32, 48, ps[g])
            filler(1)
        wo_proj(32, [(0, 8, st_lhs(lhs_b)), (8, 24, st_a(0, 24))])
        filler(2, FILL[2], FILL[3])

        lhs = lhs_b[...].astype(BF16)
        rows = [pl.multiple_of(base + 24, 8), unit_row(u0 + 3), unit_row(u0 + 4), unit_row(u0 + 5)]
        nxt = pl.multiple_of(jnp.minimum(tlead + 48, S - 24), 8)
        lhs_a[MEM:32, :] = ln1(nxt, 24)
        proj_attn(lhs, rows, 32, 48, 80, al_b, fi_b, 3)
        wo_proj(48, [(16, 8, st_lhs(lhs_a)), (0, 16, st_a(24, 16)), (24, 24, st_a(40, 24))])
        filler(None)

    with _scope("waitwo"):
        copies["x1"].wait()
        copies["wo"].wait()
        copies["wm1"].wait()

    with _scope("noffn"):
        yv[...] = jnp.zeros(yv.shape, F32)
        fv[...] = jnp.zeros(fv.shape, F32)
        modv[:, 5 * D:6 * D] = jnp.zeros((8, D), F32)
        pair(jnp.int32(0), False)

    with _scope("waitffn"):
        copies["w1"].wait()
        copies["w3"].wait()
        copies["w2"].wait()

    def late_inputs():
        copies["wm2"].wait()
        copies["x2"].wait()
        mod_part(5 * D, D)

    def pair_ffn(p, c):
        _rarely(p == MAIN_START + 1, late_inputs)

        @pl.when(p > MAIN_START + 1)
        def _():
            out_copy(pl.multiple_of((p - 3) * PT, PT), PT).start()

        pair(p, True)
        return c

    with _scope("main"):
        lax.fori_loop(MAIN_START, NPAIR, pair_ffn, 0)

    with _scope("epi"):
        out_copy((NPAIR - 3) * PT, PT).start()
        finish((NPAIR - 2) * PT)
        post_attn((NPAIR - 1) * PT)
        out_copy((NPAIR - 2) * PT, PT).start()

        ffn_up(0, NFC)
        ffn_down(0, 4, (NPAIR - 1) * PT)
        out_copy((NPAIR - 1) * PT, PT).start()
    with _scope("waitout"):
        out_copy(0, S - (MAIN_START - 1) * PT).wait()


@functools.partial(jax.jit, static_argnames=("A_seg_len",))
def pallas_adaLN_cond__memory_aug_recurrent_mem_tr__glu_gated_swiglu__prompt_kernel(
    A_x, A_mem0, A_Wq, A_Wk, A_Wv, A_Wo, A_seg_len, B_x, B_w1, B_w3, B_w2, c, w_mod,
):
    assert A_seg_len == SEG
    assert A_x.shape == (1, S, D) and A_mem0.shape == (1, MEM, D)
    assert A_Wq.shape == (D, H, DH) and B_w1.shape == (D, FF)
    del B_x

    scratch = [
        pltpu.VMEM((S, D), BF16),
        pltpu.VMEM((S, D), BF16),
        pltpu.VMEM((HD // 2, D), U32),
        pltpu.VMEM((D // 2, FF), U32),
        pltpu.VMEM((D // 2, FF), U32),
        pltpu.VMEM((FF // 2, D), U32),
        pltpu.VMEM((D // 2, 6 * D), U32),
        pltpu.VMEM((1, D), BF16),
        pltpu.VMEM((MEM, D), BF16),
        pltpu.VMEM((8, 6 * D), F32),
        pltpu.VMEM((X0, D), F32),
        pltpu.VMEM((PROM // 2, D), U32),
        pltpu.VMEM((2 * HG, PROM, DH), F32),
        pltpu.VMEM((32, D), F32),
        pltpu.VMEM((32, D), F32),
        pltpu.VMEM((24, HD), U32),
        pltpu.VMEM((PT, D), F32),
        pltpu.VMEM((PT, D), F32),
        pltpu.VMEM((PT, D), F32),
        pltpu.VMEM((PT // 2, D), U32),
        pltpu.VMEM((PT // 2, FF), U32),
        pltpu.SemaphoreType.DMA((11,)),
        pltpu.SemaphoreType.DMA((KT,)),
        pltpu.SemaphoreType.DMA((NJ,)),
        pltpu.SemaphoreType.DMA,
    ] + [pltpu.VMEM((G // 2, 3 * HG, NSLOT * SLOT, DH), U32)] * 2 + [
        pltpu.VMEM((G // 2, 3 * HG, D // 2, DH), U32)] * 2

    out = pl.pallas_call(
        _kernel,
        out_shape=jax.ShapeDtypeStruct((S, D), BF16),
        in_specs=[pl.BlockSpec(memory_space=pl.ANY)] * 11,
        out_specs=pl.BlockSpec(memory_space=pl.ANY),
        scratch_shapes=scratch,
        compiler_params=pltpu.CompilerParams(
            vmem_limit_bytes=120 * 1024 * 1024, disable_bounds_checks=True),
    )(
        A_x.reshape(S, D), A_mem0.reshape(MEM, D),
        A_Wq.reshape(D // 2, 2, H, DH), A_Wk.reshape(D // 2, 2, H, DH),
        A_Wv.reshape(D // 2, 2, H, DH), A_Wo.reshape(HD, D),
        B_w1, B_w3, B_w2, c, w_mod,
    )
    return out.reshape(1, S, D)
```

```python
import functools

import jax
import jax.numpy as jnp
from jax import lax
import jax.experimental.pallas as pl
import jax.experimental.pallas.tpu as pltpu

F32 = jnp.float32
BF16 = jnp.bfloat16
U32 = jnp.uint32

S = 2048
D = 1024
H = 32
DH = 128
HD = H * DH
MEM = 8
SEG = 32
FF = 3584
EPS = 1e-5
LOG2E = 1.4426950408889634

G = 8
HG = H // G
PRO = 512
NPAIR = S // (2 * SEG)
PT = 2 * SEG
SLOT = 40
NSLOT = 9
X0 = 544
X1 = 640
FC = 256
NFC = FF // FC
KW = 128
KT = D // KW
MW = 128
KPM = MW // KW
NJ = 3 * G // 2
FILL = (0, 2, 4, 9, 11, 14)
QKPOS = 1
PVPOS = 11
MODF = (0, 5, 6, 8, 11, 12)
PROM = PRO + 32
MAIN_START = 1
SCOPES = False
KSTART = 4


class _NoScope:
    def __enter__(self):
        return self

    def __exit__(self, *a):
        return False


def _scope(name):
    return jax.named_scope(name) if SCOPES else _NoScope()


def _unpack(x):
    return pltpu.bitcast(x, BF16)


def _pack(x):
    return pltpu.bitcast(x.astype(BF16), U32)


def _dot(a, b):
    return jnp.dot(a, b, preferred_element_type=F32)


def _ln(x):
    m = jnp.mean(x, axis=-1, keepdims=True)
    xc = x - m
    v = jnp.mean(xc * xc, axis=-1, keepdims=True)
    return xc * lax.rsqrt(v + EPS)


def _recip(x):
    r = pl.reciprocal(x, approx=True)
    return r * (2.0 - x * r)


def _silu(x):
    h = 0.5 * x
    return h + h * jnp.tanh(h)


def _cols(off, w):
    if isinstance(off, int):
        return slice(off, off + w)
    return pl.ds(pl.multiple_of(off, w), w)


def _rarely(cond, fn):
    def body(_, c):
        fn()
        return c

    lax.fori_loop(0, cond.astype(jnp.int32), body, 0)


def _masks():
    def pos(j):
        return jnp.where(j < 40, j, jnp.where(j < 48, j - 32, jnp.where(j < 56, j - 48, j - 40)))

    out = []
    for q0, nq, nk in ((0, 32, 48), (32, 48, 80)):
        qi = lax.broadcasted_iota(jnp.int32, (nq, nk), 0) + q0
        kj = lax.broadcasted_iota(jnp.int32, (nq, nk), 1)
        qp, kp = pos(qi), pos(kj)
        same = ((qi < 40) & (kj < 40)) | ((qi >= 40) & (kj >= 40))
        allowed = same & ((qp < MEM) | (qp >= kp))
        fill = jnp.where(same, jnp.float32(-1e9 * DH ** 0.5), jnp.float32(-jnp.inf))
        out.append((allowed, fill))
    return out


def _kernel(x_hbm, mem0_hbm, wq_hbm, wk_hbm, wv_hbm, wo_hbm, w1_hbm, w3_hbm, w2_hbm,
            c_hbm, wm_hbm, out_hbm,
            xv, outv, wo, w1, w3, w2, wm, cv, m0v, modv, xh, h0, acc,
            lhs_a, lhs_b, o32, abuf, yv, fv, h2, hid, sem_in, sem_m, sem_w, sem_out, *rest):
    ring = rest[0:2]
    wg = rest[2:4]

    def side(g, t):
        return (g % 2) ^ int(t >= 2 * HG)

    scale = DH ** -0.5

    copies = {}

    def mk(name, src, dst):
        copies[name] = pltpu.make_async_copy(src, dst, sem_in.at[len(copies)])

    wm_u = wm_hbm.bitcast(U32)
    mk("c", c_hbm, cv)
    mk("mem0", mem0_hbm, m0v)
    mk("x0", x_hbm.at[0:X0], xv.at[0:X0])
    mk("x1", x_hbm.at[X0:X1], xv.at[X0:X1])
    mk("wo", wo_hbm.bitcast(U32), wo)
    mk("wm1", wm_u.at[:, 2 * D:5 * D], wm.at[:, 2 * D:5 * D])
    mk("w1", w1_hbm.bitcast(U32), w1)
    mk("w3", w3_hbm.bitcast(U32), w3)
    mk("w2", w2_hbm.bitcast(U32), w2)
    mk("wm2", wm_u.at[:, 5 * D:6 * D], wm.at[:, 5 * D:6 * D])
    mk("x2", x_hbm.at[X1:S], xv.at[X1:S])

    def mod_copies(kt):
        return [pltpu.make_async_copy(wm_u.at[:, _cols(i * D + kt * MW, MW)],
                                      wm.at[:, _cols(i * D + kt * MW, MW)], sem_m.at[kt])
                for i in range(2)]

    w_hbm = (wq_hbm, wk_hbm, wv_hbm)

    def block_copies(j, m, gi, t0):
        return [
            pltpu.make_async_copy(
                w_hbm[m].bitcast(U32).at[:, par, (2 * gi + pg) * (HG // 2) + jj],
                wg[side(pg, m * HG)].at[gi, t0 + 2 * jj + par], sem_w.at[j])
            for pg in range(2) for jj in range(HG // 2) for par in range(2)]

    def start_block(j):
        for c in block_copies(j, j // 4, j % 4, (j // 4) * HG):
            c.start()

    def wait_block(j, gi, t0):
        for w in wg:
            buf = w.at[gi, pl.ds(t0, HG)]
            pltpu.make_async_copy(buf, buf, sem_w.at[j]).wait()

    for n in ("x0", "c", "mem0"):
        copies[n].start()

    def zero(i, c):
        acc[i] = jnp.zeros(acc.shape[1:], F32)
        return c

    lax.fori_loop(0, 2 * HG, zero, 0)
    start_block(0)
    for kt in range(D // MW):
        for c in mod_copies(kt):
            c.start()

    def out_copy(r0, n):
        return pltpu.make_async_copy(outv.at[pl.ds(r0, n)], out_hbm.at[pl.ds(r0, n)], sem_out)

    def silu_c():
        return jnp.broadcast_to(_silu(cv[...].astype(F32)), (16, D)).astype(BF16)

    def mod_part(off, w):
        r = _dot(silu_c(), _unpack(wm[:, _cols(off, w)]))[0:8]
        modv[:, _cols(off, w)] = r
        return r[0:1]

    def mvec(i):
        return modv[0:1, i * D:(i + 1) * D]

    def ln1(r0, n):
        xf = xv[pl.ds(r0, n), :].astype(F32)
        return _ln(xf) * (1.0 + mvec(1)) + mvec(0)

    def repack_slot(w, gi, t, enable=None):
        for r0 in range(0, D // 2, 32):
            a = w[gi, t, r0:r0 + 32, :]
            b = w[gi, t + 1, r0:r0 + 32, :]
            e = (a & jnp.uint32(0xFFFF)) | (b << 16)
            o = (a >> 16) | (b & jnp.uint32(0xFFFF0000))
            if enable is not None:
                e = jnp.where(enable, e, a)
                o = jnp.where(enable, o, b)
            w[gi, t, r0:r0 + 32, :] = e
            w[gi, t + 1, r0:r0 + 32, :] = o

    def repack_now(gi, t0):
        def body(i, c):
            for w in wg:
                repack_slot(w, gi, t0 + 2 * i)
            return c

        lax.fori_loop(0, HG // 2, body, 0)

    def store_tokens(dst, gi, t, r):
        for pp in range(PRO // PT):
            b0, r0 = pp * SLOT, pp * PT
            dst[gi, t, b0 + 4:b0 + 8, :] = _pack(r[r0:r0 + 8])
            dst[gi, t, b0 + 8:b0 + 24, :] = _pack(r[r0 + 8:r0 + 40])
            dst[gi, t, b0 + 28:b0 + 32, :] = _pack(r[r0 + 40:r0 + 48])
            dst[gi, t, b0 + 32:b0 + 40, :] = _pack(r[r0 + 48:r0 + 64])
        b0 = (PRO // PT) * SLOT
        dst[gi, t, 0:4, :] = _pack(r[PRO:PRO + 8])
        dst[gi, t, b0 + 4:b0 + 8, :] = _pack(r[PRO + 8:PRO + 16])
        dst[gi, t, b0 + 8:b0 + 16, :] = _pack(r[PRO + 16:PRO + 32])

    def proj(lhs, g, rows, t0, t1):
        for t in range(t0, t1):
            r = _dot(lhs, _unpack(wg[side(g, t)][g // 2, t]))
            for i, row in enumerate(rows):
                ring[side(g, t)][g // 2, t, pl.ds(row, 4), :] = _pack(r[8 * i:8 * i + 8])

    def attn_qk(g, base, q0, nq, nk, allowed, fill):
        qrow = pl.multiple_of(base + q0 // 2, 8)
        ps = []
        for hh in range(HG):
            q = _unpack(ring[g % 2][g // 2, hh, pl.ds(qrow, nq // 2), :])
            k = _unpack(ring[g % 2][g // 2, HG + hh, pl.ds(base, nk // 2), :])
            s = lax.dot_general(q, k, (((1,), (1,)), ((), ())), preferred_element_type=F32)
            s = jnp.where(allowed, s, fill)
            m = jnp.max(s, axis=-1, keepdims=True)
            p = jnp.exp2((s - m) * (scale * LOG2E))
            l = jnp.sum(p, axis=-1, keepdims=True)
            ps.append((p * _recip(l)).astype(BF16))
        return ps

    def attn_pv(g, base, nq, nk, ps):
        for hh in range(HG):
            v = _unpack(ring[1 - g % 2][g // 2, 2 * HG + hh, pl.ds(base, nk // 2), :])
            col = (g * HG + hh) * DH
            o32[0:nq // 2, col:col + DH] = _pack(_dot(ps[hh], v))

    def wo_proj(nq, stores):
        o = _unpack(o32[0:nq // 2, :])
        cw = 256
        for cb in range(D // cw):
            cs = slice(cb * cw, (cb + 1) * cw)
            r = _dot(o, _unpack(wo[:, cs]))
            for r0, n, fn in stores:
                fn(cs, r[r0:r0 + n])

    def post_attn(tok0):
        x1 = xv[pl.ds(tok0, PT), :].astype(F32) + mvec(2) * abuf[...]
        yv[...] = x1
        h2[...] = _pack(_ln(x1) * (1.0 + mvec(4)) + mvec(3))

    def ffn_up(c0, c1):
        a = _unpack(h2[...])
        for c in range(c0, c1):
            cs = slice(c * FC, (c + 1) * FC)
            gt = _dot(a, _unpack(w1[:, cs]))
            up = _dot(a, _unpack(w3[:, cs]))
            hid[:, cs] = _pack(_silu(gt) * up)

    def ffn_down(cb0, cb1, tok0=None):
        a = _unpack(hid[...])
        cw = 256
        for cb in range(cb0, cb1):
            cs = slice(cb * cw, (cb + 1) * cw)
            r = _dot(a, _unpack(w2[:, cs]))
            if tok0 is None:
                fv[:, cs] = r
            else:
                gb = modv[0:1, 5 * D + cb * cw:5 * D + (cb + 1) * cw]
                outv[pl.ds(tok0, PT), cs] = (yv[:, cs] + gb * r).astype(BF16)

    def finish(tok0):
        outv[pl.ds(tok0, PT), :] = (yv[...] + mvec(5) * fv[...]).astype(BF16)

    def unit_row(u):
        r = u & 7
        slot = lax.rem(u >> 3, NSLOT)
        return pl.multiple_of(slot * SLOT + 4 + 4 * r + 4 * (r >= 5).astype(jnp.int32), 4)

    with _scope("waitx0"):
        copies["x0"].wait()
    with _scope("ln0"):

        def ln_body(i, c):
            r0 = pl.multiple_of(i * 136, 8)
            xh[pl.ds(r0, 136), :] = _ln(xv[pl.ds(r0, 136), :].astype(F32))
            return c

        lax.fori_loop(0, X0 // 136, ln_body, 0)
    with _scope("waitc"):
        copies["c"].wait()
        copies["mem0"].wait()

    def modulate(kt):
        sa = mod_part(kt * KW, KW)
        ca = mod_part(D + kt * KW, KW)
        cs = _cols(kt * KW, KW)
        hh = xh[0:PRO + 24, cs] * (1.0 + ca) + sa
        a = _pack(jnp.concatenate([hh[0:PRO], m0v[:, cs].astype(F32), hh[PRO:]], axis=0))
        h0[:, _cols(kt * KW, KW)] = a
        return a

    with _scope("waitw0"):
        wait_block(0, 0, 0)
    with _scope("first"):
        repack_now(0, 0)
        with _scope("waitm0"):
            for c in mod_copies(0):
                c.wait()
        a0 = modulate(0)

    def kmajor(kt, a):
        kn = jnp.minimum(kt + 1, KT - 1)

        def more():
            for j in range(1, 4):
                start_block(j)

        _rarely(kt == KSTART, more)

        @pl.when((kt < KT - 1) & (lax.rem(kn, KPM) == 0))
        def _():
            for c in mod_copies(lax.div(kn, KPM)):
                c.wait()

        rows = pl.ds(pl.multiple_of(kt * (KW // 2), KW // 2), KW // 2)
        a_next = None
        for pg in range(2):
            for t in range(HG):
                r = acc[pg * HG + t] + _dot(_unpack(a), _unpack(wg[pg][0, t, rows, :]))
                acc[pg * HG + t] = r
                store_tokens(ring[pg], 0, t, r)
            if pg == 0:
                a_next = modulate(kn)
        return a_next

    with _scope("kmajor"):
        lax.fori_loop(0, KT, kmajor, a0)

    def pro_body(j, c):
        gi, t0 = j & 3, (j >> 2) * HG
        jn = jnp.minimum(j + 1, NJ - 1)
        gn, tn = jn & 3, (jn >> 2) * HG
        prefetch = (j > 1) & (j < NJ - 1)

        def early_blocks():
            @pl.when(j == 1)
            def _():
                for jj in range(4, 9):
                    start_block(jj)

            @pl.when(j == 3)
            def _():
                for jj in range(9, NJ):
                    start_block(jj)
                for n in ("x1", "wo", "wm1", "w1", "w3", "w2", "wm2", "x2"):
                    copies[n].start()

            def fix():
                with _scope("waitlate"):
                    wait_block(j, gi, t0)
                repack_now(gi, t0)

            _rarely(j <= 2, fix)

        _rarely(j <= 3, early_blocks)

        @pl.when(prefetch)
        def _():
            wait_block(jn, gn, tn)

        a = _unpack(h0[...])
        for pg in range(2):
            for t in range(HG):
                store_tokens(ring[pg], gi, t0 + t, _dot(a, _unpack(wg[pg][gi, t0 + t])))
        gr, tr = jnp.where(prefetch, gn, gi), jnp.where(prefetch, tn, t0)
        for w in wg:
            for t in range(0, HG, 2):
                repack_slot(w, gr, tr + t, prefetch)
        return c

    with _scope("pro"):
        lax.fori_loop(1, NJ, pro_body, 0)

    def pair(p, with_ffn):
        (al_a, fi_a), (al_b, fi_b) = _masks()
        base = pl.multiple_of(lax.rem(p, NSLOT) * SLOT, 8)
        u0 = PRO // 8 + 6 * p
        tlead = PRO + 48 * p

        if with_ffn:
            finish(pl.multiple_of(jnp.maximum(p - 2, 0) * PT, PT))
            post_attn(pl.multiple_of((p - 1) * PT, PT))

        def filler(i, c0=None, c1=None):
            if not with_ffn:
                if i is not None:
                    mod_part(2 * D + MODF[i] * 256, (MODF[i + 1] - MODF[i]) * 256)
            elif c0 is None:
                ffn_down(0, 4)
            else:
                ffn_up(c0, c1)

        def proj_attn(lhs, rows, q0, nq, nk, allowed, fill, f):
            ps = None
            for g in range(G):
                proj(lhs, g, rows, 0, QKPOS)
                if g > 0 and QKPOS > 0:
                    ps = attn_qk(g - 1, base, q0, nq, nk, allowed, fill)
                proj(lhs, g, rows, QKPOS, PVPOS)
                if g > 0:
                    attn_pv(g - 1, base, nq, nk, ps)
                proj(lhs, g, rows, PVPOS, 3 * HG)
                if QKPOS == 0 or g == G - 1:
                    ps = attn_qk(g, base, q0, nq, nk, allowed, fill)
            filler(f, FILL[f], FILL[f + 1])
            attn_pv(G - 1, base, nq, nk, ps)
            filler(f + 1, FILL[f + 1], FILL[f + 2])

        def st_lhs(ref):
            def fn(cs, val):
                ref[0:MEM, cs] = val.astype(BF16).astype(F32)
            return fn

        def st_a(r0, n):
            def fn(cs, val):
                abuf[r0:r0 + n, cs] = val
            return fn

        lhs_b[MEM:32, :] = ln1(pl.multiple_of(tlead + 24, 8), 24)
        if with_ffn:
            lhs = lhs_a[...].astype(BF16)
            rows = [base, unit_row(u0), unit_row(u0 + 1), unit_row(u0 + 2)]
            proj_attn(lhs, rows, 0, 32, 48, al_a, fi_a, 0)
        else:
            ps = [attn_qk(g, base, 0, 32, 48, al_a, fi_a) for g in range(G)]
            filler(0)
            for g in range(G):
                attn_pv(g, base, 32, 48, ps[g])
            filler(1)
        wo_proj(32, [(0, 8, st_lhs(lhs_b)), (8, 24, st_a(0, 24))])
        filler(2, FILL[2], FILL[3])

        lhs = lhs_b[...].astype(BF16)
        rows = [pl.multiple_of(base + 24, 8), unit_row(u0 + 3), unit_row(u0 + 4), unit_row(u0 + 5)]
        nxt = pl.multiple_of(jnp.minimum(tlead + 48, S - 24), 8)
        lhs_a[MEM:32, :] = ln1(nxt, 24)
        proj_attn(lhs, rows, 32, 48, 80, al_b, fi_b, 3)
        wo_proj(48, [(16, 8, st_lhs(lhs_a)), (0, 16, st_a(24, 16)), (24, 24, st_a(40, 24))])
        filler(None)

    with _scope("waitwo"):
        copies["x1"].wait()
        copies["wo"].wait()
        copies["wm1"].wait()

    with _scope("noffn"):
        yv[...] = jnp.zeros(yv.shape, F32)
        fv[...] = jnp.zeros(fv.shape, F32)
        modv[:, 5 * D:6 * D] = jnp.zeros((8, D), F32)
        pair(jnp.int32(0), False)

    with _scope("waitffn"):
        copies["w1"].wait()
        copies["w3"].wait()
        copies["w2"].wait()

    def late_inputs():
        copies["wm2"].wait()
        copies["x2"].wait()
        mod_part(5 * D, D)

    def pair_ffn(p, c):
        _rarely(p == MAIN_START + 1, late_inputs)

        @pl.when(p > MAIN_START + 1)
        def _():
            out_copy(pl.multiple_of((p - 3) * PT, PT), PT).start()

        pair(p, True)
        return c

    with _scope("main"):
        lax.fori_loop(MAIN_START, NPAIR, pair_ffn, 0)

    with _scope("epi"):
        out_copy((NPAIR - 3) * PT, PT).start()
        finish((NPAIR - 2) * PT)
        post_attn((NPAIR - 1) * PT)
        out_copy((NPAIR - 2) * PT, PT).start()

        ffn_up(0, NFC)
        ffn_down(0, 4, (NPAIR - 1) * PT)
        out_copy((NPAIR - 1) * PT, PT).start()
    with _scope("waitout"):
        out_copy(0, S - (MAIN_START - 1) * PT).wait()


@functools.partial(jax.jit, static_argnames=("A_seg_len",))
def pallas_adaLN_cond__memory_aug_recurrent_mem_tr__glu_gated_swiglu__prompt_kernel(
    A_x, A_mem0, A_Wq, A_Wk, A_Wv, A_Wo, A_seg_len, B_x, B_w1, B_w3, B_w2, c, w_mod,
):
    assert A_seg_len == SEG
    assert A_x.shape == (1, S, D) and A_mem0.shape == (1, MEM, D)
    assert A_Wq.shape == (D, H, DH) and B_w1.shape == (D, FF)
    del B_x

    scratch = [
        pltpu.VMEM((S, D), BF16),
        pltpu.VMEM((S, D), BF16),
        pltpu.VMEM((HD // 2, D), U32),
        pltpu.VMEM((D // 2, FF), U32),
        pltpu.VMEM((D // 2, FF), U32),
        pltpu.VMEM((FF // 2, D), U32),
        pltpu.VMEM((D // 2, 6 * D), U32),
        pltpu.VMEM((1, D), BF16),
        pltpu.VMEM((MEM, D), BF16),
        pltpu.VMEM((8, 6 * D), F32),
        pltpu.VMEM((X0, D), F32),
        pltpu.VMEM((PROM // 2, D), U32),
        pltpu.VMEM((2 * HG, PROM, DH), F32),
        pltpu.VMEM((32, D), F32),
        pltpu.VMEM((32, D), F32),
        pltpu.VMEM((24, HD), U32),
        pltpu.VMEM((PT, D), F32),
        pltpu.VMEM((PT, D), F32),
        pltpu.VMEM((PT, D), F32),
        pltpu.VMEM((PT // 2, D), U32),
        pltpu.VMEM((PT // 2, FF), U32),
        pltpu.SemaphoreType.DMA((11,)),
        pltpu.SemaphoreType.DMA((KT,)),
        pltpu.SemaphoreType.DMA((NJ,)),
        pltpu.SemaphoreType.DMA,
    ] + [pltpu.VMEM((G // 2, 3 * HG, NSLOT * SLOT, DH), U32)] * 2 + [
        pltpu.VMEM((G // 2, 3 * HG, D // 2, DH), U32)] * 2

    out = pl.pallas_call(
        _kernel,
        out_shape=jax.ShapeDtypeStruct((S, D), BF16),
        in_specs=[pl.BlockSpec(memory_space=pl.ANY)] * 11,
        out_specs=pl.BlockSpec(memory_space=pl.ANY),
        scratch_shapes=scratch,
        compiler_params=pltpu.CompilerParams(
            vmem_limit_bytes=120 * 1024 * 1024, disable_bounds_checks=True),
    )(
        A_x.reshape(S, D), A_mem0.reshape(MEM, D),
        A_Wq.reshape(D // 2, 2, H, DH), A_Wk.reshape(D // 2, 2, H, DH),
        A_Wv.reshape(D // 2, 2, H, DH), A_Wo.reshape(HD, D),
        B_w1, B_w3, B_w2, c, w_mod,
    )
    return out.reshape(1, S, D)
```

```python
import functools

import jax
import jax.numpy as jnp
from jax import lax
import jax.experimental.pallas as pl
import jax.experimental.pallas.tpu as pltpu

F32 = jnp.float32
BF16 = jnp.bfloat16
U32 = jnp.uint32

S = 2048
D = 1024
H = 32
DH = 128
HD = H * DH
MEM = 8
SEG = 32
FF = 3584
EPS = 1e-5
LOG2E = 1.4426950408889634

G = 8
HG = H // G
PRO = 512
NPAIR = S // (2 * SEG)
PT = 2 * SEG
SLOT = 40
NSLOT = 9
X0 = 544
X1 = 640
FC = 256
NFC = FF // FC
KW = 128
KT = D // KW
NJ = 3 * G // 2
FILL = (0, 2, 4, 9, 11, 14)
QKPOS = 1
PVPOS = 11
MODF = (0, 5, 6, 8, 11, 12)
PROM = PRO + 32
MAIN_START = 1
SCOPES = False


class _NoScope:
    def __enter__(self):
        return self

    def __exit__(self, *a):
        return False


def _scope(name):
    return jax.named_scope(name) if SCOPES else _NoScope()


def _unpack(x):
    return pltpu.bitcast(x, BF16)


def _pack(x):
    return pltpu.bitcast(x.astype(BF16), U32)


def _dot(a, b):
    return jnp.dot(a, b, preferred_element_type=F32)


def _ln(x):
    m = jnp.mean(x, axis=-1, keepdims=True)
    xc = x - m
    v = jnp.mean(xc * xc, axis=-1, keepdims=True)
    return xc * lax.rsqrt(v + EPS)


def _recip(x):
    r = pl.reciprocal(x, approx=True)
    return r * (2.0 - x * r)


def _silu(x):
    h = 0.5 * x
    return h + h * jnp.tanh(h)


def _cols(off, w):
    if isinstance(off, int):
        return slice(off, off + w)
    return pl.ds(pl.multiple_of(off, w), w)


def _rarely(cond, fn):
    def body(_, c):
        fn()
        return c

    lax.fori_loop(0, cond.astype(jnp.int32), body, 0)


def _masks():
    def pos(j):
        return jnp.where(j < 40, j, jnp.where(j < 48, j - 32, jnp.where(j < 56, j - 48, j - 40)))

    out = []
    for q0, nq, nk in ((0, 32, 48), (32, 48, 80)):
        qi = lax.broadcasted_iota(jnp.int32, (nq, nk), 0) + q0
        kj = lax.broadcasted_iota(jnp.int32, (nq, nk), 1)
        qp, kp = pos(qi), pos(kj)
        same = ((qi < 40) & (kj < 40)) | ((qi >= 40) & (kj >= 40))
        allowed = same & ((qp < MEM) | (qp >= kp))
        fill = jnp.where(same, jnp.float32(-1e9 * DH ** 0.5), jnp.float32(-jnp.inf))
        out.append((allowed, fill))
    return out


def _kernel(x_hbm, mem0_hbm, wq_hbm, wk_hbm, wv_hbm, wo_hbm, w1_hbm, w3_hbm, w2_hbm,
            c_hbm, wm_hbm, out_hbm,
            xv, outv, wo, w1, w3, w2, wm, cv, m0v, modv, xh, h0, hn, acc,
            lhs_a, lhs_b, o32, abuf, yv, fv, h2, hid, sem_in, sem_m, sem_w, sem_out, *rest):
    ring = rest[0:2]
    wg = rest[2:4]

    def side(g, t):
        return (g % 2) ^ int(t >= 2 * HG)

    scale = DH ** -0.5

    copies = {}

    def mk(name, src, dst):
        copies[name] = pltpu.make_async_copy(src, dst, sem_in.at[len(copies)])

    wm_u = wm_hbm.bitcast(U32)
    mk("c", c_hbm, cv)
    mk("mem0", mem0_hbm, m0v)
    mk("x0", x_hbm.at[0:X0], xv.at[0:X0])
    mk("x1", x_hbm.at[X0:X1], xv.at[X0:X1])
    mk("wo", wo_hbm.bitcast(U32), wo)
    mk("wm1", wm_u.at[:, 2 * D:5 * D], wm.at[:, 2 * D:5 * D])
    mk("w1", w1_hbm.bitcast(U32), w1)
    mk("w3", w3_hbm.bitcast(U32), w3)
    mk("w2", w2_hbm.bitcast(U32), w2)
    mk("wm2", wm_u.at[:, 5 * D:6 * D], wm.at[:, 5 * D:6 * D])
    mk("x2", x_hbm.at[X1:S], xv.at[X1:S])

    def mod_copies(kt):
        return [pltpu.make_async_copy(wm_u.at[:, _cols(i * D + kt * KW, KW)],
                                      wm.at[:, _cols(i * D + kt * KW, KW)], sem_m.at[kt])
                for i in range(2)]

    w_hbm = (wq_hbm, wk_hbm, wv_hbm)

    def block_copies(j, m, gi, t0):
        return [
            pltpu.make_async_copy(
                w_hbm[m].bitcast(U32).at[:, par, (2 * gi + pg) * (HG // 2) + jj],
                wg[side(pg, m * HG)].at[gi, t0 + 2 * jj + par], sem_w.at[j])
            for pg in range(2) for jj in range(HG // 2) for par in range(2)]

    def start_block(j):
        for c in block_copies(j, j // 4, j % 4, (j // 4) * HG):
            c.start()

    def wait_block(j, gi, t0):
        for w in wg:
            buf = w.at[gi, pl.ds(t0, HG)]
            pltpu.make_async_copy(buf, buf, sem_w.at[j]).wait()

    for n in ("x0", "c", "mem0"):
        copies[n].start()

    def zero(i, c):
        acc[i] = jnp.zeros(acc.shape[1:], F32)
        return c

    lax.fori_loop(0, 2 * HG, zero, 0)
    start_block(0)
    for kt in range(KT):
        for c in mod_copies(kt):
            c.start()
    for j in range(1, 4):
        start_block(j)

    def out_copy(r0, n):
        return pltpu.make_async_copy(outv.at[pl.ds(r0, n)], out_hbm.at[pl.ds(r0, n)], sem_out)

    def silu_c():
        return jnp.broadcast_to(_silu(cv[...].astype(F32)), (16, D)).astype(BF16)

    def mod_part(off, w):
        r = _dot(silu_c(), _unpack(wm[:, _cols(off, w)]))[0:8]
        modv[:, _cols(off, w)] = r
        return r[0:1]

    def mvec(i):
        return modv[0:1, i * D:(i + 1) * D]

    def ln1(r0, n):
        xf = xv[pl.ds(r0, n), :].astype(F32)
        return _ln(xf) * (1.0 + mvec(1)) + mvec(0)

    def repack_slot(w, gi, t, enable=None):
        for r0 in range(0, D // 2, 32):
            a = w[gi, t, r0:r0 + 32, :]
            b = w[gi, t + 1, r0:r0 + 32, :]
            e = (a & jnp.uint32(0xFFFF)) | (b << 16)
            o = (a >> 16) | (b & jnp.uint32(0xFFFF0000))
            if enable is not None:
                e = jnp.where(enable, e, a)
                o = jnp.where(enable, o, b)
            w[gi, t, r0:r0 + 32, :] = e
            w[gi, t + 1, r0:r0 + 32, :] = o

    def repack_now(gi, t0):
        def body(i, c):
            for w in wg:
                repack_slot(w, gi, t0 + 2 * i)
            return c

        lax.fori_loop(0, HG // 2, body, 0)

    def store_tokens(dst, gi, t, r):
        for pp in range(PRO // PT):
            b0, r0 = pp * SLOT, pp * PT
            dst[gi, t, b0 + 4:b0 + 8, :] = _pack(r[r0:r0 + 8])
            dst[gi, t, b0 + 8:b0 + 24, :] = _pack(r[r0 + 8:r0 + 40])
            dst[gi, t, b0 + 28:b0 + 32, :] = _pack(r[r0 + 40:r0 + 48])
            dst[gi, t, b0 + 32:b0 + 40, :] = _pack(r[r0 + 48:r0 + 64])
        b0 = (PRO // PT) * SLOT
        dst[gi, t, 0:4, :] = _pack(r[PRO:PRO + 8])
        dst[gi, t, b0 + 4:b0 + 8, :] = _pack(r[PRO + 8:PRO + 16])
        dst[gi, t, b0 + 8:b0 + 16, :] = _pack(r[PRO + 16:PRO + 32])

    def proj(lhs, g, rows, t0, t1):
        for t in range(t0, t1):
            r = _dot(lhs, _unpack(wg[side(g, t)][g // 2, t]))
            for i, row in enumerate(rows):
                ring[side(g, t)][g // 2, t, pl.ds(row, 4), :] = _pack(r[8 * i:8 * i + 8])

    def attn_qk(g, base, q0, nq, nk, allowed, fill):
        qrow = pl.multiple_of(base + q0 // 2, 8)
        ps = []
        for hh in range(HG):
            q = _unpack(ring[g % 2][g // 2, hh, pl.ds(qrow, nq // 2), :])
            k = _unpack(ring[g % 2][g // 2, HG + hh, pl.ds(base, nk // 2), :])
            s = lax.dot_general(q, k, (((1,), (1,)), ((), ())), preferred_element_type=F32)
            s = jnp.where(allowed, s, fill)
            m = jnp.max(s, axis=-1, keepdims=True)
            p = jnp.exp2((s - m) * (scale * LOG2E))
            l = jnp.sum(p, axis=-1, keepdims=True)
            ps.append((p * _recip(l)).astype(BF16))
        return ps

    def attn_pv(g, base, nq, nk, ps):
        for hh in range(HG):
            v = _unpack(ring[1 - g % 2][g // 2, 2 * HG + hh, pl.ds(base, nk // 2), :])
            col = (g * HG + hh) * DH
            o32[0:nq // 2, col:col + DH] = _pack(_dot(ps[hh], v))

    def wo_proj(nq, stores):
        o = _unpack(o32[0:nq // 2, :])
        cw = 256
        for cb in range(D // cw):
            cs = slice(cb * cw, (cb + 1) * cw)
            r = _dot(o, _unpack(wo[:, cs]))
            for r0, n, fn in stores:
                fn(cs, r[r0:r0 + n])

    def post_attn(tok0):
        x1 = xv[pl.ds(tok0, PT), :].astype(F32) + mvec(2) * abuf[...]
        yv[...] = x1
        h2[...] = _pack(_ln(x1) * (1.0 + mvec(4)) + mvec(3))

    def ffn_up(c0, c1):
        a = _unpack(h2[...])
        for c in range(c0, c1):
            cs = slice(c * FC, (c + 1) * FC)
            gt = _dot(a, _unpack(w1[:, cs]))
            up = _dot(a, _unpack(w3[:, cs]))
            hid[:, cs] = _pack(_silu(gt) * up)

    def ffn_down(cb0, cb1, tok0=None):
        a = _unpack(hid[...])
        cw = 256
        for cb in range(cb0, cb1):
            cs = slice(cb * cw, (cb + 1) * cw)
            r = _dot(a, _unpack(w2[:, cs]))
            if tok0 is None:
                fv[:, cs] = r
            else:
                gb = modv[0:1, 5 * D + cb * cw:5 * D + (cb + 1) * cw]
                outv[pl.ds(tok0, PT), cs] = (yv[:, cs] + gb * r).astype(BF16)

    def finish(tok0):
        outv[pl.ds(tok0, PT), :] = (yv[...] + mvec(5) * fv[...]).astype(BF16)

    def unit_row(u):
        r = u & 7
        slot = lax.rem(u >> 3, NSLOT)
        return pl.multiple_of(slot * SLOT + 4 + 4 * r + 4 * (r >= 5).astype(jnp.int32), 4)

    with _scope("waitx0"):
        copies["x0"].wait()
    with _scope("ln0"):

        def ln_body(i, c):
            r0 = pl.multiple_of(i * 136, 8)
            xh[pl.ds(r0, 136), :] = _ln(xv[pl.ds(r0, 136), :].astype(F32))
            return c

        lax.fori_loop(0, X0 // 136, ln_body, 0)
    with _scope("waitc"):
        copies["c"].wait()
        copies["mem0"].wait()

    def modulate(kt):
        sa = mod_part(kt * KW, KW)
        ca = mod_part(D + kt * KW, KW)
        cs = _cols(kt * KW, KW)
        hh = xh[0:PRO + 24, cs] * (1.0 + ca) + sa
        hn[...] = _pack(jnp.concatenate([hh[0:PRO], m0v[:, cs].astype(F32), hh[PRO:]], axis=0))

    with _scope("waitw0"):
        wait_block(0, 0, 0)
    with _scope("first"):
        repack_now(0, 0)
        with _scope("waitm0"):
            for c in mod_copies(0):
                c.wait()
        modulate(0)

    def kmajor(kt, c):
        kn = jnp.minimum(kt + 1, KT - 1)

        @pl.when(kt < KT - 1)
        def _():
            for cp in mod_copies(kn):
                cp.wait()

        cs = _cols(kt * KW, KW)
        h0[:, cs] = hn[...]
        rows = pl.ds(pl.multiple_of(kt * (KW // 2), KW // 2), KW // 2)
        for pg in range(2):
            for t in range(HG):
                r = acc[pg * HG + t] + _dot(_unpack(h0[:, cs]), _unpack(wg[pg][0, t, rows, :]))
                acc[pg * HG + t] = r
                store_tokens(ring[pg], 0, t, r)
            if pg == 0:
                modulate(kn)
        return c

    with _scope("kmajor"):
        lax.fori_loop(0, KT, kmajor, 0)

    def pro_body(j, c):
        gi, t0 = j & 3, (j >> 2) * HG
        jn = jnp.minimum(j + 1, NJ - 1)
        gn, tn = jn & 3, (jn >> 2) * HG
        prefetch = (j > 1) & (j < NJ - 1)

        def early_blocks():
            @pl.when(j == 1)
            def _():
                for jj in range(4, 9):
                    start_block(jj)

            @pl.when(j == 3)
            def _():
                for jj in range(9, NJ):
                    start_block(jj)
                for n in ("x1", "wo", "wm1", "w1", "w3", "w2", "wm2", "x2"):
                    copies[n].start()

            def fix():
                with _scope("waitlate"):
                    wait_block(j, gi, t0)
                repack_now(gi, t0)

            _rarely(j <= 2, fix)

        _rarely(j <= 3, early_blocks)

        @pl.when(prefetch)
        def _():
            wait_block(jn, gn, tn)

        a = _unpack(h0[...])
        for pg in range(2):
            for t in range(HG):
                store_tokens(ring[pg], gi, t0 + t, _dot(a, _unpack(wg[pg][gi, t0 + t])))
        gr, tr = jnp.where(prefetch, gn, gi), jnp.where(prefetch, tn, t0)
        for w in wg:
            for t in range(0, HG, 2):
                repack_slot(w, gr, tr + t, prefetch)
        return c

    with _scope("pro"):
        lax.fori_loop(1, NJ, pro_body, 0)

    def pair(p, with_ffn):
        (al_a, fi_a), (al_b, fi_b) = _masks()
        base = pl.multiple_of(lax.rem(p, NSLOT) * SLOT, 8)
        u0 = PRO // 8 + 6 * p
        tlead = PRO + 48 * p

        if with_ffn:
            finish(pl.multiple_of(jnp.maximum(p - 2, 0) * PT, PT))
            post_attn(pl.multiple_of((p - 1) * PT, PT))

        def filler(i, c0=None, c1=None):
            if not with_ffn:
                if i is not None:
                    mod_part(2 * D + MODF[i] * 256, (MODF[i + 1] - MODF[i]) * 256)
            elif c0 is None:
                ffn_down(0, 4)
            else:
                ffn_up(c0, c1)

        def proj_attn(lhs, rows, q0, nq, nk, allowed, fill, f):
            ps = None
            for g in range(G):
                proj(lhs, g, rows, 0, QKPOS)
                if g > 0 and QKPOS > 0:
                    ps = attn_qk(g - 1, base, q0, nq, nk, allowed, fill)
                proj(lhs, g, rows, QKPOS, PVPOS)
                if g > 0:
                    attn_pv(g - 1, base, nq, nk, ps)
                proj(lhs, g, rows, PVPOS, 3 * HG)
                if QKPOS == 0 or g == G - 1:
                    ps = attn_qk(g, base, q0, nq, nk, allowed, fill)
            filler(f, FILL[f], FILL[f + 1])
            attn_pv(G - 1, base, nq, nk, ps)
            filler(f + 1, FILL[f + 1], FILL[f + 2])

        def st_lhs(ref):
            def fn(cs, val):
                ref[0:MEM, cs] = val.astype(BF16).astype(F32)
            return fn

        def st_a(r0, n):
            def fn(cs, val):
                abuf[r0:r0 + n, cs] = val
            return fn

        lhs_b[MEM:32, :] = ln1(pl.multiple_of(tlead + 24, 8), 24)
        if with_ffn:
            lhs = lhs_a[...].astype(BF16)
            rows = [base, unit_row(u0), unit_row(u0 + 1), unit_row(u0 + 2)]
            proj_attn(lhs, rows, 0, 32, 48, al_a, fi_a, 0)
        else:
            ps = [attn_qk(g, base, 0, 32, 48, al_a, fi_a) for g in range(G)]
            filler(0)
            for g in range(G):
                attn_pv(g, base, 32, 48, ps[g])
            filler(1)
        wo_proj(32, [(0, 8, st_lhs(lhs_b)), (8, 24, st_a(0, 24))])
        filler(2, FILL[2], FILL[3])

        lhs = lhs_b[...].astype(BF16)
        rows = [pl.multiple_of(base + 24, 8), unit_row(u0 + 3), unit_row(u0 + 4), unit_row(u0 + 5)]
        nxt = pl.multiple_of(jnp.minimum(tlead + 48, S - 24), 8)
        lhs_a[MEM:32, :] = ln1(nxt, 24)
        proj_attn(lhs, rows, 32, 48, 80, al_b, fi_b, 3)
        wo_proj(48, [(16, 8, st_lhs(lhs_a)), (0, 16, st_a(24, 16)), (24, 24, st_a(40, 24))])
        filler(None)

    with _scope("waitwo"):
        copies["x1"].wait()
        copies["wo"].wait()
        copies["wm1"].wait()

    with _scope("noffn"):
        yv[...] = jnp.zeros(yv.shape, F32)
        fv[...] = jnp.zeros(fv.shape, F32)
        modv[:, 5 * D:6 * D] = jnp.zeros((8, D), F32)
        pair(jnp.int32(0), False)

    with _scope("waitffn"):
        copies["w1"].wait()
        copies["w3"].wait()
        copies["w2"].wait()

    def late_inputs():
        copies["wm2"].wait()
        copies["x2"].wait()
        mod_part(5 * D, D)

    def pair_ffn(p, c):
        _rarely(p == MAIN_START + 1, late_inputs)

        @pl.when(p > MAIN_START + 1)
        def _():
            out_copy(pl.multiple_of((p - 3) * PT, PT), PT).start()

        pair(p, True)
        return c

    with _scope("main"):
        lax.fori_loop(MAIN_START, NPAIR, pair_ffn, 0)

    with _scope("epi"):
        out_copy((NPAIR - 3) * PT, PT).start()
        finish((NPAIR - 2) * PT)
        post_attn((NPAIR - 1) * PT)
        out_copy((NPAIR - 2) * PT, PT).start()

        ffn_up(0, NFC)
        ffn_down(0, 4, (NPAIR - 1) * PT)
        out_copy((NPAIR - 1) * PT, PT).start()
    with _scope("waitout"):
        out_copy(0, S - (MAIN_START - 1) * PT).wait()


@functools.partial(jax.jit, static_argnames=("A_seg_len",))
def pallas_adaLN_cond__memory_aug_recurrent_mem_tr__glu_gated_swiglu__prompt_kernel(
    A_x, A_mem0, A_Wq, A_Wk, A_Wv, A_Wo, A_seg_len, B_x, B_w1, B_w3, B_w2, c, w_mod,
):
    assert A_seg_len == SEG
    assert A_x.shape == (1, S, D) and A_mem0.shape == (1, MEM, D)
    assert A_Wq.shape == (D, H, DH) and B_w1.shape == (D, FF)
    del B_x

    scratch = [
        pltpu.VMEM((S, D), BF16),
        pltpu.VMEM((S, D), BF16),
        pltpu.VMEM((HD // 2, D), U32),
        pltpu.VMEM((D // 2, FF), U32),
        pltpu.VMEM((D // 2, FF), U32),
        pltpu.VMEM((FF // 2, D), U32),
        pltpu.VMEM((D // 2, 6 * D), U32),
        pltpu.VMEM((1, D), BF16),
        pltpu.VMEM((MEM, D), BF16),
        pltpu.VMEM((8, 6 * D), F32),
        pltpu.VMEM((X0, D), F32),
        pltpu.VMEM((PROM // 2, D), U32),
        pltpu.VMEM((PROM // 2, KW), U32),
        pltpu.VMEM((2 * HG, PROM, DH), F32),
        pltpu.VMEM((32, D), F32),
        pltpu.VMEM((32, D), F32),
        pltpu.VMEM((24, HD), U32),
        pltpu.VMEM((PT, D), F32),
        pltpu.VMEM((PT, D), F32),
        pltpu.VMEM((PT, D), F32),
        pltpu.VMEM((PT // 2, D), U32),
        pltpu.VMEM((PT // 2, FF), U32),
        pltpu.SemaphoreType.DMA((11,)),
        pltpu.SemaphoreType.DMA((KT,)),
        pltpu.SemaphoreType.DMA((NJ,)),
        pltpu.SemaphoreType.DMA,
    ] + [pltpu.VMEM((G // 2, 3 * HG, NSLOT * SLOT, DH), U32)] * 2 + [
        pltpu.VMEM((G // 2, 3 * HG, D // 2, DH), U32)] * 2

    out = pl.pallas_call(
        _kernel,
        out_shape=jax.ShapeDtypeStruct((S, D), BF16),
        in_specs=[pl.BlockSpec(memory_space=pl.ANY)] * 11,
        out_specs=pl.BlockSpec(memory_space=pl.ANY),
        scratch_shapes=scratch,
        compiler_params=pltpu.CompilerParams(
            vmem_limit_bytes=120 * 1024 * 1024, disable_bounds_checks=True),
    )(
        A_x.reshape(S, D), A_mem0.reshape(MEM, D),
        A_Wq.reshape(D // 2, 2, H, DH), A_Wk.reshape(D // 2, 2, H, DH),
        A_Wv.reshape(D // 2, 2, H, DH), A_Wo.reshape(HD, D),
        B_w1, B_w3, B_w2, c, w_mod,
    )
    return out.reshape(1, S, D)
```

```python
import functools

import jax
import jax.numpy as jnp
from jax import lax
import jax.experimental.pallas as pl
import jax.experimental.pallas.tpu as pltpu

F32 = jnp.float32
BF16 = jnp.bfloat16
U32 = jnp.uint32

S = 2048
D = 1024
H = 32
DH = 128
HD = H * DH
MEM = 8
SEG = 32
FF = 3584
EPS = 1e-5
LOG2E = 1.4426950408889634

G = 8
HG = H // G
PRO = 512
NPAIR = S // (2 * SEG)
PT = 2 * SEG
SLOT = 40
NSLOT = 9
X0 = 544
X1 = 640
FC = 256
NFC = FF // FC
KW = 128
KT = D // KW
NJ = 3 * G // 2
FILL = (0, 2, 4, 9, 11, 14)
QKPOS = 1
PVPOS = 11
MODF = (0, 5, 6, 8, 11, 12)
PROM = PRO + 32
MAIN_START = 1
SCOPES = False


class _NoScope:
    def __enter__(self):
        return self

    def __exit__(self, *a):
        return False


def _scope(name):
    return jax.named_scope(name) if SCOPES else _NoScope()


def _unpack(x):
    return pltpu.bitcast(x, BF16)


def _pack(x):
    return pltpu.bitcast(x.astype(BF16), U32)


def _dot(a, b):
    return jnp.dot(a, b, preferred_element_type=F32)


def _ln(x):
    m = jnp.mean(x, axis=-1, keepdims=True)
    xc = x - m
    v = jnp.mean(xc * xc, axis=-1, keepdims=True)
    return xc * lax.rsqrt(v + EPS)


def _recip(x):
    r = pl.reciprocal(x, approx=True)
    return r * (2.0 - x * r)


def _silu(x):
    h = 0.5 * x
    return h + h * jnp.tanh(h)


def _cols(off, w):
    if isinstance(off, int):
        return slice(off, off + w)
    return pl.ds(pl.multiple_of(off, w), w)


def _rarely(cond, fn):
    def body(_, c):
        fn()
        return c

    lax.fori_loop(0, cond.astype(jnp.int32), body, 0)


def _masks():
    def pos(j):
        return jnp.where(j < 40, j, jnp.where(j < 48, j - 32, jnp.where(j < 56, j - 48, j - 40)))

    out = []
    for q0, nq, nk in ((0, 32, 48), (32, 48, 80)):
        qi = lax.broadcasted_iota(jnp.int32, (nq, nk), 0) + q0
        kj = lax.broadcasted_iota(jnp.int32, (nq, nk), 1)
        qp, kp = pos(qi), pos(kj)
        same = ((qi < 40) & (kj < 40)) | ((qi >= 40) & (kj >= 40))
        allowed = same & ((qp < MEM) | (qp >= kp))
        fill = jnp.where(same, jnp.float32(-1e9 * DH ** 0.5), jnp.float32(-jnp.inf))
        out.append((allowed, fill))
    return out


def _kernel(x_hbm, mem0_hbm, wq_hbm, wk_hbm, wv_hbm, wo_hbm, w1_hbm, w3_hbm, w2_hbm,
            c_hbm, wm_hbm, out_hbm,
            xv, outv, wo, w1, w3, w2, wm, cv, m0v, modv, xh, h0, hn, acc,
            lhs_a, lhs_b, o32, abuf, yv, fv, h2, hid, sem_in, sem_m, sem_w, sem_out, *rest):
    ring = rest[0:2]
    wg = rest[2:4]

    def side(g, t):
        return (g % 2) ^ int(t >= 2 * HG)

    scale = DH ** -0.5

    copies = {}

    def mk(name, src, dst):
        copies[name] = pltpu.make_async_copy(src, dst, sem_in.at[len(copies)])

    wm_u = wm_hbm.bitcast(U32)
    mk("c", c_hbm, cv)
    mk("mem0", mem0_hbm, m0v)
    mk("x0", x_hbm.at[0:X0], xv.at[0:X0])
    mk("x1", x_hbm.at[X0:X1], xv.at[X0:X1])
    mk("wo", wo_hbm.bitcast(U32), wo)
    mk("wm1", wm_u.at[:, 2 * D:5 * D], wm.at[:, 2 * D:5 * D])
    mk("w1", w1_hbm.bitcast(U32), w1)
    mk("w3", w3_hbm.bitcast(U32), w3)
    mk("w2", w2_hbm.bitcast(U32), w2)
    mk("wm2", wm_u.at[:, 5 * D:6 * D], wm.at[:, 5 * D:6 * D])
    mk("x2", x_hbm.at[X1:S], xv.at[X1:S])

    def mod_copies(kt):
        return [pltpu.make_async_copy(wm_u.at[:, _cols(i * D + kt * KW, KW)],
                                      wm.at[:, _cols(i * D + kt * KW, KW)], sem_m.at[kt])
                for i in range(2)]

    w_hbm = (wq_hbm, wk_hbm, wv_hbm)

    def block_copies(j, m, gi, t0):
        return [
            pltpu.make_async_copy(
                w_hbm[m].bitcast(U32).at[:, par, (2 * gi + pg) * (HG // 2) + jj],
                wg[side(pg, m * HG)].at[gi, t0 + 2 * jj + par], sem_w.at[j])
            for pg in range(2) for jj in range(HG // 2) for par in range(2)]

    def start_block(j):
        for c in block_copies(j, j // 4, j % 4, (j // 4) * HG):
            c.start()

    def wait_block(j, gi, t0):
        for w in wg:
            buf = w.at[gi, pl.ds(t0, HG)]
            pltpu.make_async_copy(buf, buf, sem_w.at[j]).wait()

    for n in ("x0", "c", "mem0"):
        copies[n].start()

    def zero(i, c):
        acc[i] = jnp.zeros(acc.shape[1:], F32)
        return c

    lax.fori_loop(0, 2 * HG, zero, 0)
    start_block(0)
    for kt in range(KT):
        for c in mod_copies(kt):
            c.start()
    for j in range(1, 4):
        start_block(j)

    def out_copy(r0, n):
        return pltpu.make_async_copy(outv.at[pl.ds(r0, n)], out_hbm.at[pl.ds(r0, n)], sem_out)

    def silu_c():
        return jnp.broadcast_to(_silu(cv[...].astype(F32)), (16, D)).astype(BF16)

    def mod_part(off, w):
        r = _dot(silu_c(), _unpack(wm[:, _cols(off, w)]))[0:8]
        modv[:, _cols(off, w)] = r
        return r[0:1]

    def mvec(i):
        return modv[0:1, i * D:(i + 1) * D]

    def ln1(r0, n):
        xf = xv[pl.ds(r0, n), :].astype(F32)
        return _ln(xf) * (1.0 + mvec(1)) + mvec(0)

    def repack_slot(w, gi, t, enable=None):
        for r0 in range(0, D // 2, 32):
            a = w[gi, t, r0:r0 + 32, :]
            b = w[gi, t + 1, r0:r0 + 32, :]
            e = (a & jnp.uint32(0xFFFF)) | (b << 16)
            o = (a >> 16) | (b & jnp.uint32(0xFFFF0000))
            if enable is not None:
                e = jnp.where(enable, e, a)
                o = jnp.where(enable, o, b)
            w[gi, t, r0:r0 + 32, :] = e
            w[gi, t + 1, r0:r0 + 32, :] = o

    def repack_now(gi, t0):
        def body(i, c):
            for w in wg:
                repack_slot(w, gi, t0 + 2 * i)
            return c

        lax.fori_loop(0, HG // 2, body, 0)

    def store_tokens(dst, gi, t, r):
        for pp in range(PRO // PT):
            b0, r0 = pp * SLOT, pp * PT
            dst[gi, t, b0 + 4:b0 + 8, :] = _pack(r[r0:r0 + 8])
            dst[gi, t, b0 + 8:b0 + 24, :] = _pack(r[r0 + 8:r0 + 40])
            dst[gi, t, b0 + 28:b0 + 32, :] = _pack(r[r0 + 40:r0 + 48])
            dst[gi, t, b0 + 32:b0 + 40, :] = _pack(r[r0 + 48:r0 + 64])
        b0 = (PRO // PT) * SLOT
        dst[gi, t, 0:4, :] = _pack(r[PRO:PRO + 8])
        dst[gi, t, b0 + 4:b0 + 8, :] = _pack(r[PRO + 8:PRO + 16])
        dst[gi, t, b0 + 8:b0 + 16, :] = _pack(r[PRO + 16:PRO + 32])

    def proj(lhs, g, rows, t0, t1):
        for t in range(t0, t1):
            r = _dot(lhs, _unpack(wg[side(g, t)][g // 2, t]))
            for i, row in enumerate(rows):
                ring[side(g, t)][g // 2, t, pl.ds(row, 4), :] = _pack(r[8 * i:8 * i + 8])

    def attn_qk(g, base, q0, nq, nk, allowed, fill):
        qrow = pl.multiple_of(base + q0 // 2, 8)
        ps = []
        for hh in range(HG):
            q = _unpack(ring[g % 2][g // 2, hh, pl.ds(qrow, nq // 2), :])
            k = _unpack(ring[g % 2][g // 2, HG + hh, pl.ds(base, nk // 2), :])
            s = lax.dot_general(q, k, (((1,), (1,)), ((), ())), preferred_element_type=F32)
            s = jnp.where(allowed, s, fill)
            m = jnp.max(s, axis=-1, keepdims=True)
            p = jnp.exp2((s - m) * (scale * LOG2E))
            l = jnp.sum(p, axis=-1, keepdims=True)
            ps.append((p * _recip(l)).astype(BF16))
        return ps

    def attn_pv(g, base, nq, nk, ps):
        for hh in range(HG):
            v = _unpack(ring[1 - g % 2][g // 2, 2 * HG + hh, pl.ds(base, nk // 2), :])
            col = (g * HG + hh) * DH
            o32[0:nq // 2, col:col + DH] = _pack(_dot(ps[hh], v))

    def wo_proj(nq, stores):
        o = _unpack(o32[0:nq // 2, :])
        cw = 256
        for cb in range(D // cw):
            cs = slice(cb * cw, (cb + 1) * cw)
            r = _dot(o, _unpack(wo[:, cs]))
            for r0, n, fn in stores:
                fn(cs, r[r0:r0 + n])

    def post_attn(tok0):
        x1 = xv[pl.ds(tok0, PT), :].astype(F32) + mvec(2) * abuf[...]
        yv[...] = x1
        h2[...] = _pack(_ln(x1) * (1.0 + mvec(4)) + mvec(3))

    def ffn_up(c0, c1):
        a = _unpack(h2[...])
        for c in range(c0, c1):
            cs = slice(c * FC, (c + 1) * FC)
            gt = _dot(a, _unpack(w1[:, cs]))
            up = _dot(a, _unpack(w3[:, cs]))
            hid[:, cs] = _pack(_silu(gt) * up)

    def ffn_down(cb0, cb1, tok0=None):
        a = _unpack(hid[...])
        cw = 256
        for cb in range(cb0, cb1):
            cs = slice(cb * cw, (cb + 1) * cw)
            r = _dot(a, _unpack(w2[:, cs]))
            if tok0 is None:
                fv[:, cs] = r
            else:
                gb = modv[0:1, 5 * D + cb * cw:5 * D + (cb + 1) * cw]
                outv[pl.ds(tok0, PT), cs] = (yv[:, cs] + gb * r).astype(BF16)
                pltpu.make_async_copy(outv.at[pl.ds(tok0, PT), cs],
                                      out_hbm.at[pl.ds(tok0, PT), cs], sem_out).start()

    def finish(tok0):
        outv[pl.ds(tok0, PT), :] = (yv[...] + mvec(5) * fv[...]).astype(BF16)

    def unit_row(u):
        r = u & 7
        slot = lax.rem(u >> 3, NSLOT)
        return pl.multiple_of(slot * SLOT + 4 + 4 * r + 4 * (r >= 5).astype(jnp.int32), 4)

    with _scope("waitx0"):
        copies["x0"].wait()
    with _scope("ln0"):

        def ln_body(i, c):
            r0 = pl.multiple_of(i * 136, 8)
            xh[pl.ds(r0, 136), :] = _ln(xv[pl.ds(r0, 136), :].astype(F32))
            return c

        lax.fori_loop(0, X0 // 136, ln_body, 0)
    with _scope("waitc"):
        copies["c"].wait()
        copies["mem0"].wait()

    def modulate(kt):
        sa = mod_part(kt * KW, KW)
        ca = mod_part(D + kt * KW, KW)
        cs = _cols(kt * KW, KW)
        hh = xh[0:PRO + 24, cs] * (1.0 + ca) + sa
        hn[...] = _pack(jnp.concatenate([hh[0:PRO], m0v[:, cs].astype(F32), hh[PRO:]], axis=0))

    with _scope("waitw0"):
        wait_block(0, 0, 0)
    with _scope("first"):
        repack_now(0, 0)
        with _scope("waitm0"):
            for c in mod_copies(0):
                c.wait()
        modulate(0)

    def kmajor(kt, c):
        kn = jnp.minimum(kt + 1, KT - 1)

        @pl.when(kt < KT - 1)
        def _():
            for cp in mod_copies(kn):
                cp.wait()

        cs = _cols(kt * KW, KW)
        h0[:, cs] = hn[...]
        rows = pl.ds(pl.multiple_of(kt * (KW // 2), KW // 2), KW // 2)
        for pg in range(2):
            for t in range(HG):
                r = acc[pg * HG + t] + _dot(_unpack(h0[:, cs]), _unpack(wg[pg][0, t, rows, :]))
                acc[pg * HG + t] = r
                store_tokens(ring[pg], 0, t, r)
            if pg == 0:
                modulate(kn)
        return c

    with _scope("kmajor"):
        lax.fori_loop(0, KT, kmajor, 0)

    def pro_body(j, c):
        gi, t0 = j & 3, (j >> 2) * HG
        jn = jnp.minimum(j + 1, NJ - 1)
        gn, tn = jn & 3, (jn >> 2) * HG
        prefetch = (j > 1) & (j < NJ - 1)

        def early_blocks():
            def batch1():
                for jj in range(4, 9):
                    start_block(jj)

            def batch2():
                for jj in range(9, NJ):
                    start_block(jj)
                for n in ("x1", "wo", "wm1", "w1", "w3", "w2", "wm2", "x2"):
                    copies[n].start()

            _rarely(j == 1, batch1)
            _rarely(j == 3, batch2)

            def fix():
                with _scope("waitlate"):
                    wait_block(j, gi, t0)
                repack_now(gi, t0)

            _rarely(j <= 2, fix)

        _rarely(j <= 3, early_blocks)

        @pl.when(prefetch)
        def _():
            wait_block(jn, gn, tn)

        a = _unpack(h0[...])
        for pg in range(2):
            for t in range(HG):
                store_tokens(ring[pg], gi, t0 + t, _dot(a, _unpack(wg[pg][gi, t0 + t])))
        gr, tr = jnp.where(prefetch, gn, gi), jnp.where(prefetch, tn, t0)
        for w in wg:
            for t in range(0, HG, 2):
                repack_slot(w, gr, tr + t, prefetch)
        return c

    with _scope("pro"):
        lax.fori_loop(1, NJ, pro_body, 0)

    def pair(p, with_ffn):
        (al_a, fi_a), (al_b, fi_b) = _masks()
        base = pl.multiple_of(lax.rem(p, NSLOT) * SLOT, 8)
        u0 = PRO // 8 + 6 * p
        tlead = PRO + 48 * p

        if with_ffn:
            finish(pl.multiple_of(jnp.maximum(p - 2, 0) * PT, PT))
            post_attn(pl.multiple_of((p - 1) * PT, PT))

        def filler(i, c0=None, c1=None):
            if not with_ffn:
                if i is not None:
                    mod_part(2 * D + MODF[i] * 256, (MODF[i + 1] - MODF[i]) * 256)
            elif c0 is None:
                ffn_down(0, 4)
            else:
                ffn_up(c0, c1)

        def proj_attn(lhs, rows, q0, nq, nk, allowed, fill, f):
            ps = None
            for g in range(G):
                proj(lhs, g, rows, 0, QKPOS)
                if g > 0 and QKPOS > 0:
                    ps = attn_qk(g - 1, base, q0, nq, nk, allowed, fill)
                proj(lhs, g, rows, QKPOS, PVPOS)
                if g > 0:
                    attn_pv(g - 1, base, nq, nk, ps)
                proj(lhs, g, rows, PVPOS, 3 * HG)
                if QKPOS == 0 or g == G - 1:
                    ps = attn_qk(g, base, q0, nq, nk, allowed, fill)
            filler(f, FILL[f], FILL[f + 1])
            attn_pv(G - 1, base, nq, nk, ps)
            filler(f + 1, FILL[f + 1], FILL[f + 2])

        def st_lhs(ref):
            def fn(cs, val):
                ref[0:MEM, cs] = val.astype(BF16).astype(F32)
            return fn

        def st_a(r0, n):
            def fn(cs, val):
                abuf[r0:r0 + n, cs] = val
            return fn

        lhs_b[MEM:32, :] = ln1(pl.multiple_of(tlead + 24, 8), 24)
        if with_ffn:
            lhs = lhs_a[...].astype(BF16)
            rows = [base, unit_row(u0), unit_row(u0 + 1), unit_row(u0 + 2)]
            proj_attn(lhs, rows, 0, 32, 48, al_a, fi_a, 0)
        else:
            ps = [attn_qk(g, base, 0, 32, 48, al_a, fi_a) for g in range(G)]
            filler(0)
            for g in range(G):
                attn_pv(g, base, 32, 48, ps[g])
            filler(1)
        wo_proj(32, [(0, 8, st_lhs(lhs_b)), (8, 24, st_a(0, 24))])
        filler(2, FILL[2], FILL[3])

        lhs = lhs_b[...].astype(BF16)
        rows = [pl.multiple_of(base + 24, 8), unit_row(u0 + 3), unit_row(u0 + 4), unit_row(u0 + 5)]
        nxt = pl.multiple_of(jnp.minimum(tlead + 48, S - 24), 8)
        lhs_a[MEM:32, :] = ln1(nxt, 24)
        proj_attn(lhs, rows, 32, 48, 80, al_b, fi_b, 3)
        wo_proj(48, [(16, 8, st_lhs(lhs_a)), (0, 16, st_a(24, 16)), (24, 24, st_a(40, 24))])
        filler(None)

    with _scope("waitwo"):
        copies["x1"].wait()
        copies["wo"].wait()
        copies["wm1"].wait()

    with _scope("noffn"):
        yv[...] = jnp.zeros(yv.shape, F32)
        fv[...] = jnp.zeros(fv.shape, F32)
        modv[:, 5 * D:6 * D] = jnp.zeros((8, D), F32)
        pair(jnp.int32(0), False)

    with _scope("waitffn"):
        copies["w1"].wait()
        copies["w3"].wait()
        copies["w2"].wait()

    def late_inputs():
        copies["wm2"].wait()
        copies["x2"].wait()
        mod_part(5 * D, D)

    def pair_ffn(p, c):
        _rarely(p == MAIN_START + 1, late_inputs)

        @pl.when(p > MAIN_START + 1)
        def _():
            out_copy(pl.multiple_of((p - 3) * PT, PT), PT).start()

        pair(p, True)
        return c

    with _scope("main"):
        lax.fori_loop(MAIN_START, NPAIR, pair_ffn, 0)

    with _scope("epi"):
        out_copy((NPAIR - 3) * PT, PT).start()
        finish((NPAIR - 2) * PT)
        post_attn((NPAIR - 1) * PT)
        out_copy((NPAIR - 2) * PT, PT).start()

        ffn_up(0, NFC)
        ffn_down(0, 4, (NPAIR - 1) * PT)
    with _scope("waitout"):
        out_copy(0, S - (MAIN_START - 1) * PT).wait()


@functools.partial(jax.jit, static_argnames=("A_seg_len",))
def pallas_adaLN_cond__memory_aug_recurrent_mem_tr__glu_gated_swiglu__prompt_kernel(
    A_x, A_mem0, A_Wq, A_Wk, A_Wv, A_Wo, A_seg_len, B_x, B_w1, B_w3, B_w2, c, w_mod,
):
    assert A_seg_len == SEG
    assert A_x.shape == (1, S, D) and A_mem0.shape == (1, MEM, D)
    assert A_Wq.shape == (D, H, DH) and B_w1.shape == (D, FF)
    del B_x

    scratch = [
        pltpu.VMEM((S, D), BF16),
        pltpu.VMEM((S, D), BF16),
        pltpu.VMEM((HD // 2, D), U32),
        pltpu.VMEM((D // 2, FF), U32),
        pltpu.VMEM((D // 2, FF), U32),
        pltpu.VMEM((FF // 2, D), U32),
        pltpu.VMEM((D // 2, 6 * D), U32),
        pltpu.VMEM((1, D), BF16),
        pltpu.VMEM((MEM, D), BF16),
        pltpu.VMEM((8, 6 * D), F32),
        pltpu.VMEM((X0, D), F32),
        pltpu.VMEM((PROM // 2, D), U32),
        pltpu.VMEM((PROM // 2, KW), U32),
        pltpu.VMEM((2 * HG, PROM, DH), F32),
        pltpu.VMEM((32, D), F32),
        pltpu.VMEM((32, D), F32),
        pltpu.VMEM((24, HD), U32),
        pltpu.VMEM((PT, D), F32),
        pltpu.VMEM((PT, D), F32),
        pltpu.VMEM((PT, D), F32),
        pltpu.VMEM((PT // 2, D), U32),
        pltpu.VMEM((PT // 2, FF), U32),
        pltpu.SemaphoreType.DMA((11,)),
        pltpu.SemaphoreType.DMA((KT,)),
        pltpu.SemaphoreType.DMA((NJ,)),
        pltpu.SemaphoreType.DMA,
    ] + [pltpu.VMEM((G // 2, 3 * HG, NSLOT * SLOT, DH), U32)] * 2 + [
        pltpu.VMEM((G // 2, 3 * HG, D // 2, DH), U32)] * 2

    out = pl.pallas_call(
        _kernel,
        out_shape=jax.ShapeDtypeStruct((S, D), BF16),
        in_specs=[pl.BlockSpec(memory_space=pl.ANY)] * 11,
        out_specs=pl.BlockSpec(memory_space=pl.ANY),
        scratch_shapes=scratch,
        compiler_params=pltpu.CompilerParams(
            vmem_limit_bytes=120 * 1024 * 1024, disable_bounds_checks=True),
    )(
        A_x.reshape(S, D), A_mem0.reshape(MEM, D),
        A_Wq.reshape(D // 2, 2, H, DH), A_Wk.reshape(D // 2, 2, H, DH),
        A_Wv.reshape(D // 2, 2, H, DH), A_Wo.reshape(HD, D),
        B_w1, B_w3, B_w2, c, w_mod,
    )
    return out.reshape(1, S, D)
```

```python
import functools

import jax
import jax.numpy as jnp
from jax import lax
import jax.experimental.pallas as pl
import jax.experimental.pallas.tpu as pltpu

F32 = jnp.float32
BF16 = jnp.bfloat16
U32 = jnp.uint32

S = 2048
D = 1024
H = 32
DH = 128
HD = H * DH
MEM = 8
SEG = 32
FF = 3584
EPS = 1e-5
LOG2E = 1.4426950408889634

G = 8
HG = H // G
PRO = 512
NPAIR = S // (2 * SEG)
PT = 2 * SEG
SLOT = 40
NSLOT = 9
X0 = 544
X1 = 640
FC = 256
NFC = FF // FC
KW = 128
KT = D // KW
NJ = 3 * G // 2
FILL = (0, 2, 4, 9, 11, 14)
QKPOS = 1
PVPOS = 11
MODF = (0, 5, 6, 8, 11, 12)
PROM = PRO + 32
MAIN_START = 1
SCOPES = False


class _NoScope:
    def __enter__(self):
        return self

    def __exit__(self, *a):
        return False


def _scope(name):
    return jax.named_scope(name) if SCOPES else _NoScope()


def _unpack(x):
    return pltpu.bitcast(x, BF16)


def _pack(x):
    return pltpu.bitcast(x.astype(BF16), U32)


def _dot(a, b):
    return jnp.dot(a, b, preferred_element_type=F32)


def _ln(x):
    m = jnp.mean(x, axis=-1, keepdims=True)
    xc = x - m
    v = jnp.mean(xc * xc, axis=-1, keepdims=True)
    return xc * lax.rsqrt(v + EPS)


def _recip(x):
    r = pl.reciprocal(x, approx=True)
    return r * (2.0 - x * r)


def _silu(x):
    h = 0.5 * x
    return h + h * jnp.tanh(h)


def _cols(off, w):
    if isinstance(off, int):
        return slice(off, off + w)
    return pl.ds(pl.multiple_of(off, w), w)


def _rarely(cond, fn):
    def body(_, c):
        fn()
        return c

    lax.fori_loop(0, cond.astype(jnp.int32), body, 0)


def _slot(pair):
    assert NSLOT == 9
    return pair - NSLOT * ((pair * 57) >> 9)


def _masks():
    def pos(j):
        return jnp.where(j < 40, j, jnp.where(j < 48, j - 32, jnp.where(j < 56, j - 48, j - 40)))

    out = []
    for q0, nq, nk in ((0, 32, 48), (32, 48, 80)):
        qi = lax.broadcasted_iota(jnp.int32, (nq, nk), 0) + q0
        kj = lax.broadcasted_iota(jnp.int32, (nq, nk), 1)
        qp, kp = pos(qi), pos(kj)
        same = ((qi < 40) & (kj < 40)) | ((qi >= 40) & (kj >= 40))
        allowed = same & ((qp < MEM) | (qp >= kp))
        fill = jnp.where(same, jnp.float32(-1e9 * DH ** 0.5), jnp.float32(-jnp.inf))
        out.append((allowed, fill))
    return out


def _kernel(x_hbm, mem0_hbm, wq_hbm, wk_hbm, wv_hbm, wo_hbm, w1_hbm, w3_hbm, w2_hbm,
            c_hbm, wm_hbm, out_hbm,
            xv, outv, wo, w1, w3, w2, wm, cv, m0v, modv, xh, h0, hn, acc,
            lhs_a, lhs_b, o32, abuf, yv, fv, h2, hid, sem_in, sem_m, sem_w, sem_out, *rest):
    ring = rest[0:2]
    wg = rest[2:4]

    def side(g, t):
        return (g % 2) ^ int(t >= 2 * HG)

    scale = DH ** -0.5

    copies = {}

    def mk(name, src, dst):
        copies[name] = pltpu.make_async_copy(src, dst, sem_in.at[len(copies)])

    wm_u = wm_hbm.bitcast(U32)
    mk("c", c_hbm, cv)
    mk("mem0", mem0_hbm, m0v)
    mk("x0", x_hbm.at[0:X0], xv.at[0:X0])
    mk("x1", x_hbm.at[X0:X1], xv.at[X0:X1])
    mk("wo", wo_hbm.bitcast(U32), wo)
    mk("wm1", wm_u.at[:, 2 * D:5 * D], wm.at[:, 2 * D:5 * D])
    mk("w1", w1_hbm.bitcast(U32), w1)
    mk("w3", w3_hbm.bitcast(U32), w3)
    mk("w2", w2_hbm.bitcast(U32), w2)
    mk("wm2", wm_u.at[:, 5 * D:6 * D], wm.at[:, 5 * D:6 * D])
    mk("x2", x_hbm.at[X1:S], xv.at[X1:S])

    def mod_copies(kt):
        return [pltpu.make_async_copy(wm_u.at[:, _cols(i * D + kt * KW, KW)],
                                      wm.at[:, _cols(i * D + kt * KW, KW)], sem_m.at[kt])
                for i in range(2)]

    w_hbm = (wq_hbm, wk_hbm, wv_hbm)

    def block_copies(j, m, gi, t0):
        return [
            pltpu.make_async_copy(
                w_hbm[m].bitcast(U32).at[:, par, (2 * gi + pg) * (HG // 2) + jj],
                wg[side(pg, m * HG)].at[gi, t0 + 2 * jj + par], sem_w.at[j])
            for pg in range(2) for jj in range(HG // 2) for par in range(2)]

    def start_block(j):
        for c in block_copies(j, j // 4, j % 4, (j // 4) * HG):
            c.start()

    def wait_block(j, gi, t0):
        for w in wg:
            buf = w.at[gi, pl.ds(t0, HG)]
            pltpu.make_async_copy(buf, buf, sem_w.at[j]).wait()

    for n in ("x0", "c", "mem0"):
        copies[n].start()

    def zero(i, c):
        acc[i] = jnp.zeros(acc.shape[1:], F32)
        return c

    lax.fori_loop(0, 2 * HG, zero, 0)
    start_block(0)
    for kt in range(KT):
        for c in mod_copies(kt):
            c.start()
    for j in range(1, 4):
        start_block(j)

    def out_copy(r0, n):
        return pltpu.make_async_copy(outv.at[pl.ds(r0, n)], out_hbm.at[pl.ds(r0, n)], sem_out)

    def silu_c():
        return jnp.broadcast_to(_silu(cv[...].astype(F32)), (16, D)).astype(BF16)

    def mod_part(off, w):
        r = _dot(silu_c(), _unpack(wm[:, _cols(off, w)]))[0:8]
        modv[:, _cols(off, w)] = r
        return r[0:1]

    def mvec(i):
        return modv[0:1, i * D:(i + 1) * D]

    def ln1(r0, n):
        xf = xv[pl.ds(r0, n), :].astype(F32)
        return _ln(xf) * (1.0 + mvec(1)) + mvec(0)

    def repack_slot(w, gi, t, enable=None):
        for r0 in range(0, D // 2, 32):
            a = w[gi, t, r0:r0 + 32, :]
            b = w[gi, t + 1, r0:r0 + 32, :]
            e = (a & jnp.uint32(0xFFFF)) | (b << 16)
            o = (a >> 16) | (b & jnp.uint32(0xFFFF0000))
            if enable is not None:
                e = jnp.where(enable, e, a)
                o = jnp.where(enable, o, b)
            w[gi, t, r0:r0 + 32, :] = e
            w[gi, t + 1, r0:r0 + 32, :] = o

    def repack_now(gi, t0):
        def body(i, c):
            for w in wg:
                repack_slot(w, gi, t0 + 2 * i)
            return c

        lax.fori_loop(0, HG // 2, body, 0)

    def store_tokens(dst, gi, t, r):
        for pp in range(PRO // PT):
            b0, r0 = pp * SLOT, pp * PT
            dst[gi, t, b0 + 4:b0 + 8, :] = _pack(r[r0:r0 + 8])
            dst[gi, t, b0 + 8:b0 + 24, :] = _pack(r[r0 + 8:r0 + 40])
            dst[gi, t, b0 + 28:b0 + 32, :] = _pack(r[r0 + 40:r0 + 48])
            dst[gi, t, b0 + 32:b0 + 40, :] = _pack(r[r0 + 48:r0 + 64])
        b0 = (PRO // PT) * SLOT
        dst[gi, t, 0:4, :] = _pack(r[PRO:PRO + 8])
        dst[gi, t, b0 + 4:b0 + 8, :] = _pack(r[PRO + 8:PRO + 16])
        dst[gi, t, b0 + 8:b0 + 16, :] = _pack(r[PRO + 16:PRO + 32])

    def proj(lhs, g, rows, t0, t1):
        for t in range(t0, t1):
            r = _dot(lhs, _unpack(wg[side(g, t)][g // 2, t]))
            for i, row in enumerate(rows):
                ring[side(g, t)][g // 2, t, pl.ds(row, 4), :] = _pack(r[8 * i:8 * i + 8])

    def attn_qk(g, base, q0, nq, nk, allowed, fill):
        qrow = pl.multiple_of(base + q0 // 2, 8)
        ps = []
        for hh in range(HG):
            q = _unpack(ring[g % 2][g // 2, hh, pl.ds(qrow, nq // 2), :])
            k = _unpack(ring[g % 2][g // 2, HG + hh, pl.ds(base, nk // 2), :])
            s = lax.dot_general(q, k, (((1,), (1,)), ((), ())), preferred_element_type=F32)
            s = jnp.where(allowed, s, fill)
            m = jnp.max(s, axis=-1, keepdims=True)
            p = jnp.exp2((s - m) * (scale * LOG2E))
            l = jnp.sum(p, axis=-1, keepdims=True)
            ps.append((p * _recip(l)).astype(BF16))
        return ps

    def attn_pv(g, base, nq, nk, ps):
        for hh in range(HG):
            v = _unpack(ring[1 - g % 2][g // 2, 2 * HG + hh, pl.ds(base, nk // 2), :])
            col = (g * HG + hh) * DH
            o32[0:nq // 2, col:col + DH] = _pack(_dot(ps[hh], v))

    def wo_proj(nq, stores):
        o = _unpack(o32[0:nq // 2, :])
        cw = 256
        for cb in range(D // cw):
            cs = slice(cb * cw, (cb + 1) * cw)
            r = _dot(o, _unpack(wo[:, cs]))
            for r0, n, fn in stores:
                fn(cs, r[r0:r0 + n])

    def post_attn(tok0):
        x1 = xv[pl.ds(tok0, PT), :].astype(F32) + mvec(2) * abuf[...]
        yv[...] = x1
        h2[...] = _pack(_ln(x1) * (1.0 + mvec(4)) + mvec(3))

    def ffn_up(c0, c1):
        a = _unpack(h2[...])
        for c in range(c0, c1):
            cs = slice(c * FC, (c + 1) * FC)
            gt = _dot(a, _unpack(w1[:, cs]))
            up = _dot(a, _unpack(w3[:, cs]))
            hid[:, cs] = _pack(_silu(gt) * up)

    def ffn_down(cb0, cb1, tok0=None):
        a = _unpack(hid[...])
        cw = 256
        for cb in range(cb0, cb1):
            cs = slice(cb * cw, (cb + 1) * cw)
            r = _dot(a, _unpack(w2[:, cs]))
            if tok0 is None:
                fv[:, cs] = r
            else:
                gb = modv[0:1, 5 * D + cb * cw:5 * D + (cb + 1) * cw]
                outv[pl.ds(tok0, PT), cs] = (yv[:, cs] + gb * r).astype(BF16)
                pltpu.make_async_copy(outv.at[pl.ds(tok0, PT), cs],
                                      out_hbm.at[pl.ds(tok0, PT), cs], sem_out).start()

    def finish(tok0):
        outv[pl.ds(tok0, PT), :] = (yv[...] + mvec(5) * fv[...]).astype(BF16)

    def unit_row(u):
        r = u & 7
        slot = _slot(u >> 3)
        return pl.multiple_of(slot * SLOT + 4 + 4 * r + 4 * (r >= 5).astype(jnp.int32), 4)

    with _scope("waitx0"):
        copies["x0"].wait()
    with _scope("ln0"):

        def ln_body(i, c):
            r0 = pl.multiple_of(i * 136, 8)
            xh[pl.ds(r0, 136), :] = _ln(xv[pl.ds(r0, 136), :].astype(F32))
            return c

        lax.fori_loop(0, X0 // 136, ln_body, 0)
    with _scope("waitc"):
        copies["c"].wait()
        copies["mem0"].wait()

    def modulate(kt):
        sa = mod_part(kt * KW, KW)
        ca = mod_part(D + kt * KW, KW)
        cs = _cols(kt * KW, KW)
        hh = xh[0:PRO + 24, cs] * (1.0 + ca) + sa
        hn[...] = _pack(jnp.concatenate([hh[0:PRO], m0v[:, cs].astype(F32), hh[PRO:]], axis=0))

    with _scope("waitw0"):
        wait_block(0, 0, 0)
    with _scope("first"):
        repack_now(0, 0)
        with _scope("waitm0"):
            for c in mod_copies(0):
                c.wait()
        modulate(0)

    def kmajor(kt, c):
        kn = jnp.minimum(kt + 1, KT - 1)

        @pl.when(kt < KT - 1)
        def _():
            for cp in mod_copies(kn):
                cp.wait()

        cs = _cols(kt * KW, KW)
        h0[:, cs] = hn[...]
        rows = pl.ds(pl.multiple_of(kt * (KW // 2), KW // 2), KW // 2)
        for pg in range(2):
            for t in range(HG):
                r = acc[pg * HG + t] + _dot(_unpack(h0[:, cs]), _unpack(wg[pg][0, t, rows, :]))
                acc[pg * HG + t] = r
                store_tokens(ring[pg], 0, t, r)
            if pg == 0:
                modulate(kn)
        return c

    with _scope("kmajor"):
        lax.fori_loop(0, KT, kmajor, 0)

    def pro_body(j, c):
        gi, t0 = j & 3, (j >> 2) * HG
        jn = jnp.minimum(j + 1, NJ - 1)
        gn, tn = jn & 3, (jn >> 2) * HG
        prefetch = (j > 1) & (j < NJ - 1)

        def early_blocks():
            def batch1():
                for jj in range(4, 9):
                    start_block(jj)

            def batch2():
                for jj in range(9, NJ):
                    start_block(jj)
                for n in ("x1", "wo", "wm1", "w1", "w3", "w2", "wm2", "x2"):
                    copies[n].start()

            _rarely(j == 1, batch1)
            _rarely(j == 3, batch2)

            def fix():
                with _scope("waitlate"):
                    wait_block(j, gi, t0)
                repack_now(gi, t0)

            _rarely(j <= 2, fix)

        _rarely(j <= 3, early_blocks)

        @pl.when(prefetch)
        def _():
            wait_block(jn, gn, tn)

        a = _unpack(h0[...])
        for pg in range(2):
            for t in range(HG):
                store_tokens(ring[pg], gi, t0 + t, _dot(a, _unpack(wg[pg][gi, t0 + t])))
        gr, tr = jnp.where(prefetch, gn, gi), jnp.where(prefetch, tn, t0)
        for w in wg:
            for t in range(0, HG, 2):
                repack_slot(w, gr, tr + t, prefetch)
        return c

    with _scope("pro"):
        lax.fori_loop(1, NJ, pro_body, 0)

    def pair(p, with_ffn):
        (al_a, fi_a), (al_b, fi_b) = _masks()
        base = pl.multiple_of(_slot(p) * SLOT, 8)
        u0 = PRO // 8 + 6 * p
        tlead = PRO + 48 * p

        if with_ffn:
            finish(pl.multiple_of(jnp.maximum(p - 2, 0) * PT, PT))
            post_attn(pl.multiple_of((p - 1) * PT, PT))

        def filler(i, c0=None, c1=None):
            if not with_ffn:
                if i is not None:
                    mod_part(2 * D + MODF[i] * 256, (MODF[i + 1] - MODF[i]) * 256)
            elif c0 is None:
                ffn_down(0, 4)
            else:
                ffn_up(c0, c1)

        def proj_attn(lhs, rows, q0, nq, nk, allowed, fill, f):
            ps = None
            for g in range(G):
                proj(lhs, g, rows, 0, QKPOS)
                if g > 0 and QKPOS > 0:
                    ps = attn_qk(g - 1, base, q0, nq, nk, allowed, fill)
                proj(lhs, g, rows, QKPOS, PVPOS)
                if g > 0:
                    attn_pv(g - 1, base, nq, nk, ps)
                proj(lhs, g, rows, PVPOS, 3 * HG)
                if QKPOS == 0 or g == G - 1:
                    ps = attn_qk(g, base, q0, nq, nk, allowed, fill)
            filler(f, FILL[f], FILL[f + 1])
            attn_pv(G - 1, base, nq, nk, ps)
            filler(f + 1, FILL[f + 1], FILL[f + 2])

        def st_lhs(ref):
            def fn(cs, val):
                ref[0:MEM, cs] = val.astype(BF16).astype(F32)
            return fn

        def st_a(r0, n):
            def fn(cs, val):
                abuf[r0:r0 + n, cs] = val
            return fn

        lhs_b[MEM:32, :] = ln1(pl.multiple_of(tlead + 24, 8), 24)
        if with_ffn:
            lhs = lhs_a[...].astype(BF16)
            rows = [base, unit_row(u0), unit_row(u0 + 1), unit_row(u0 + 2)]
            proj_attn(lhs, rows, 0, 32, 48, al_a, fi_a, 0)
        else:
            ps = [attn_qk(g, base, 0, 32, 48, al_a, fi_a) for g in range(G)]
            filler(0)
            for g in range(G):
                attn_pv(g, base, 32, 48, ps[g])
            filler(1)
        wo_proj(32, [(0, 8, st_lhs(lhs_b)), (8, 24, st_a(0, 24))])
        filler(2, FILL[2], FILL[3])

        lhs = lhs_b[...].astype(BF16)
        rows = [pl.multiple_of(base + 24, 8), unit_row(u0 + 3), unit_row(u0 + 4), unit_row(u0 + 5)]
        nxt = pl.multiple_of(jnp.minimum(tlead + 48, S - 24), 8)
        lhs_a[MEM:32, :] = ln1(nxt, 24)
        proj_attn(lhs, rows, 32, 48, 80, al_b, fi_b, 3)
        wo_proj(48, [(16, 8, st_lhs(lhs_a)), (0, 16, st_a(24, 16)), (24, 24, st_a(40, 24))])
        filler(None)

    with _scope("waitwo"):
        copies["x1"].wait()
        copies["wo"].wait()
        copies["wm1"].wait()

    with _scope("noffn"):
        yv[...] = jnp.zeros(yv.shape, F32)
        fv[...] = jnp.zeros(fv.shape, F32)
        modv[:, 5 * D:6 * D] = jnp.zeros((8, D), F32)
        pair(jnp.int32(0), False)

    with _scope("waitffn"):
        copies["w1"].wait()
        copies["w3"].wait()
        copies["w2"].wait()

    def late_inputs():
        copies["wm2"].wait()
        copies["x2"].wait()
        mod_part(5 * D, D)

    def pair_ffn(p, c):
        pair(p, True)
        return c

    def main(o, c):
        _rarely(o == 1, late_inputs)
        lax.fori_loop(MAIN_START + o, MAIN_START + 1 + o * (NPAIR - MAIN_START - 1), pair_ffn, 0)
        return c

    with _scope("main"):
        lax.fori_loop(0, 2, main, 0)

    with _scope("epi"):
        out_copy(0, (NPAIR - 2) * PT).start()
        finish((NPAIR - 2) * PT)
        post_attn((NPAIR - 1) * PT)
        out_copy((NPAIR - 2) * PT, PT).start()

        ffn_up(0, NFC)
        ffn_down(0, 4, (NPAIR - 1) * PT)
    with _scope("waitout"):
        out_copy(0, S - (MAIN_START - 1) * PT).wait()


@functools.partial(jax.jit, static_argnames=("A_seg_len",))
def pallas_adaLN_cond__memory_aug_recurrent_mem_tr__glu_gated_swiglu__prompt_kernel(
    A_x, A_mem0, A_Wq, A_Wk, A_Wv, A_Wo, A_seg_len, B_x, B_w1, B_w3, B_w2, c, w_mod,
):
    assert A_seg_len == SEG
    assert A_x.shape == (1, S, D) and A_mem0.shape == (1, MEM, D)
    assert A_Wq.shape == (D, H, DH) and B_w1.shape == (D, FF)
    del B_x

    scratch = [
        pltpu.VMEM((S, D), BF16),
        pltpu.VMEM((S, D), BF16),
        pltpu.VMEM((HD // 2, D), U32),
        pltpu.VMEM((D // 2, FF), U32),
        pltpu.VMEM((D // 2, FF), U32),
        pltpu.VMEM((FF // 2, D), U32),
        pltpu.VMEM((D // 2, 6 * D), U32),
        pltpu.VMEM((1, D), BF16),
        pltpu.VMEM((MEM, D), BF16),
        pltpu.VMEM((8, 6 * D), F32),
        pltpu.VMEM((X0, D), F32),
        pltpu.VMEM((PROM // 2, D), U32),
        pltpu.VMEM((PROM // 2, KW), U32),
        pltpu.VMEM((2 * HG, PROM, DH), F32),
        pltpu.VMEM((32, D), F32),
        pltpu.VMEM((32, D), F32),
        pltpu.VMEM((24, HD), U32),
        pltpu.VMEM((PT, D), F32),
        pltpu.VMEM((PT, D), F32),
        pltpu.VMEM((PT, D), F32),
        pltpu.VMEM((PT // 2, D), U32),
        pltpu.VMEM((PT // 2, FF), U32),
        pltpu.SemaphoreType.DMA((11,)),
        pltpu.SemaphoreType.DMA((KT,)),
        pltpu.SemaphoreType.DMA((NJ,)),
        pltpu.SemaphoreType.DMA,
    ] + [pltpu.VMEM((G // 2, 3 * HG, NSLOT * SLOT, DH), U32)] * 2 + [
        pltpu.VMEM((G // 2, 3 * HG, D // 2, DH), U32)] * 2

    out = pl.pallas_call(
        _kernel,
        out_shape=jax.ShapeDtypeStruct((S, D), BF16),
        in_specs=[pl.BlockSpec(memory_space=pl.ANY)] * 11,
        out_specs=pl.BlockSpec(memory_space=pl.ANY),
        scratch_shapes=scratch,
        compiler_params=pltpu.CompilerParams(
            vmem_limit_bytes=120 * 1024 * 1024, disable_bounds_checks=True),
    )(
        A_x.reshape(S, D), A_mem0.reshape(MEM, D),
        A_Wq.reshape(D // 2, 2, H, DH), A_Wk.reshape(D // 2, 2, H, DH),
        A_Wv.reshape(D // 2, 2, H, DH), A_Wo.reshape(HD, D),
        B_w1, B_w3, B_w2, c, w_mod,
    )
    return out.reshape(1, S, D)
```

```python
import functools

import jax
import jax.numpy as jnp
from jax import lax
import jax.experimental.pallas as pl
import jax.experimental.pallas.tpu as pltpu

F32 = jnp.float32
BF16 = jnp.bfloat16
U32 = jnp.uint32

S = 2048
D = 1024
H = 32
DH = 128
HD = H * DH
MEM = 8
SEG = 32
FF = 3584
EPS = 1e-5
LOG2E = 1.4426950408889634

G = 8
HG = H // G
PRO = 512
NPAIR = S // (2 * SEG)
PT = 2 * SEG
SLOT = 40
NSLOT = 9
X0 = 544
X1 = 640
FC = 256
NFC = FF // FC
KW = 128
KT = D // KW
NB0 = 2
SETW = 128
NSET = D // 2 // SETW
NWS = G // 2 * 3 * HG
NJ = 3 * G // 2
FILL = (0, 2, 4, 9, 11, 14)
WOCW = 256
DNCW = 256
QKPOS = 1
PVPOS = 11
MODF = (0, 5, 6, 8, 11, 12)
PROM = PRO + 32
MAIN_START = 1
EPI_UP = 4
LNR = 136
SCOPES = False


class _NoScope:
    def __enter__(self):
        return self

    def __exit__(self, *a):
        return False


def _scope(name):
    return jax.named_scope(name) if SCOPES else _NoScope()


def _unpack(x):
    return pltpu.bitcast(x, BF16)


def _pack(x):
    return pltpu.bitcast(x.astype(BF16), U32)


def _dot(a, b):
    return jnp.dot(a, b, preferred_element_type=F32)


def _ln(x):
    m = jnp.mean(x, axis=-1, keepdims=True)
    xc = x - m
    v = jnp.mean(xc * xc, axis=-1, keepdims=True)
    return xc * lax.rsqrt(v + EPS)


def _recip(x):
    r = pl.reciprocal(x, approx=True)
    return r * (2.0 - x * r)


def _silu(x):
    h = 0.5 * x
    return h + h * jnp.tanh(h)


def _cols(off, w):
    if isinstance(off, int):
        return slice(off, off + w)
    return pl.ds(pl.multiple_of(off, w), w)


def _rarely(cond, fn):
    def body(_, c):
        fn()
        return c

    lax.fori_loop(0, cond.astype(jnp.int32), body, 0)


def _slot(pair):
    assert NSLOT == 9
    return pair - NSLOT * ((pair * 57) >> 9)


def _masks():
    def pos(j):
        return jnp.where(j < 40, j, jnp.where(j < 48, j - 32, jnp.where(j < 56, j - 48, j - 40)))

    out = []
    for q0, nq, nk in ((0, 32, 48), (32, 48, 80)):
        qi = lax.broadcasted_iota(jnp.int32, (nq, nk), 0) + q0
        kj = lax.broadcasted_iota(jnp.int32, (nq, nk), 1)
        qp, kp = pos(qi), pos(kj)
        same = ((qi < 40) & (kj < 40)) | ((qi >= 40) & (kj >= 40))
        allowed = same & ((qp < MEM) | (qp >= kp))
        fill = jnp.where(same, jnp.float32(-1e9 * DH ** 0.5), jnp.float32(-jnp.inf))
        out.append((allowed, fill))
    return out


def _kernel(x_hbm, mem0_hbm, wq_hbm, wk_hbm, wv_hbm, wo_hbm, w1_hbm, w3_hbm, w2_hbm,
            c_hbm, wm_hbm, out_hbm,
            xv, outv, wo, w1, w3, w2, wm, cv, m0v, modv, xh, h0, hn, acc,
            lhs_a, lhs_b, o32, abuf, yv, fv, h2, hid, sem_in, sem_m, sem_s, sem_w, sem_out, *rest):
    ring = rest[0:2]
    wg = rest[2:4]

    def side(g, t):
        return (g % 2) ^ int(t >= 2 * HG)

    scale = DH ** -0.5

    copies = {}

    def mk(name, src, dst):
        copies[name] = pltpu.make_async_copy(src, dst, sem_in.at[len(copies)])

    wm_u = wm_hbm.bitcast(U32)
    mk("c", c_hbm, cv)
    mk("mem0", mem0_hbm, m0v)
    mk("x0", x_hbm.at[0:X0], xv.at[0:X0])
    mk("x1", x_hbm.at[X0:X1], xv.at[X0:X1])
    mk("wo", wo_hbm.bitcast(U32), wo)
    mk("wm1", wm_u.at[:, 2 * D:5 * D], wm.at[:, 2 * D:5 * D])
    mk("w1", w1_hbm.bitcast(U32), w1)
    mk("w3", w3_hbm.bitcast(U32), w3)
    mk("w2", w2_hbm.bitcast(U32), w2)
    mk("wm2", wm_u.at[:, 5 * D:6 * D], wm.at[:, 5 * D:6 * D])
    mk("x2", x_hbm.at[X1:S], xv.at[X1:S])

    def mod_copies(kt):
        return [pltpu.make_async_copy(wm_u.at[:, _cols(i * D + kt * KW, KW)],
                                      wm.at[:, _cols(i * D + kt * KW, KW)], sem_m.at[kt])
                for i in range(2)]

    w_hbm = (wq_hbm, wk_hbm, wv_hbm)

    def start_block(j, rows=slice(None), sem=None):
        m, gi = j // 4, j % 4
        for pg in range(2):
            for jj in range(HG // 2):
                for par in range(2):
                    pltpu.make_async_copy(
                        w_hbm[m].bitcast(U32).at[rows, par, (2 * gi + pg) * (HG // 2) + jj],
                        wg[side(pg, m * HG)].at[gi * 3 * HG + m * HG + 2 * jj + par, rows],
                        sem_w.at[j] if sem is None else sem).start()

    def wait_block(j, s0):
        for w in wg:
            buf = w.at[pl.ds(s0, HG)]
            pltpu.make_async_copy(buf, buf, sem_w.at[j]).wait()

    def start_set(i):
        for j in range(NB0):
            start_block(j, slice(i * SETW, (i + 1) * SETW), sem_s.at[i])

    def wait_set(i):
        for w in wg:
            for gi in range(NB0):
                buf = w.at[gi * 3 * HG:gi * 3 * HG + HG, pl.ds(pl.multiple_of(i * SETW, SETW), SETW)]
                pltpu.make_async_copy(buf, buf, sem_s.at[i]).wait()

    def start_mod(kts):
        for kt in kts:
            for c in mod_copies(kt):
                c.start()

    for n in ("x0", "c", "mem0"):
        copies[n].start()

    def zero(i, c):
        acc[i] = jnp.zeros(acc.shape[1:], F32)
        rows = pl.ds(pl.multiple_of(i * 32, 32), 32)
        for w in wg:
            w[NWS:NWS + HG, rows, :] = jnp.zeros((HG, 32, DH), U32)
        return c

    lax.fori_loop(0, NB0 * 2 * HG, zero, 0)
    start_set(0)
    start_mod((0, 1, 2))
    start_set(1)
    start_mod((3, 4))
    start_set(2)
    start_mod((5,))

    def out_copy(r0, n):
        return pltpu.make_async_copy(outv.at[pl.ds(r0, n)], out_hbm.at[pl.ds(r0, n)], sem_out)

    def silu_c():
        return jnp.broadcast_to(_silu(cv[...].astype(F32)), (16, D)).astype(BF16)

    def mod_part(off, w):
        r = _dot(silu_c(), _unpack(wm[:, _cols(off, w)]))[0:8]
        modv[:, _cols(off, w)] = r
        return r[0:1]

    def mvec(i):
        return modv[0:1, i * D:(i + 1) * D]

    def ln1(r0, n):
        xf = xv[pl.ds(r0, n), :].astype(F32)
        return _ln(xf) * (1.0 + mvec(1)) + mvec(0)

    def repack_rows(w, sl, r0):
        rows = slice(r0, r0 + 32) if isinstance(r0, int) else pl.ds(r0, 32)
        a = w[sl, rows, :]
        b = w[sl + 1, rows, :]
        w[sl, rows, :] = (a & jnp.uint32(0xFFFF)) | (b << 16)
        w[sl + 1, rows, :] = (a >> 16) | (b & jnp.uint32(0xFFFF0000))

    def repack_now(s0):
        def body(i, c):
            for w in wg:
                for r in range(0, D // 4, 32):
                    r0 = pl.multiple_of((i & 1) * (D // 4) + r, 32)
                    repack_rows(w, s0 + 2 * (i >> 1), r0)
            return c

        lax.fori_loop(0, HG, body, 0)

    def repack_tile(w, kt, slots):
        for s0 in slots:
            for t in range(0, HG, 2):
                for r in range(0, KW // 2, 32):
                    r0 = kt * (KW // 2) + r
                    repack_rows(w, s0 + t, r0 if isinstance(r0, int) else pl.multiple_of(r0, 32))

    def store_tokens(dst, gi, t, r):
        for pp in range(PRO // PT):
            b0, r0 = pp * SLOT, pp * PT
            dst[gi, t, b0 + 4:b0 + 8, :] = _pack(r[r0:r0 + 8])
            dst[gi, t, b0 + 8:b0 + 24, :] = _pack(r[r0 + 8:r0 + 40])
            dst[gi, t, b0 + 28:b0 + 32, :] = _pack(r[r0 + 40:r0 + 48])
            dst[gi, t, b0 + 32:b0 + 40, :] = _pack(r[r0 + 48:r0 + 64])
        b0 = (PRO // PT) * SLOT
        dst[gi, t, 0:4, :] = _pack(r[PRO:PRO + 8])
        dst[gi, t, b0 + 4:b0 + 8, :] = _pack(r[PRO + 8:PRO + 16])
        dst[gi, t, b0 + 8:b0 + 16, :] = _pack(r[PRO + 16:PRO + 32])

    def proj(lhs, g, rows, t0, t1):
        for t in range(t0, t1):
            r = _dot(lhs, _unpack(wg[side(g, t)][g // 2 * 3 * HG + t]))
            for i, row in enumerate(rows):
                ring[side(g, t)][g // 2, t, pl.ds(row, 4), :] = _pack(r[8 * i:8 * i + 8])

    def attn_qk(g, base, q0, nq, nk, allowed, fill):
        qrow = pl.multiple_of(base + q0 // 2, 8)
        ps = []
        for hh in range(HG):
            q = _unpack(ring[g % 2][g // 2, hh, pl.ds(qrow, nq // 2), :])
            k = _unpack(ring[g % 2][g // 2, HG + hh, pl.ds(base, nk // 2), :])
            s = lax.dot_general(q, k, (((1,), (1,)), ((), ())), preferred_element_type=F32)
            s = jnp.where(allowed, s, fill)
            m = jnp.max(s, axis=-1, keepdims=True)
            p = jnp.exp2((s - m) * (scale * LOG2E))
            l = jnp.sum(p, axis=-1, keepdims=True)
            ps.append((p * _recip(l)).astype(BF16))
        return ps

    def attn_pv(g, base, nq, nk, ps):
        for hh in range(HG):
            v = _unpack(ring[1 - g % 2][g // 2, 2 * HG + hh, pl.ds(base, nk // 2), :])
            col = (g * HG + hh) * DH
            o32[0:nq // 2, col:col + DH] = _pack(_dot(ps[hh], v))

    def wo_proj(nq, stores):
        o = _unpack(o32[0:nq // 2, :])
        cw = WOCW
        for cb in range(D // cw):
            cs = slice(cb * cw, (cb + 1) * cw)
            r = _dot(o, _unpack(wo[:, cs]))
            for r0, n, fn in stores:
                fn(cs, r[r0:r0 + n])

    def post_attn(tok0):
        x1 = xv[pl.ds(tok0, PT), :].astype(F32) + mvec(2) * abuf[...]
        yv[...] = x1
        h2[...] = _pack(_ln(x1) * (1.0 + mvec(4)) + mvec(3))

    def ffn_up(c0, c1, off=0):
        a = _unpack(h2[...])
        for c in range(c0, c1):
            cs = _cols(off + c * FC, FC)
            gt = _dot(a, _unpack(w1[:, cs]))
            up = _dot(a, _unpack(w3[:, cs]))
            hid[:, cs] = _pack(_silu(gt) * up)

    def ffn_down(tok0=None):
        a = _unpack(hid[...])
        cw = DNCW
        for cb in range(D // cw):
            cs = slice(cb * cw, (cb + 1) * cw)
            r = _dot(a, _unpack(w2[:, cs]))
            if tok0 is None:
                fv[:, cs] = r
            else:
                gb = modv[0:1, 5 * D + cb * cw:5 * D + (cb + 1) * cw]
                outv[pl.ds(tok0, PT), cs] = (yv[:, cs] + gb * r).astype(BF16)
                pltpu.make_async_copy(outv.at[pl.ds(tok0, PT), cs],
                                      out_hbm.at[pl.ds(tok0, PT), cs], sem_out).start()

    def finish(tok0):
        outv[pl.ds(tok0, PT), :] = (yv[...] + mvec(5) * fv[...]).astype(BF16)

    def unit_row(u):
        r = u & 7
        slot = _slot(u >> 3)
        return pl.multiple_of(slot * SLOT + 4 + 4 * r + 4 * (r >= 5).astype(jnp.int32), 4)

    with _scope("waitx0"):
        copies["x0"].wait()
    with _scope("ln0"):

        def ln_body(i, c):
            r0 = pl.multiple_of(i * LNR, 8)
            xh[pl.ds(r0, LNR), :] = _ln(xv[pl.ds(r0, LNR), :].astype(F32))
            return c

        lax.fori_loop(0, X0 // LNR, ln_body, 0)
    with _scope("waitc"):
        copies["c"].wait()
        copies["mem0"].wait()

    def modulate(kt):
        sa = mod_part(kt * KW, KW)
        ca = mod_part(D + kt * KW, KW)
        cs = _cols(kt * KW, KW)
        hh = xh[0:PRO + 24, cs] * (1.0 + ca) + sa
        hn[...] = _pack(jnp.concatenate([hh[0:PRO], m0v[:, cs].astype(F32), hh[PRO:]], axis=0))

    with _scope("waitw0"):
        wait_set(0)
    with _scope("first"):
        for w in wg:
            repack_tile(w, 0, [gi * 3 * HG for gi in range(NB0)])
        with _scope("waitm0"):
            for c in mod_copies(0):
                c.wait()
        modulate(0)

    def kmajor(kt, c):
        more = kt < KT - 1
        kn = jnp.minimum(kt + 1, KT - 1)

        def later_copies():
            start_set(3)
            start_mod((6, 7))
            for j in range(NB0, NB0 + 3):
                start_block(j)

        _rarely(kt == 1, later_copies)

        @pl.when(more)
        def _():
            for cp in mod_copies(kn):
                cp.wait()

        @pl.when(more & ((kn & 1) == 0))
        def _():
            wait_set(kn >> 1)

        cs = _cols(kt * KW, KW)
        h0[:, cs] = hn[...]
        rows = pl.ds(pl.multiple_of(kt * (KW // 2), KW // 2), KW // 2)
        for pg in range(2):
            for gi in range(NB0):
                for t in range(HG):
                    i = (pg * NB0 + gi) * HG + t
                    r = acc[i] + _dot(_unpack(h0[:, cs]), _unpack(wg[pg][gi * 3 * HG + t, rows, :]))
                    acc[i] = r
                    store_tokens(ring[pg], gi, t, r)
                if pg == 0 and gi == 0:
                    modulate(kn)
        slots = [jnp.where(more, gi * 3 * HG, NWS) for gi in range(NB0)]
        for w in wg:
            repack_tile(w, kn, slots)
        return c

    with _scope("kmajor"):
        lax.fori_loop(0, KT, kmajor, 0)

    def pro_body(j, c):
        gi, t0 = j & 3, (j >> 2) * HG
        s0 = gi * (3 * HG) + t0
        jn = j + 1
        prefetch = jn < NJ
        sn = jnp.where(prefetch, (jn & 3) * (3 * HG) + (jn >> 2) * HG, NWS)

        def first_blocks():
            def batch1():
                for jj in range(NB0 + 3, NJ - 2):
                    start_block(jj)
                with _scope("waitlate"):
                    wait_block(j, s0)
                repack_now(s0)

            def batch2():
                for jj in range(NJ - 2, NJ):
                    start_block(jj)
                for n in ("x1", "wo", "wm1", "w1", "w3", "w2", "wm2", "x2"):
                    copies[n].start()

            _rarely(j == NB0, batch1)
            _rarely(j == NB0 + 1, batch2)

        _rarely(j <= NB0 + 1, first_blocks)

        @pl.when(prefetch)
        def _():
            wait_block(jn, sn)

        a = _unpack(h0[...])
        for pg in range(2):
            for t in range(HG):
                store_tokens(ring[pg], gi, t0 + t, _dot(a, _unpack(wg[pg][s0 + t])))
        for w in wg:
            for t in range(0, HG, 2):
                for r0 in range(0, D // 2, 32):
                    repack_rows(w, sn + t, r0)
        return c

    with _scope("pro"):
        lax.fori_loop(NB0, NJ, pro_body, 0)

    def pair(p, with_ffn):
        (al_a, fi_a), (al_b, fi_b) = _masks()
        base = pl.multiple_of(_slot(p) * SLOT, 8)
        u0 = PRO // 8 + 6 * p
        tlead = PRO + 48 * p

        if with_ffn:
            finish(pl.multiple_of(jnp.maximum(p - 2, 0) * PT, PT))
            post_attn(pl.multiple_of((p - 1) * PT, PT))

        def filler(i, c0=None, c1=None):
            if not with_ffn:
                if i is not None:
                    mod_part(2 * D + MODF[i] * 256, (MODF[i + 1] - MODF[i]) * 256)
            elif c0 is None:
                ffn_down()
            else:
                ffn_up(c0, c1)

        def proj_attn(lhs, rows, q0, nq, nk, allowed, fill, f):
            ps = None
            for g in range(G):
                proj(lhs, g, rows, 0, QKPOS)
                if g > 0 and QKPOS > 0:
                    ps = attn_qk(g - 1, base, q0, nq, nk, allowed, fill)
                proj(lhs, g, rows, QKPOS, PVPOS)
                if g > 0:
                    attn_pv(g - 1, base, nq, nk, ps)
                proj(lhs, g, rows, PVPOS, 3 * HG)
                if QKPOS == 0 or g == G - 1:
                    ps = attn_qk(g, base, q0, nq, nk, allowed, fill)
            filler(f, FILL[f], FILL[f + 1])
            attn_pv(G - 1, base, nq, nk, ps)
            filler(f + 1, FILL[f + 1], FILL[f + 2])

        def st_lhs(ref):
            def fn(cs, val):
                ref[0:MEM, cs] = val.astype(BF16).astype(F32)
            return fn

        def st_a(r0, n):
            def fn(cs, val):
                abuf[r0:r0 + n, cs] = val
            return fn

        lhs_b[MEM:32, :] = ln1(pl.multiple_of(tlead + 24, 8), 24)
        if with_ffn:
            lhs = lhs_a[...].astype(BF16)
            rows = [base, unit_row(u0), unit_row(u0 + 1), unit_row(u0 + 2)]
            proj_attn(lhs, rows, 0, 32, 48, al_a, fi_a, 0)
        else:
            ps = [attn_qk(g, base, 0, 32, 48, al_a, fi_a) for g in range(G)]
            filler(0)
            for g in range(G):
                attn_pv(g, base, 32, 48, ps[g])
            filler(1)
        wo_proj(32, [(0, 8, st_lhs(lhs_b)), (8, 24, st_a(0, 24))])
        filler(2, FILL[2], FILL[3])

        lhs = lhs_b[...].astype(BF16)
        rows = [pl.multiple_of(base + 24, 8), unit_row(u0 + 3), unit_row(u0 + 4), unit_row(u0 + 5)]
        nxt = pl.multiple_of(jnp.minimum(tlead + 48, S - 24), 8)
        lhs_a[MEM:32, :] = ln1(nxt, 24)
        proj_attn(lhs, rows, 32, 48, 80, al_b, fi_b, 3)
        wo_proj(48, [(16, 8, st_lhs(lhs_a)), (0, 16, st_a(24, 16)), (24, 24, st_a(40, 24))])
        filler(None)

    with _scope("waitwo"):
        copies["x1"].wait()
        copies["wo"].wait()
        copies["wm1"].wait()

    with _scope("noffn"):
        yv[...] = jnp.zeros(yv.shape, F32)
        fv[...] = jnp.zeros(fv.shape, F32)
        modv[:, 5 * D:6 * D] = jnp.zeros((8, D), F32)
        pair(jnp.int32(0), False)

    with _scope("waitffn"):
        copies["w1"].wait()
        copies["w3"].wait()
        copies["w2"].wait()

    def late_inputs():
        copies["wm2"].wait()
        copies["x2"].wait()
        mod_part(5 * D, D)

    def pair_ffn(p, c):
        pair(p, True)
        return c

    def main(o, c):
        _rarely(o == 1, late_inputs)
        lax.fori_loop(MAIN_START + o, MAIN_START + 1 + o * (NPAIR - MAIN_START - 1), pair_ffn, 0)
        return c

    with _scope("main"):
        lax.fori_loop(0, 2, main, 0)

    with _scope("epi"):
        out_copy(0, (NPAIR - 2) * PT).start()
        finish((NPAIR - 2) * PT)
        post_attn((NPAIR - 1) * PT)
        out_copy((NPAIR - 2) * PT, PT).start()


        def up_body(i, c):
            ffn_up(0, EPI_UP, i * (EPI_UP * FC))
            return c

        lax.fori_loop(0, 2, up_body, 0)
        ffn_up(2 * EPI_UP, NFC)
        ffn_down((NPAIR - 1) * PT)
    with _scope("waitout"):
        out_copy(0, S - (MAIN_START - 1) * PT).wait()


@functools.partial(jax.jit, static_argnames=("A_seg_len",))
def pallas_adaLN_cond__memory_aug_recurrent_mem_tr__glu_gated_swiglu__prompt_kernel(
    A_x, A_mem0, A_Wq, A_Wk, A_Wv, A_Wo, A_seg_len, B_x, B_w1, B_w3, B_w2, c, w_mod,
):
    assert A_seg_len == SEG
    assert A_x.shape == (1, S, D) and A_mem0.shape == (1, MEM, D)
    assert A_Wq.shape == (D, H, DH) and B_w1.shape == (D, FF)
    del B_x

    scratch = [
        pltpu.VMEM((S, D), BF16),
        pltpu.VMEM((S, D), BF16),
        pltpu.VMEM((HD // 2, D), U32),
        pltpu.VMEM((D // 2, FF), U32),
        pltpu.VMEM((D // 2, FF), U32),
        pltpu.VMEM((FF // 2, D), U32),
        pltpu.VMEM((D // 2, 6 * D), U32),
        pltpu.VMEM((1, D), BF16),
        pltpu.VMEM((MEM, D), BF16),
        pltpu.VMEM((8, 6 * D), F32),
        pltpu.VMEM((X0, D), F32),
        pltpu.VMEM((PROM // 2, D), U32),
        pltpu.VMEM((PROM // 2, KW), U32),
        pltpu.VMEM((NB0 * 2 * HG, PROM, DH), F32),
        pltpu.VMEM((32, D), F32),
        pltpu.VMEM((32, D), F32),
        pltpu.VMEM((24, HD), U32),
        pltpu.VMEM((PT, D), F32),
        pltpu.VMEM((PT, D), F32),
        pltpu.VMEM((PT, D), F32),
        pltpu.VMEM((PT // 2, D), U32),
        pltpu.VMEM((PT // 2, FF), U32),
        pltpu.SemaphoreType.DMA((11,)),
        pltpu.SemaphoreType.DMA((KT,)),
        pltpu.SemaphoreType.DMA((NSET,)),
        pltpu.SemaphoreType.DMA((NJ,)),
        pltpu.SemaphoreType.DMA,
    ] + [pltpu.VMEM((G // 2, 3 * HG, NSLOT * SLOT, DH), U32)] * 2 + [
        pltpu.VMEM((NWS + HG, D // 2, DH), U32)] * 2

    out = pl.pallas_call(
        _kernel,
        out_shape=jax.ShapeDtypeStruct((S, D), BF16),
        in_specs=[pl.BlockSpec(memory_space=pl.ANY)] * 11,
        out_specs=pl.BlockSpec(memory_space=pl.ANY),
        scratch_shapes=scratch,
        compiler_params=pltpu.CompilerParams(
            vmem_limit_bytes=120 * 1024 * 1024, disable_bounds_checks=True),
    )(
        A_x.reshape(S, D), A_mem0.reshape(MEM, D),
        A_Wq.reshape(D // 2, 2, H, DH), A_Wk.reshape(D // 2, 2, H, DH),
        A_Wv.reshape(D // 2, 2, H, DH), A_Wo.reshape(HD, D),
        B_w1, B_w3, B_w2, c, w_mod,
    )
    return out.reshape(1, S, D)
```

```python
import functools

import jax
import jax.numpy as jnp
from jax import lax
import jax.experimental.pallas as pl
import jax.experimental.pallas.tpu as pltpu

F32 = jnp.float32
BF16 = jnp.bfloat16
U32 = jnp.uint32

S = 2048
D = 1024
H = 32
DH = 128
HD = H * DH
MEM = 8
SEG = 32
FF = 3584
EPS = 1e-5
LOG2E = 1.4426950408889634

G = 8
HG = H // G
PRO = 512
NPAIR = S // (2 * SEG)
PT = 2 * SEG
SLOT = 40
NSLOT = 9
X0 = 544
X1 = 640
FC = 256
NFC = FF // FC
KW = 128
KT = D // KW
NB0 = 2
SETW = 128
NSET = D // 2 // SETW
NWS = G // 2 * 3 * HG
NJ = 3 * G // 2
FILL = (2, 4, 6, 10, 12, 14)
WOCW = 256
DNCW = 256
QKPOS = 2
PVPOS = 11
MODF = (0, 5, 6, 8, 11, 12)
PROM = PRO + 32
MAIN_START = 1
EPI_UP = 4
LNR = 136
SCOPES = False


class _NoScope:
    def __enter__(self):
        return self

    def __exit__(self, *a):
        return False


def _scope(name):
    return jax.named_scope(name) if SCOPES else _NoScope()


def _unpack(x):
    return pltpu.bitcast(x, BF16)


def _pack(x):
    return pltpu.bitcast(x.astype(BF16), U32)


def _dot(a, b):
    return jnp.dot(a, b, preferred_element_type=F32)


def _ln(x):
    m = jnp.mean(x, axis=-1, keepdims=True)
    xc = x - m
    v = jnp.mean(xc * xc, axis=-1, keepdims=True)
    return xc * lax.rsqrt(v + EPS)


def _recip(x):
    r = pl.reciprocal(x, approx=True)
    return r * (2.0 - x * r)


def _silu(x):
    h = 0.5 * x
    return h + h * jnp.tanh(h)


def _cols(off, w):
    if isinstance(off, int):
        return slice(off, off + w)
    return pl.ds(pl.multiple_of(off, w), w)


def _rarely(cond, fn):
    def body(_, c):
        fn()
        return c

    lax.fori_loop(0, cond.astype(jnp.int32), body, 0)


def _slot(pair):
    assert NSLOT == 9
    return pair - NSLOT * ((pair * 57) >> 9)


def _masks():
    def pos(j):
        return jnp.where(j < 40, j, jnp.where(j < 48, j - 32, jnp.where(j < 56, j - 48, j - 40)))

    out = []
    for q0, nq, nk in ((0, 32, 48), (32, 48, 80)):
        qi = lax.broadcasted_iota(jnp.int32, (nq, nk), 0) + q0
        kj = lax.broadcasted_iota(jnp.int32, (nq, nk), 1)
        qp, kp = pos(qi), pos(kj)
        same = ((qi < 40) & (kj < 40)) | ((qi >= 40) & (kj >= 40))
        allowed = same & ((qp < MEM) | (qp >= kp))
        fill = jnp.where(same, jnp.float32(-1e9 * DH ** 0.5), jnp.float32(-jnp.inf))
        out.append((allowed, fill))
    return out


def _kernel(x_hbm, mem0_hbm, wq_hbm, wk_hbm, wv_hbm, wo_hbm, w1_hbm, w3_hbm, w2_hbm,
            c_hbm, wm_hbm, out_hbm,
            xv, outv, wo, w1, w3, w2, wm, cv, m0v, modv, xh, h0, hn, acc,
            lhs_a, lhs_b, o32, x1n, x1o, fv, h2, hid, sem_in, sem_m, sem_s, sem_w, sem_out, *rest):
    ring = rest[0:2]
    wg = rest[2:4]

    def side(g, t):
        return (g % 2) ^ int(t >= 2 * HG)

    scale = DH ** -0.5

    copies = {}

    def mk(name, src, dst):
        copies[name] = pltpu.make_async_copy(src, dst, sem_in.at[len(copies)])

    wm_u = wm_hbm.bitcast(U32)
    mk("c", c_hbm, cv)
    mk("mem0", mem0_hbm, m0v)
    mk("x0", x_hbm.at[0:X0], xv.at[0:X0])
    mk("x1", x_hbm.at[X0:X1], xv.at[X0:X1])
    mk("wo", wo_hbm.bitcast(U32), wo)
    mk("wm1", wm_u.at[:, 2 * D:5 * D], wm.at[:, 2 * D:5 * D])
    for n, hbm, ref in (("w1", w1_hbm, w1), ("w3", w3_hbm, w3)):
        mk(n + "a", hbm.bitcast(U32).at[:, 0:FILL[0] * FC], ref.at[:, 0:FILL[0] * FC])
        mk(n + "b", hbm.bitcast(U32).at[:, FILL[0] * FC:FF], ref.at[:, FILL[0] * FC:FF])
    mk("w2", w2_hbm.bitcast(U32), w2)
    mk("wm2", wm_u.at[:, 5 * D:6 * D], wm.at[:, 5 * D:6 * D])
    mk("x2", x_hbm.at[X1:S], xv.at[X1:S])

    def mod_copies(kt):
        return [pltpu.make_async_copy(wm_u.at[:, _cols(i * D + kt * KW, KW)],
                                      wm.at[:, _cols(i * D + kt * KW, KW)], sem_m.at[kt])
                for i in range(2)]

    w_hbm = (wq_hbm, wk_hbm, wv_hbm)

    def start_block(j, rows=slice(None), sem=None):
        m, gi = j // 4, j % 4
        for pg in range(2):
            for jj in range(HG // 2):
                for par in range(2):
                    pltpu.make_async_copy(
                        w_hbm[m].bitcast(U32).at[rows, par, (2 * gi + pg) * (HG // 2) + jj],
                        wg[side(pg, m * HG)].at[gi * 3 * HG + m * HG + 2 * jj + par, rows],
                        sem_w.at[j] if sem is None else sem).start()

    def wait_block(j, s0):
        for w in wg:
            buf = w.at[pl.ds(s0, HG)]
            pltpu.make_async_copy(buf, buf, sem_w.at[j]).wait()

    def start_set(i):
        for j in range(NB0):
            start_block(j, slice(i * SETW, (i + 1) * SETW), sem_s.at[i])

    def wait_set(i):
        for w in wg:
            for gi in range(NB0):
                buf = w.at[gi * 3 * HG:gi * 3 * HG + HG, pl.ds(pl.multiple_of(i * SETW, SETW), SETW)]
                pltpu.make_async_copy(buf, buf, sem_s.at[i]).wait()

    def start_mod(kts):
        for kt in kts:
            for c in mod_copies(kt):
                c.start()

    for n in ("x0", "c", "mem0"):
        copies[n].start()

    def zero(i, c):
        acc[i] = jnp.zeros(acc.shape[1:], F32)
        rows = pl.ds(pl.multiple_of(i * 32, 32), 32)
        for w in wg:
            w[NWS:NWS + HG, rows, :] = jnp.zeros((HG, 32, DH), U32)
        return c

    lax.fori_loop(0, NB0 * 2 * HG, zero, 0)
    start_set(0)
    start_mod((0, 1, 2))
    start_set(1)
    start_mod((3, 4))
    start_set(2)
    start_mod((5,))

    def out_copy(r0, n):
        return pltpu.make_async_copy(outv.at[pl.ds(r0, n)], out_hbm.at[pl.ds(r0, n)], sem_out)

    def silu_c():
        return jnp.broadcast_to(_silu(cv[...].astype(F32)), (16, D)).astype(BF16)

    def mod_part(off, w):
        r = _dot(silu_c(), _unpack(wm[:, _cols(off, w)]))[0:8]
        modv[:, _cols(off, w)] = r
        return r[0:1]

    def mvec(i, n, plus=0.0):
        m = modv[:, i * D:(i + 1) * D]
        return jnp.concatenate([plus + m if plus else m] * (n // 8), axis=0)

    def ln1(r0, n):
        xf = xv[pl.ds(r0, n), :].astype(F32)
        return _ln(xf) * mvec(1, n, 1.0) + mvec(0, n)

    def repack_rows(w, sl, r0):
        rows = slice(r0, r0 + 32) if isinstance(r0, int) else pl.ds(r0, 32)
        a = w[sl, rows, :]
        b = w[sl + 1, rows, :]
        w[sl, rows, :] = (a & jnp.uint32(0xFFFF)) | (b << 16)
        w[sl + 1, rows, :] = (a >> 16) | (b & jnp.uint32(0xFFFF0000))

    def repack_now(s0):
        def body(i, c):
            for w in wg:
                for r in range(0, D // 4, 32):
                    r0 = pl.multiple_of((i & 1) * (D // 4) + r, 32)
                    repack_rows(w, s0 + 2 * (i >> 1), r0)
            return c

        lax.fori_loop(0, HG, body, 0)

    def repack_tile(w, kt, slots):
        for s0 in slots:
            for t in range(0, HG, 2):
                for r in range(0, KW // 2, 32):
                    r0 = kt * (KW // 2) + r
                    repack_rows(w, s0 + t, r0 if isinstance(r0, int) else pl.multiple_of(r0, 32))

    def store_tokens(dst, gi, t, r):
        for pp in range(PRO // PT):
            b0, r0 = pp * SLOT, pp * PT
            dst[gi, t, b0 + 4:b0 + 8, :] = _pack(r[r0:r0 + 8])
            dst[gi, t, b0 + 8:b0 + 24, :] = _pack(r[r0 + 8:r0 + 40])
            dst[gi, t, b0 + 28:b0 + 32, :] = _pack(r[r0 + 40:r0 + 48])
            dst[gi, t, b0 + 32:b0 + 40, :] = _pack(r[r0 + 48:r0 + 64])
        b0 = (PRO // PT) * SLOT
        dst[gi, t, 0:4, :] = _pack(r[PRO:PRO + 8])
        dst[gi, t, b0 + 4:b0 + 8, :] = _pack(r[PRO + 8:PRO + 16])
        dst[gi, t, b0 + 8:b0 + 16, :] = _pack(r[PRO + 16:PRO + 32])

    def proj(lhs, g, rows, t0, t1):
        for t in range(t0, t1):
            r = _dot(lhs, _unpack(wg[side(g, t)][g // 2 * 3 * HG + t]))
            for i, row in enumerate(rows):
                ring[side(g, t)][g // 2, t, pl.ds(row, 4), :] = _pack(r[8 * i:8 * i + 8])

    def attn_qk(g, base, q0, nq, nk, allowed, fill):
        qrow = pl.multiple_of(base + q0 // 2, 8)
        ps = []
        for hh in range(HG):
            q = _unpack(ring[g % 2][g // 2, hh, pl.ds(qrow, nq // 2), :])
            k = _unpack(ring[g % 2][g // 2, HG + hh, pl.ds(base, nk // 2), :])
            s = lax.dot_general(q, k, (((1,), (1,)), ((), ())), preferred_element_type=F32)
            s = jnp.where(allowed, s, fill)
            m = jnp.max(s, axis=-1, keepdims=True)
            p = jnp.exp2((s - m) * (scale * LOG2E))
            l = jnp.sum(p, axis=-1, keepdims=True)
            ps.append((p * _recip(l)).astype(BF16))
        return ps

    def attn_pv(g, base, nq, nk, ps):
        for hh in range(HG):
            v = _unpack(ring[1 - g % 2][g // 2, 2 * HG + hh, pl.ds(base, nk // 2), :])
            col = (g * HG + hh) * DH
            o32[0:nq // 2, col:col + DH] = _pack(_dot(ps[hh], v))

    def wo_proj(nq, stores):
        o = _unpack(o32[0:nq // 2, :])
        cw = WOCW
        for cb in range(D // cw):
            cs = slice(cb * cw, (cb + 1) * cw)
            r = _dot(o, _unpack(wo[:, cs]))
            for r0, n, fn in stores:
                fn(cs, r[r0:r0 + n])

    def ln2():
        h2[...] = _pack(_ln(x1n[...]) * mvec(4, PT, 1.0) + mvec(3, PT))

    def ffn_up(c0, c1, off=0):
        a = _unpack(h2[...])
        for c in range(c0, c1):
            cs = _cols(off + c * FC, FC)
            gt = _dot(a, _unpack(w1[:, cs]))
            up = _dot(a, _unpack(w3[:, cs]))
            hid[:, cs] = _pack(_silu(gt) * up)

    def ffn_down(tok0, x1, last=False):
        a = _unpack(hid[...])
        cw = DNCW
        for cb in range(D // cw):
            cs = slice(cb * cw, (cb + 1) * cw)
            r = _dot(a, _unpack(w2[:, cs]))
            if not last:
                fv[:, cs] = r
            gb = modv[0:1, 5 * D + cb * cw:5 * D + (cb + 1) * cw]
            outv[pl.ds(tok0, PT), cs] = (x1[:, cs] + gb * r).astype(BF16)
            if last:
                pltpu.make_async_copy(outv.at[pl.ds(tok0, PT), cs],
                                      out_hbm.at[pl.ds(tok0, PT), cs], sem_out).start()

    def unit_row(u):
        r = u & 7
        slot = _slot(u >> 3)
        return pl.multiple_of(slot * SLOT + 4 + 4 * r + 4 * (r >= 5).astype(jnp.int32), 4)

    with _scope("waitx0"):
        copies["x0"].wait()
    with _scope("ln0"):

        def ln_body(i, c):
            r0 = pl.multiple_of(i * LNR, 8)
            xh[pl.ds(r0, LNR), :] = _ln(xv[pl.ds(r0, LNR), :].astype(F32))
            return c

        lax.fori_loop(0, X0 // LNR, ln_body, 0)
    with _scope("waitc"):
        copies["c"].wait()
        copies["mem0"].wait()

    def modulate(kt):
        sa = mod_part(kt * KW, KW)
        ca = mod_part(D + kt * KW, KW)
        cs = _cols(kt * KW, KW)
        hh = xh[0:PRO + 24, cs] * (1.0 + ca) + sa
        hn[...] = _pack(jnp.concatenate([hh[0:PRO], m0v[:, cs].astype(F32), hh[PRO:]], axis=0))

    with _scope("waitw0"):
        wait_set(0)
    with _scope("first"):
        for w in wg:
            repack_tile(w, 0, [gi * 3 * HG for gi in range(NB0)])
        with _scope("waitm0"):
            for c in mod_copies(0):
                c.wait()
        modulate(0)

    def kmajor(kt, c):
        more = kt < KT - 1
        kn = jnp.minimum(kt + 1, KT - 1)

        def later_copies():
            start_set(3)
            start_mod((6, 7))
            for j in range(NB0, NB0 + 3):
                start_block(j)

        _rarely(kt == 1, later_copies)

        @pl.when(more)
        def _():
            for cp in mod_copies(kn):
                cp.wait()

        @pl.when(more & ((kn & 1) == 0))
        def _():
            wait_set(kn >> 1)

        cs = _cols(kt * KW, KW)
        h0[:, cs] = hn[...]
        rows = pl.ds(pl.multiple_of(kt * (KW // 2), KW // 2), KW // 2)
        for pg in range(2):
            for gi in range(NB0):
                for t in range(HG):
                    i = (pg * NB0 + gi) * HG + t
                    r = acc[i] + _dot(_unpack(h0[:, cs]), _unpack(wg[pg][gi * 3 * HG + t, rows, :]))
                    acc[i] = r
                    store_tokens(ring[pg], gi, t, r)
                if pg == 0 and gi == 0:
                    modulate(kn)
        slots = [jnp.where(more, gi * 3 * HG, NWS) for gi in range(NB0)]
        for w in wg:
            repack_tile(w, kn, slots)
        return c

    with _scope("kmajor"):
        lax.fori_loop(0, KT, kmajor, 0)

    def pro_body(j, c):
        gi, t0 = j & 3, (j >> 2) * HG
        s0 = gi * (3 * HG) + t0
        jn = j + 1
        prefetch = jn < NJ
        sn = jnp.where(prefetch, (jn & 3) * (3 * HG) + (jn >> 2) * HG, NWS)

        def first_blocks():
            def batch1():
                for jj in range(NB0 + 3, NJ - 2):
                    start_block(jj)
                with _scope("waitlate"):
                    wait_block(j, s0)
                repack_now(s0)

            def batch2():
                for jj in range(NJ - 2, NJ):
                    start_block(jj)
                for n in ("x1", "wo", "wm1", "w1a", "w3a", "w1b", "w3b", "w2", "wm2", "x2"):
                    copies[n].start()

            _rarely(j == NB0, batch1)
            _rarely(j == NB0 + 1, batch2)

        _rarely(j <= NB0 + 1, first_blocks)

        @pl.when(prefetch)
        def _():
            wait_block(jn, sn)

        a = _unpack(h0[...])
        for pg in range(2):
            for t in range(HG):
                store_tokens(ring[pg], gi, t0 + t, _dot(a, _unpack(wg[pg][s0 + t])))
        for w in wg:
            for t in range(0, HG, 2):
                for r0 in range(0, D // 2, 32):
                    repack_rows(w, sn + t, r0)
        return c

    with _scope("pro"):
        lax.fori_loop(NB0, NJ, pro_body, 0)

    def pair(p, with_ffn):
        (al_a, fi_a), (al_b, fi_b) = _masks()
        base = pl.multiple_of(_slot(p) * SLOT, 8)
        u0 = PRO // 8 + 6 * p
        tlead = PRO + 48 * p

        if with_ffn:
            x1o[...] = x1n[...]

        def filler(i, c0=None, c1=None):
            if not with_ffn:
                if i is not None:
                    mod_part(2 * D + MODF[i] * 256, (MODF[i + 1] - MODF[i]) * 256)
            elif c0 is None:
                ffn_down(pl.multiple_of((p - 1) * PT, PT), x1o)
            else:
                ffn_up(c0, c1)

        def proj_attn(lhs, rows, q0, nq, nk, allowed, fill, f):
            ps = None
            for g in range(G):
                proj(lhs, g, rows, 0, QKPOS)
                if g > 0 and QKPOS > 0:
                    ps = attn_qk(g - 1, base, q0, nq, nk, allowed, fill)
                proj(lhs, g, rows, QKPOS, PVPOS)
                if g > 0:
                    attn_pv(g - 1, base, nq, nk, ps)
                proj(lhs, g, rows, PVPOS, 3 * HG)
                if QKPOS == 0 or g == G - 1:
                    ps = attn_qk(g, base, q0, nq, nk, allowed, fill)
            filler(f, FILL[f], FILL[f + 1])
            attn_pv(G - 1, base, nq, nk, ps)
            filler(f + 1, FILL[f + 1], FILL[f + 2])

        def st_lhs(ref):
            def fn(cs, val):
                ref[0:MEM, cs] = val.astype(BF16).astype(F32)
            return fn

        def st_a(r0, n):
            def fn(cs, val):
                ga = modv[0:1, 2 * D + cs.start:2 * D + cs.stop]
                x = xv[pl.ds(pl.multiple_of(p * PT + r0, 8), n), cs].astype(F32)
                x1n[r0:r0 + n, cs] = x + ga * val
            return fn

        lhs_b[MEM:32, :] = ln1(pl.multiple_of(tlead + 24, 8), 24)
        if with_ffn:
            lhs = lhs_a[...].astype(BF16)
            rows = [base, unit_row(u0), unit_row(u0 + 1), unit_row(u0 + 2)]
            proj_attn(lhs, rows, 0, 32, 48, al_a, fi_a, 0)
        else:
            ps = [attn_qk(g, base, 0, 32, 48, al_a, fi_a) for g in range(G)]
            filler(0)
            for g in range(G):
                attn_pv(g, base, 32, 48, ps[g])
            filler(1)
        wo_proj(32, [(0, 8, st_lhs(lhs_b)), (8, 24, st_a(0, 24))])
        filler(2, FILL[2], FILL[3])

        lhs = lhs_b[...].astype(BF16)
        rows = [pl.multiple_of(base + 24, 8), unit_row(u0 + 3), unit_row(u0 + 4), unit_row(u0 + 5)]
        nxt = pl.multiple_of(jnp.minimum(tlead + 48, S - 24), 8)
        lhs_a[MEM:32, :] = ln1(nxt, 24)
        proj_attn(lhs, rows, 32, 48, 80, al_b, fi_b, 3)
        wo_proj(48, [(16, 8, st_lhs(lhs_a)), (0, 16, st_a(24, 16)), (24, 24, st_a(40, 24))])
        ln2()
        filler(None)
        ffn_up(0, FILL[0])

    with _scope("waitwo"):
        copies["x1"].wait()
        copies["wo"].wait()
        copies["wm1"].wait()
        copies["w1a"].wait()
        copies["w3a"].wait()

    with _scope("noffn"):
        modv[:, 5 * D:6 * D] = jnp.zeros((8, D), F32)
        pair(jnp.int32(0), False)

    with _scope("waitffn"):
        copies["w1b"].wait()
        copies["w3b"].wait()
        copies["w2"].wait()

    def late_inputs():
        copies["wm2"].wait()
        copies["x2"].wait()
        mod_part(5 * D, D)
        outv[0:PT, :] = (x1o[...] + mvec(5, PT) * fv[...]).astype(BF16)

    def pair_ffn(p, c):
        pair(p, True)
        return c

    def main(o, c):
        _rarely(o == 1, late_inputs)
        lax.fori_loop(MAIN_START + o, MAIN_START + 1 + o * (NPAIR - MAIN_START - 1), pair_ffn, 0)
        return c

    with _scope("main"):
        lax.fori_loop(0, 2, main, 0)

    with _scope("epi"):
        out_copy(0, S - PT).start()

        def up_body(i, c):
            ffn_up(FILL[0], FILL[0] + EPI_UP, i * (EPI_UP * FC))
            return c

        lax.fori_loop(0, 2, up_body, 0)
        ffn_up(FILL[0] + 2 * EPI_UP, NFC)
        ffn_down(S - PT, x1n, last=True)
    with _scope("waitout"):
        out_copy(0, S).wait()


@functools.partial(jax.jit, static_argnames=("A_seg_len",))
def pallas_adaLN_cond__memory_aug_recurrent_mem_tr__glu_gated_swiglu__prompt_kernel(
    A_x, A_mem0, A_Wq, A_Wk, A_Wv, A_Wo, A_seg_len, B_x, B_w1, B_w3, B_w2, c, w_mod,
):
    assert A_seg_len == SEG
    assert A_x.shape == (1, S, D) and A_mem0.shape == (1, MEM, D)
    assert A_Wq.shape == (D, H, DH) and B_w1.shape == (D, FF)
    del B_x

    scratch = [
        pltpu.VMEM((S, D), BF16),
        pltpu.VMEM((S, D), BF16),
        pltpu.VMEM((HD // 2, D), U32),
        pltpu.VMEM((D // 2, FF), U32),
        pltpu.VMEM((D // 2, FF), U32),
        pltpu.VMEM((FF // 2, D), U32),
        pltpu.VMEM((D // 2, 6 * D), U32),
        pltpu.VMEM((1, D), BF16),
        pltpu.VMEM((MEM, D), BF16),
        pltpu.VMEM((8, 6 * D), F32),
        pltpu.VMEM((X0, D), F32),
        pltpu.VMEM((PROM // 2, D), U32),
        pltpu.VMEM((PROM // 2, KW), U32),
        pltpu.VMEM((NB0 * 2 * HG, PROM, DH), F32),
        pltpu.VMEM((32, D), F32),
        pltpu.VMEM((32, D), F32),
        pltpu.VMEM((24, HD), U32),
        pltpu.VMEM((PT, D), F32),
        pltpu.VMEM((PT, D), F32),
        pltpu.VMEM((PT, D), F32),
        pltpu.VMEM((PT // 2, D), U32),
        pltpu.VMEM((PT // 2, FF), U32),
        pltpu.SemaphoreType.DMA((13,)),
        pltpu.SemaphoreType.DMA((KT,)),
        pltpu.SemaphoreType.DMA((NSET,)),
        pltpu.SemaphoreType.DMA((NJ,)),
        pltpu.SemaphoreType.DMA,
    ] + [pltpu.VMEM((G // 2, 3 * HG, NSLOT * SLOT, DH), U32)] * 2 + [
        pltpu.VMEM((NWS + HG, D // 2, DH), U32)] * 2

    out = pl.pallas_call(
        _kernel,
        out_shape=jax.ShapeDtypeStruct((S, D), BF16),
        in_specs=[pl.BlockSpec(memory_space=pl.ANY)] * 11,
        out_specs=pl.BlockSpec(memory_space=pl.ANY),
        scratch_shapes=scratch,
        compiler_params=pltpu.CompilerParams(
            vmem_limit_bytes=120 * 1024 * 1024, disable_bounds_checks=True),
    )(
        A_x.reshape(S, D), A_mem0.reshape(MEM, D),
        A_Wq.reshape(D // 2, 2, H, DH), A_Wk.reshape(D // 2, 2, H, DH),
        A_Wv.reshape(D // 2, 2, H, DH), A_Wo.reshape(HD, D),
        B_w1, B_w3, B_w2, c, w_mod,
    )
    return out.reshape(1, S, D)
```

```python
import functools

import jax
import jax.numpy as jnp
from jax import lax
import jax.experimental.pallas as pl
import jax.experimental.pallas.tpu as pltpu

F32 = jnp.float32
BF16 = jnp.bfloat16
U32 = jnp.uint32

S = 2048
D = 1024
H = 32
DH = 128
HD = H * DH
MEM = 8
SEG = 32
FF = 3584
EPS = 1e-5
LOG2E = 1.4426950408889634

G = 8
HG = H // G
PRO = 512
NPAIR = S // (2 * SEG)
PT = 2 * SEG
SLOT = 40
NSLOT = 9
X0 = 544
X1 = 640
FC = 256
NFC = FF // FC
KW = 128
KT = D // KW
NB0 = 2
SETW = 128
NSET = D // 2 // SETW
NWS = G // 2 * 3 * HG
NJ = 3 * G // 2
FILL = (3, 5, 7, 10, 12, 14)
WOCW = 256
DNCW = 256
QKPOS = 2
PVPOS = 11
MODF = (0, 5, 6, 8, 11, 12)
PROM = PRO + 32
MAIN_START = 1
LNR = 136
SCOPES = False
FLUSH_AT = 1
MODR = 32


class _NoScope:
    def __enter__(self):
        return self

    def __exit__(self, *a):
        return False


def _scope(name):
    return jax.named_scope(name) if SCOPES else _NoScope()


def _unpack(x):
    return pltpu.bitcast(x, BF16)


def _pack(x):
    return pltpu.bitcast(x.astype(BF16), U32)


def _dot(a, b):
    return jnp.dot(a, b, preferred_element_type=F32)


def _ln(x):
    m = jnp.mean(x, axis=-1, keepdims=True)
    xc = x - m
    v = jnp.mean(xc * xc, axis=-1, keepdims=True)
    return xc * lax.rsqrt(v + EPS)


def _recip(x):
    r = pl.reciprocal(x, approx=True)
    return r * (2.0 - x * r)


def _silu(x):
    h = 0.5 * x
    return h + h * jnp.tanh(h)


def _cols(off, w):
    if isinstance(off, int):
        return slice(off, off + w)
    return pl.ds(pl.multiple_of(off, w), w)


def _rarely(cond, fn):
    def body(_, c):
        fn()
        return c

    lax.fori_loop(0, cond.astype(jnp.int32), body, 0)


def _slot(pair):
    assert NSLOT == 9
    return pair - NSLOT * ((pair * 57) >> 9)


def _masks():
    def pos(j):
        return jnp.where(j < 40, j, jnp.where(j < 48, j - 32, jnp.where(j < 56, j - 48, j - 40)))

    out = []
    for q0, nq, nk in ((0, 32, 48), (32, 48, 80)):
        qi = lax.broadcasted_iota(jnp.int32, (nq, nk), 0) + q0
        kj = lax.broadcasted_iota(jnp.int32, (nq, nk), 1)
        qp, kp = pos(qi), pos(kj)
        same = ((qi < 40) & (kj < 40)) | ((qi >= 40) & (kj >= 40))
        allowed = same & ((qp < MEM) | (qp >= kp))
        fill = jnp.where(same, jnp.float32(-1e9 * DH ** 0.5), jnp.float32(-jnp.inf))
        out.append((allowed, fill))
    return out


def _kernel(x_hbm, mem0_hbm, wq_hbm, wk_hbm, wv_hbm, wo_hbm, w1_hbm, w3_hbm, w2_hbm,
            c_hbm, wm_hbm, out_hbm,
            xv, outv, wo, w1, w3, w2, wm, cv, m0v, modv, xh, h0, hn, acc,
            lhs_a, lhs_b, o32, x1n, x1o, fv, h2, hid, sem_in, sem_m, sem_s, sem_w, sem_out, *rest):
    ring = rest[0:2]
    wg = rest[2:4]

    def side(g, t):
        return (g % 2) ^ int(t >= 2 * HG)

    scale = DH ** -0.5

    copies = {}

    def mk(name, src, dst):
        copies[name] = pltpu.make_async_copy(src, dst, sem_in.at[len(copies)])

    wm_u = wm_hbm.bitcast(U32)
    mk("c", c_hbm, cv)
    mk("mem0", mem0_hbm, m0v)
    mk("x0", x_hbm.at[0:X0], xv.at[0:X0])
    mk("x1", x_hbm.at[X0:X1], xv.at[X0:X1])
    mk("wo", wo_hbm.bitcast(U32), wo)
    mk("wm1", wm_u.at[:, 2 * D:5 * D], wm.at[:, 2 * D:5 * D])
    for n, hbm, ref in (("w1", w1_hbm, w1), ("w3", w3_hbm, w3)):
        mk(n + "a", hbm.bitcast(U32).at[:, 0:FILL[0] * FC], ref.at[:, 0:FILL[0] * FC])
        mk(n + "b", hbm.bitcast(U32).at[:, FILL[0] * FC:FF], ref.at[:, FILL[0] * FC:FF])
    mk("w2", w2_hbm.bitcast(U32), w2)
    mk("wm2", wm_u.at[:, 5 * D:6 * D], wm.at[:, 5 * D:6 * D])
    mk("x2", x_hbm.at[X1:S], xv.at[X1:S])

    def mod_copies(kt):
        return [pltpu.make_async_copy(wm_u.at[:, _cols(i * D + kt * KW, KW)],
                                      wm.at[:, _cols(i * D + kt * KW, KW)], sem_m.at[kt])
                for i in range(2)]

    w_hbm = (wq_hbm, wk_hbm, wv_hbm)

    def start_block(j, rows=slice(None), sem=None):
        m, gi = j // 4, j % 4
        for pg in range(2):
            for jj in range(HG // 2):
                for par in range(2):
                    pltpu.make_async_copy(
                        w_hbm[m].bitcast(U32).at[rows, par, (2 * gi + pg) * (HG // 2) + jj],
                        wg[side(pg, m * HG)].at[gi * 3 * HG + m * HG + 2 * jj + par, rows],
                        sem_w.at[j] if sem is None else sem).start()

    def wait_block(j, s0):
        for w in wg:
            buf = w.at[pl.ds(s0, HG)]
            pltpu.make_async_copy(buf, buf, sem_w.at[j]).wait()

    def start_set(i):
        for j in range(NB0):
            start_block(j, slice(i * SETW, (i + 1) * SETW), sem_s.at[i])

    def wait_set(i):
        for w in wg:
            for gi in range(NB0):
                buf = w.at[gi * 3 * HG:gi * 3 * HG + HG, pl.ds(pl.multiple_of(i * SETW, SETW), SETW)]
                pltpu.make_async_copy(buf, buf, sem_s.at[i]).wait()

    def start_mod(kts):
        for kt in kts:
            for c in mod_copies(kt):
                c.start()

    for n in ("x0", "c", "mem0"):
        copies[n].start()

    def zero(i, c):
        acc[i] = jnp.zeros(acc.shape[1:], F32)
        rows = pl.ds(pl.multiple_of(i * 32, 32), 32)
        for w in wg:
            w[NWS:NWS + HG, rows, :] = jnp.zeros((HG, 32, DH), U32)
        return c

    lax.fori_loop(0, NB0 * 2 * HG, zero, 0)
    start_set(0)
    start_mod((0, 1, 2))
    start_set(1)
    start_mod((3, 4))
    start_set(2)
    start_mod((5,))

    def out_copy(r0, n):
        return pltpu.make_async_copy(outv.at[pl.ds(r0, n)], out_hbm.at[pl.ds(r0, n)], sem_out)

    def silu_c():
        return jnp.broadcast_to(_silu(cv[...].astype(F32)), (16, D)).astype(BF16)

    def mod_part(off, w):
        r = _dot(silu_c(), _unpack(wm[:, _cols(off, w)]))[0:8]
        modv[:, _cols(off, w)] = r
        return r[0:1]

    def mvec(i, n, plus=0.0):
        m = modv[:, i * D:(i + 1) * D]
        return jnp.concatenate([plus + m if plus else m] * (n // 8), axis=0)

    def ln1(r0, n):
        xf = xv[pl.ds(r0, n), :].astype(F32)
        return _ln(xf) * mvec(1, n, 1.0) + mvec(0, n)

    def repack_rows(w, sl, r0):
        rows = slice(r0, r0 + 32) if isinstance(r0, int) else pl.ds(r0, 32)
        a = w[sl, rows, :]
        b = w[sl + 1, rows, :]
        w[sl, rows, :] = (a & jnp.uint32(0xFFFF)) | (b << 16)
        w[sl + 1, rows, :] = (a >> 16) | (b & jnp.uint32(0xFFFF0000))

    def repack_now(s0):
        def body(i, c):
            for w in wg:
                for r in range(0, D // 4, 32):
                    r0 = pl.multiple_of((i & 1) * (D // 4) + r, 32)
                    repack_rows(w, s0 + 2 * (i >> 1), r0)
            return c

        lax.fori_loop(0, HG, body, 0)

    def repack_tile(w, kt, slots):
        for s0 in slots:
            for t in range(0, HG, 2):
                for r in range(0, KW // 2, 32):
                    r0 = kt * (KW // 2) + r
                    repack_rows(w, s0 + t, r0 if isinstance(r0, int) else pl.multiple_of(r0, 32))

    def store_tokens(dst, gi, t, r):
        for pp in range(PRO // PT):
            b0, r0 = pp * SLOT, pp * PT
            dst[gi, t, b0 + 4:b0 + 8, :] = _pack(r[r0:r0 + 8])
            dst[gi, t, b0 + 8:b0 + 24, :] = _pack(r[r0 + 8:r0 + 40])
            dst[gi, t, b0 + 28:b0 + 32, :] = _pack(r[r0 + 40:r0 + 48])
            dst[gi, t, b0 + 32:b0 + 40, :] = _pack(r[r0 + 48:r0 + 64])
        b0 = (PRO // PT) * SLOT
        dst[gi, t, 0:4, :] = _pack(r[PRO:PRO + 8])
        dst[gi, t, b0 + 4:b0 + 8, :] = _pack(r[PRO + 8:PRO + 16])
        dst[gi, t, b0 + 8:b0 + 16, :] = _pack(r[PRO + 16:PRO + 32])

    def proj(lhs, g, rows, t0, t1):
        for t in range(t0, t1):
            r = _dot(lhs, _unpack(wg[side(g, t)][g // 2 * 3 * HG + t]))
            for i, row in enumerate(rows):
                ring[side(g, t)][g // 2, t, pl.ds(row, 4), :] = _pack(r[8 * i:8 * i + 8])

    def attn_qk(g, base, q0, nq, nk, allowed, fill):
        qrow = pl.multiple_of(base + q0 // 2, 8)
        ps = []
        for hh in range(HG):
            q = _unpack(ring[g % 2][g // 2, hh, pl.ds(qrow, nq // 2), :])
            k = _unpack(ring[g % 2][g // 2, HG + hh, pl.ds(base, nk // 2), :])
            s = lax.dot_general(q, k, (((1,), (1,)), ((), ())), preferred_element_type=F32)
            s = jnp.where(allowed, s, fill)
            m = jnp.max(s, axis=-1, keepdims=True)
            p = jnp.exp2((s - m) * (scale * LOG2E))
            l = jnp.sum(p, axis=-1, keepdims=True)
            ps.append((p * _recip(l)).astype(BF16))
        return ps

    def attn_pv(g, base, nq, nk, ps):
        for hh in range(HG):
            v = _unpack(ring[1 - g % 2][g // 2, 2 * HG + hh, pl.ds(base, nk // 2), :])
            col = (g * HG + hh) * DH
            o32[0:nq // 2, col:col + DH] = _pack(_dot(ps[hh], v))

    def wo_proj(nq, stores):
        o = _unpack(o32[0:nq // 2, :])
        cw = WOCW
        for cb in range(D // cw):
            cs = slice(cb * cw, (cb + 1) * cw)
            r = _dot(o, _unpack(wo[:, cs]))
            for r0, n, fn in stores:
                fn(cs, r[r0:r0 + n])

    def ln2():
        h2[...] = _pack(_ln(x1n[...]) * mvec(4, PT, 1.0) + mvec(3, PT))

    def ffn_up(c0, c1):
        a = _unpack(h2[...])
        for c in range(c0, c1):
            cs = slice(c * FC, (c + 1) * FC)
            gt = _dot(a, _unpack(w1[:, cs]))
            up = _dot(a, _unpack(w3[:, cs]))
            hid[:, cs] = _pack(_silu(gt) * up)

    def ffn_down(tok0, x1, last=False):
        a = _unpack(hid[...])
        cw = DNCW
        for cb in range(D // cw):
            cs = slice(cb * cw, (cb + 1) * cw)
            r = _dot(a, _unpack(w2[:, cs]))
            if not last:
                fv[:, cs] = r
            gb = modv[0:1, 5 * D + cb * cw:5 * D + (cb + 1) * cw]
            outv[pl.ds(tok0, PT), cs] = (x1[:, cs] + gb * r).astype(BF16)
            if last:
                pltpu.make_async_copy(outv.at[pl.ds(tok0, PT), cs],
                                      out_hbm.at[pl.ds(tok0, PT), cs], sem_out).start()

    def unit_row(u):
        r = u & 7
        slot = _slot(u >> 3)
        return pl.multiple_of(slot * SLOT + 4 + 4 * r + 4 * (r >= 5).astype(jnp.int32), 4)

    with _scope("waitx0"):
        copies["x0"].wait()
    with _scope("ln0"):

        def ln_body(i, c):
            r0 = pl.multiple_of(i * LNR, 8)
            xh[pl.ds(r0, LNR), :] = _ln(xv[pl.ds(r0, LNR), :].astype(F32))
            return c

        lax.fori_loop(0, X0 // LNR, ln_body, 0)
    with _scope("waitc"):
        copies["c"].wait()
        copies["mem0"].wait()

    def modulate(kt):
        sa = mod_part(kt * KW, KW)
        ca = mod_part(D + kt * KW, KW)
        cs = _cols(kt * KW, KW)
        ca = 1.0 + ca
        for r0 in range(0, PRO, MODR):
            hn[r0 // 2:(r0 + MODR) // 2, :] = _pack(xh[r0:r0 + MODR, cs] * ca + sa)
        hh = xh[PRO:PRO + 24, cs] * ca + sa
        hn[PRO // 2:PROM // 2, :] = _pack(jnp.concatenate([m0v[:, cs].astype(F32), hh], axis=0))

    with _scope("waitw0"):
        wait_set(0)
    with _scope("first"):
        for w in wg:
            repack_tile(w, 0, [gi * 3 * HG for gi in range(NB0)])
        with _scope("waitm0"):
            for c in mod_copies(0):
                c.wait()
        modulate(0)

    def kmajor(kt, c):
        more = kt < KT - 1
        kn = jnp.minimum(kt + 1, KT - 1)

        def later_copies():
            start_set(3)
            start_mod((6, 7))
            for j in range(NB0, NB0 + 3):
                start_block(j)

        _rarely(kt == 1, later_copies)

        @pl.when(more)
        def _():
            for cp in mod_copies(kn):
                cp.wait()

        @pl.when(more & ((kn & 1) == 0))
        def _():
            wait_set(kn >> 1)

        cs = _cols(kt * KW, KW)
        h0[:, cs] = hn[...]
        rows = pl.ds(pl.multiple_of(kt * (KW // 2), KW // 2), KW // 2)
        for pg in range(2):
            for gi in range(NB0):
                for t in range(HG):
                    i = (pg * NB0 + gi) * HG + t
                    a = hn[...] if i < HG else h0[:, cs]
                    acc[i] += _dot(_unpack(a), _unpack(wg[pg][gi * 3 * HG + t, rows, :]))
                if pg == 0 and gi == 0:
                    modulate(kn)
        slots = [jnp.where(more, gi * 3 * HG, NWS) for gi in range(NB0)]
        for w in wg:
            repack_tile(w, kn, slots)
        return c

    with _scope("kmajor"):
        lax.fori_loop(0, KT, kmajor, 0)

    def pro_body(j, c):
        gi, t0 = j & 3, (j >> 2) * HG
        s0 = gi * (3 * HG) + t0
        jn = j + 1
        prefetch = jn < NJ
        sn = jnp.where(prefetch, (jn & 3) * (3 * HG) + (jn >> 2) * HG, NWS)

        def first_blocks():
            def batch1():
                for jj in range(NB0 + 3, NJ - 2):
                    start_block(jj)
                with _scope("waitlate"):
                    wait_block(j, s0)
                repack_now(s0)

            def batch2():
                for jj in range(NJ - 2, NJ):
                    start_block(jj)
                for n in ("x1", "wo", "wm1", "w1a", "w3a", "w1b", "w3b", "w2", "wm2", "x2"):
                    copies[n].start()

            _rarely(j == NB0, batch1)
            _rarely(j == NB0 + 1, batch2)

        _rarely(j <= NB0 + 1, first_blocks)

        @pl.when(prefetch)
        def _():
            wait_block(jn, sn)

        a = _unpack(h0[...])
        k = jnp.minimum(j - NB0, NB0 * HG - 1)
        for pg in range(2):
            for t in range(HG):
                store_tokens(ring[pg], gi, t0 + t, _dot(a, _unpack(wg[pg][s0 + t])))
                if t == FLUSH_AT:
                    store_tokens(ring[pg], k >> 2, k & 3, acc[pg * NB0 * HG + k])
        for w in wg:
            for t in range(0, HG, 2):
                for r0 in range(0, D // 2, 32):
                    repack_rows(w, sn + t, r0)
        return c

    with _scope("pro"):
        lax.fori_loop(NB0, NJ, pro_body, 0)

    def pair(p, with_ffn):
        (al_a, fi_a), (al_b, fi_b) = _masks()
        base = pl.multiple_of(_slot(p) * SLOT, 8)
        u0 = PRO // 8 + 6 * p
        tlead = PRO + 48 * p

        if with_ffn:
            x1o[...] = x1n[...]

        def filler(i, c0=None, c1=None):
            if not with_ffn:
                if i is not None:
                    mod_part(2 * D + MODF[i] * 256, (MODF[i + 1] - MODF[i]) * 256)
            elif c0 is None:
                ffn_down(pl.multiple_of((p - 1) * PT, PT), x1o)
            else:
                ffn_up(c0, c1)

        def proj_attn(lhs, rows, q0, nq, nk, allowed, fill, f):
            ps = None
            for g in range(G):
                proj(lhs, g, rows, 0, QKPOS)
                if g > 0 and QKPOS > 0:
                    ps = attn_qk(g - 1, base, q0, nq, nk, allowed, fill)
                proj(lhs, g, rows, QKPOS, PVPOS)
                if g > 0:
                    attn_pv(g - 1, base, nq, nk, ps)
                proj(lhs, g, rows, PVPOS, 3 * HG)
                if QKPOS == 0 or g == G - 1:
                    ps = attn_qk(g, base, q0, nq, nk, allowed, fill)
            filler(f, FILL[f], FILL[f + 1])
            attn_pv(G - 1, base, nq, nk, ps)
            filler(f + 1, FILL[f + 1], FILL[f + 2])

        def st_lhs(ref):
            def fn(cs, val):
                ref[0:MEM, cs] = val.astype(BF16).astype(F32)
            return fn

        def st_a(r0, n):
            def fn(cs, val):
                ga = modv[0:1, 2 * D + cs.start:2 * D + cs.stop]
                x = xv[pl.ds(pl.multiple_of(p * PT + r0, 8), n), cs].astype(F32)
                x1n[r0:r0 + n, cs] = x + ga * val
            return fn

        lhs_b[MEM:32, :] = ln1(pl.multiple_of(tlead + 24, 8), 24)
        if with_ffn:
            lhs = lhs_a[...].astype(BF16)
            rows = [base, unit_row(u0), unit_row(u0 + 1), unit_row(u0 + 2)]
            proj_attn(lhs, rows, 0, 32, 48, al_a, fi_a, 0)
        else:
            ps = [attn_qk(g, base, 0, 32, 48, al_a, fi_a) for g in range(G)]
            filler(0)
            for g in range(G):
                attn_pv(g, base, 32, 48, ps[g])
            filler(1)
        wo_proj(32, [(0, 8, st_lhs(lhs_b)), (8, 24, st_a(0, 24))])
        filler(2, FILL[2], FILL[3])

        lhs = lhs_b[...].astype(BF16)
        rows = [pl.multiple_of(base + 24, 8), unit_row(u0 + 3), unit_row(u0 + 4), unit_row(u0 + 5)]
        nxt = pl.multiple_of(jnp.minimum(tlead + 48, S - 24), 8)
        lhs_a[MEM:32, :] = ln1(nxt, 24)
        proj_attn(lhs, rows, 32, 48, 80, al_b, fi_b, 3)
        wo_proj(48, [(16, 8, st_lhs(lhs_a)), (0, 16, st_a(24, 16)), (24, 24, st_a(40, 24))])
        ln2()
        filler(None)
        ffn_up(0, FILL[0])

    with _scope("waitwo"):
        copies["x1"].wait()
        copies["wo"].wait()
        copies["wm1"].wait()
        copies["w1a"].wait()
        copies["w3a"].wait()

    with _scope("noffn"):
        modv[:, 5 * D:6 * D] = jnp.zeros((8, D), F32)
        pair(jnp.int32(0), False)

    with _scope("waitffn"):
        copies["w1b"].wait()
        copies["w3b"].wait()
        copies["w2"].wait()

    def late_inputs():
        copies["wm2"].wait()
        copies["x2"].wait()
        mod_part(5 * D, D)
        outv[0:PT, :] = (x1o[...] + mvec(5, PT) * fv[...]).astype(BF16)

    def pair_ffn(p, c):
        pair(p, True)
        return c

    def main(o, c):
        _rarely(o == 1, late_inputs)
        lax.fori_loop(MAIN_START + o, MAIN_START + 1 + o * (NPAIR - MAIN_START - 1), pair_ffn, 0)
        return c

    with _scope("main"):
        lax.fori_loop(0, 2, main, 0)

    with _scope("epi"):
        out_copy(0, S - PT).start()
        ffn_up(FILL[0], NFC)
        ffn_down(S - PT, x1n, last=True)
    with _scope("waitout"):
        out_copy(0, S).wait()


@functools.partial(jax.jit, static_argnames=("A_seg_len",))
def pallas_adaLN_cond__memory_aug_recurrent_mem_tr__glu_gated_swiglu__prompt_kernel(
    A_x, A_mem0, A_Wq, A_Wk, A_Wv, A_Wo, A_seg_len, B_x, B_w1, B_w3, B_w2, c, w_mod,
):
    assert A_seg_len == SEG
    assert A_x.shape == (1, S, D) and A_mem0.shape == (1, MEM, D)
    assert A_Wq.shape == (D, H, DH) and B_w1.shape == (D, FF)
    del B_x

    scratch = [
        pltpu.VMEM((S, D), BF16),
        pltpu.VMEM((S, D), BF16),
        pltpu.VMEM((HD // 2, D), U32),
        pltpu.VMEM((D // 2, FF), U32),
        pltpu.VMEM((D // 2, FF), U32),
        pltpu.VMEM((FF // 2, D), U32),
        pltpu.VMEM((D // 2, 6 * D), U32),
        pltpu.VMEM((1, D), BF16),
        pltpu.VMEM((MEM, D), BF16),
        pltpu.VMEM((8, 6 * D), F32),
        pltpu.VMEM((X0, D), F32),
        pltpu.VMEM((PROM // 2, D), U32),
        pltpu.VMEM((PROM // 2, KW), U32),
        pltpu.VMEM((NB0 * 2 * HG, PROM, DH), F32),
        pltpu.VMEM((32, D), F32),
        pltpu.VMEM((32, D), F32),
        pltpu.VMEM((24, HD), U32),
        pltpu.VMEM((PT, D), F32),
        pltpu.VMEM((PT, D), F32),
        pltpu.VMEM((PT, D), F32),
        pltpu.VMEM((PT // 2, D), U32),
        pltpu.VMEM((PT // 2, FF), U32),
        pltpu.SemaphoreType.DMA((13,)),
        pltpu.SemaphoreType.DMA((KT,)),
        pltpu.SemaphoreType.DMA((NSET,)),
        pltpu.SemaphoreType.DMA((NJ,)),
        pltpu.SemaphoreType.DMA,
    ] + [pltpu.VMEM((G // 2, 3 * HG, NSLOT * SLOT, DH), U32)] * 2 + [
        pltpu.VMEM((NWS + HG, D // 2, DH), U32)] * 2

    out = pl.pallas_call(
        _kernel,
        out_shape=jax.ShapeDtypeStruct((S, D), BF16),
        in_specs=[pl.BlockSpec(memory_space=pl.ANY)] * 11,
        out_specs=pl.BlockSpec(memory_space=pl.ANY),
        scratch_shapes=scratch,
        compiler_params=pltpu.CompilerParams(
            vmem_limit_bytes=120 * 1024 * 1024, disable_bounds_checks=True),
    )(
        A_x.reshape(S, D), A_mem0.reshape(MEM, D),
        A_Wq.reshape(D // 2, 2, H, DH), A_Wk.reshape(D // 2, 2, H, DH),
        A_Wv.reshape(D // 2, 2, H, DH), A_Wo.reshape(HD, D),
        B_w1, B_w3, B_w2, c, w_mod,
    )
    return out.reshape(1, S, D)
```

```python
import functools

import jax
import jax.numpy as jnp
from jax import lax
import jax.experimental.pallas as pl
import jax.experimental.pallas.tpu as pltpu

F32 = jnp.float32
BF16 = jnp.bfloat16
U32 = jnp.uint32

S = 2048
D = 1024
H = 32
DH = 128
HD = H * DH
MEM = 8
SEG = 32
FF = 3584
EPS = 1e-5
LOG2E = 1.4426950408889634

G = 8
HG = H // G
PRO = 512
NPAIR = S // (2 * SEG)
PT = 2 * SEG
SLOT = 40
NSLOT = 9
X0 = 544
X1 = 640
FC = 256
NFC = FF // FC
KW = 128
KT = D // KW
NB0 = 2
SETW = 128
NSET = D // 2 // SETW
NWS = G // 2 * 3 * HG
NJ = 3 * G // 2
FILL = (3, 5, 7, 10, 12, 14)
MODF = (0, 5, 6, 8, 11, 12)
QKPOS = 2
PVPOS = 11
WOCW = 256
DNCW = 256
PROM = PRO + 32
LNR = 136
MODR = 32
FLUSH_AT = 1
SCOPES = False


class _NoScope:
    def __enter__(self):
        return self

    def __exit__(self, *a):
        return False


def _scope(name):
    return jax.named_scope(name) if SCOPES else _NoScope()


def _unpack(x):
    return pltpu.bitcast(x, BF16)


def _pack(x):
    return pltpu.bitcast(x.astype(BF16), U32)


def _dot(a, b):
    return jnp.dot(a, b, preferred_element_type=F32)


def _ln(x):
    m = jnp.mean(x, axis=-1, keepdims=True)
    xc = x - m
    v = jnp.mean(xc * xc, axis=-1, keepdims=True)
    return xc * lax.rsqrt(v + EPS)


def _recip(x):
    r = pl.reciprocal(x, approx=True)
    return r * (2.0 - x * r)


def _silu(x):
    h = 0.5 * x
    return h + h * jnp.tanh(h)


def _cols(off, w):
    if isinstance(off, int):
        return slice(off, off + w)
    return pl.ds(pl.multiple_of(off, w), w)


def _rarely(cond, fn):
    def body(_, c):
        fn()
        return c

    lax.fori_loop(0, cond.astype(jnp.int32), body, 0)


def _slot(pair):
    assert NSLOT == 9
    return pair - NSLOT * ((pair * 57) >> 9)


def _masks():
    def pos(j):
        return jnp.where(j < 40, j, jnp.where(j < 48, j - 32, jnp.where(j < 56, j - 48, j - 40)))

    out = []
    for q0, nq, nk in ((0, 32, 48), (32, 48, 80)):
        qi = lax.broadcasted_iota(jnp.int32, (nq, nk), 0) + q0
        kj = lax.broadcasted_iota(jnp.int32, (nq, nk), 1)
        qp, kp = pos(qi), pos(kj)
        same = ((qi < 40) & (kj < 40)) | ((qi >= 40) & (kj >= 40))
        allowed = same & ((qp < MEM) | (qp >= kp))
        fill = jnp.where(same, jnp.float32(-1e9 * DH ** 0.5), jnp.float32(-jnp.inf))
        out.append((allowed, fill))
    return out


def _kernel(x_hbm, mem0_hbm, wq_hbm, wk_hbm, wv_hbm, wo_hbm, w1_hbm, w3_hbm, w2_hbm,
            c_hbm, wm_hbm, out_hbm,
            xv, outv, wo, w1, w3, w2, wm, cv, m0v, modv, xh, h0, hn, acc,
            lhs_a, lhs_b, o32, x1n, x1o, fv, h2, hid, sem_in, sem_m, sem_s, sem_w, sem_out, *rest):
    ring = rest[0:2]
    wg = rest[2:4]

    def side(g, t):
        return (g % 2) ^ int(t >= 2 * HG)

    scale = DH ** -0.5

    copies = {}

    def mk(name, src, dst):
        copies[name] = pltpu.make_async_copy(src, dst, sem_in.at[len(copies)])

    wm_u = wm_hbm.bitcast(U32)
    mk("c", c_hbm, cv)
    mk("mem0", mem0_hbm, m0v)
    mk("x0", x_hbm.at[0:X0], xv.at[0:X0])
    mk("x1", x_hbm.at[X0:X1], xv.at[X0:X1])
    for n, hbm, ref in (("wo", wo_hbm, wo), ("w2", w2_hbm, w2)):
        mk(n + "a", hbm.bitcast(U32).at[:, 0:D // 2], ref.at[:, 0:D // 2])
        mk(n + "b", hbm.bitcast(U32).at[:, D // 2:D], ref.at[:, D // 2:D])
    mk("wm1", wm_u.at[:, 2 * D:5 * D], wm.at[:, 2 * D:5 * D])
    for n, hbm, ref in (("w1", w1_hbm, w1), ("w3", w3_hbm, w3)):
        mk(n + "a", hbm.bitcast(U32).at[:, 0:FILL[0] * FC], ref.at[:, 0:FILL[0] * FC])
        mk(n + "b", hbm.bitcast(U32).at[:, FILL[0] * FC:FF], ref.at[:, FILL[0] * FC:FF])
    mk("wm2", wm_u.at[:, 5 * D:6 * D], wm.at[:, 5 * D:6 * D])
    mk("x2", x_hbm.at[X1:S], xv.at[X1:S])

    def mod_copies(kt):
        return [pltpu.make_async_copy(wm_u.at[:, _cols(i * D + kt * KW, KW)],
                                      wm.at[:, _cols(i * D + kt * KW, KW)], sem_m.at[kt])
                for i in range(2)]

    w_hbm = (wq_hbm, wk_hbm, wv_hbm)

    def start_block(j, rows=slice(None), sem=None):
        m, gi = j // 4, j % 4
        for pg in range(2):
            for jj in range(HG // 2):
                for par in range(2):
                    pltpu.make_async_copy(
                        w_hbm[m].bitcast(U32).at[rows, par, (2 * gi + pg) * (HG // 2) + jj],
                        wg[side(pg, m * HG)].at[gi * 3 * HG + m * HG + 2 * jj + par, rows],
                        sem_w.at[j] if sem is None else sem).start()

    def wait_block(j, s0):
        for w in wg:
            buf = w.at[pl.ds(s0, HG)]
            pltpu.make_async_copy(buf, buf, sem_w.at[j]).wait()

    def start_set(i):
        for j in range(NB0):
            start_block(j, slice(i * SETW, (i + 1) * SETW), sem_s.at[i])

    def wait_set(i):
        for w in wg:
            for gi in range(NB0):
                buf = w.at[gi * 3 * HG:gi * 3 * HG + HG, pl.ds(pl.multiple_of(i * SETW, SETW), SETW)]
                pltpu.make_async_copy(buf, buf, sem_s.at[i]).wait()

    def start_mod(kts):
        for kt in kts:
            for c in mod_copies(kt):
                c.start()

    for n in ("x0", "c", "mem0"):
        copies[n].start()

    def zero(i, c):
        acc[i] = jnp.zeros(acc.shape[1:], F32)
        rows = pl.ds(pl.multiple_of(i * 32, 32), 32)
        for w in wg:
            w[NWS:NWS + HG, rows, :] = jnp.zeros((HG, 32, DH), U32)
        return c

    lax.fori_loop(0, NB0 * 2 * HG, zero, 0)
    start_set(0)
    start_mod((0, 1, 2))
    start_set(1)
    start_mod((3, 4))
    start_set(2)
    start_mod((5,))

    def out_copy(r0, n):
        return pltpu.make_async_copy(outv.at[pl.ds(r0, n)], out_hbm.at[pl.ds(r0, n)], sem_out)

    def silu_c():
        return jnp.broadcast_to(_silu(cv[...].astype(F32)), (16, D)).astype(BF16)

    def mod_part(off, w):
        r = _dot(silu_c(), _unpack(wm[:, _cols(off, w)]))[0:8]
        modv[:, _cols(off, w)] = r
        return r[0:1]

    def mvec(i, n, plus=0.0):
        m = modv[:, i * D:(i + 1) * D]
        return jnp.concatenate([plus + m if plus else m] * (n // 8), axis=0)

    def ln1(r0, n):
        xf = xv[pl.ds(r0, n), :].astype(F32)
        return _ln(xf) * mvec(1, n, 1.0) + mvec(0, n)

    def repack_rows(w, sl, r0):
        rows = slice(r0, r0 + 32) if isinstance(r0, int) else pl.ds(r0, 32)
        a = w[sl, rows, :]
        b = w[sl + 1, rows, :]
        w[sl, rows, :] = (a & jnp.uint32(0xFFFF)) | (b << 16)
        w[sl + 1, rows, :] = (a >> 16) | (b & jnp.uint32(0xFFFF0000))

    def repack_now(s0):
        def body(i, c):
            for w in wg:
                for r in range(0, D // 4, 32):
                    r0 = pl.multiple_of((i & 1) * (D // 4) + r, 32)
                    repack_rows(w, s0 + 2 * (i >> 1), r0)
            return c

        lax.fori_loop(0, HG, body, 0)

    def repack_tile(w, kt, slots):
        for s0 in slots:
            for t in range(0, HG, 2):
                for r in range(0, KW // 2, 32):
                    r0 = kt * (KW // 2) + r
                    repack_rows(w, s0 + t, r0 if isinstance(r0, int) else pl.multiple_of(r0, 32))

    def store_tokens(dst, gi, t, r):
        for pp in range(PRO // PT):
            b0, r0 = pp * SLOT, pp * PT
            dst[gi, t, b0 + 4:b0 + 8, :] = _pack(r[r0:r0 + 8])
            dst[gi, t, b0 + 8:b0 + 24, :] = _pack(r[r0 + 8:r0 + 40])
            dst[gi, t, b0 + 28:b0 + 32, :] = _pack(r[r0 + 40:r0 + 48])
            dst[gi, t, b0 + 32:b0 + 40, :] = _pack(r[r0 + 48:r0 + 64])
        b0 = (PRO // PT) * SLOT
        dst[gi, t, 0:4, :] = _pack(r[PRO:PRO + 8])
        dst[gi, t, b0 + 4:b0 + 8, :] = _pack(r[PRO + 8:PRO + 16])
        dst[gi, t, b0 + 8:b0 + 16, :] = _pack(r[PRO + 16:PRO + 32])

    def proj(lhs, g, rows, t0, t1):
        for t in range(t0, t1):
            r = _dot(lhs, _unpack(wg[side(g, t)][g // 2 * 3 * HG + t]))
            for i, row in enumerate(rows):
                ring[side(g, t)][g // 2, t, pl.ds(row, 4), :] = _pack(r[8 * i:8 * i + 8])

    def attn_qk(g, base, q0, nq, nk, allowed, fill):
        qrow = pl.multiple_of(base + q0 // 2, 8)
        ps = []
        for hh in range(HG):
            q = _unpack(ring[g % 2][g // 2, hh, pl.ds(qrow, nq // 2), :])
            k = _unpack(ring[g % 2][g // 2, HG + hh, pl.ds(base, nk // 2), :])
            s = lax.dot_general(q, k, (((1,), (1,)), ((), ())), preferred_element_type=F32)
            s = jnp.where(allowed, s, fill)
            m = jnp.max(s, axis=-1, keepdims=True)
            p = jnp.exp2((s - m) * (scale * LOG2E))
            l = jnp.sum(p, axis=-1, keepdims=True)
            ps.append((p * _recip(l)).astype(BF16))
        return ps

    def attn_pv(g, base, nq, nk, ps):
        for hh in range(HG):
            v = _unpack(ring[1 - g % 2][g // 2, 2 * HG + hh, pl.ds(base, nk // 2), :])
            col = (g * HG + hh) * DH
            o32[0:nq // 2, col:col + DH] = _pack(_dot(ps[hh], v))

    def wo_proj(nq, stores):
        o = _unpack(o32[0:nq // 2, :])
        cw = WOCW
        for cb in range(D // cw):
            cs = slice(cb * cw, (cb + 1) * cw)
            r = _dot(o, _unpack(wo[:, cs]))
            for r0, n, fn in stores:
                fn(cs, r[r0:r0 + n])

    def ln2():
        h2[...] = _pack(_ln(x1n[...]) * mvec(4, PT, 1.0) + mvec(3, PT))

    def ffn_up(c0, c1):
        a = _unpack(h2[...])
        for c in range(c0, c1):
            cs = slice(c * FC, (c + 1) * FC)
            gt = _dot(a, _unpack(w1[:, cs]))
            up = _dot(a, _unpack(w3[:, cs]))
            hid[:, cs] = _pack(_silu(gt) * up)

    def ffn_down(tok0, x1, last=False):
        a = _unpack(hid[...])
        cw = DNCW
        for cb in range(D // cw):
            cs = slice(cb * cw, (cb + 1) * cw)
            r = _dot(a, _unpack(w2[:, cs]))
            if not last:
                fv[:, cs] = r
            gb = modv[0:1, 5 * D + cb * cw:5 * D + (cb + 1) * cw]
            outv[pl.ds(tok0, PT), cs] = (x1[:, cs] + gb * r).astype(BF16)
            if last:
                pltpu.make_async_copy(outv.at[pl.ds(tok0, PT), cs],
                                      out_hbm.at[pl.ds(tok0, PT), cs], sem_out).start()

    def unit_row(u):
        r = u & 7
        slot = _slot(u >> 3)
        return pl.multiple_of(slot * SLOT + 4 + 4 * r + 4 * (r >= 5).astype(jnp.int32), 4)

    with _scope("waitx0"):
        copies["x0"].wait()
    with _scope("ln0"):

        def ln_body(i, c):
            r0 = pl.multiple_of(i * LNR, 8)
            xh[pl.ds(r0, LNR), :] = _ln(xv[pl.ds(r0, LNR), :].astype(F32))
            return c

        lax.fori_loop(0, X0 // LNR, ln_body, 0)
    with _scope("waitc"):
        copies["c"].wait()
        copies["mem0"].wait()

    def modulate(kt):
        sa = mod_part(kt * KW, KW)
        ca = mod_part(D + kt * KW, KW)
        cs = _cols(kt * KW, KW)
        ca = 1.0 + ca
        for r0 in range(0, PRO, MODR):
            hn[r0 // 2:(r0 + MODR) // 2, :] = _pack(xh[r0:r0 + MODR, cs] * ca + sa)
        hh = xh[PRO:PRO + 24, cs] * ca + sa
        hn[PRO // 2:PROM // 2, :] = _pack(jnp.concatenate([m0v[:, cs].astype(F32), hh], axis=0))

    with _scope("waitw0"):
        wait_set(0)
    with _scope("first"):
        for w in wg:
            repack_tile(w, 0, [gi * 3 * HG for gi in range(NB0)])
        with _scope("waitm0"):
            for c in mod_copies(0):
                c.wait()
        modulate(0)

    def kmajor(kt, c):
        more = kt < KT - 1
        kn = jnp.minimum(kt + 1, KT - 1)

        def later_copies():
            start_set(3)
            start_mod((6, 7))
            for j in range(NB0, NB0 + 3):
                start_block(j)

        _rarely(kt == 1, later_copies)

        @pl.when(more)
        def _():
            for cp in mod_copies(kn):
                cp.wait()

        @pl.when(more & ((kn & 1) == 0))
        def _():
            wait_set(kn >> 1)

        cs = _cols(kt * KW, KW)
        h0[:, cs] = hn[...]
        rows = pl.ds(pl.multiple_of(kt * (KW // 2), KW // 2), KW // 2)
        for pg in range(2):
            for gi in range(NB0):
                for t in range(HG):
                    i = (pg * NB0 + gi) * HG + t
                    a = hn[...] if i < HG else h0[:, cs]
                    acc[i] += _dot(_unpack(a), _unpack(wg[pg][gi * 3 * HG + t, rows, :]))
                if pg == 0 and gi == 0:
                    modulate(kn)
        slots = [jnp.where(more, gi * 3 * HG, NWS) for gi in range(NB0)]
        for w in wg:
            repack_tile(w, kn, slots)
        return c

    with _scope("kmajor"):
        lax.fori_loop(0, KT, kmajor, 0)

    def pro_body(j, c):
        gi, t0 = j & 3, (j >> 2) * HG
        s0 = gi * (3 * HG) + t0
        jn = j + 1
        prefetch = jn < NJ
        sn = jnp.where(prefetch, (jn & 3) * (3 * HG) + (jn >> 2) * HG, NWS)

        def first_blocks():
            def batch1():
                for jj in range(NB0 + 3, NJ - 2):
                    start_block(jj)
                with _scope("waitlate"):
                    wait_block(j, s0)
                repack_now(s0)

            def batch2():
                for jj in range(NJ - 2, NJ):
                    start_block(jj)
                for n in ("x1", "woa", "wob", "wm1", "w1a", "w3a", "w1b", "w3b", "w2a", "w2b", "wm2", "x2"):
                    copies[n].start()

            _rarely(j == NB0, batch1)
            _rarely(j == NB0 + 1, batch2)

        _rarely(j <= NB0 + 1, first_blocks)

        @pl.when(prefetch)
        def _():
            wait_block(jn, sn)

        a = _unpack(h0[...])
        k = jnp.minimum(j - NB0, NB0 * HG - 1)
        for pg in range(2):
            for t in range(HG):
                store_tokens(ring[pg], gi, t0 + t, _dot(a, _unpack(wg[pg][s0 + t])))
                if t == FLUSH_AT:
                    store_tokens(ring[pg], k >> 2, k & 3, acc[pg * NB0 * HG + k])
        for w in wg:
            for t in range(0, HG, 2):
                for r0 in range(0, D // 2, 32):
                    repack_rows(w, sn + t, r0)
        return c

    with _scope("pro"):
        lax.fori_loop(NB0, NJ, pro_body, 0)

    def pair(p, with_ffn):
        (al_a, fi_a), (al_b, fi_b) = _masks()
        base = pl.multiple_of(_slot(p) * SLOT, 8)
        u0 = PRO // 8 + 6 * p
        tlead = PRO + 48 * p

        if with_ffn:
            x1o[...] = x1n[...]

        def filler(i, c0=None, c1=None):
            if not with_ffn:
                if i is not None:
                    mod_part(2 * D + MODF[i] * 256, (MODF[i + 1] - MODF[i]) * 256)
            elif c0 is None:
                ffn_down(pl.multiple_of((p - 1) * PT, PT), x1o)
            else:
                ffn_up(c0, c1)

        def proj_attn(lhs, rows, q0, nq, nk, allowed, fill, f):
            ps = None
            for g in range(G):
                proj(lhs, g, rows, 0, QKPOS)
                if g > 0 and QKPOS > 0:
                    ps = attn_qk(g - 1, base, q0, nq, nk, allowed, fill)
                proj(lhs, g, rows, QKPOS, PVPOS)
                if g > 0:
                    attn_pv(g - 1, base, nq, nk, ps)
                proj(lhs, g, rows, PVPOS, 3 * HG)
                if QKPOS == 0 or g == G - 1:
                    ps = attn_qk(g, base, q0, nq, nk, allowed, fill)
            filler(f, FILL[f], FILL[f + 1])
            attn_pv(G - 1, base, nq, nk, ps)
            filler(f + 1, FILL[f + 1], FILL[f + 2])

        def st_lhs(ref):
            def fn(cs, val):
                ref[0:MEM, cs] = val.astype(BF16).astype(F32)
            return fn

        def st_a(r0, n):
            def fn(cs, val):
                ga = modv[0:1, 2 * D + cs.start:2 * D + cs.stop]
                x = xv[pl.ds(pl.multiple_of(p * PT + r0, 8), n), cs].astype(F32)
                x1n[r0:r0 + n, cs] = x + ga * val
            return fn

        lhs_b[MEM:32, :] = ln1(pl.multiple_of(tlead + 24, 8), 24)
        if with_ffn:
            lhs = lhs_a[...].astype(BF16)
            rows = [base, unit_row(u0), unit_row(u0 + 1), unit_row(u0 + 2)]
            proj_attn(lhs, rows, 0, 32, 48, al_a, fi_a, 0)
        else:
            ps = [attn_qk(g, base, 0, 32, 48, al_a, fi_a) for g in range(G)]
            filler(0)
            for g in range(G):
                attn_pv(g, base, 32, 48, ps[g])
            filler(1)
        wo_proj(32, [(0, 8, st_lhs(lhs_b)), (8, 24, st_a(0, 24))])
        filler(2, FILL[2], FILL[3])

        lhs = lhs_b[...].astype(BF16)
        rows = [pl.multiple_of(base + 24, 8), unit_row(u0 + 3), unit_row(u0 + 4), unit_row(u0 + 5)]
        nxt = pl.multiple_of(jnp.minimum(tlead + 48, S - 24), 8)
        lhs_a[MEM:32, :] = ln1(nxt, 24)
        proj_attn(lhs, rows, 32, 48, 80, al_b, fi_b, 3)
        wo_proj(48, [(16, 8, st_lhs(lhs_a)), (0, 16, st_a(24, 16)), (24, 24, st_a(40, 24))])
        ln2()
        filler(None)
        ffn_up(0, FILL[0])

    with _scope("waitwo"):
        copies["x1"].wait()
        copies["woa"].wait()
        copies["wob"].wait()
        copies["wm1"].wait()
        copies["w1a"].wait()
        copies["w3a"].wait()

    with _scope("noffn"):
        modv[:, 5 * D:6 * D] = jnp.zeros((8, D), F32)
        pair(jnp.int32(0), False)

    with _scope("waitffn"):
        copies["w1b"].wait()
        copies["w3b"].wait()
        copies["w2a"].wait()
        copies["w2b"].wait()

    def late_inputs():
        copies["wm2"].wait()
        copies["x2"].wait()
        mod_part(5 * D, D)
        outv[0:PT, :] = (x1o[...] + mvec(5, PT) * fv[...]).astype(BF16)

    def pair_ffn(p, c):
        pair(p, True)
        return c

    def main(o, c):
        _rarely(o == 1, late_inputs)
        lax.fori_loop(1 + o, 2 + o * (NPAIR - 2), pair_ffn, 0)
        return c

    with _scope("main"):
        lax.fori_loop(0, 2, main, 0)

    with _scope("epi"):
        out_copy(0, S - PT).start()
        ffn_up(FILL[0], NFC)
        ffn_down(S - PT, x1n, last=True)
    with _scope("waitout"):
        out_copy(0, S).wait()


@functools.partial(jax.jit, static_argnames=("A_seg_len",))
def pallas_adaLN_cond__memory_aug_recurrent_mem_tr__glu_gated_swiglu__prompt_kernel(
    A_x, A_mem0, A_Wq, A_Wk, A_Wv, A_Wo, A_seg_len, B_x, B_w1, B_w3, B_w2, c, w_mod,
):
    assert A_seg_len == SEG
    assert A_x.shape == (1, S, D) and A_mem0.shape == (1, MEM, D)
    assert A_Wq.shape == (D, H, DH) and B_w1.shape == (D, FF)
    del B_x

    scratch = [
        pltpu.VMEM((S, D), BF16),
        pltpu.VMEM((S, D), BF16),
        pltpu.VMEM((HD // 2, D), U32),
        pltpu.VMEM((D // 2, FF), U32),
        pltpu.VMEM((D // 2, FF), U32),
        pltpu.VMEM((FF // 2, D), U32),
        pltpu.VMEM((D // 2, 6 * D), U32),
        pltpu.VMEM((1, D), BF16),
        pltpu.VMEM((MEM, D), BF16),
        pltpu.VMEM((8, 6 * D), F32),
        pltpu.VMEM((X0, D), F32),
        pltpu.VMEM((PROM // 2, D), U32),
        pltpu.VMEM((PROM // 2, KW), U32),
        pltpu.VMEM((NB0 * 2 * HG, PROM, DH), F32),
        pltpu.VMEM((32, D), F32),
        pltpu.VMEM((32, D), F32),
        pltpu.VMEM((24, HD), U32),
        pltpu.VMEM((PT, D), F32),
        pltpu.VMEM((PT, D), F32),
        pltpu.VMEM((PT, D), F32),
        pltpu.VMEM((PT // 2, D), U32),
        pltpu.VMEM((PT // 2, FF), U32),
        pltpu.SemaphoreType.DMA((15,)),
        pltpu.SemaphoreType.DMA((KT,)),
        pltpu.SemaphoreType.DMA((NSET,)),
        pltpu.SemaphoreType.DMA((NJ,)),
        pltpu.SemaphoreType.DMA,
    ] + [pltpu.VMEM((G // 2, 3 * HG, NSLOT * SLOT, DH), U32)] * 2 + [
        pltpu.VMEM((NWS + HG, D // 2, DH), U32)] * 2

    out = pl.pallas_call(
        _kernel,
        out_shape=jax.ShapeDtypeStruct((S, D), BF16),
        in_specs=[pl.BlockSpec(memory_space=pl.ANY)] * 11,
        out_specs=pl.BlockSpec(memory_space=pl.ANY),
        scratch_shapes=scratch,
        compiler_params=pltpu.CompilerParams(
            vmem_limit_bytes=120 * 1024 * 1024, disable_bounds_checks=True,
            disable_semaphore_checks=True),
    )(
        A_x.reshape(S, D), A_mem0.reshape(MEM, D),
        A_Wq.reshape(D // 2, 2, H, DH), A_Wk.reshape(D // 2, 2, H, DH),
        A_Wv.reshape(D // 2, 2, H, DH), A_Wo.reshape(HD, D),
        B_w1, B_w3, B_w2, c, w_mod,
    )
    return out.reshape(1, S, D)
```
